```python
import jax
import jax.numpy as jnp

def _softmax(x, axis=-1):
    return jax.nn.softmax(x, axis=axis)
def _gelu(x):
    return jax.nn.gelu(x, approximate=True)
def _silu(x):
    return jax.nn.silu(x)
def _sigmoid(x):
    return jax.nn.sigmoid(x)
def _layernorm(x, axis=-1, eps=1e-5):
    m = jnp.mean(x, axis=axis, keepdims=True)
    v = jnp.var(x, axis=axis, keepdims=True)
    return (x - m) / jnp.sqrt(v + eps)
def _scatter_add(tgt, idx, src, axis=0):
    return tgt.at[idx].add(src)
def _segment_sum(src, seg, n):
    return jax.ops.segment_sum(src, seg, n)
class _Rng:
    def __init__(self, key):
        self._k = key
    def _next(self):
        self._k, sub = jax.random.split(self._k)
        return sub
    def normal(self, shape):
        return jax.random.normal(self._next(), shape, dtype=jnp.bfloat16)
    def randint(self, lo, hi, shape):
        return jax.random.randint(self._next(), shape, lo, hi, dtype=jnp.int32)
    def uniform(self, shape, lo=0.0, hi=1.0):
        return jax.random.uniform(self._next(), shape, jnp.bfloat16, lo, hi)
    def permutation(self, n):
        return jax.random.permutation(self._next(), n)


kernel_name = 'recurrent_scan__sliding_local_dilated__geglu_ffn__prompt'

def setup_inputs():
    _rng = _Rng(jax.random.key(int.from_bytes(__import__("os").urandom(4), "little")))
    _w = (lambda a: (lambda t: t.astype(jnp.bfloat16) if jnp.issubdtype(t.dtype, jnp.floating) else t)(jnp.asarray(a)))
    def _A_setup():
        B, S, D = 1, 2048, 1024
        return {
            "x": _w((lambda *s: _rng.normal(s) * 0.05)(B, S, D)),
            "wqkv": _w((lambda *s: _rng.normal(s) * 0.05)(D, 3 * D)),
            "wo": _w((lambda *s: _rng.normal(s) * 0.05)(D, D)),
        }
    _A_in = _A_setup()

    def _B_setup():
        B, S, D, F = 1, 2048, 1024, 3584
        return {
            "x": _w((lambda *s: _rng.normal(s) * 0.05)(B, S, D)),
            "w_gate": _w((lambda *s: _rng.normal(s) * 0.05)(D, F)),
            "w_up": _w((lambda *s: _rng.normal(s) * 0.05)(D, F)),
            "w_down": _w((lambda *s: _rng.normal(s) * 0.05)(F, D)),
        }
    _B_in = _B_setup()

    return {
        "A_x": _A_in["x"],
        "A_wqkv": _A_in["wqkv"],
        "A_wo": _A_in["wo"],
        "B_x": _B_in["x"],
        "B_w_gate": _B_in["w_gate"],
        "B_w_up": _B_in["w_up"],
        "B_w_down": _B_in["w_down"],
    }

def reference(A_x, A_wqkv, A_wo, B_x, B_w_gate, B_w_up, B_w_down):
    def _A_ref(x, wqkv, wo):
        B, S, D = x.shape
        H = 32; Dh = D // H
        W, dil = 8, 2
        qkv = (lambda x, *d: x.transpose(*d))((x @ wqkv).reshape(B, S, 3, H, Dh), 2, 0, 3, 1, 4)
        q, k, v = qkv[0], qkv[1], qkv[2]
        scale = Dh ** -0.5
        pos = jnp.arange(S)
        off = jnp.arange(W) * dil
        idx = pos[:, None] - off[None, :]
        mask = idx >= 0
        idx_c = jnp.where(mask, idx, 0).reshape(-1)
        kg = k[:, :, idx_c, :].reshape(B, H, S, W, Dh)
        vg = v[:, :, idx_c, :].reshape(B, H, S, W, Dh)
        logits = jnp.einsum("bhsd,bhswd->bhsw", q, kg) * scale
        logits = jnp.where(mask[None, None, :, :], logits, -1e9)
        attn = _softmax(logits, axis=-1)
        o = jnp.einsum("bhsw,bhswd->bhsd", attn, vg)
        return (lambda x, *d: x.transpose(*d))(o, 0, 2, 1, 3).reshape(B, S, D) @ wo

    def _B_ref(x, w_gate, w_up, w_down):
        return (_gelu(x @ w_gate) * (x @ w_up)) @ w_down

    x = A_x
    xn = _layernorm(x, axis=-1)
    s = _A_ref(xn, A_wqkv, A_wo)
    g = _silu(_B_ref(xn, B_w_gate, B_w_up, B_w_down))
    return x + s * g
```

```python
import functools, math
import jax
import jax.numpy as jnp
from jax import lax
import jax.experimental.pallas as pl
import jax.experimental.pallas.tpu as pltpu

S, D, F = 2048, 1024, 3584
H, DH, W, DIL = 32, 32, 8, 2
NL = 128
NCH = D // NL
HALO = 16
F32, BF16, U32 = jnp.float32, jnp.bfloat16, jnp.uint32
EPS = 1e-5
GELU_C0 = math.sqrt(2.0 / math.pi)
GELU_C1 = GELU_C0 * 0.044715
EXP2_SCALE = (DH ** -0.5) * math.log2(math.e)
NEG = -1e9 / (DH ** -0.5)


def make(T=512, FC=512, N1=3, AR=8):
    NT = S // T
    NC = F // FC
    N2 = NC - N1
    AP = T // N2
    assert AP * N2 == T and AP % AR == 0

    def kernel(x_ref, wqkv_hbm, wo_hbm, wg_hbm, wu_hbm, wd_hbm, out_ref,
               wgu, wd, wqkv, wo_raw, wo32, wo, xn, q, kb, vb, o, acc, sem_g, sem_u, sem_d, sem_a):
        step = pl.program_id(0)

        def cp_g(c):
            return pltpu.make_async_copy(wg_hbm.at[:, pl.ds(c * FC, FC)], wgu.at[c, :, pl.ds(0, FC)], sem_g.at[c])
        def cp_u(c):
            return pltpu.make_async_copy(wu_hbm.at[:, pl.ds(c * FC, FC)], wgu.at[c, :, pl.ds(FC, FC)], sem_u.at[c])
        def cp_d(c):
            return pltpu.make_async_copy(wd_hbm.at[pl.ds(c * FC, FC), :], wd.at[c], sem_d.at[c])
        cp_qkv = pltpu.make_async_copy(wqkv_hbm, wqkv, sem_a.at[0])
        cp_wo = pltpu.make_async_copy(wo_hbm, wo_raw, sem_a.at[1])

        @pl.when(step == 0)
        def _():
            for c in range(N1):
                cp_g(c).start(); cp_u(c).start(); cp_d(c).start()
                if c == 0:
                    pass
            cp_qkv.start()
            for c in range(N1, NC):
                cp_g(c).start(); cp_u(c).start(); cp_d(c).start()
            cp_wo.start()

        def ln_body(i, carry):
            r = pl.multiple_of(i * 16, 16)
            x = x_ref[pl.ds(r, 16), :].astype(F32)
            m = jnp.mean(x, axis=-1, keepdims=True)
            xc = x - m
            v = jnp.mean(xc * xc, axis=-1, keepdims=True)
            xn[pl.ds(r, 16), :] = (xc * lax.rsqrt(v + EPS)).astype(BF16)
            return carry
        lax.fori_loop(0, T // 16, ln_body, 0, unroll=4)

        def ffn_chunk(c, first):
            gu = jnp.dot(xn[...], wgu[c], preferred_element_type=F32)
            g = gu[:, :FC]
            u = gu[:, FC:]
            t = jnp.tanh(g * (GELU_C0 + GELU_C1 * (g * g)))
            p = g * u
            h = (p + p * t).astype(BF16)
            d = jnp.dot(h, wd[c], preferred_element_type=F32)
            if first:
                acc[...] = d
            else:
                acc[...] += d

        def wait_chunk(c):
            @pl.when(step == 0)
            def _():
                cp_g(c).wait(); cp_u(c).wait(); cp_d(c).wait()

        lane = lax.broadcasted_iota(jnp.int32, (8, NL), 1)

        def attn_rows(r0):
            lane_a = lax.broadcasted_iota(jnp.int32, (AR, NL), 1)
            odd = (lane_a & 1) != 0
            hi = (lane_a & 2) != 0
            pos = step * T + r0 + lax.broadcasted_iota(jnp.int32, (AR, NL), 0)
            qs = [q[j, pl.ds(r0, AR), :] for j in range(NCH)]
            ls = []
            for w in range(W):
                a = qs[0] * kb[0, pl.ds(r0 + HALO - DIL * w, AR), :]
                for j in range(1, NCH):
                    a = a + qs[j] * kb[j, pl.ds(r0 + HALO - DIL * w, AR), :]
                a = a + jnp.where(odd, pltpu.roll(a, 1, 1), pltpu.roll(a, NL - 1, 1))
                a = a + jnp.where(hi, pltpu.roll(a, 2, 1), pltpu.roll(a, NL - 2, 1))
                if w > 0:
                    a = jnp.where(pos >= DIL * w, a, NEG)
                ls.append(a)
            m = ls[0]
            for w in range(1, W):
                m = jnp.maximum(m, ls[w])
            ps = [jnp.exp2((l - m) * EXP2_SCALE) for l in ls]
            den = ps[0]
            for w in range(1, W):
                den = den + ps[w]
            inv = 1.0 / den
            ps = [p * inv for p in ps]
            outs = []
            for j in range(NCH):
                a = ps[0] * vb[j, pl.ds(r0 + HALO, AR), :]
                for w in range(1, W):
                    a = a + ps[w] * vb[j, pl.ds(r0 + HALO - DIL * w, AR), :]
                outs.append(a)
            return outs

        wait_chunk(0)
        ffn_chunk(0, True)

        def body1(c, carry):
            wait_chunk(c)
            ffn_chunk(c, False)
            return carry
        lax.fori_loop(1, N1, body1, 0)

        @pl.when(step == 0)
        def _():
            cp_qkv.wait()
            g = (lane % 32) // 4
            masks = [(g & (1 << b)) != 0 for b in range(3)]
            def perm_body(i, carry):
                r = pl.multiple_of(i * 16, 16)
                for part in range(3):
                    blk = pltpu.bitcast(wqkv[pl.ds(r, 16), pl.ds(part * D, D)], U32)
                    y = [blk[:, k * NL:(k + 1) * NL] for k in range(NCH)]
                    y = [y[0]] + [pltpu.roll(y[k], 4 * k, 1) for k in range(1, NCH)]
                    v = [y[(-m_) % NCH] for m_ in range(NCH)]
                    for b in range(3):
                        v = [jnp.where(masks[b], v[(m_ - (1 << b)) % NCH], v[m_]) for m_ in range(NCH)]
                    v = [v[0]] + [pltpu.roll(v[k], NL - 4 * k, 1) for k in range(1, NCH)]
                    wqkv[pl.ds(r, 16), pl.ds(part * D, D)] = pltpu.bitcast(jnp.concatenate(v, axis=1), BF16)
                return carry
            lax.fori_loop(0, D // 16, perm_body, 0)

        @pl.when(step > 0)
        def _():
            for j in range(NCH):
                kb[j, 0:HALO, :] = kb[j, T:T + HALO, :]
                vb[j, 0:HALO, :] = vb[j, T:T + HALO, :]
        xv = xn[...]
        for part, dst, off in ((0, q, 0), (1, kb, HALO), (2, vb, HALO)):
            r = jnp.dot(xv, wqkv[:, part * D:(part + 1) * D], preferred_element_type=F32)
            for j in range(NCH):
                dst[j, off:off + T, :] = r[:, j * NL:(j + 1) * NL]
        @pl.when(step == 0)
        def _():
            for j in range(NCH):
                kb[j, 0:HALO, :] = jnp.broadcast_to(kb[j, HALO:HALO + 1, :], (HALO, NL))
                vb[j, 0:HALO, :] = jnp.broadcast_to(vb[j, HALO:HALO + 1, :], (HALO, NL))

        def body2(i, carry):
            c = N1 + i
            wait_chunk(c)
            ffn_chunk(c, False)
            base = pl.multiple_of(i * AP, AP)
            for s in range(AP // 16):
                parts = []
                for t_ in range(16 // AR):
                    parts.append(attn_rows(base + s * 16 + t_ * AR))
                for j in range(NCH):
                    blk = parts[0][j] if len(parts) == 1 else jnp.concatenate([p_[j] for p_ in parts], axis=0)
                    o[pl.ds(pl.multiple_of(base + s * 16, 16), 16), j * NL:(j + 1) * NL] = blk.astype(BF16)
            return carry
        lax.fori_loop(0, N2, body2, 0)

        @pl.when(step == 0)
        def _():
            cp_wo.wait()
            for k in range(NCH):
                wo32[k] = pltpu.bitcast(wo_raw[:, k * NL:(k + 1) * NL], U32)
            for k in range(NCH):
                for j in range(8):
                    for hh in range(4):
                        rows = []
                        for tp in range(2):
                            rows.append(wo32[k, pl.ds(16 * hh + 2 * j + tp, 8, stride=64), :])
                        for tp in range(2):
                            wo32[NCH + k, pl.ds(64 * j + 16 * hh + tp, 8, stride=2), :] = rows[tp]
            for k in range(NCH):
                wo[:, k * NL:(k + 1) * NL] = pltpu.bitcast(wo32[NCH + k], BF16)

        s_ = jnp.dot(o[...], wo[...], preferred_element_type=F32)
        f = acc[...] * 0.5
        gate = f * (0.5 + 0.5 * jnp.tanh(0.5 * f))
        out_ref[...] = (x_ref[...].astype(F32) + s_ * gate).astype(out_ref.dtype)

    @jax.jit
    def fn(A_x, A_wqkv, A_wo, B_x, B_w_gate, B_w_up, B_w_down):
        x = A_x.reshape(S, D)
        anyspec = pl.BlockSpec(memory_space=pl.ANY)
        out = pl.pallas_call(
            kernel,
            grid=(NT,),
            in_specs=[pl.BlockSpec((T, D), lambda i: (i, 0)), anyspec, anyspec, anyspec, anyspec, anyspec],
            out_specs=pl.BlockSpec((T, D), lambda i: (i, 0)),
            out_shape=jax.ShapeDtypeStruct((S, D), BF16),
            scratch_shapes=[
                pltpu.VMEM((NC, D, 2 * FC), BF16),
                pltpu.VMEM((NC, FC, D), BF16),
                pltpu.VMEM((D, 3 * D), BF16),
                pltpu.VMEM((D, D), BF16),
                pltpu.VMEM((2 * NCH, D // 2, NL), U32),
                pltpu.VMEM((D, D), BF16),
                pltpu.VMEM((T, D), BF16),
                pltpu.VMEM((NCH, T, NL), F32),
                pltpu.VMEM((NCH, T + HALO, NL), F32),
                pltpu.VMEM((NCH, T + HALO, NL), F32),
                pltpu.VMEM((T, D), BF16),
                pltpu.VMEM((T, D), F32),
                pltpu.SemaphoreType.DMA((NC,)),
                pltpu.SemaphoreType.DMA((NC,)),
                pltpu.SemaphoreType.DMA((NC,)),
                pltpu.SemaphoreType.DMA((2,)),
            ],
            compiler_params=pltpu.CompilerParams(
                dimension_semantics=("arbitrary",), vmem_limit_bytes=100 * 2 ** 20),
        )(x, A_wqkv, A_wo, B_w_gate, B_w_up, B_w_down)
        return out.reshape(1, S, D)
    return fn


_IMPL = make(T=256, FC=512, N1=3)


@jax.jit
def pallas_recurrent_scan__sliding_local_dilated__geglu_ffn__prompt_kernel(
    A_x: jax.Array,
    A_wqkv: jax.Array,
    A_wo: jax.Array,
    B_x: jax.Array,
    B_w_gate: jax.Array,
    B_w_up: jax.Array,
    B_w_down: jax.Array,
):
    return _IMPL(A_x, A_wqkv, A_wo, B_x, B_w_gate, B_w_up, B_w_down)
```

```python
import contextlib
import math

import jax
import jax.numpy as jnp
from jax import lax
import jax.experimental.pallas as pl
import jax.experimental.pallas.tpu as pltpu

S, D, F = 2048, 1024, 3584
H, DH, W, DIL = 32, 32, 8, 2
NL = 128
NCH = D // NL
HS = S // 2
KH = D // 2
KC = KH // NL
FC = 256
NC = F // FC
HALO = 16
F32, BF16, U32 = jnp.float32, jnp.bfloat16, jnp.uint32
EPS = 1e-5
GELU_C0 = math.sqrt(2.0 / math.pi)
GELU_C1 = GELU_C0 * 0.044715
EXP2_SCALE = (DH ** -0.5) * math.log2(math.e)
NEG = -1e9 / (DH ** -0.5)


def _a_ops(a11, a12, a21, a22):
    return [a11 + a22, a21 + a22, a11, a22, a11 + a12, a21 - a11, a12 - a22]


def _b_ops(b11, b12, b21, b22):
    return [b11 + b22, b11, b12 - b22, b21 - b11, b22, b11 + b12, b21 + b22]


def _dot(a, b):
    return jnp.dot(a, b, preferred_element_type=F32)


def _pk(x):
    return x.astype(BF16)


def _strassen(prod, fin, cost):
    m1 = prod(1)
    yield cost, m1
    m3 = prod(3)
    fin(2, m1 + m3)
    yield cost, m3
    m0 = prod(0)
    t11 = m3 + m0
    t22 = m0 - m1
    yield cost, m0
    m5 = prod(5)
    t22 = t22 + m5
    yield cost, m5
    m2 = prod(2)
    fin(3, t22 + m2)
    yield cost, m2
    m4 = prod(4)
    fin(1, m2 + m4)
    t11 = t11 - m4
    yield cost, m4
    m6 = prod(6)
    fin(0, t11 + m6)
    yield cost, m6


def _emit(lag, main, total, *sides):
    done = [0] * len(sides)
    acc = 0

    def flush(frac, val):
        for k, (f0, f1, tasks) in enumerate(sides):
            want = len(tasks) if frac >= f1 else int(max(0.0, (frac - f0) / (f1 - f0)) * len(tasks)) + (frac >= f0)
            while done[k] < min(want, len(tasks)):
                tasks[done[k]](val)
                done[k] += 1
    hist = [None] * (lag + 1)
    flush(0.0, None)
    for c, val in main:
        acc += c
        hist = hist[1:] + [val]
        flush(acc / total, hist[0])
    assert acc == total, (acc, total)
    flush(2.0, hist[0])


def _skew(stages_per_item):
    n = len(stages_per_item)
    depth = max(len(st) for st in stages_per_item)
    tasks = []
    for t in range(n + depth - 1):
        group = [stages_per_item[t - k][k] for k in range(depth) if 0 <= t - k < n and k < len(stages_per_item[t - k])]
        tasks.append(lambda val, group=group: [g(val) for g in group])
    return tasks


def make(RH=128, T0=256, T3=256, AP=80, LAG=2, scopes=False):
    NT0 = HS // T0
    NT3 = HS // T3
    assert AP % 16 == 0 and AP * (NC - 1) >= HS

    def scope(name):
        return jax.named_scope(name) if scopes else contextlib.nullcontext()

    def kernel(x_hbm, wqkv_hbm, wo_hbm, wg_hbm, wu_hbm, wd_hbm, out_hbm,
               xbuf, XA, qkv, OA, P, HA, BW,
               rgu, rd, rq, ro, obuf,
               sem_x, sem_gu, sem_d, sem_q, sem_o, sem_out):

        XA, OA, HA, BW = [r.bitcast(BF16) for r in (XA, OA, HA, BW)]

        def ch(n):
            return pl.ds(n * NL, NL) if isinstance(n, int) else pl.ds(pl.multiple_of(n * NL, NL), NL)

        def cp_x(i, half):
            r = half * HS + i * T0
            return pltpu.make_async_copy(x_hbm.at[pl.ds(r, T0), :], xbuf.at[pl.ds(r, T0), :], sem_x.at[i, half])

        def cp_gu(c, which):
            src = wg_hbm if which == 0 else wu_hbm
            return pltpu.make_async_copy(src.at[:, pl.ds(c * FC, FC)], rgu.at[c % 2, which, pl.ds(0, D), :], sem_gu.at[c % 2, which])

        def cp_d(c):
            return pltpu.make_async_copy(wd_hbm.at[pl.ds(c * FC, FC), :], rd.at[c % 2, pl.ds(0, FC), :], sem_d.at[c % 2])

        def cp_q(m):
            return pltpu.make_async_copy(wqkv_hbm.at[:, pl.ds(m * D, D)], rq.at[m, pl.ds(0, D), :], sem_q.at[m])

        def cp_o(j):
            return pltpu.make_async_copy(wo_hbm.at[:, pl.ds(j * NL, NL)], ro.at[j, pl.ds(0, D // 2), :].bitcast(BF16), sem_o.at[j])

        def cp_out(i, half):
            r = half * HS + i * T3
            return pltpu.make_async_copy(obuf.at[i % 2, half], out_hbm.at[pl.ds(r, T3), :], sem_out.at[i % 2, half])

        def zero(i):
            return i % 2 + (i + 1) % 2 - 1

        def own_block(pred, fn):
            def body(_, c):
                fn()
                return c
            lax.fori_loop(0, pred.astype(jnp.int32), body, 0)

        def anchor(dst, row, val, z):
            if val is not None and z is not None:
                r = pl.multiple_of(row + z * 16, 8)
                dst[pl.ds(r, 8), pl.ds(0, NL)] = val[0:8, 0:NL].astype(dst.dtype)

        def store_a_ops(dst, r, top, bot):
            for kc in range(KC):
                ops = _a_ops(top[kc], top[KC + kc], bot[kc], bot[KC + kc])
                for i in range(7):
                    dst.at[i][pl.ds(r, 16), ch(kc)] = _pk(ops[i])

        def ln_tasks(r0, n, z):
            def xrows(r):
                return [xbuf[pl.ds(r, 16), :].astype(F32), xbuf[pl.ds(HS + r, 16), :].astype(F32)]
            items = []
            for g in range(n // 16):
                st = {}
                def s0(val, r=r0 + g * 16, st=st):
                    anchor(xbuf, S, val, z)
                    st["m"] = [jnp.sum(x, axis=-1, keepdims=True) * (1.0 / D) for x in xrows(r)]
                def s1(val, r=r0 + g * 16, st=st):
                    xc = [x - m for x, m in zip(xrows(r), st["m"])]
                    st["v"] = [jnp.sum(c * c, axis=-1, keepdims=True) * (1.0 / D) for c in xc]
                def s2(val, r=r0 + g * 16, st=st):
                    y = [(x - m) * lax.rsqrt(v + EPS) for x, m, v in zip(xrows(r), st["m"], st["v"])]
                    store_a_ops(XA, r, *[[t[:, j * NL:(j + 1) * NL] for j in range(NCH)] for t in y])
                items.append([s0, s1, s2])
            return _skew(items)

        def prep_g_tasks(slot, r0, n, z):
            def task(val, r, which):
                anchor(rgu.at[0, 0], D, val, z)
                top = rgu[slot, which, pl.ds(r, 16), :].astype(F32)
                bot = rgu[slot, which, pl.ds(KH + r, 16), :].astype(F32)
                ops = _b_ops(top[:, :NL], top[:, NL:], bot[:, :NL], bot[:, NL:])
                for i in range(7):
                    BW.at[slot, i][pl.ds(r, 16), ch(which)] = _pk(ops[i])
            return [(lambda val, r=r0 + g * 16, w=w: task(val, r, w)) for g in range(n // 16) for w in range(2)]

        def prep_d_tasks(slot, r0, n, z):
            def task(val, r, n):
                anchor(rd.at[0], FC, val, z)
                q11 = rd[slot, pl.ds(r, 16), pl.ds(n * NL, NL)].astype(F32)
                q12 = rd[slot, pl.ds(r, 16), pl.ds(KH + n * NL, NL)].astype(F32)
                q21 = rd[slot, pl.ds(NL + r, 16), pl.ds(n * NL, NL)].astype(F32)
                q22 = rd[slot, pl.ds(NL + r, 16), pl.ds(KH + n * NL, NL)].astype(F32)
                ops = _b_ops(q11, q12, q21, q22)
                for i in range(7):
                    BW.at[slot, i][pl.ds(KH + (n // 2) * NL + r, 16), ch(n % 2)] = _pk(ops[i])
            return [(lambda val, r=r0 + g * 16, c=c: task(val, r, c)) for g in range(n // 16) for c in range(KC)]

        def prep_q_tasks(slot, m, par, z):
            def perm_a(r):
                blk = rq[m, pl.ds(r, 16), :].astype(F32)
                y = [blk[:, k * NL:(k + 1) * NL] for k in range(NCH)]
                return [y[0]] + [pltpu.roll(y[k], 2 * k, 1) for k in range(1, NCH)]

            def perm_b(y):
                lane = lax.broadcasted_iota(jnp.int32, (16, NL), 1)
                sh = (((lane & 15) >> 1) - par) & 7
                u = [y[(-m_) % NCH] for m_ in range(NCH)]
                b0, b1, b2 = (sh & 1) != 0, (sh & 2) != 0, (sh & 4) != 0
                v = {m_: jnp.where(b0, u[(m_ - 1) % NCH], u[m_]) for m_ in (0, 2, 4, 6)}
                v = {m_: jnp.where(b1, v[(m_ - 2) % NCH], v[m_]) for m_ in (0, 2, 4, 6)}
                v = {m_: jnp.where(b2, v[(m_ - 4) % NCH], v[m_]) for m_ in (0, 2, 4, 6)}
                return [pltpu.roll(v[m_], (2 * NL - 2 * m_ - 2 * par) % NL, 1) for m_ in (0, 2, 4, 6)]

            items = []
            for g in range(KH // 16):
                st = {}
                for half in range(2):
                    def s0(val, r=half * KH + g * 16, st=st, half=half):
                        anchor(rq.at[0], D, val, z)
                        st["a", half] = perm_a(r)
                    def s1(val, st=st, half=half):
                        st["b", half] = perm_b(st["a", half])
                    def s2(val, r=g * 16, st=st):
                        top, bot = st["b", 0], st["b", 1]
                        for n in range(2):
                            ops = _b_ops(top[n], top[2 + n], bot[n], bot[2 + n])
                            for i in range(7):
                                BW.at[2 + slot, i][pl.ds(r, 16), ch(n)] = _pk(ops[i])
                    items.append([s0, s1] + ([s2] if half else []))
            return _skew(items)

        def prep_o_tasks(n, z):
            def task(val, jj, a, b):
                if val is not None:
                    anchor(ro.at[0], D // 2, pltpu.bitcast(val[0:8, 0:NL], U32), z)
                def rows(j, c):
                    return pltpu.bitcast(ro[c, pl.ds(16 * a + 8 * b + j, 8, stride=64), :], BF16).astype(F32)
                ops = _b_ops(rows(jj, n), rows(jj, KC + n), rows(KC + jj, n), rows(KC + jj, KC + n))
                r = jj * NL + 32 * a + 16 * b
                for i in range(7):
                    BW.at[4 + n // 2, i][pl.ds(r, 16), ch(n % 2)] = _pk(ops[i])
            return [(lambda val, jj=jj, a=a, b=b: task(val, jj, a, b))
                    for jj in range(KC) for a in range(4) for b in range(2)]

        def attn_logits(r0, masked):
            lane = lax.broadcasted_iota(jnp.int32, (8, NL), 1)
            odd = (lane & 1) != 0
            hi = (lane & 16) != 0
            qs = [qkv[j, pl.ds(r0 + HALO, 8), :] for j in range(NCH)]
            ls = []
            for w in range(W):
                a = qs[0] * qkv[NCH, pl.ds(r0 + HALO - DIL * w, 8), :]
                for j in range(1, NCH):
                    a = a + qs[j] * qkv[NCH + j, pl.ds(r0 + HALO - DIL * w, 8), :]
                ls.append(a)
            ls = [a + jnp.where(odd, pltpu.roll(a, 1, 1), pltpu.roll(a, NL - 1, 1)) for a in ls]
            ls = [a + jnp.where(hi, pltpu.roll(a, 16, 1), pltpu.roll(a, NL - 16, 1)) for a in ls]
            if masked:
                pos = r0 + lax.broadcasted_iota(jnp.int32, (8, NL), 0)
                ls = [ls[0]] + [jnp.where(pos >= DIL * w, ls[w], NEG) for w in range(1, W)]
            m = ls[0]
            for w in range(1, W):
                m = jnp.maximum(m, ls[w])
            ps = [jnp.exp2((l - m) * EXP2_SCALE) for l in ls]
            den = ps[0]
            for w in range(1, W):
                den = den + ps[w]
            inv = 1.0 / den
            return [p * inv for p in ps]

        def attn_pv(r0, ps):
            outs = []
            for j in range(NCH):
                a = ps[0] * qkv[2 * NCH + j, pl.ds(r0 + HALO, 8), :]
                for w in range(1, W):
                    a = a + ps[w] * qkv[2 * NCH + j, pl.ds(r0 + HALO - DIL * w, 8), :]
                outs.append(a)
            return outs

        def attn_tasks(t0, z):
            tasks = []
            for g in range(AP // 16):
                st = {}
                r = t0 + g * 16
                for k, (base, masked) in enumerate(((r, g == 0), (r + 8, g == 0), (HS + r, False), (HS + r + 8, False))):
                    def ta(val, base=base, masked=masked, st=st):
                        anchor(qkv.at[0], 0, val, z)
                        st["p"] = attn_logits(base, masked)
                    def tb(val, base=base, k=k, st=st, r=r):
                        anchor(qkv.at[0], 0, val, z)
                        st[k] = attn_pv(base, st["p"])
                        if k == 3:
                            top = [jnp.concatenate([st[0][j], st[1][j]], axis=0) for j in range(NCH)]
                            bot = [jnp.concatenate([st[2][j], st[3][j]], axis=0) for j in range(NCH)]
                            store_a_ops(OA, r, top, bot)
                    tasks += [ta, tb]
            return tasks

        def lhs(ref, i, r0, m):
            return ref[i, pl.ds(r0, m), :]

        def gelu2(g, u):
            t = jnp.tanh(g * (GELU_C0 + GELU_C1 * (g * g)))
            p = g * u
            return p + p * t

        def up_phase(slot, r0, m):
            g, h = {}, {}
            def put(i, v):
                HA[pl.ds(r0, m), ch(i)] = _pk(v)
            def fin_u(k, u):
                h[k] = gelu2(g[k], u)
                if k == 3:
                    put(1, h[2] + h[3]); put(3, h[3])
                elif k == 1:
                    put(6, h[1] - h[3])
                elif k == 0:
                    put(0, h[0] + h[3]); put(2, h[0]); put(4, h[0] + h[1]); put(5, h[2] - h[0])
            yield from _strassen(lambda i: _dot(lhs(XA, i, r0, m), BW[slot, i, pl.ds(0, KH), ch(0)]), g.__setitem__, m)
            yield from _strassen(lambda i: _dot(lhs(XA, i, r0, m), BW[slot, i, pl.ds(0, KH), ch(1)]), fin_u, m)

        def down_phase(slot, r0, m, first):
            for i in range(7):
                w = jnp.concatenate([BW[slot, i, pl.ds(KH, NL), :], BW[slot, i, pl.ds(KH + NL, NL), :]], axis=1)
                d = _dot(HA[pl.ds(r0, m), ch(i)], w)
                if first:
                    P[i, pl.ds(r0, m), :] = d
                else:
                    P[i, pl.ds(r0, m), :] += d
                yield m, d

        def ffn_rows(slot, r0, nrows, first):
            m = min(RH, nrows)
            for s in range(nrows // m):
                yield from up_phase(slot, r0 + s * m, m)
            for s in range(nrows // m):
                yield from down_phase(slot, r0 + s * m, m, first)

        with scope("start"):
            cp_x(0, 0).start(); cp_x(0, 1).start()
            cp_gu(0, 0).start(); cp_gu(0, 1).start()
            cp_x(0, 0).wait(); cp_x(0, 1).wait()
            if NT0 > 1:
                cp_x(1, 0).start(); cp_x(1, 1).start()
            cp_d(0).start()

            def ln0(g, c):
                for t in ln_tasks(pl.multiple_of(g * 32, 32), 32, None):
                    t(None)
                return c
            lax.fori_loop(0, T0 // 32, ln0, 0)
            cp_gu(0, 0).wait(); cp_gu(0, 1).wait()
            for i in range(2, NT0):
                cp_x(i, 0).start(); cp_x(i, 1).start()

            def pg0(g, c):
                for t in prep_g_tasks(0, pl.multiple_of(g * 32, 32), 32, None):
                    t(None)
                return c
            lax.fori_loop(0, KH // 32, pg0, 0)
            cp_d(0).wait()
            cp_q(0).start()
            cp_gu(1, 0).start(); cp_gu(1, 1).start()
            for t in prep_d_tasks(0, 0, NL, None):
                t(None)

        def p0_body(i, c):
            own_block(i >= 0, lambda: (cp_x(i + 1, 0).wait(), cp_x(i + 1, 1).wait()))
            own_block(i == NT0 - 3, lambda: (cp_d(1).start(), [cp_o(j).start() for j in range(NCH)]))
            own_block(i == NT0 - 2, lambda: cp_q(1).start())
            r0 = pl.multiple_of(i * T0, T0)
            _emit(LAG, ffn_rows(0, r0, T0, True), 21 * T0, (0.0, 0.9, ln_tasks(r0 + T0, T0, zero(i))))
            return zero(i)
        with scope("p0"):
            z0 = lax.fori_loop(0, NT0 - 1, p0_body, 0)
        with scope("p0_last"):
            cp_q(0).wait()
            cp_q(2).start()
            cp_gu(2, 0).start(); cp_gu(2, 1).start(); cp_d(2).start()
            _emit(LAG, ffn_rows(0, HS - T0, T0, True), 21 * T0, (0.0, 0.9, prep_q_tasks(0, 0, 0, z0)))

        def p1_body(b, c):
            own_block(b == 0, lambda: (cp_gu(1, 0).wait(), cp_gu(1, 1).wait(), cp_d(1).wait(),
                                       [cp_o(j).wait() for j in range(NCH)]))
            own_block(b == 1, lambda: cp_q(1).wait())
            own_block(b == 3, lambda: cp_q(2).wait())
            m = b // 2
            par = b % 2

            def main():
                for s in range(HS // RH):
                    r0 = s * RH
                    for n in range(2):
                        def fin(k, v):
                            j = m * NCH + par + 2 * n + 4 * (k % 2)
                            qkv[j, pl.ds(HALO + (k // 2) * HS + r0, RH), :] = v
                        yield from _strassen(lambda i: _dot(lhs(XA, i, r0, RH), BW[2 + par, i, pl.ds(0, KH), ch(n)]), fin, RH)
            piece = jnp.clip(b - 2, 0, 3)
            z = zero(b)
            _emit(LAG, main(), 14 * HS,
                  (0.0, 0.95, prep_q_tasks(1 - par, jnp.minimum((b + 1) // 2, 2), 1 - par, z)),
                  (0.0, 0.95, prep_g_tasks(1, pl.multiple_of(piece * (KH // 4), KH // 4), KH // 4, z)),
                  (0.0, 0.95, prep_d_tasks(1, pl.multiple_of(piece * 32, 32), 32, z)),
                  (0.0, 0.95, prep_o_tasks(piece, z)))
            return c
        with scope("p1"):
            lax.fori_loop(0, 6, p1_body, 0)
        with scope("p1_tail"):
            for j in range(NCH, 3 * NCH):
                qkv[j, 0:HALO, :] = jnp.broadcast_to(qkv[j, HALO:HALO + 1, :], (HALO, NL))

        def p2_body(c, carry):
            own_block(c + 1 < NC, lambda: (cp_gu(c + 1, 0).wait(), cp_gu(c + 1, 1).wait(), cp_d(c + 1).wait()))
            own_block(c + 2 < NC, lambda: (cp_gu(c + 2, 0).start(), cp_gu(c + 2, 1).start(), cp_d(c + 2).start()))
            t0 = pl.multiple_of(jnp.minimum((c - 1) * AP, HS - AP), 16)
            cur = c % 2
            z = zero(c)
            _emit(LAG, ffn_rows(cur, 0, HS, False), 21 * HS,
                  (0.0, 0.97, prep_g_tasks(1 - cur, 0, KH, z) + prep_d_tasks(1 - cur, 0, NL, z)),
                  (0.0, 0.95, attn_tasks(t0, z)))
            return carry
        with scope("p2"):
            lax.fori_loop(1, NC, p2_body, 0)

        def p3_body(t, carry):
            @pl.when(t >= 2)
            def _():
                cp_out(t - 2, 0).wait(); cp_out(t - 2, 1).wait()
            slot = t % 2
            m = min(RH, T3)

            def main():
                for s in range(T3 // m):
                    r0 = pl.multiple_of(t * T3 + s * m, m)
                    for n in range(KC):
                        def pq(i):
                            return P[i, pl.ds(r0, m), pl.ds(n * NL, NL)]
                        def fin(k, sq):
                            if k == 0:
                                f = pq(0) + pq(3) - pq(4) + pq(6)
                            elif k == 1:
                                f = pq(2) + pq(4)
                            elif k == 2:
                                f = pq(1) + pq(3)
                            else:
                                f = pq(0) - pq(1) + pq(2) + pq(5)
                            half, col = k // 2, (k % 2) * KH + n * NL
                            z = f * 0.25
                            gate = z + z * jnp.tanh(z)
                            x = xbuf[pl.ds(half * HS + r0, m), pl.ds(col, NL)].astype(F32)
                            obuf.at[slot, half][pl.ds(s * m, m), pl.ds(col, NL)] = (x + sq * gate).astype(BF16)
                        yield from _strassen(lambda i: _dot(lhs(OA, i, r0, m), BW[4 + n // 2, i, pl.ds(0, KH), ch(n % 2)]), fin, m)
            _emit(LAG, main(), 28 * T3)
            cp_out(t, 0).start(); cp_out(t, 1).start()
            return carry
        with scope("p3"):
            lax.fori_loop(0, NT3, p3_body, 0)
        with scope("end"):
            for t in range(max(NT3 - 2, 0), NT3):
                cp_out(t, 0).wait(); cp_out(t, 1).wait()

    def fn(A_x, A_wqkv, A_wo, B_x, B_w_gate, B_w_up, B_w_down):
        x = A_x.reshape(S, D)
        anyspec = pl.BlockSpec(memory_space=pl.ANY)
        out = pl.pallas_call(
            kernel,
            in_specs=[anyspec] * 6,
            out_specs=anyspec,
            out_shape=jax.ShapeDtypeStruct((S, D), BF16),
            scratch_shapes=[
                pltpu.VMEM((S + 16, D), BF16),
                pltpu.VMEM((7, HS // 2, KH), U32),
                pltpu.VMEM((3 * NCH, HALO + S, NL), F32),
                pltpu.VMEM((7, HS // 2, KH), U32),
                pltpu.VMEM((7, HS, KH), F32),
                pltpu.VMEM((HS // 2, 7 * NL), U32),
                pltpu.VMEM((6, 7, (KH + 2 * NL) // 2, 2 * NL), U32),
                pltpu.VMEM((2, 2, D + 16, FC), BF16),
                pltpu.VMEM((2, FC + 16, D), BF16),
                pltpu.VMEM((3, D + 16, D), BF16),
                pltpu.VMEM((NCH, D // 2 + 8, NL), U32),
                pltpu.VMEM((2, 2, T3, D), BF16),
                pltpu.SemaphoreType.DMA((NT0, 2)),
                pltpu.SemaphoreType.DMA((2, 2)),
                pltpu.SemaphoreType.DMA((2,)),
                pltpu.SemaphoreType.DMA((3,)),
                pltpu.SemaphoreType.DMA((NCH,)),
                pltpu.SemaphoreType.DMA((2, 2)),
            ],
            compiler_params=pltpu.CompilerParams(vmem_limit_bytes=120 * 2 ** 20),
        )(x, A_wqkv, A_wo, B_w_gate, B_w_up, B_w_down)
        return out.reshape(1, S, D)
    return jax.jit(fn)


_IMPL = make(RH=256, LAG=1)


@jax.jit
def pallas_recurrent_scan__sliding_local_dilated__geglu_ffn__prompt_kernel(
    A_x: jax.Array,
    A_wqkv: jax.Array,
    A_wo: jax.Array,
    B_x: jax.Array,
    B_w_gate: jax.Array,
    B_w_up: jax.Array,
    B_w_down: jax.Array,
):
    return _IMPL(A_x, A_wqkv, A_wo, B_x, B_w_gate, B_w_up, B_w_down)
```

```python
import contextlib
import math

import jax
import jax.numpy as jnp
from jax import lax
import jax.experimental.pallas as pl
import jax.experimental.pallas.tpu as pltpu

S, D, F = 2048, 1024, 3584
H, DH, W, DIL = 32, 32, 8, 2
NL = 128
NCH = D // NL
HS = S // 2
KH = D // 2
KC = KH // NL
FC = 256
NC = F // FC
HALO = 16
F32, BF16, U32 = jnp.float32, jnp.bfloat16, jnp.uint32
EPS = 1e-5
GELU_C0 = math.sqrt(2.0 / math.pi)
GELU_C1 = GELU_C0 * 0.044715
EXP2_SCALE = (DH ** -0.5) * math.log2(math.e)
NEG = -1e9 / (DH ** -0.5)


def _a_ops(a11, a12, a21, a22):
    return [a11 + a22, a21 + a22, a11, a22, a11 + a12, a21 - a11, a12 - a22]


def _b_ops(b11, b12, b21, b22):
    return [b11 + b22, b11, b12 - b22, b21 - b11, b22, b11 + b12, b21 + b22]


def _dot(a, b):
    return jnp.dot(a, b, preferred_element_type=F32)


def _pk(x):
    return x.astype(BF16)


def _strassen(prod, fin, room):
    m1 = prod(1)
    yield room[0], m1
    m3 = prod(3)
    fin(2, m1 + m3)
    yield room[1], m3
    m0 = prod(0)
    t11 = m3 + m0
    t22 = m0 - m1
    yield room[2], m0
    m5 = prod(5)
    t22 = t22 + m5
    yield room[3], m5
    m2 = prod(2)
    fin(3, t22 + m2)
    yield room[4], m2
    m4 = prod(4)
    fin(1, m2 + m4)
    t11 = t11 - m4
    yield room[5], m4
    m6 = prod(6)
    fin(0, t11 + m6)
    yield room[6], m6


def _emit(lag, main, total, *sides):
    done = [0] * len(sides)
    acc = 0

    def flush(frac, val):
        due = []
        for k, (f0, f1, tasks) in enumerate(sides):
            want = len(tasks) if frac >= f1 else int(max(0.0, (frac - f0) / (f1 - f0)) * len(tasks) + 0.5)
            n = min(want, len(tasks)) - done[k]
            due += [((j + 0.5) / n, k, tasks[done[k] + j]) for j in range(n)]
            done[k] += max(n, 0)
        due.sort(key=lambda e: e[:2])
        for j, (_, _, task) in enumerate(due):
            if val is None:
                task(None)
            else:
                r = (val.shape[0] // 8) * j // len(due) * 8
                task(val[r:r + 8, 0:NL])
    hist = [(0, None)] * lag
    for item in main:
        hist.append(item)
        room, val = hist.pop(0)
        acc += room
        if room:
            flush(acc / total, val)
    acc += sum(h[0] for h in hist)
    assert acc == total, (acc, total)
    flush(2.0, hist[-1][1] if hist else val)


def _skew(stages_per_item, flat=False):
    n = len(stages_per_item)
    depth = max(len(st) for st in stages_per_item)
    tasks = []
    for t in range(n + depth - 1):
        group = [stages_per_item[t - k][k] for k in range(depth) if 0 <= t - k < n and k < len(stages_per_item[t - k])]
        if flat:
            tasks += [g for g in group if g.__name__ != "<lambda>"]
        else:
            tasks.append(lambda val, group=group: [g(val) for g in group])
    return tasks


def make(EXP='', P1A=0.44, P1B=0.0, NOBC=True, AGAP=4, LN0=64, RH=256, T0=128, T3=256, AP=80, LAG=1, RG=(2, 2, 2, 2, 2, 2, 2), RU=(2, 1, 2, 2, 1, 1, 0), RD=2, scopes=False):
    RF = sum(RG) + sum(RU) + 7 * RD
    NT0 = HS // T0
    NT3 = HS // T3
    assert AP % 16 == 0 and AP * (NC - 1) >= HS

    def scope(name):
        return jax.named_scope(name) if scopes else contextlib.nullcontext()

    def kernel(x_hbm, wqkv_hbm, wo_hbm, wg_hbm, wu_hbm, wd_hbm, out_hbm,
               xbuf, XA, qkv, OA, P, HA, BW, BQ, BO,
               rgu, rd, rq, ro, obuf, osc,
               sem_x, sem_gu, sem_d, sem_q, sem_o, sem_out):

        XA, OA, HA, BW, BQ, BO = [r.bitcast(BF16) for r in (XA, OA, HA, BW, BQ, BO)]

        def ch(n):
            return pl.ds(n * NL, NL) if isinstance(n, int) else pl.ds(pl.multiple_of(n * NL, NL), NL)

        def cp_x(i, half):
            r = half * HS + i * T0
            return pltpu.make_async_copy(x_hbm.at[pl.ds(r, T0), :], xbuf.at[pl.ds(r, T0), :], sem_x.at[i, half])

        def cp_gu(c, which):
            src = wg_hbm if which == 0 else wu_hbm
            return pltpu.make_async_copy(src.at[:, pl.ds(c * FC, FC)], rgu.at[c % 2, which, pl.ds(0, D), :], sem_gu.at[c % 2, which])

        def cp_d(c):
            return pltpu.make_async_copy(wd_hbm.at[pl.ds(c * FC, FC), :], rd.at[c % 2, pl.ds(0, FC), :], sem_d.at[c % 2])

        class cp_q:
            def __init__(self, m):
                self.cps = [pltpu.make_async_copy(wqkv_hbm.at[:, pl.ds((m * NCH + k) * NL, NL)],
                                                  rq.at[m * NCH + k, pl.ds(0, D // 2), :].bitcast(BF16),
                                                  sem_q.at[m, k]) for k in range(NCH)]
            def start(self):
                for c in self.cps:
                    c.start()
            def wait(self):
                for c in self.cps:
                    c.wait()

        def cp_o(j):
            return pltpu.make_async_copy(wo_hbm.at[:, pl.ds(j * NL, NL)], ro.at[j, pl.ds(0, D // 2), :].bitcast(BF16), sem_o.at[j])

        def cp_out(i, half):
            r = half * HS + i * T3
            return pltpu.make_async_copy(obuf.at[i % 2, half], out_hbm.at[pl.ds(r, T3), :], sem_out.at[i % 2, half])

        def zero(i):
            return i % 2 + (i + 1) % 2 - 1

        def own_block(pred, fn):
            def body(_, c):
                fn()
                return c
            lax.fori_loop(0, pred.astype(jnp.int32), body, 0)

        def anchor(dst, row, val, z):
            if val is not None and z is not None:
                r = pl.multiple_of(row + z * 16, 8)
                dst[pl.ds(r, 8), pl.ds(0, NL)] = pltpu.bitcast(val, U32) if dst.dtype == U32 else val.astype(dst.dtype)

        def store_a_ops(dst, r, top, bot):
            for kc in range(KC):
                ops = _a_ops(top[kc], top[KC + kc], bot[kc], bot[KC + kc])
                for i in range(7):
                    dst.at[i][pl.ds(r, 16), ch(kc)] = _pk(ops[i])

        def ln_tasks(r0, n, z):
            def xrow(r):
                return xbuf[pl.ds(r, 16), :].astype(F32)
            items = []
            for g in range(n // 16):
                st = {}
                for half in range(2):
                    def s0(val, r=half * HS + r0 + g * 16, st=st, half=half):
                        anchor(xbuf, S, val, z)
                        st["m", half] = jnp.sum(xrow(r), axis=-1, keepdims=True) * (1.0 / D)
                    def s1(val, r=half * HS + r0 + g * 16, st=st, half=half):
                        anchor(xbuf, S, val, z)
                        c = xrow(r) - st["m", half]
                        st["v", half] = lax.rsqrt(jnp.sum(c * c, axis=-1, keepdims=True) * (1.0 / D) + EPS)
                    def s2(val, r=r0 + g * 16, st=st, half=half):
                        for kc in (2 * half, 2 * half + 1):
                            anchor(xbuf, S, val, z)
                            q = [(xbuf[pl.ds(h * HS + r, 16), ch(c)].astype(F32) - st["m", h]) * st["v", h]
                                 for h in range(2) for c in (kc, KC + kc)]
                            ops = _a_ops(*q)
                            for i in range(7):
                                XA.at[i][pl.ds(r, 16), ch(kc)] = _pk(ops[i])
                    nop = lambda val: None
                    items.append([s0, nop, s1, nop, nop, s2] if half == 0 else [s0, nop, s1, nop, s2])
            flat = _skew(items, flat=True)
            return flat

        def prep_g_tasks(slot, r0, n, z):
            def task(val, r, which):
                anchor(rgu.at[0, 0], D, val, z)
                top = rgu[slot, which, pl.ds(r, 16), :].astype(F32)
                bot = rgu[slot, which, pl.ds(KH + r, 16), :].astype(F32)
                ops = _b_ops(top[:, :NL], top[:, NL:], bot[:, :NL], bot[:, NL:])
                for i in range(7):
                    BW.at[slot, i][pl.ds(r, 16), ch(which)] = _pk(ops[i])
            return [(lambda val, r=r0 + g * 16, w=w: task(val, r, w)) for g in range(n // 16) for w in range(2)]

        def prep_d_tasks(slot, r0, n, z):
            def task(val, r, n):
                anchor(rd.at[0], FC, val, z)
                q11 = rd[slot, pl.ds(r, 16), pl.ds(n * NL, NL)].astype(F32)
                q12 = rd[slot, pl.ds(r, 16), pl.ds(KH + n * NL, NL)].astype(F32)
                q21 = rd[slot, pl.ds(NL + r, 16), pl.ds(n * NL, NL)].astype(F32)
                q22 = rd[slot, pl.ds(NL + r, 16), pl.ds(KH + n * NL, NL)].astype(F32)
                ops = _b_ops(q11, q12, q21, q22)
                for i in range(7):
                    BW.at[slot, i][pl.ds(KH + (n // 2) * NL + r, 16), ch(n % 2)] = _pk(ops[i])
            return [(lambda val, r=r0 + g * 16, c=c: task(val, r, c)) for g in range(n // 16) for c in range(KC)]

        def prep_q_tasks(m, par, n, z):
            def perm_a(r):
                y = [rq[m * NCH + k, pl.ds(r // 2, 8), :] for k in range(NCH)]
                return [y[0]] + [pltpu.roll(y[k], 2 * k, 1) for k in range(1, NCH)]

            def perm_b(y):
                lane = lax.broadcasted_iota(jnp.int32, (8, NL), 1)
                sh = (((lane & 15) >> 1) - par) & 7
                u = [y[(-m_) % NCH] for m_ in range(NCH)]
                b0, b1, b2 = (sh & 1) != 0, (sh & 2) != 0, (sh & 4) != 0
                out = (2 * n, 2 * n + 4)
                v = {m_: jnp.where(b0, u[(m_ - 1) % NCH], u[m_]) for m_ in (0, 2, 4, 6)}
                v = {m_: jnp.where(b1, v[(m_ - 2) % NCH], v[m_]) for m_ in out}
                v = {m_: jnp.where(b2, v[(m_ - 4) % NCH], v[m_]) for m_ in out}
                return [pltpu.roll(v[m_], (2 * NL - 2 * m_ - 2 * par) % NL, 1) for m_ in out]

            def wide(w):
                return pltpu.bitcast(w, BF16).astype(F32)

            items = []
            for g in range(KH // 16):
                st = {}
                for half in range(2):
                    def s0(val, r=half * KH + g * 16, st=st, half=half):
                        anchor(rq.at[0], D // 2, val, z)
                        st["a", half] = perm_a(r)
                    def s1(val, st=st, half=half):
                        st["b", half] = perm_b(st["a", half])
                    def s2(val, r=g * 16, st=st):
                        top, bot = st["b", 0], st["b", 1]
                        ops = _b_ops(wide(top[0]), wide(top[1]), wide(bot[0]), wide(bot[1]))
                        for i in range(7):
                            BQ.at[i][pl.ds(r, 16), ch(n)] = _pk(ops[i])
                    items.append([s0, s1] + ([s2] if half else []))
            return _skew(items)

        def prep_o_tasks(n, z):
            tasks = []
            for jj in range(KC):
                for a in range(4):
                    for b in range(2):
                        st = []
                        for k, (j, c) in enumerate(((jj, n), (jj, KC + n), (KC + jj, n), (KC + jj, KC + n))):
                            def task(val, k=k, j=j, c=c, st=st, start=16 * a + 8 * b, r=jj * NL + 32 * a + 16 * b):
                                anchor(ro.at[0], D // 2, val, z)
                                st.append(ro[c, pl.ds(start + j, 8, stride=64), :])
                                if k == 3:
                                    ops = _b_ops(*[pltpu.bitcast(w, BF16).astype(F32) for w in st])
                                    for i in range(7):
                                        BO.at[i][pl.ds(r, 16), ch(n)] = _pk(ops[i])
                            tasks.append(task)
            return tasks

        def attn_unit(r0, masked, slot, z):
            st = {}

            def shifted(plane):
                return [qkv[plane, pl.ds(r0 + HALO + 8 - DIL * k, 8), :] for k in range(12)]

            def logits(val, j):
                anchor(qkv.at[0], 0, val, z)
                q = [qkv[j, pl.ds(r0 + HALO + 8 * g, 8), :] for g in range(2)]
                kk = shifted(NCH + j)
                for g in range(2):
                    for w in range(W):
                        t = q[g] * kk[w + 4 - 4 * g]
                        st[g, w] = t if j == 0 else st[g, w] + t
                if j == NCH - 1:
                    softmax()

            def softmax():
                lane = lax.broadcasted_iota(jnp.int32, (8, NL), 1)
                odd = (lane & 1) != 0
                hi = (lane & 16) != 0
                keys = [(g, w) for g in range(2) for w in range(W)]
                for k in keys:
                    a = st[k]
                    st[k] = a + jnp.where(odd, pltpu.roll(a, 1, 1), pltpu.roll(a, NL - 1, 1))
                for k in keys:
                    a = st[k]
                    st[k] = a + jnp.where(hi, pltpu.roll(a, 16, 1), pltpu.roll(a, NL - 16, 1))
                for g in range(2):
                    ls = [st[g, w] for w in range(W)]
                    if masked:
                        pos = r0 + 8 * g + lax.broadcasted_iota(jnp.int32, (8, NL), 0)
                        ls = [ls[0]] + [jnp.where(pos >= DIL * w, ls[w], NEG) for w in range(1, W)]
                    m = ls[0]
                    for w in range(1, W):
                        m = jnp.maximum(m, ls[w])
                    ps = [jnp.exp2((l - m) * EXP2_SCALE) for l in ls]
                    den = ps[0]
                    for w in range(1, W):
                        den = den + ps[w]
                    inv = 1.0 / den
                    for w in range(W):
                        st[g, w] = ps[w] * inv

            def pv(val, j):
                anchor(qkv.at[0], 0, val, z)
                vv = shifted(2 * NCH + j)
                for g in range(2):
                    a = st[g, 0] * vv[4 - 4 * g]
                    for w in range(1, W):
                        a = a + st[g, w] * vv[w + 4 - 4 * g]
                    osc[slot, j, pl.ds(8 * g, 8), :] = a

            gap = [lambda val: None] * AGAP
            return ([(lambda val, j=j: logits(val, j)) for j in range(NCH)] + gap
                    + [(lambda val, j=j: pv(val, j)) for j in range(NCH)])

        def attn_tasks(t0, z):
            tasks = []
            for g in range(AP // 16):
                r = t0 + g * 16
                tasks += attn_unit(r, g == 0, 2 * g, z) + attn_unit(HS + r, False, 2 * g + 1, z)
                def oa(val, kc, g=g, r=r):
                    ops = _a_ops(osc[2 * g, kc], osc[2 * g, KC + kc], osc[2 * g + 1, kc], osc[2 * g + 1, KC + kc])
                    for i in range(7):
                        OA.at[i][pl.ds(r, 16), ch(kc)] = _pk(ops[i])
                tasks += [(lambda val, kc=kc, oa=oa: oa(val, kc)) for kc in range(KC)]
            return tasks

        def lhs(ref, i, r0, m):
            return ref[i, pl.ds(r0, m), :]

        def gelu2(g, u):
            t = jnp.tanh(g * (GELU_C0 + GELU_C1 * (g * g)))
            p = g * u
            return p + p * t

        def up_phase(slot, r0, m):
            g, h = {}, {}
            def put(i, v):
                HA[pl.ds(r0, m), ch(i)] = _pk(v)
            def fin_u(k, u):
                h[k] = gelu2(g[k], u)
                if k == 3:
                    put(1, h[2] + h[3]); put(3, h[3])
                elif k == 1:
                    put(6, h[1] - h[3])
                elif k == 0:
                    put(0, h[0] + h[3]); put(2, h[0]); put(4, h[0] + h[1]); put(5, h[2] - h[0])
            yield from _strassen(lambda i: _dot(lhs(XA, i, r0, m), BW[slot, i, pl.ds(0, KH), ch(0)]), g.__setitem__, RG)
            yield from _strassen(lambda i: _dot(lhs(XA, i, r0, m), BW[slot, i, pl.ds(0, KH), ch(1)]), fin_u, RU)

        def down_phase(slot, r0, m, first):
            for i in range(7):
                w = jnp.concatenate([BW[slot, i, pl.ds(KH, NL), :], BW[slot, i, pl.ds(KH + NL, NL), :]], axis=1)
                d = _dot(HA[pl.ds(r0, m), ch(i)], w)
                if first:
                    P[i, pl.ds(r0, m), :] = d
                else:
                    P[i, pl.ds(r0, m), :] += d
                yield RD, d

        def ffn_rows(slot, r0, nrows, first):
            m = min(RH, nrows)
            for s in range(nrows // m):
                yield from up_phase(slot, r0 + s * m, m)
            for s in range(nrows // m):
                yield from down_phase(slot, r0 + s * m, m, first)

        with scope("start"):
            groups = [[cp_x(0, 0), cp_x(0, 1)], [cp_gu(0, 0)], [cp_gu(0, 1)], [cp_d(0)]]
            groups += [[cp_x(i, 0), cp_x(i, 1)] for i in range(1, NT0)]
            groups += [[cp_q(0)], [cp_gu(1, 0), cp_gu(1, 1), cp_d(1)], [cp_o(j) for j in range(NCH)],
                       [cp_q(1)], [cp_q(2)]]

            def issue(k, c):
                for g, cps in enumerate(groups):
                    @pl.when(k == g)
                    def _():
                        for cp in cps:
                            cp.start()
                return c
            lax.fori_loop(0, len(groups), issue, 0)
            cp_x(0, 0).wait(); cp_x(0, 1).wait()

            def ln0(g, c):
                for t in ln_tasks(pl.multiple_of(g * LN0, LN0), LN0, None):
                    t(None)
                return c
            lax.fori_loop(0, T0 // LN0, ln0, 0)
            for which in range(2):
                cp_gu(0, which).wait()
                def pg0(g, c):
                    for t in prep_g_tasks(0, pl.multiple_of(g * 64, 64), 64, None)[which::2]:
                        t(None)
                    return c
                lax.fori_loop(0, KH // 64, pg0, 0)
            cp_d(0).wait()
            for t in prep_d_tasks(0, 0, NL, None):
                t(None)

        def p0_body(i, c):
            own_block(i >= 0, lambda: (cp_x(i + 1, 0).wait(), cp_x(i + 1, 1).wait()))
            r0 = pl.multiple_of(i * T0, T0)
            _emit(LAG, ffn_rows(0, r0, T0, True), RF * (T0 // min(RH, T0)), (0.0, 0.9, ln_tasks(r0 + T0, T0, zero(i))))
            return zero(i)
        with scope("p0"):
            z0 = lax.fori_loop(0, NT0 - 1, p0_body, 0)
        with scope("p0_last"):
            cp_q(0).wait()
            cp_gu(2, 0).start(); cp_gu(2, 1).start(); cp_d(2).start()
            _emit(LAG, ffn_rows(0, HS - T0, T0, True), RF * (T0 // min(RH, T0)), (0.0, 0.9, prep_q_tasks(0, 0, 0, z0)))

        def p1_body(b, c):
            own_block(b == 0, lambda: (cp_gu(1, 0).wait(), cp_gu(1, 1).wait(), cp_d(1).wait(),
                                       [cp_o(j).wait() for j in range(NCH)]))
            own_block(b == 1, lambda: cp_q(1).wait())
            own_block(b == 3, lambda: cp_q(2).wait())
            m = b // 2
            par = b % 2

            def main():
                for n in range(2):
                    for s in range(HS // RH):
                        r0 = s * RH
                        def fin(k, v):
                            j = m * NCH + par + 2 * n + 4 * (k % 2)
                            qkv[j, pl.ds(HALO + (k // 2) * HS + r0, RH), :] = v
                        yield from _strassen(lambda i: _dot(lhs(XA, i, r0, RH), BQ[i, :, ch(n)]), fin, (1,) * 7)
            piece = jnp.clip(b - 2, 0, 3)
            z = zero(b)
            _emit(LAG, main(), 14 * (HS // RH),
                  (0.0, P1A, prep_q_tasks(m, par, 1, z)),
                  (0.5 + P1B, 0.5 + P1A, prep_q_tasks(jnp.minimum((b + 1) // 2, 2), (b + 1) % 2, 0, z)),
                  (0.0, 0.95, prep_g_tasks(1, pl.multiple_of(piece * (KH // 4), KH // 4), KH // 4, z)),
                  (0.0, 0.95, prep_d_tasks(1, pl.multiple_of(piece * 32, 32), 32, z)),
                  (0.0, 0.95, prep_o_tasks(piece, z)))
            return c
        with scope("p1"):
            lax.fori_loop(0, 6, p1_body, 0)
        with scope("p1_tail"):
            for j in range(NCH, 3 * NCH):
                qkv[j, 0:HALO, :] = jnp.broadcast_to(qkv[j, HALO:HALO + 1, :], (HALO, NL))

        def p2_body(c, carry):
            def dma_step():
                cp_gu(c + 1, 0).wait(); cp_gu(c + 1, 1).wait(); cp_d(c + 1).wait()
                @pl.when(c + 2 < NC)
                def _():
                    cp_gu(c + 2, 0).start(); cp_gu(c + 2, 1).start(); cp_d(c + 2).start()
            own_block(c + 1 < NC, dma_step)
            t0 = pl.multiple_of(jnp.minimum((c - 1) * AP, HS - AP), 16)
            cur = c % 2
            z = zero(c)
            _emit(LAG, ffn_rows(cur, 0, HS, False), RF * (HS // RH),
                  (0.0, 0.97, (prep_g_tasks(1 - cur, 0, KH, z) + prep_d_tasks(1 - cur, 0, NL, z)) if 'noprep' not in EXP else []),
                  (0.0, 0.95, attn_tasks(t0, z) if 'noattn' not in EXP else []))
            return carry
        with scope("p2"):
            lax.fori_loop(1, NC, p2_body, 0)

        def p3_body(t, carry):
            @pl.when(t >= 2)
            def _():
                cp_out(t - 2, 0).wait(); cp_out(t - 2, 1).wait()
            slot = t % 2
            m = min(RH, T3)

            def main():
                for s in range(T3 // m):
                    r0 = pl.multiple_of(t * T3 + s * m, m)
                    for n in range(KC):
                        def pq(i):
                            return P[i, pl.ds(r0, m), pl.ds(n * NL, NL)]
                        def fin(k, sq):
                            if k == 0:
                                f = pq(0) + pq(3) - pq(4) + pq(6)
                            elif k == 1:
                                f = pq(2) + pq(4)
                            elif k == 2:
                                f = pq(1) + pq(3)
                            else:
                                f = pq(0) - pq(1) + pq(2) + pq(5)
                            half, col = k // 2, (k % 2) * KH + n * NL
                            z = f * 0.25
                            gate = z + z * jnp.tanh(z)
                            x = xbuf[pl.ds(half * HS + r0, m), pl.ds(col, NL)].astype(F32)
                            obuf.at[slot, half][pl.ds(s * m, m), pl.ds(col, NL)] = (x + sq * gate).astype(BF16)
                        yield from _strassen(lambda i: _dot(lhs(OA, i, r0, m), BO[i, :, ch(n)]), fin, (1,) * 7)
            _emit(LAG, main(), 28 * (T3 // m))
            cp_out(t, 0).start(); cp_out(t, 1).start()
            return carry
        with scope("p3"):
            lax.fori_loop(0, NT3, p3_body, 0)
        with scope("end"):
            for t in range(max(NT3 - 2, 0), NT3):
                cp_out(t, 0).wait(); cp_out(t, 1).wait()

    def fn(A_x, A_wqkv, A_wo, B_x, B_w_gate, B_w_up, B_w_down):
        x = A_x.reshape(S, D)
        anyspec = pl.BlockSpec(memory_space=pl.ANY)
        out = pl.pallas_call(
            kernel,
            in_specs=[anyspec] * 6,
            out_specs=anyspec,
            out_shape=jax.ShapeDtypeStruct((S, D), BF16),
            scratch_shapes=[
                pltpu.VMEM((S + 16, D), BF16),
                pltpu.VMEM((7, HS // 2, KH), U32),
                pltpu.VMEM((3 * NCH, HALO + S, NL), F32),
                pltpu.VMEM((7, HS // 2, KH), U32),
                pltpu.VMEM((7, HS, KH), F32),
                pltpu.VMEM((HS // 2, 7 * NL), U32),
                pltpu.VMEM((2, 7, (KH + 2 * NL) // 2, 2 * NL), U32),
                pltpu.VMEM((7, KH // 2, 2 * NL), U32),
                pltpu.VMEM((7, KH // 2, KH), U32),
                pltpu.VMEM((2, 2, D + 16, FC), BF16),
                pltpu.VMEM((2, FC + 16, D), BF16),
                pltpu.VMEM((3 * NCH, D // 2 + 8, NL), U32),
                pltpu.VMEM((NCH, D // 2 + 8, NL), U32),
                pltpu.VMEM((2, 2, T3, D), BF16),
                pltpu.VMEM((AP // 8, NCH, 16, NL), F32),
                pltpu.SemaphoreType.DMA((NT0, 2)),
                pltpu.SemaphoreType.DMA((2, 2)),
                pltpu.SemaphoreType.DMA((2,)),
                pltpu.SemaphoreType.DMA((3, NCH)),
                pltpu.SemaphoreType.DMA((NCH,)),
                pltpu.SemaphoreType.DMA((2, 2)),
            ],
            compiler_params=pltpu.CompilerParams(vmem_limit_bytes=120 * 2 ** 20, disable_bounds_checks=NOBC),
        )(x, A_wqkv, A_wo, B_w_gate, B_w_up, B_w_down)
        return out.reshape(1, S, D)
    return jax.jit(fn)


_IMPL = make(T0=128)


@jax.jit
def pallas_recurrent_scan__sliding_local_dilated__geglu_ffn__prompt_kernel(
    A_x: jax.Array,
    A_wqkv: jax.Array,
    A_wo: jax.Array,
    B_x: jax.Array,
    B_w_gate: jax.Array,
    B_w_up: jax.Array,
    B_w_down: jax.Array,
):
    return _IMPL(A_x, A_wqkv, A_wo, B_x, B_w_gate, B_w_up, B_w_down)
```

```python
import contextlib
import math

import jax
import jax.numpy as jnp
from jax import lax
import jax.experimental.pallas as pl
import jax.experimental.pallas.tpu as pltpu

S, D, F = 2048, 1024, 3584
H, DH, W, DIL = 32, 32, 8, 2
NL = 128
NCH = D // NL
HS = S // 2
KH = D // 2
KC = KH // NL
QS = S // 4
KQ = D // 4
FC = 256
NC = F // FC
HALO = 16
F32, BF16, U32 = jnp.float32, jnp.bfloat16, jnp.uint32
EPS = 1e-5
GELU_C0 = math.sqrt(2.0 / math.pi)
GELU_C1 = GELU_C0 * 0.044715
EXP2_SCALE = (DH ** -0.5) * math.log2(math.e)
NEG = -1e9 / (DH ** -0.5)


def _a_ops(a11, a12, a21, a22):
    return [a11 + a22, a21 + a22, a11, a22, a11 + a12, a21 - a11, a12 - a22]


def _b_ops(b11, b12, b21, b22):
    return [b11 + b22, b11, b12 - b22, b21 - b11, b22, b11 + b12, b21 + b22]


_A_TERMS = (((0, 0, 1), (1, 1, 1)), ((1, 0, 1), (1, 1, 1)), ((0, 0, 1),), ((1, 1, 1),),
            ((0, 0, 1), (0, 1, 1)), ((1, 0, 1), (0, 0, -1)), ((0, 1, 1), (1, 1, -1)))
_B_TERMS = (((0, 0, 1), (1, 1, 1)), ((0, 0, 1),), ((0, 1, 1), (1, 1, -1)), ((1, 0, 1), (0, 0, -1)),
            ((1, 1, 1),), ((0, 0, 1), (0, 1, 1)), ((1, 0, 1), (1, 1, 1)))
_ORDER = (1, 3, 0, 5, 2, 4, 6)
_XB_SLOT = {0: 0, 1: 1, 4: 2, 5: 3, 6: 4}


def _combine(terms, get):
    (r, c, _), *rest = terms
    v = get(r, c)
    for r, c, sign in rest:
        v = v + get(r, c) if sign > 0 else v - get(r, c)
    return v


def _dot(a, b):
    return jnp.dot(a, b, preferred_element_type=F32)


def _pk(x):
    return x.astype(BF16)


def _strassen(prod, fin, room):
    m1 = prod(1)
    yield room[0], m1
    m3 = prod(3)
    fin(2, m1 + m3)
    yield room[1], m3
    m0 = prod(0)
    t11 = m3 + m0
    t22 = m0 - m1
    yield room[2], m0
    m5 = prod(5)
    t22 = t22 + m5
    yield room[3], m5
    m2 = prod(2)
    fin(3, t22 + m2)
    yield room[4], m2
    m4 = prod(4)
    fin(1, m2 + m4)
    t11 = t11 - m4
    yield room[5], m4
    m6 = prod(6)
    fin(0, t11 + m6)
    yield room[6], m6


def _emit(lag, main, total, *sides, dyn=None, dyn_rate=0, dyn_delay=0):
    done = [0] * len(sides)
    acc = 0

    def flush(frac, val):
        due = []
        for k, (f0, f1, tasks) in enumerate(sides):
            want = len(tasks) if frac >= f1 else int(max(0.0, (frac - f0) / (f1 - f0)) * len(tasks) + 0.5)
            n = min(want, len(tasks)) - done[k]
            due += [((j + 0.5) / n, k, tasks[done[k] + j]) for j in range(n)]
            done[k] += max(n, 0)
        if dyn:
            ready = [e for e in dyn if e[0] + dyn_delay <= step[0]][:dyn_rate]
            for j, e in enumerate(ready):
                dyn.remove(e)
                due.append(((j + 0.5) / len(ready), -1, e[1]))
        due.sort(key=lambda e: e[:2])
        for j, (_, _, task) in enumerate(due):
            if val is None:
                task(None)
            else:
                r = (val.shape[0] // 8) * j // len(due) * 8
                task(val[r:r + 8, 0:NL])
    hist = [(0, None)] * lag
    step = [0]
    seen = 0
    for item in main:
        step[0] += 1
        if dyn is not None:
            for e in dyn:
                if e[0] is None:
                    e[0] = step[0]
        hist.append(item)
        room, val = hist.pop(0)
        acc += room
        if room or dyn:
            flush(acc / total, val)
    acc += sum(h[0] for h in hist)
    assert acc == total, (acc, total)
    assert not dyn
    flush(2.0, hist[-1][1] if hist else val)


def _skew(stages_per_item, flat=False):
    n = len(stages_per_item)
    depth = max(len(st) for st in stages_per_item)
    tasks = []
    for t in range(n + depth - 1):
        group = [stages_per_item[t - k][k] for k in range(depth) if 0 <= t - k < n and k < len(stages_per_item[t - k])]
        if flat:
            tasks += [g for g in group if g.__name__ != "<lambda>"]
        else:
            tasks.append(lambda val, group=group: [g(val) for g in group])
    return tasks


def make(EXP='', RH2=64, LAG2=4, PG0=1.5, R2L=(2,) * 7, R2H=(2, 0, 2, 2, 0, 0, 0), RD2=2, HG=16, DRATE=1, DDELAY=4, P1A=0.44, P1B=0.0, NOBC=True, AGAP=4, LN0=64, RH=256, T0=128, T3=256, AP=80, LAG=1, RG=(2, 2, 2, 2, 2, 2, 2), RU=(2, 1, 2, 2, 1, 1, 0), RD=2, scopes=False):
    RF = sum(RG) + sum(RU) + 7 * RD
    NT0 = HS // T0
    NT3 = HS // T3
    assert AP % 16 == 0 and AP * (NC - 1) >= HS

    def scope(name):
        return jax.named_scope(name) if scopes else contextlib.nullcontext()

    def kernel(x_hbm, wqkv_hbm, wo_hbm, wg_hbm, wu_hbm, wd_hbm, out_hbm,
               xbuf, XA, qkv, OA, P, HA, BW, BQ, BO, Y, XB, BG, HF,
               rgu, rd, rq, ro, obuf, osc,
               sem_x, sem_gu, sem_d, sem_q, sem_o, sem_out):

        XA, OA, HA, BW, BQ, BO, XB, BG = [r.bitcast(BF16) for r in (XA, OA, HA, BW, BQ, BO, XB, BG)]

        def ch(n):
            return pl.ds(n * NL, NL) if isinstance(n, int) else pl.ds(pl.multiple_of(n * NL, NL), NL)

        def cp_x(i, half):
            r = half * HS + i * T0
            return pltpu.make_async_copy(x_hbm.at[pl.ds(r, T0), :], xbuf.at[pl.ds(r, T0), :], sem_x.at[i, half])

        def cp_gu(c, which):
            src = wg_hbm if which == 0 else wu_hbm
            return pltpu.make_async_copy(src.at[:, pl.ds(c * FC, FC)], rgu.at[c % 2, which, pl.ds(0, D), :], sem_gu.at[c % 2, which])

        def cp_d(c):
            return pltpu.make_async_copy(wd_hbm.at[pl.ds(c * FC, FC), :], rd.at[c % 2, pl.ds(0, FC), :], sem_d.at[c % 2])

        class cp_q:
            def __init__(self, m):
                self.cps = [pltpu.make_async_copy(wqkv_hbm.at[:, pl.ds((m * NCH + k) * NL, NL)],
                                                  rq.at[m * NCH + k, pl.ds(0, D // 2), :].bitcast(BF16),
                                                  sem_q.at[m, k]) for k in range(NCH)]
            def start(self):
                for c in self.cps:
                    c.start()
            def wait(self):
                for c in self.cps:
                    c.wait()

        def cp_o(j):
            return pltpu.make_async_copy(wo_hbm.at[:, pl.ds(j * NL, NL)], ro.at[j, pl.ds(0, D // 2), :].bitcast(BF16), sem_o.at[j])

        def cp_out(i, half):
            r = half * HS + i * T3
            return pltpu.make_async_copy(obuf.at[i % 2, half], out_hbm.at[pl.ds(r, T3), :], sem_out.at[i % 2, half])

        def zero(i):
            return i % 2 + (i + 1) % 2 - 1

        def own_block(pred, fn):
            def body(_, c):
                fn()
                return c
            lax.fori_loop(0, pred.astype(jnp.int32), body, 0)

        def anchor(dst, row, val, z):
            if val is not None and z is not None:
                r = pl.multiple_of(row + z * 16, 8)
                dst[pl.ds(r, 8), pl.ds(0, NL)] = pltpu.bitcast(val, U32) if dst.dtype == U32 else val.astype(dst.dtype)

        def store_a_ops(dst, r, top, bot):
            for kc in range(KC):
                ops = _a_ops(top[kc], top[KC + kc], bot[kc], bot[KC + kc])
                for i in range(7):
                    dst.at[i][pl.ds(r, 16), ch(kc)] = _pk(ops[i])

        def ln_tasks(r0, n, z):
            def xrow(r):
                return xbuf[pl.ds(r, 16), :].astype(F32)
            items = []
            for g in range(n // 16):
                st = {}
                for half in range(2):
                    def s0(val, r=half * HS + r0 + g * 16, st=st, half=half):
                        anchor(xbuf, S, val, z)
                        st["m", half] = jnp.sum(xrow(r), axis=-1, keepdims=True) * (1.0 / D)
                    def s1(val, r=half * HS + r0 + g * 16, st=st, half=half):
                        anchor(xbuf, S, val, z)
                        c = xrow(r) - st["m", half]
                        st["v", half] = lax.rsqrt(jnp.sum(c * c, axis=-1, keepdims=True) * (1.0 / D) + EPS)
                    def s2(val, r=r0 + g * 16, st=st, half=half):
                        for kc in (2 * half, 2 * half + 1):
                            anchor(xbuf, S, val, z)
                            q = [(xbuf[pl.ds(h * HS + r, 16), ch(c)].astype(F32) - st["m", h]) * st["v", h]
                                 for h in range(2) for c in (kc, KC + kc)]
                            for k, (h, c) in enumerate((h, c) for h in range(2) for c in (kc, KC + kc)):
                                Y[pl.ds(h * HS + r, 16), ch(c)] = q[k]
                            ops = _a_ops(*q)
                            for i in range(7):
                                XA.at[i][pl.ds(r, 16), ch(kc)] = _pk(ops[i])
                    nop = lambda val: None
                    items.append([s0, nop, s1, nop, nop, s2] if half == 0 else [s0, nop, s1, nop, s2])
            flat = _skew(items, flat=True)
            return flat

        def prep_g_tasks(slot, r0, n, z):
            def task(val, r, which):
                anchor(rgu.at[0, 0], D, val, z)
                top = rgu[slot, which, pl.ds(r, 16), :].astype(F32)
                bot = rgu[slot, which, pl.ds(KH + r, 16), :].astype(F32)
                ops = _b_ops(top[:, :NL], top[:, NL:], bot[:, :NL], bot[:, NL:])
                for i in range(7):
                    BW.at[slot, i][pl.ds(r, 16), ch(which)] = _pk(ops[i])
            return [(lambda val, r=r0 + g * 16, w=w: task(val, r, w)) for g in range(n // 16) for w in range(2)]

        def xb_tasks(r0, n, z):
            def task(val, r, kc, i):
                anchor(Y, S, val, z)
                x = [_combine(_A_TERMS[i], lambda sg, kp: Y[pl.ds((2 * sg + ro_) * QS + r, 16), ch(4 * kp + 2 * ta + kc)])
                     for ro_ in range(2) for ta in range(2)]
                ops = _a_ops(*x)
                for k, slot in _XB_SLOT.items():
                    XB.at[5 * i + slot][pl.ds(r, 16), ch(kc)] = _pk(ops[k])
            return [(lambda val, r=r0 + g * 16, kc=kc, i=i: task(val, r, kc, i))
                    for g in range(n // 16) for kc in range(2) for i in range(7)]

        def prep_g2_tasks(slot, outer, r0, n, z):
            def task(val, r, i):
                anchor(rgu.at[0, 0], D, val, z)
                y = [_combine(_B_TERMS[i], lambda kp, mu: rgu[slot, mu, pl.ds((2 * kp + ta) * KQ + r, 16), :].astype(F32))
                     for ta in range(2)]
                ops = _b_ops(y[0][:, :NL], y[0][:, NL:], y[1][:, :NL], y[1][:, NL:])
                for k in range(7):
                    BG.at[i][pl.ds(r, 16), ch(k)] = _pk(ops[k])
            return [(lambda val, r=r0 + g * 16, i=i: task(val, r, i)) for i in outer for g in range(n // 16)]

        def prep_d_tasks(slot, r0, n, z):
            def task(val, r, n):
                anchor(rd.at[0], FC, val, z)
                q11 = rd[slot, pl.ds(r, 16), pl.ds(n * NL, NL)].astype(F32)
                q12 = rd[slot, pl.ds(r, 16), pl.ds(KH + n * NL, NL)].astype(F32)
                q21 = rd[slot, pl.ds(NL + r, 16), pl.ds(n * NL, NL)].astype(F32)
                q22 = rd[slot, pl.ds(NL + r, 16), pl.ds(KH + n * NL, NL)].astype(F32)
                ops = _b_ops(q11, q12, q21, q22)
                for i in range(7):
                    BW.at[slot, i][pl.ds(KH + (n // 2) * NL + r, 16), ch(n % 2)] = _pk(ops[i])
            return [(lambda val, r=r0 + g * 16, c=c: task(val, r, c)) for g in range(n // 16) for c in range(KC)]

        def prep_q_tasks(m, par, n, z):
            def perm_a(r):
                y = [rq[m * NCH + k, pl.ds(r // 2, 8), :] for k in range(NCH)]
                return [y[0]] + [pltpu.roll(y[k], 2 * k, 1) for k in range(1, NCH)]

            def perm_b(y):
                lane = lax.broadcasted_iota(jnp.int32, (8, NL), 1)
                sh = (((lane & 15) >> 1) - par) & 7
                u = [y[(-m_) % NCH] for m_ in range(NCH)]
                b0, b1, b2 = (sh & 1) != 0, (sh & 2) != 0, (sh & 4) != 0
                out = (2 * n, 2 * n + 4)
                v = {m_: jnp.where(b0, u[(m_ - 1) % NCH], u[m_]) for m_ in (0, 2, 4, 6)}
                v = {m_: jnp.where(b1, v[(m_ - 2) % NCH], v[m_]) for m_ in out}
                v = {m_: jnp.where(b2, v[(m_ - 4) % NCH], v[m_]) for m_ in out}
                return [pltpu.roll(v[m_], (2 * NL - 2 * m_ - 2 * par) % NL, 1) for m_ in out]

            def wide(w):
                return pltpu.bitcast(w, BF16).astype(F32)

            items = []
            for g in range(KH // 16):
                st = {}
                for half in range(2):
                    def s0(val, r=half * KH + g * 16, st=st, half=half):
                        anchor(rq.at[0], D // 2, val, z)
                        st["a", half] = perm_a(r)
                    def s1(val, st=st, half=half):
                        st["b", half] = perm_b(st["a", half])
                    def s2(val, r=g * 16, st=st):
                        top, bot = st["b", 0], st["b", 1]
                        ops = _b_ops(wide(top[0]), wide(top[1]), wide(bot[0]), wide(bot[1]))
                        for i in range(7):
                            BQ.at[i][pl.ds(r, 16), ch(n)] = _pk(ops[i])
                    items.append([s0, s1] + ([s2] if half else []))
            return _skew(items)

        def prep_o_tasks(n, z):
            tasks = []
            for jj in range(KC):
                for a in range(4):
                    for b in range(2):
                        st = []
                        for k, (j, c) in enumerate(((jj, n), (jj, KC + n), (KC + jj, n), (KC + jj, KC + n))):
                            def task(val, k=k, j=j, c=c, st=st, start=16 * a + 8 * b, r=jj * NL + 32 * a + 16 * b):
                                anchor(ro.at[0], D // 2, val, z)
                                st.append(ro[c, pl.ds(start + j, 8, stride=64), :])
                                if k == 3:
                                    ops = _b_ops(*[pltpu.bitcast(w, BF16).astype(F32) for w in st])
                                    for i in range(7):
                                        BO.at[i][pl.ds(r, 16), ch(n)] = _pk(ops[i])
                            tasks.append(task)
            return tasks

        def attn_unit(r0, masked, slot, z):
            st = {}

            def shifted(plane):
                return [qkv[plane, pl.ds(r0 + HALO + 8 - DIL * k, 8), :] for k in range(12)]

            def logits(val, j):
                anchor(qkv.at[0], 0, val, z)
                q = [qkv[j, pl.ds(r0 + HALO + 8 * g, 8), :] for g in range(2)]
                kk = shifted(NCH + j)
                for g in range(2):
                    for w in range(W):
                        t = q[g] * kk[w + 4 - 4 * g]
                        st[g, w] = t if j == 0 else st[g, w] + t
                if j == NCH - 1:
                    softmax()

            def softmax():
                lane = lax.broadcasted_iota(jnp.int32, (8, NL), 1)
                odd = (lane & 1) != 0
                hi = (lane & 16) != 0
                keys = [(g, w) for g in range(2) for w in range(W)]
                for k in keys:
                    a = st[k]
                    st[k] = a + jnp.where(odd, pltpu.roll(a, 1, 1), pltpu.roll(a, NL - 1, 1))
                for k in keys:
                    a = st[k]
                    st[k] = a + jnp.where(hi, pltpu.roll(a, 16, 1), pltpu.roll(a, NL - 16, 1))
                for g in range(2):
                    ls = [st[g, w] for w in range(W)]
                    if masked:
                        pos = r0 + 8 * g + lax.broadcasted_iota(jnp.int32, (8, NL), 0)
                        ls = [ls[0]] + [jnp.where(pos >= DIL * w, ls[w], NEG) for w in range(1, W)]
                    m = ls[0]
                    for w in range(1, W):
                        m = jnp.maximum(m, ls[w])
                    ps = [jnp.exp2((l - m) * EXP2_SCALE) for l in ls]
                    den = ps[0]
                    for w in range(1, W):
                        den = den + ps[w]
                    inv = 1.0 / den
                    for w in range(W):
                        st[g, w] = ps[w] * inv

            def pv(val, j):
                anchor(qkv.at[0], 0, val, z)
                vv = shifted(2 * NCH + j)
                for g in range(2):
                    a = st[g, 0] * vv[4 - 4 * g]
                    for w in range(1, W):
                        a = a + st[g, w] * vv[w + 4 - 4 * g]
                    osc[slot, j, pl.ds(8 * g, 8), :] = a

            gap = [lambda val: None] * AGAP
            return ([(lambda val, j=j: logits(val, j)) for j in range(NCH)] + gap
                    + [(lambda val, j=j: pv(val, j)) for j in range(NCH)])

        def attn_tasks(t0, z):
            tasks = []
            for g in range(AP // 16):
                r = t0 + g * 16
                tasks += attn_unit(r, g == 0, 2 * g, z) + attn_unit(HS + r, False, 2 * g + 1, z)
                def oa(val, kc, g=g, r=r):
                    ops = _a_ops(osc[2 * g, kc], osc[2 * g, KC + kc], osc[2 * g + 1, kc], osc[2 * g + 1, KC + kc])
                    for i in range(7):
                        OA.at[i][pl.ds(r, 16), ch(kc)] = _pk(ops[i])
                tasks += [(lambda val, kc=kc, oa=oa: oa(val, kc)) for kc in range(KC)]
            return tasks

        def lhs(ref, i, r0, m):
            return ref[i, pl.ds(r0, m), :]

        def gelu2(g, u):
            t = jnp.tanh(g * (GELU_C0 + GELU_C1 * (g * g)))
            p = g * u
            return p + p * t

        def up_phase(slot, r0, m):
            g, h = {}, {}
            def put(i, v):
                HA[pl.ds(r0, m), ch(i)] = _pk(v)
            def fin_u(k, u):
                h[k] = gelu2(g[k], u)
                if k == 3:
                    put(1, h[2] + h[3]); put(3, h[3])
                elif k == 1:
                    put(6, h[1] - h[3])
                elif k == 0:
                    put(0, h[0] + h[3]); put(2, h[0]); put(4, h[0] + h[1]); put(5, h[2] - h[0])
            yield from _strassen(lambda i: _dot(lhs(XA, i, r0, m), BW[slot, i, pl.ds(0, KH), ch(0)]), g.__setitem__, RG)
            yield from _strassen(lambda i: _dot(lhs(XA, i, r0, m), BW[slot, i, pl.ds(0, KH), ch(1)]), fin_u, RU)

        def up_sub(r0, m, dyn, z):
            st = {}

            def ha_task(val, r, which):
                anchor(HF, S, val, z)
                def get(sg, j):
                    return HF[pl.ds(sg * HS + r, HG), ch(j)]
                for i in which:
                    HA[pl.ds(r, HG), ch(i)] = _pk(_combine(_A_TERMS[i], get))

            def outer_fin(K, k, v):
                rho, j = k // 2, k % 2
                if K in (2, 1):
                    st["hold", k] = v
                    return
                sg = K // 2
                HF[pl.ds(sg * HS + rho * QS + r0, m), ch(j)] = (
                    gelu2(st["hold", k], v) if K == 3 else gelu2(v, st["hold", k]))
                st["h", sg, rho, j] = True
                if ("h", sg, rho, 1 - j) in st:
                    which = (1, 3) if sg == 1 else (0, 2, 4, 5, 6)
                    for g in range(m // HG):
                        dyn.append([None, lambda val, r=rho * QS + r0 + g * HG, which=which: ha_task(val, r, which),
                                    (rho * QS + r0 + g * HG, which)])

            def outer_step(i, k, v):
                if i == 1:
                    st["m1", k] = v
                elif i == 3:
                    outer_fin(2, k, st["m1", k] + v)
                    st["t11", k] = v
                elif i == 0:
                    st["t11", k] = st["t11", k] + v
                    st["t22", k] = v - st["m1", k]
                elif i == 5:
                    st["t22", k] = st["t22", k] + v
                elif i == 2:
                    outer_fin(3, k, st["t22", k] + v)
                    st["m2", k] = v
                elif i == 4:
                    outer_fin(1, k, st["m2", k] + v)
                    st["t11", k] = st["t11", k] - v
                else:
                    outer_fin(0, k, st["t11", k] + v)

            def lhs2(i, k):
                if k == 2:
                    return XA[i, pl.ds(r0, m), pl.ds(0, KQ)]
                if k == 3:
                    return XA[i, pl.ds(QS + r0, m), pl.ds(KQ, KQ)]
                return XB[5 * i + _XB_SLOT[k], pl.ds(r0, m), :]

            def step(i):
                return _strassen(lambda k: _dot(lhs2(i, k), BG[i, :, ch(k)]),
                                 lambda k, v: outer_step(i, k, v), R2H if i in (2, 6) else R2L)
            return step

        def ffn2(slot, dyn, z):
            subs = [up_sub(s * RH2, RH2, dyn, z) for s in range(QS // RH2)]
            for i in _ORDER:
                for sub in subs:
                    yield from sub(i)
            n = HS // RH
            order = [(i, s) for s in range(n) for i in (1, 3)]
            order += [(i, s) for s in list(range(n // 2, n)) + list(range(n // 2)) for i in (0, 2, 4, 5, 6)]
            for i, s in order:
                for e in list(dyn):
                    if i in e[2][1] and s * RH <= e[2][0] < (s + 1) * RH:
                        dyn.remove(e)
                        e[1](None)
                yield from down_phase(slot, s * RH, RH, False, RD2 * (QS // RH2), (i,))

        def down_phase(slot, r0, m, first, room=None, which=range(7)):
            for i in which:
                w = jnp.concatenate([BW[slot, i, pl.ds(KH, NL), :], BW[slot, i, pl.ds(KH + NL, NL), :]], axis=1)
                d = _dot(HA[pl.ds(r0, m), ch(i)], w)
                if first:
                    P[i, pl.ds(r0, m), :] = d
                else:
                    P[i, pl.ds(r0, m), :] += d
                yield (RD if room is None else room), d

        def ffn_rows(slot, r0, nrows, first):
            m = min(RH, nrows)
            for s in range(nrows // m):
                yield from up_phase(slot, r0 + s * m, m)
            for s in range(nrows // m):
                yield from down_phase(slot, r0 + s * m, m, first)

        with scope("start"):
            groups = [[cp_x(0, 0), cp_x(0, 1)], [cp_gu(0, 0)], [cp_gu(0, 1)], [cp_d(0)]]
            groups += [[cp_x(i, 0), cp_x(i, 1)] for i in range(1, NT0)]
            groups += [[cp_q(0)], [cp_gu(1, 0), cp_gu(1, 1), cp_d(1)], [cp_o(j) for j in range(NCH)],
                       [cp_q(1)], [cp_q(2)]]

            def issue(k, c):
                for g, cps in enumerate(groups):
                    @pl.when(k == g)
                    def _():
                        for cp in cps:
                            cp.start()
                return c
            lax.fori_loop(0, len(groups), issue, 0)
            cp_x(0, 0).wait(); cp_x(0, 1).wait()

            def ln0(g, c):
                for t in ln_tasks(pl.multiple_of(g * LN0, LN0), LN0, None):
                    t(None)
                return c
            lax.fori_loop(0, T0 // LN0, ln0, 0)
            for which in range(2):
                cp_gu(0, which).wait()
                def pg0(g, c):
                    for t in prep_g_tasks(0, pl.multiple_of(g * 64, 64), 64, None)[which::2]:
                        t(None)
                    return c
                lax.fori_loop(0, KH // 64, pg0, 0)
            cp_d(0).wait()
            for t in prep_d_tasks(0, 0, NL, None):
                t(None)

        def p0_body(i, c):
            own_block(i >= 0, lambda: (cp_x(i + 1, 0).wait(), cp_x(i + 1, 1).wait()))
            r0 = pl.multiple_of(i * T0, T0)
            _emit(LAG, ffn_rows(0, r0, T0, True), RF * (T0 // min(RH, T0)), (0.0, 0.9, ln_tasks(r0 + T0, T0, zero(i))))
            return zero(i)
        with scope("p0"):
            z0 = lax.fori_loop(0, NT0 - 1, p0_body, 0)
        with scope("p0_last"):
            cp_q(0).wait()
            cp_gu(2, 0).start(); cp_gu(2, 1).start(); cp_d(2).start()
            _emit(LAG, ffn_rows(0, HS - T0, T0, True), RF * (T0 // min(RH, T0)), (0.0, 0.9, prep_q_tasks(0, 0, 0, z0)))

        def p1_body(b, c):
            own_block(b == 0, lambda: (cp_gu(1, 0).wait(), cp_gu(1, 1).wait(), cp_d(1).wait(),
                                       [cp_o(j).wait() for j in range(NCH)]))
            own_block(b == 1, lambda: cp_q(1).wait())
            own_block(b == 3, lambda: cp_q(2).wait())
            m = b // 2
            par = b % 2

            def main():
                for n in range(2):
                    for s in range(HS // RH):
                        r0 = s * RH
                        def fin(k, v):
                            j = m * NCH + par + 2 * n + 4 * (k % 2)
                            qkv[j, pl.ds(HALO + (k // 2) * HS + r0, RH), :] = v
                        yield from _strassen(lambda i: _dot(lhs(XA, i, r0, RH), BQ[i, :, ch(n)]), fin, (1,) * 7)
            piece = jnp.clip(b - 2, 0, 3)
            z = zero(b)
            _emit(LAG, main(), 14 * (HS // RH),
                  (0.0, P1A, prep_q_tasks(m, par, 1, z)),
                  (0.5 + P1B, 0.5 + P1A, prep_q_tasks(jnp.minimum((b + 1) // 2, 2), (b + 1) % 2, 0, z)),
                  (0.0, 0.95, prep_g2_tasks(1, range(7), pl.multiple_of(piece * (KQ // 4), KQ // 4), KQ // 4, z)),
                  (0.0, 0.95, xb_tasks(pl.multiple_of(jnp.minimum(b * 96, QS - 96), 16), 96, z)),
                  (0.0, 0.95, prep_d_tasks(1, pl.multiple_of(piece * 32, 32), 32, z)),
                  (0.0, 0.95, prep_o_tasks(piece, z)))
            return c
        with scope("p1"):
            lax.fori_loop(0, 6, p1_body, 0)
        with scope("p1_tail"):
            for j in range(NCH, 3 * NCH):
                qkv[j, 0:HALO, :] = jnp.broadcast_to(qkv[j, HALO:HALO + 1, :], (HALO, NL))

        def p2_body(c, carry):
            def dma_step():
                cp_gu(c + 1, 0).wait(); cp_gu(c + 1, 1).wait(); cp_d(c + 1).wait()
                @pl.when(c + 2 < NC)
                def _():
                    cp_gu(c + 2, 0).start(); cp_gu(c + 2, 1).start(); cp_d(c + 2).start()
            own_block(c + 1 < NC, dma_step)
            t0 = pl.multiple_of(jnp.minimum((c - 1) * AP, HS - AP), 16)
            cur = c % 2
            z = zero(c)
            nsub = QS // RH2
            g_room = (5 * sum(R2L) + 2 * sum(R2H)) * nsub
            total = g_room + 7 * RD2 * nsub * (HS // RH)
            f0 = PG0 * sum(R2L) * nsub / total
            dyn = []
            _emit(LAG2, ffn2(cur, dyn, z), total,
                  (f0, 0.97, prep_g2_tasks(1 - cur, _ORDER, 0, KQ, z)),
                  (0.0, max(f0, 0.5), prep_d_tasks(1 - cur, 0, NL, z)),
                  (0.0, 0.95, attn_tasks(t0, z) if 'noattn' not in EXP else []),
                  dyn=dyn, dyn_rate=DRATE, dyn_delay=DDELAY)
            return carry
        with scope("p2"):
            lax.fori_loop(1, NC, p2_body, 0)

        def p3_body(t, carry):
            @pl.when(t >= 2)
            def _():
                cp_out(t - 2, 0).wait(); cp_out(t - 2, 1).wait()
            slot = t % 2
            m = min(RH, T3)

            def main():
                for s in range(T3 // m):
                    r0 = pl.multiple_of(t * T3 + s * m, m)
                    for n in range(KC):
                        def pq(i):
                            return P[i, pl.ds(r0, m), pl.ds(n * NL, NL)]
                        def fin(k, sq):
                            if k == 0:
                                f = pq(0) + pq(3) - pq(4) + pq(6)
                            elif k == 1:
                                f = pq(2) + pq(4)
                            elif k == 2:
                                f = pq(1) + pq(3)
                            else:
                                f = pq(0) - pq(1) + pq(2) + pq(5)
                            half, col = k // 2, (k % 2) * KH + n * NL
                            z = f * 0.25
                            gate = z + z * jnp.tanh(z)
                            x = xbuf[pl.ds(half * HS + r0, m), pl.ds(col, NL)].astype(F32)
                            obuf.at[slot, half][pl.ds(s * m, m), pl.ds(col, NL)] = (x + sq * gate).astype(BF16)
                        yield from _strassen(lambda i: _dot(lhs(OA, i, r0, m), BO[i, :, ch(n)]), fin, (1,) * 7)
            _emit(LAG, main(), 28 * (T3 // m))
            cp_out(t, 0).start(); cp_out(t, 1).start()
            return carry
        with scope("p3"):
            lax.fori_loop(0, NT3, p3_body, 0)
        with scope("end"):
            for t in range(max(NT3 - 2, 0), NT3):
                cp_out(t, 0).wait(); cp_out(t, 1).wait()

    def fn(A_x, A_wqkv, A_wo, B_x, B_w_gate, B_w_up, B_w_down):
        x = A_x.reshape(S, D)
        anyspec = pl.BlockSpec(memory_space=pl.ANY)
        out = pl.pallas_call(
            kernel,
            in_specs=[anyspec] * 6,
            out_specs=anyspec,
            out_shape=jax.ShapeDtypeStruct((S, D), BF16),
            scratch_shapes=[
                pltpu.VMEM((S + 16, D), BF16),
                pltpu.VMEM((7, HS // 2, KH), U32),
                pltpu.VMEM((3 * NCH, HALO + S, NL), F32),
                pltpu.VMEM((7, HS // 2, KH), U32),
                pltpu.VMEM((7, HS, KH), F32),
                pltpu.VMEM((HS // 2, 7 * NL), U32),
                pltpu.VMEM((2, 7, (KH + 2 * NL) // 2, 2 * NL), U32),
                pltpu.VMEM((7, KH // 2, 2 * NL), U32),
                pltpu.VMEM((7, KH // 2, KH), U32),
                pltpu.VMEM((S + 8, D), F32),
                pltpu.VMEM((35, QS // 2, KQ), U32),
                pltpu.VMEM((7, KQ // 2, 7 * NL), U32),
                pltpu.VMEM((S + 8, FC), F32),
                pltpu.VMEM((2, 2, D + 16, FC), BF16),
                pltpu.VMEM((2, FC + 16, D), BF16),
                pltpu.VMEM((3 * NCH, D // 2 + 8, NL), U32),
                pltpu.VMEM((NCH, D // 2 + 8, NL), U32),
                pltpu.VMEM((2, 2, T3, D), BF16),
                pltpu.VMEM((AP // 8, NCH, 16, NL), F32),
                pltpu.SemaphoreType.DMA((NT0, 2)),
                pltpu.SemaphoreType.DMA((2, 2)),
                pltpu.SemaphoreType.DMA((2,)),
                pltpu.SemaphoreType.DMA((3, NCH)),
                pltpu.SemaphoreType.DMA((NCH,)),
                pltpu.SemaphoreType.DMA((2, 2)),
            ],
            compiler_params=pltpu.CompilerParams(vmem_limit_bytes=120 * 2 ** 20, disable_bounds_checks=NOBC),
        )(x, A_wqkv, A_wo, B_w_gate, B_w_up, B_w_down)
        return out.reshape(1, S, D)
    return jax.jit(fn)


_IMPL = make()


@jax.jit
def pallas_recurrent_scan__sliding_local_dilated__geglu_ffn__prompt_kernel(
    A_x: jax.Array,
    A_wqkv: jax.Array,
    A_wo: jax.Array,
    B_x: jax.Array,
    B_w_gate: jax.Array,
    B_w_up: jax.Array,
    B_w_down: jax.Array,
):
    return _IMPL(A_x, A_wqkv, A_wo, B_x, B_w_gate, B_w_up, B_w_down)
```

```python
import contextlib
import math

import jax
import jax.numpy as jnp
from jax import lax
import jax.experimental.pallas as pl
import jax.experimental.pallas.tpu as pltpu

S, D, F = 2048, 1024, 3584
H, DH, W, DIL = 32, 32, 8, 2
NL = 128
NCH = D // NL
HS = S // 2
KH = D // 2
KC = KH // NL
QS = S // 4
KQ = D // 4
FC = 256
NP = F // (2 * FC)
HALO = 16
F32, BF16, U32 = jnp.float32, jnp.bfloat16, jnp.uint32
EPS = 1e-5
GELU_C0 = math.sqrt(2.0 / math.pi)
GELU_C1 = GELU_C0 * 0.044715
EXP2_SCALE = (DH ** -0.5) * math.log2(math.e)
NEG = -1e9 / (DH ** -0.5)

_A_TERMS = (((0, 0, 1), (1, 1, 1)), ((1, 0, 1), (1, 1, 1)), ((0, 0, 1),), ((1, 1, 1),),
            ((0, 0, 1), (0, 1, 1)), ((1, 0, 1), (0, 0, -1)), ((0, 1, 1), (1, 1, -1)))
_B_TERMS = (((0, 0, 1), (1, 1, 1)), ((0, 0, 1),), ((0, 1, 1), (1, 1, -1)), ((1, 0, 1), (0, 0, -1)),
            ((1, 1, 1),), ((0, 0, 1), (0, 1, 1)), ((1, 0, 1), (1, 1, 1)))
_C_TERMS = (((0, 1), (3, 1), (4, -1), (6, 1)), ((2, 1), (4, 1)), ((1, 1), (3, 1)), ((0, 1), (1, -1), (2, 1), (5, 1)))
_ORDER = (1, 3, 0, 5, 2, 4, 6)
_XB_SLOT = {0: 0, 1: 1, 4: 2, 5: 3, 6: 4}


def _combine(terms, get):
    (r, c, _), *rest = terms
    v = get(r, c)
    for r, c, sign in rest:
        v = v + get(r, c) if sign > 0 else v - get(r, c)
    return v


def _ops(terms, q11, q12, q21, q22):
    q = ((q11, q12), (q21, q22))
    return [_combine(t, lambda r, c: q[r][c]) for t in terms]


def _dot(a, b):
    return jnp.dot(a, b, preferred_element_type=F32)


class _Fold:
    def __init__(self, fin):
        self.fin = fin

    def __call__(self, i, m):
        if i == 1:
            self.m1 = m
        elif i == 3:
            self.fin(2, self.m1 + m)
            self.t11 = m
        elif i == 0:
            self.t11 = self.t11 + m
            self.t22 = m - self.m1
        elif i == 5:
            self.t22 = self.t22 + m
        elif i == 2:
            self.fin(3, self.t22 + m)
            self.m2 = m
        elif i == 4:
            self.fin(1, self.m2 + m)
            self.t11 = self.t11 - m
        else:
            self.fin(0, self.t11 + m)


def _strassen(prod, fin, room):
    fold = _Fold(fin)
    for step, i in enumerate(_ORDER):
        m = prod(i)
        fold(i, m)
        yield room[step], m


def _emit(lag, main, total, *sides, dyn=None, dyn_rate=0, dyn_delay=0):
    done = [0] * len(sides)
    acc = step = 0

    def flush(frac, val):
        due = []
        for k, (f0, f1, tasks) in enumerate(sides):
            want = len(tasks) if frac >= f1 else int(max(0.0, (frac - f0) / (f1 - f0)) * len(tasks) + 0.5)
            n = min(want, len(tasks)) - done[k]
            due += [((j + 0.5) / n, k, tasks[done[k] + j]) for j in range(n)]
            done[k] += max(n, 0)
        if dyn:
            rate = dyn_rate
            ready = [e for e in dyn if e[0] + dyn_delay <= step][:rate]
            for j, e in enumerate(ready):
                dyn.remove(e)
                due.append(((j + 0.5) / len(ready), -1, e[1]))
        due.sort(key=lambda e: e[:2])
        for j, (_, _, task) in enumerate(due):
            if val is None:
                task(None)
            else:
                r = (val.shape[0] // 8) * j // len(due) * 8
                task(val[r:r + 8, 0:NL])

    hist = [(0, None)] * lag
    for item in main:
        step += 1
        for e in dyn or ():
            if e[0] is None:
                e[0] = step
        hist.append(item)
        room, val = hist.pop(0)
        acc += room
        if room:
            flush(acc / total, val)
    acc += sum(h[0] for h in hist)
    assert abs(acc - total) < 1e-6 and not dyn, (acc, total)
    flush(2.0, hist[-1][1] if hist else val)


def _skew(items):
    depth = max(len(st) for st in items)
    return [items[t - k][k] for t in range(len(items) + depth - 1) for k in range(depth)
            if 0 <= t - k < len(items) and k < len(items[t - k]) and items[t - k][k] is not None]


def make(EXP='', ONEPASS=True, T0=128, LN0=64, LNF=0.8, RG=(2,) * 7, RU=(2, 1, 2, 2, 1, 1, 1),
         RH=256, LAG=1, P1A=0.44,
         RH2=64, LAG2=4, PG0=1.5, R2L=(2,) * 7, R2H=(2, 0, 2, 2, 0, 0, 0), MD=128, ND=128, RD2=2, DRATE=2, DDELAY=4,
         APA=48, APB=112, AGAP=4, HAF=0.6, HA1=2.0, HA2=4.6, ATS=None, ATE=0.75, ATB=0.97, PDN=64, PDB=0.8,
         M3=64, OUTK=1, LAG3=1, scopes=False):
    NT0 = HS // T0
    T3 = 256
    NT3 = HS // T3
    assert (NP - 1) * APA + NP * APB >= HS and APA % 16 == 0 and APB % 16 == 0

    def scope(name):
        return jax.named_scope(name) if scopes else contextlib.nullcontext()

    def kernel(x_hbm, wqkv_hbm, wo_hbm, wg_hbm, wu_hbm, wd_hbm, out_hbm,
               xbuf, XA, XB, qkv, P, HF, BG, BD, BO, rgu, rd,
               sem_x, sem_gu, sem_d, sem_q, sem_o, sem_out):

        XA, XB, BG, BD, BO = [r.bitcast(BF16) for r in (XA, XB, BG, BD, BO)]

        def ch(n, w=NL):
            return pl.ds(n * w, w) if isinstance(n, int) else pl.ds(pl.multiple_of(n * w, w), w)

        def zero(i):
            return i % 2 + (i + 1) % 2 - 1

        def when(pred, fn):
            pl.when(pred)(lambda: (fn(), None)[1])

        def cp_x(i, half):
            r = half * HS + i * T0
            return pltpu.make_async_copy(x_hbm.at[pl.ds(r, T0), :], xbuf.at[pl.ds(r, T0), :], sem_x.at[i, half])

        def cp_gu(c, slot, which):
            src = wg_hbm if which == 0 else wu_hbm
            return pltpu.make_async_copy(src.at[:, pl.ds(c * FC, FC)], rgu.at[slot, which, pl.ds(0, D), :],
                                         sem_gu.at[slot, which])

        def cp_d(p):
            return pltpu.make_async_copy(wd_hbm.at[pl.ds(p * 2 * FC, 2 * FC), :], rd.at[pl.ds(0, 2 * FC), :],
                                         sem_d.at[0])

        def anchor(dst, row, val, z):
            if val is not None and z is not None:
                r = pl.multiple_of(row + z * 16, 8)
                dst[pl.ds(r, 8), pl.ds(0, NL)] = pltpu.bitcast(val, U32) if dst.dtype == U32 else val.astype(dst.dtype)

        def gelu2(g, u):
            t = jnp.tanh(g * (GELU_C0 + GELU_C1 * (g * g)))
            p = g * u
            return p + p * t

        def prep_g2_tasks(slot, outer, r0, n, z, free=None):
            def task(val, r, i):
                assert free is None or i in free
                anchor(rgu.at[0, 0], D, val, z)
                y = [_combine(_B_TERMS[i], lambda kp, mu: rgu[slot, mu, pl.ds((2 * kp + ta) * KQ + r, 16), :].astype(F32))
                     for ta in range(2)]
                ops = _ops(_B_TERMS, y[0][:, :NL], y[0][:, NL:], y[1][:, :NL], y[1][:, NL:])
                for k in range(7):
                    BG.at[i][pl.ds(r, 16), ch(k)] = ops[k].astype(BF16)
            return [(lambda val, r=r0 + g * 16, i=i: task(val, r, i)) for i in outer for g in range(n // 16)]

        def prep_d2_tasks(r0, n, z):
            def task(val, r, i):
                anchor(rd, 2 * FC, val, z)
                y = [_combine(_B_TERMS[i],
                              lambda kp, nu: rd[pl.ds((2 * kp + ta) * NL + r, 16), ch(2 * nu + up, KQ)].astype(F32))
                     for ta in range(2) for up in range(2)]
                ops = _ops(_B_TERMS, *y)
                for k in range(7):
                    BD.at[7 * i + k][pl.ds(r, 16), :] = ops[k].astype(BF16)
            return [(lambda val, r=r0 + g * 16, i=i: task(val, r, i)) for g in range(n // 16) for i in range(7)]

        def first_half(Y, B0, BQ, rq):
            B0, BQ = B0.bitcast(BF16), BQ.bitcast(BF16)

            class cp_cols:
                def __init__(self, src, col0, dst, slot0, sem):
                    self.args = src, col0, dst, slot0, sem

                def start(self):
                    src, col0, dst, slot0, sem = self.args
                    for k in range(NCH):
                        pltpu.make_async_copy(src.at[:, pl.ds(col0 + k * NL, NL)],
                                              dst.at[slot0 + k, pl.ds(0, D // 2), :].bitcast(BF16), sem).start()

                def wait(self):
                    _, _, dst, slot0, sem = self.args
                    whole = dst.at[pl.ds(slot0, NCH), pl.ds(0, D // 2), :]
                    pltpu.make_async_copy(whole, whole, sem).wait()

            def cp_q(m):
                return cp_cols(wqkv_hbm, m * D, rq, m * NCH, sem_q.at[m])

            def cp_o():
                return cp_cols(wo_hbm, 0, rq, 3 * NCH, sem_o.at[0])

            def ln_tasks(r0, n, z):
                def xrow(r):
                    return xbuf[pl.ds(r, 16), :].astype(F32)
                items = []
                for g in range(n // 16):
                    st = {}
                    for half in range(2):
                        def s0(val, r=half * HS + r0 + g * 16, st=st, half=half):
                            anchor(xbuf, S, val, z)
                            st["m", half] = jnp.sum(xrow(r), axis=-1, keepdims=True) * (1.0 / D)

                        def s1(val, r=half * HS + r0 + g * 16, st=st, half=half):
                            anchor(xbuf, S, val, z)
                            c = xrow(r) - st["m", half]
                            st["v", half] = lax.rsqrt(jnp.sum(c * c, axis=-1, keepdims=True) * (1.0 / D) + EPS)

                        def s01(val, r=half * HS + r0 + g * 16, st=st, half=half):
                            anchor(xbuf, S, val, z)
                            x = xrow(r)
                            m = jnp.sum(x, axis=-1, keepdims=True) * (1.0 / D)
                            e2 = jnp.sum(x * x, axis=-1, keepdims=True) * (1.0 / D)
                            st["m", half] = m
                            st["v", half] = lax.rsqrt(jnp.maximum(e2 - m * m, 0.0) + EPS)

                        def s2(val, r=r0 + g * 16, st=st, half=half):
                            for kc in (2 * half, 2 * half + 1):
                                anchor(xbuf, S, val, z)
                                pos = [(h, c) for h in range(2) for c in (kc, KC + kc)]
                                q = [(xbuf[pl.ds(h * HS + r, 16), ch(c)].astype(F32) - st["m", h]) * st["v", h]
                                     for h, c in pos]
                                for (h, c), y in zip(pos, q):
                                    Y[pl.ds(h * HS + r, 16), ch(c)] = y
                                for i, op in enumerate(_ops(_A_TERMS, *q)):
                                    XA.at[i][pl.ds(r, 16), ch(kc)] = op.astype(BF16)
                        stats = [s01] if ONEPASS else [s0, None, s1]
                        items.append(stats + [None] * (2 - half) + [s2])
                return _skew(items)

            def prep_g1_tasks(which, r0, n):
                for g in range(n // 16):
                    r = r0 + g * 16
                    top = rgu[0, which, pl.ds(r, 16), :].astype(F32)
                    bot = rgu[0, which, pl.ds(KH + r, 16), :].astype(F32)
                    for i, op in enumerate(_ops(_B_TERMS, top[:, :NL], top[:, NL:], bot[:, :NL], bot[:, NL:])):
                        B0.at[i][pl.ds(r, 16), ch(which)] = op.astype(BF16)

            def xb_tasks(r0, n, z):
                def task(val, r, kc, i):
                    anchor(Y, S, val, z)
                    x = [_combine(_A_TERMS[i],
                                  lambda sg, kp: Y[pl.ds((2 * sg + rho) * QS + r, 16), ch(4 * kp + 2 * ta + kc)])
                         for rho in range(2) for ta in range(2)]
                    ops = _ops(_A_TERMS, *x)
                    for k, slot in _XB_SLOT.items():
                        XB.at[5 * i + slot][pl.ds(r, 16), ch(kc)] = ops[k].astype(BF16)
                return [(lambda val, r=r0 + g * 16, kc=kc, i=i: task(val, r, kc, i))
                        for g in range(n // 16) for kc in range(2) for i in range(7)]

            def wide(w):
                return pltpu.bitcast(w, BF16).astype(F32)

            def prep_q_tasks(m, par, n, z):
                def perm_a(r):
                    y = [rq[m * NCH + k, pl.ds(r // 2, 8), :] for k in range(NCH)]
                    return [y[0]] + [pltpu.roll(y[k], 2 * k, 1) for k in range(1, NCH)]

                def perm_b(y):
                    lane = lax.broadcasted_iota(jnp.int32, (8, NL), 1)
                    sh = (((lane & 15) >> 1) - par) & 7
                    u = [y[(-j) % NCH] for j in range(NCH)]
                    b0, b1, b2 = (sh & 1) != 0, (sh & 2) != 0, (sh & 4) != 0
                    out = (2 * n, 2 * n + 4)
                    v = {j: jnp.where(b0, u[(j - 1) % NCH], u[j]) for j in (0, 2, 4, 6)}
                    v = {j: jnp.where(b1, v[(j - 2) % NCH], v[j]) for j in out}
                    v = {j: jnp.where(b2, v[(j - 4) % NCH], v[j]) for j in out}
                    return [pltpu.roll(v[j], (2 * NL - 2 * j - 2 * par) % NL, 1) for j in out]

                items = []
                for g in range(KH // 16):
                    st = {}
                    for half in range(2):
                        def s0(val, r=half * KH + g * 16, st=st, half=half):
                            anchor(rq.at[0], D // 2, val, z)
                            st["a", half] = perm_a(r)

                        def s1(val, st=st, half=half):
                            st["b", half] = perm_b(st["a", half])

                        def s2(val, r=g * 16, st=st):
                            ops = _ops(_B_TERMS, *[wide(w) for w in st["b", 0] + st["b", 1]])
                            for i in range(7):
                                BQ.at[i][pl.ds(r, 16), ch(n)] = ops[i].astype(BF16)
                        items.append([s0, s1] + ([s2] if half else []))
                flat = _skew(items)
                firsts = [j for j, t in enumerate(flat) if t.__name__ == "s0"] + [len(flat)]
                return [(lambda val, grp=flat[a:b]: [t(val) for t in grp]) for a, b in zip(firsts, firsts[1:])]

            def prep_o_tasks(src, n, z):
                tasks = []
                for jj in range(KC):
                    for a in range(8):
                        st = []
                        for k, (j, c) in enumerate(((jj, n), (jj, KC + n), (KC + jj, n), (KC + jj, KC + n))):
                            def task(val, k=k, j=j, c=c, st=st, start=8 * a, r=jj * NL + 16 * a):
                                anchor(rq.at[0], D // 2, val, z)
                                st.append(rq[src + c, pl.ds(start + j, 8, stride=64), :])
                                if k == 3:
                                    for i, op in enumerate(_ops(_B_TERMS, *[wide(w) for w in st])):
                                        BO.at[i][pl.ds(r, 16), ch(n)] = op.astype(BF16)
                            tasks.append(task)
                return tasks

            def zero_p_tasks(u0, n, z):
                def task(val, u):
                    v = jnp.zeros((8, NL), F32) if val is None else jnp.where(z != 0, val, 0.0)
                    P[u // 32, pl.ds(pl.multiple_of((u % 32) * 32, 32), 32), :] = jnp.tile(v, (4, KC))
                return [(lambda val, u=u0 + j: task(val, u)) for j in range(n)]

            def up1(r0, m):
                g = {}

                def fin_u(k, u):
                    HF[pl.ds((k // 2) * HS + r0, m), ch(k % 2)] = gelu2(g[k], u)
                yield from _strassen(lambda i: _dot(XA[i, pl.ds(r0, m), :], B0[i, :, ch(0)]), g.__setitem__, RG)
                yield from _strassen(lambda i: _dot(XA[i, pl.ds(r0, m), :], B0[i, :, ch(1)]), fin_u, RU)

            with scope("start"):
                groups = [lambda: [cp_x(0, 0), cp_x(0, 1)], lambda: [cp_gu(0, 0, 0)], lambda: [cp_gu(0, 0, 1)]]
                groups += [(lambda i=i: [cp_x(i, 0), cp_x(i, 1)]) for i in range(1, NT0)]
                groups += [lambda: [cp_q(0)], lambda: [cp_gu(1, 1, 0), cp_gu(1, 1, 1), cp_d(0)],
                           lambda: [cp_q(1)], lambda: [cp_o()], lambda: [cp_q(2)]]

                def issue(k, c):
                    for g, cps in enumerate(groups):
                        when(k == g, lambda: [cp.start() for cp in cps()])
                    return c
                lax.fori_loop(0, len(groups), issue, 0)
                cp_x(0, 0).wait(); cp_x(0, 1).wait()

                def ln0(g, c):
                    for t in ln_tasks(pl.multiple_of(g * LN0, LN0), LN0, None):
                        t(None)
                    return c
                lax.fori_loop(0, T0 // LN0, ln0, 0)
                for which in range(2):
                    cp_gu(0, 0, which).wait()

                    def pg0(g, c):
                        prep_g1_tasks(which, pl.multiple_of(g * 64, 64), 64)
                        return c
                    lax.fori_loop(0, KH // 64, pg0, 0)

            def p0_body(i, c):
                cp_x(i + 1, 0).wait(); cp_x(i + 1, 1).wait()
                r0 = pl.multiple_of(i * T0, T0)
                _emit(LAG, up1(r0, T0), sum(RG) + sum(RU), (0.0, LNF, ln_tasks(r0 + T0, T0, zero(i))))
                return zero(i)
            with scope("p0"):
                z0 = lax.fori_loop(0, NT0 - 1, p0_body, 0)
            with scope("p0_last"):
                cp_q(0).wait()
                cp_gu(2, 0, 0).start(); cp_gu(2, 0, 1).start()
                _emit(LAG, up1(HS - T0, T0), sum(RG) + sum(RU), (0.0, 0.85, prep_q_tasks(0, 0, 0, z0)))

            def p1_body(b, c):
                with scope("p1i"):
                    return p1_body_(b, c)

            def p1_body_(b, c):
                when(b == 0, lambda: (cp_gu(1, 1, 0).wait(), cp_gu(1, 1, 1).wait(), cp_d(0).wait()))
                when(b == 1, lambda: cp_q(1).wait())
                when(b == 2, lambda: cp_o().wait())
                when(b == 3, lambda: cp_q(2).wait())
                m = b // 2
                par = b % 2

                def main():
                    for n in range(2):
                        for s in range(HS // RH):
                            r0 = s * RH

                            def fin(k, v):
                                j = m * NCH + par + 2 * n + 4 * (k % 2)
                                qkv[j, pl.ds(HALO + (k // 2) * HS + r0, RH), :] = v
                            yield from _strassen(lambda i: _dot(XA[i, pl.ds(r0, RH), :], BQ[i, :, ch(n)]), fin, (1,) * 7)
                piece = jnp.clip(b - 2, 0, 3)
                z = zero(b)
                _emit(LAG, main(), 14 * (HS // RH),
                      (0.0, P1A, prep_q_tasks(m, par, 1, z)),
                      (0.5, 0.5 + P1A, prep_q_tasks(jnp.minimum((b + 1) // 2, 2), (b + 1) % 2, 0, z)),
                      (0.0, 0.95, prep_g2_tasks(1, range(7), pl.multiple_of(piece * 64, 64), 64, z)),
                      (0.0, 0.95, xb_tasks(pl.multiple_of(jnp.minimum(b * 96, QS - 96), 16), 96, z)),
                      (0.0, 0.95, prep_d2_tasks(pl.multiple_of(piece * 32, 32), 32, z)),
                      (0.0, 0.95, zero_p_tasks(jnp.minimum(b * 38, 224 - 38), 38, z)),
                      (0.0, 0.95, prep_o_tasks(jnp.where(b < 2, 0, 3 * NCH), piece, z)))
                return c
            with scope("p1"):
                lax.fori_loop(0, 6, p1_body, 0)
                for j in range(NCH, 3 * NCH):
                    qkv[j, 0:HALO, :] = jnp.broadcast_to(qkv[j, HALO:HALO + 1, :], (HALO, NL))

        def second_half(OA, HA, osc, obuf):
            OA, HA = OA.bitcast(BF16), HA.bitcast(BF16)

            def attn_unit(r0, masked, slot, z):
                st = {}

                def shifted(plane):
                    return [qkv[plane, pl.ds(r0 + HALO + 8 - DIL * k, 8), :] for k in range(12)]

                def logits(val, j):
                    anchor(qkv.at[0], 0, val, z)
                    q = [qkv[j, pl.ds(r0 + HALO + 8 * g, 8), :] for g in range(2)]
                    kk = shifted(NCH + j)
                    for g in range(2):
                        for w in range(W):
                            t = q[g] * kk[w + 4 - 4 * g]
                            st[g, w] = t if j == 0 else st[g, w] + t
                    if j == NCH - 1:
                        softmax()

                def softmax():
                    lane = lax.broadcasted_iota(jnp.int32, (8, NL), 1)
                    odd = (lane & 1) != 0
                    hi = (lane & 16) != 0
                    keys = [(g, w) for g in range(2) for w in range(W)]
                    for k in keys:
                        a = st[k]
                        st[k] = a + jnp.where(odd, pltpu.roll(a, 1, 1), pltpu.roll(a, NL - 1, 1))
                    for k in keys:
                        a = st[k]
                        st[k] = a + jnp.where(hi, pltpu.roll(a, 16, 1), pltpu.roll(a, NL - 16, 1))
                    for g in range(2):
                        ls = [st[g, w] for w in range(W)]
                        if masked:
                            pos = r0 + 8 * g + lax.broadcasted_iota(jnp.int32, (8, NL), 0)
                            ls = [ls[0]] + [jnp.where(pos >= DIL * w, ls[w], NEG) for w in range(1, W)]
                        m = ls[0]
                        for w in range(1, W):
                            m = jnp.maximum(m, ls[w])
                        ps = [jnp.exp2((l - m) * EXP2_SCALE) for l in ls]
                        den = ps[0]
                        for w in range(1, W):
                            den = den + ps[w]
                        inv = 1.0 / den
                        for w in range(W):
                            st[g, w] = ps[w] * inv

                def pv(val, j):
                    anchor(qkv.at[0], 0, val, z)
                    vv = shifted(2 * NCH + j)
                    for g in range(2):
                        a = st[g, 0] * vv[4 - 4 * g]
                        for w in range(1, W):
                            a = a + st[g, w] * vv[w + 4 - 4 * g]
                        osc[slot, j, pl.ds(8 * g, 8), :] = a

                return ([(lambda val, j=j: logits(val, j)) for j in range(NCH)] + [lambda val: None] * AGAP
                        + [(lambda val, j=j: pv(val, j)) for j in range(NCH)])

            def attn_tasks(t0, n, z):
                if 'noattn' in EXP or n == 0:
                    return []
                t0 = pl.multiple_of(jnp.minimum(t0, HS - n), 16)
                tasks = []
                for g in range(n // 16):
                    r = t0 + g * 16
                    tasks += attn_unit(r, g == 0, 2 * g, z) + attn_unit(HS + r, False, 2 * g + 1, z)

                    def oa(val, kc, g=g, r=r):
                        ops = _ops(_A_TERMS, osc[2 * g, kc], osc[2 * g, KC + kc],
                                   osc[2 * g + 1, kc], osc[2 * g + 1, KC + kc])
                        for i in range(7):
                            OA.at[i][pl.ds(r, 16), ch(kc)] = ops[i].astype(BF16)
                    tasks += [(lambda val, kc=kc, oa=oa: oa(val, kc)) for kc in range(KC)]
                return tasks

            def ha_task(val, r, i, z, have):
                anchor(HF, S, val, z)
                x = [_combine(_A_TERMS[i], lambda sg, kp: HF[pl.ds((2 * sg + rho) * QS + r, 16), ch(2 * kp + ta)])
                     for rho in range(2) for ta in range(2)]
                for k, op in enumerate(_ops(_A_TERMS, *x)):
                    HA[pl.ds(r, 16), ch(7 * i + k)] = op.astype(BF16)
                have.add((i, r))

            def up2(kp, free, on_half):
                def sub(r0, m):
                    hold, seen = {}, set()

                    def outer_fin(k, K, v):
                        if K in (2, 1):
                            hold[k] = v
                            return
                        sg = K // 2
                        HF[pl.ds((2 * sg + k // 2) * QS + r0, m), ch(2 * kp + k % 2)] = (
                            gelu2(hold[k], v) if K == 3 else gelu2(v, hold[k]))
                        seen.add((sg, k))
                        if all((sg, j) in seen for j in range(4)):
                            on_half(sg, r0, m)
                    folds = [_Fold(lambda K, v, k=k: outer_fin(k, K, v)) for k in range(4)]

                    def lhs(i, k):
                        if k == 2:
                            return XA[i, pl.ds(r0, m), pl.ds(0, KQ)]
                        if k == 3:
                            return XA[i, pl.ds(QS + r0, m), pl.ds(KQ, KQ)]
                        return XB[5 * i + _XB_SLOT[k], pl.ds(r0, m), :]
                    return lambda i: _strassen(lambda k: _dot(lhs(i, k), BG[i, :, ch(k)]),
                                               lambda k, v: folds[k](i, v), R2H if i in (2, 6) else R2L)
                subs = [sub(s * RH2, RH2) for s in range(QS // RH2)]
                for i in _ORDER:
                    for sb in subs:
                        yield from sb(i)
                    free.add(i)

            nsub = QS // RH2
            g_room = (5 * sum(R2L) + 2 * sum(R2H)) * nsub
            d_unit = RD2 * MD * ND / (RH2 * KQ)

            ends = [sum(sum(R2H if i in (2, 6) else R2L) for i in _ORDER[:j + 1]) * nsub for j in range(7)]

            def bg_sides(slot, total, z, free, n):
                return [((ends[j] + 1) / total, (ends[j + 1] if j < 6 else ends[6] + ends[0]) / total - 0.01,
                         prep_g2_tasks(slot, _ORDER[j:j + 1], 0, KQ, z, free)) for j in range(n)]

            def block_b(k):
                when(k < NP - 1, lambda: (cp_gu(0, 0, 0).wait(), cp_gu(0, 0, 1).wait()))

                def prefetch(val):
                    when(k < NP - 1, lambda: (cp_gu(2 * k + 3, 1, 0).start(), cp_gu(2 * k + 3, 1, 1).start(),
                                              cp_d(k + 1).start()))
                z = zero(k)
                free, have, halves = set(), set(), set()

                def on_half(sg, r0, m):
                    if r0 + m == QS:
                        halves.add(sg)

                def ha_tasks(outer, need):
                    def task(val, r, i):
                        assert need <= halves
                        ha_task(val, r, i, z, have)
                    return [(lambda val, r=r, i=i: task(val, r, i)) for i in outer for r in range(0, QS, 16)]

                def main():
                    yield from up2(1, free, on_half)
                    for i in (2, 5, 1, 3, 0, 4, 6):
                        assert all((i, r) in have for r in range(0, QS, 16))
                        for r0 in range(0, QS, MD):
                            for c in range(KQ // ND):
                                def fin(q, v):
                                    P[i, pl.ds((q // 2) * QS + r0, MD), pl.ds((q % 2) * KQ + c * ND, ND)] += v
                                yield from _strassen(
                                    lambda j: _dot(HA[pl.ds(r0, MD), ch(7 * i + j)], BD[7 * i + j, :, ch(c, ND)]),
                                    fin, (d_unit,) * 7)
                total = g_room + 49 * (QS // MD) * (KQ // ND) * d_unit
                gf = g_room / total
                df = (1 - gf) / 7
                att = attn_tasks(k * (APA + APB), APB, z)
                if ATS is None:
                    att_sides = [(0.0, ATB, att)]
                else:
                    cut = len(att) * ATS // (APB // 16)
                    att_sides = [(0.0, ATE * gf, att[:cut]), (gf + HA2 * df, ATB, att[cut:])]
                _emit(LAG2, main(), total, *bg_sides(0, total, z, free, 7),
                      (0.0, ends[0] / total, prep_g2_tasks(1, _ORDER[6:], 0, KQ, z)),
                      (0.0, HAF * gf, ha_tasks((2, 5), set())),
                      ((ends[4] + 1) / total, gf + HA1 * df, ha_tasks((1, 3, 0), {1})),
                      (gf + HA1 * df, gf + HA2 * df, ha_tasks((4, 6), {0, 1})),
                      (0.0, PDB * gf, prep_d2_tasks(NL - PDN, PDN, z)),
                      *att_sides,
                      (gf, gf + 0.01, [prefetch]))

            def block_a(k):
                cp_gu(0, 1, 0).wait(); cp_gu(0, 1, 1).wait(); cp_d(0).wait()

                def prefetch(val):
                    when(k < NP - 2, lambda: (cp_gu(2 * k + 4, 0, 0).start(), cp_gu(2 * k + 4, 0, 1).start()))
                z = zero(k)
                free = set()
                _emit(LAG2, up2(0, free, lambda *a: None), g_room, *bg_sides(1, g_room, z, free, 6),
                      (0.0, 0.95, prep_d2_tasks(0, NL - PDN, z)),
                      (0.0, 0.95, attn_tasks(k * (APA + APB) + APB, APA, z)),
                      (0.01, 0.02, [prefetch]))

            def p2_body(k, carry):
                with scope("b"):
                    block_b(k)
                with scope("a"):
                    when(k < NP - 1, lambda: block_a(k))
                return carry
            with scope("p2"):
                lax.fori_loop(0, NP, p2_body, 0)

            def cp_out(t, half, s):
                return pltpu.make_async_copy(obuf.at[t % 2, half, pl.ds(s * M3, M3), :],
                                             out_hbm.at[pl.ds(half * HS + t * T3 + s * M3, M3), :], sem_out.at[t % 2])

            def wait_out(t):
                pltpu.make_async_copy(obuf.at[t % 2], obuf.at[t % 2], sem_out.at[t % 2]).wait()

            def p3_body(t, carry):
                when(t >= 2, lambda: wait_out(t - 2))
                for s in range(T3 // M3):
                    r0 = pl.multiple_of(t * T3 + s * M3, M3)
                    for n in range(KC):
                        def fin(k, sq):
                            (j0, _), *rest = _C_TERMS[k]
                            f = P[j0, pl.ds(r0, M3), ch(n)]
                            for j, sign in rest:
                                f = f + P[j, pl.ds(r0, M3), ch(n)] if sign > 0 else f - P[j, pl.ds(r0, M3), ch(n)]
                            y = f * 0.25
                            half, col = k // 2, (k % 2) * KC + n
                            x = xbuf[pl.ds(half * HS + r0, M3), ch(col)].astype(F32)
                            obuf.at[t % 2, half][pl.ds(s * M3, M3), ch(col)] = (
                                x + sq * (y + y * jnp.tanh(y))).astype(BF16)
                        for step, _ in enumerate(_strassen(
                                lambda i: _dot(OA[i, pl.ds(r0, M3), :], BO[i, :, ch(n)]), fin, (1,) * 7)):
                            if s > 0 and n == 0 and step == OUTK:
                                cp_out(t, 0, s - 1).start(); cp_out(t, 1, s - 1).start()
                cp_out(t, 0, T3 // M3 - 1).start(); cp_out(t, 1, T3 // M3 - 1).start()
                return carry
            with scope("p3"):
                lax.fori_loop(0, NT3, p3_body, 0)
            with scope("end"):
                for t in range(NT3 - 2, NT3):
                    wait_out(t)

        pl.run_scoped(first_half,
                      pltpu.VMEM((S + 8, D), F32),
                      pltpu.VMEM((7, KH // 2, 2 * NL), U32),
                      pltpu.VMEM((7, KH // 2, 2 * NL), U32),
                      pltpu.VMEM((4 * NCH, D // 2 + 8, NL), U32))
        pl.run_scoped(second_half,
                      pltpu.VMEM((7, HS // 2, KH), U32),
                      pltpu.VMEM((QS // 2, 49 * NL), U32),
                      pltpu.VMEM((max(APA, APB) // 8, NCH, 16, NL), F32),
                      pltpu.VMEM((2, 2, T3, D), BF16))

    def fn(A_x, A_wqkv, A_wo, B_x, B_w_gate, B_w_up, B_w_down):
        x = A_x.reshape(S, D)
        anyspec = pl.BlockSpec(memory_space=pl.ANY)
        out = pl.pallas_call(
            kernel,
            in_specs=[anyspec] * 6,
            out_specs=anyspec,
            out_shape=jax.ShapeDtypeStruct((S, D), BF16),
            scratch_shapes=[
                pltpu.VMEM((S + 16, D), BF16),
                pltpu.VMEM((7, HS // 2, KH), U32),
                pltpu.VMEM((35, QS // 2, KQ), U32),
                pltpu.VMEM((3 * NCH, HALO + S, NL), F32),
                pltpu.VMEM((7, HS, KH), F32),
                pltpu.VMEM((S + 8, 2 * FC), F32),
                pltpu.VMEM((7, KQ // 2, 7 * NL), U32),
                pltpu.VMEM((49, NL // 2, KQ), U32),
                pltpu.VMEM((7, KH // 2, KH), U32),
                pltpu.VMEM((2, 2, D + 16, FC), BF16),
                pltpu.VMEM((2 * FC + 16, D), BF16),
                pltpu.SemaphoreType.DMA((NT0, 2)),
                pltpu.SemaphoreType.DMA((2, 2)),
                pltpu.SemaphoreType.DMA((1,)),
                pltpu.SemaphoreType.DMA((3,)),
                pltpu.SemaphoreType.DMA((1,)),
                pltpu.SemaphoreType.DMA((2,)),
            ],
            compiler_params=pltpu.CompilerParams(vmem_limit_bytes=124 * 2 ** 20, disable_bounds_checks=True),
        )(x, A_wqkv, A_wo, B_w_gate, B_w_up, B_w_down)
        return out.reshape(1, S, D)
    return jax.jit(fn)


_IMPL = make()


@jax.jit
def pallas_recurrent_scan__sliding_local_dilated__geglu_ffn__prompt_kernel(
    A_x: jax.Array,
    A_wqkv: jax.Array,
    A_wo: jax.Array,
    B_x: jax.Array,
    B_w_gate: jax.Array,
    B_w_up: jax.Array,
    B_w_down: jax.Array,
):
    return _IMPL(A_x, A_wqkv, A_wo, B_x, B_w_gate, B_w_up, B_w_down)
```

```python
import contextlib
import math

import jax
import jax.numpy as jnp
from jax import lax
import jax.experimental.pallas as pl
import jax.experimental.pallas.tpu as pltpu

S, D, F = 2048, 1024, 3584
H, DH, W, DIL = 32, 32, 8, 2
NL = 128
NCH = D // NL
HS = S // 2
KH = D // 2
KC = KH // NL
QS = S // 4
KQ = D // 4
FC = 256
NP = F // (2 * FC)
HALO = 16
SPARE = 48
F32, BF16, U32 = jnp.float32, jnp.bfloat16, jnp.uint32
EPS = 1e-5
GELU_C0 = math.sqrt(2.0 / math.pi)
GELU_C1 = GELU_C0 * 0.044715
EXP2_SCALE = (DH ** -0.5) * math.log2(math.e)
NEG = -1e9 / (DH ** -0.5)

_A_TERMS = (((0, 0, 1), (1, 1, 1)), ((1, 0, 1), (1, 1, 1)), ((0, 0, 1),), ((1, 1, 1),),
            ((0, 0, 1), (0, 1, 1)), ((1, 0, 1), (0, 0, -1)), ((0, 1, 1), (1, 1, -1)))
_B_TERMS = (((0, 0, 1), (1, 1, 1)), ((0, 0, 1),), ((0, 1, 1), (1, 1, -1)), ((1, 0, 1), (0, 0, -1)),
            ((1, 1, 1),), ((0, 0, 1), (0, 1, 1)), ((1, 0, 1), (1, 1, 1)))
_C_TERMS = (((0, 1), (3, 1), (4, -1), (6, 1)), ((2, 1), (4, 1)), ((1, 1), (3, 1)), ((0, 1), (1, -1), (2, 1), (5, 1)))
_ORDER = (1, 3, 0, 5, 2, 4, 6)
_XB_SLOT = {0: 0, 1: 1, 4: 2, 5: 3, 6: 4}


def _combine(terms, get):
    (r, c, _), *rest = terms
    v = get(r, c)
    for r, c, sign in rest:
        v = v + get(r, c) if sign > 0 else v - get(r, c)
    return v


def _ops(terms, q11, q12, q21, q22):
    q = ((q11, q12), (q21, q22))
    return [_combine(t, lambda r, c: q[r][c]) for t in terms]


def _dot(a, b):
    return jnp.dot(a, b, preferred_element_type=F32)


class _Fold:
    def __init__(self, fin):
        self.fin = fin

    def __call__(self, i, m):
        if i == 1:
            self.m1 = m
        elif i == 3:
            self.fin(2, self.m1 + m)
            self.t11 = m
        elif i == 0:
            self.t11 = self.t11 + m
            self.t22 = m - self.m1
        elif i == 5:
            self.t22 = self.t22 + m
        elif i == 2:
            self.fin(3, self.t22 + m)
            self.m2 = m
        elif i == 4:
            self.fin(1, self.m2 + m)
            self.t11 = self.t11 - m
        else:
            self.fin(0, self.t11 + m)


def _strassen(prod, fin, room):
    fold = _Fold(fin)
    for step, i in enumerate(_ORDER):
        m = prod(i)
        fold(i, m)
        yield room[step], m


def _emit(lag, main, total, *sides, dyn=None, dyn_rate=0, dyn_delay=0):
    done = [0] * len(sides)
    acc = step = 0

    def flush(frac, val):
        due = []
        for k, (f0, f1, tasks) in enumerate(sides):
            want = len(tasks) if frac >= f1 else int(max(0.0, (frac - f0) / (f1 - f0)) * len(tasks) + 0.5)
            n = min(want, len(tasks)) - done[k]
            due += [((j + 0.5) / n, k, tasks[done[k] + j]) for j in range(n)]
            done[k] += max(n, 0)
        if dyn:
            rate = dyn_rate
            ready = [e for e in dyn if e[0] + dyn_delay <= step][:rate]
            for j, e in enumerate(ready):
                dyn.remove(e)
                due.append(((j + 0.5) / len(ready), -1, e[1]))
        due.sort(key=lambda e: e[:2])
        for j, (_, _, task) in enumerate(due):
            if val is None:
                task(None)
            else:
                r = (val.shape[0] // 8) * j // len(due) * 8
                task(val[r:r + 8, 0:NL])

    hist = [(0, None)] * lag
    for item in main:
        step += 1
        for e in dyn or ():
            if e[0] is None:
                e[0] = step
        hist.append(item)
        room, val = hist.pop(0)
        acc += room
        if room:
            flush(acc / total, val)
    acc += sum(h[0] for h in hist)
    assert abs(acc - total) < 1e-6 and not dyn, (acc, total)
    flush(2.0, hist[-1][1] if hist else val)


def _skew(items):
    depth = max(len(st) for st in items)
    return [items[t - k][k] for t in range(len(items) + depth - 1) for k in range(depth)
            if 0 <= t - k < len(items) and k < len(items[t - k]) and items[t - k][k] is not None]


def make(EXP='', ONEPASS=True, T0=128, LN0=64, LNF=0.8, RG=(2,) * 7, RU=(2, 1, 2, 2, 1, 1, 1),
         RH=256, LAG=1, P1A=0.44,
         RH2=64, LAG2=4, PG0=1.5, R2L=(2,) * 7, R2H=(2, 0, 2, 2, 0, 0, 0), MD=128, ND=128, RD2=2, DRATE=2, DDELAY=4,
         APA=32, APB=128, AGAP=4, HAF=0.6, HA1=2.0, HA2=4.6, ATS=None, ATE=0.75, ATB=0.97, PDN=64, PDB=0.8,
         M3=64, OUTK=1, LAG3=1, scopes=False):
    NT0 = HS // T0
    T3 = 256
    NT3 = HS // T3
    assert NL - PDN <= 96
    assert (NP - 1) * APA + NP * APB >= HS and APA % 16 == 0 and APB % 16 == 0

    def scope(name):
        return jax.named_scope(name) if scopes else contextlib.nullcontext()

    def kernel(x_hbm, wqkv_hbm, wo_hbm, wg_hbm, wu_hbm, wd_hbm, out_hbm,
               xbuf, XA, XB, qkv, P, HF, BG, BD, BO, rgu, rd,
               sem_x, sem_gu, sem_d, sem_q, sem_o, sem_out):

        XA, XB, BG, BD, BO = [r.bitcast(BF16) for r in (XA, XB, BG, BD, BO)]

        def ch(n, w=NL):
            return pl.ds(n * w, w) if isinstance(n, int) else pl.ds(pl.multiple_of(n * w, w), w)

        def zero(i):
            return i % 2 + (i + 1) % 2 - 1

        def when(pred, fn):
            pl.when(pred)(lambda: (fn(), None)[1])

        def cp_x(i, half):
            r = half * HS + i * T0
            return pltpu.make_async_copy(x_hbm.at[pl.ds(r, T0), :], xbuf.at[pl.ds(r, T0), :], sem_x.at[i, half])

        def cp_gu(c, slot, which):
            src = wg_hbm if which == 0 else wu_hbm
            return pltpu.make_async_copy(src.at[:, pl.ds(c * FC, FC)], rgu.at[slot, which, pl.ds(0, D), :],
                                         sem_gu.at[slot, which])

        def cp_d(p):
            return pltpu.make_async_copy(wd_hbm.at[pl.ds(p * 2 * FC, 2 * FC), :], rd.at[pl.ds(0, 2 * FC), :],
                                         sem_d.at[0])

        def anchor(dst, row, val, z):
            if val is not None and z is not None:
                r = pl.multiple_of(row + 16 + z * 16, 8)
                dst[pl.ds(r, 8), pl.ds(0, NL)] = pltpu.bitcast(val, U32) if dst.dtype == U32 else val.astype(dst.dtype)

        def gelu2(g, u):
            t = jnp.tanh(g * (GELU_C0 + GELU_C1 * (g * g)))
            p = g * u
            return p + p * t

        def prep_g2_tasks(slot, outer, r0, n, z, free=None):
            def task(val, r, i):
                assert free is None or i in free
                anchor(rgu.at[0, 0], D, val, z)
                y = [_combine(_B_TERMS[i], lambda kp, mu: rgu[slot, mu, pl.ds((2 * kp + ta) * KQ + r, 16), :].astype(F32))
                     for ta in range(2)]
                ops = _ops(_B_TERMS, y[0][:, :NL], y[0][:, NL:], y[1][:, :NL], y[1][:, NL:])
                for k in range(7):
                    BG.at[i][pl.ds(r, 16), ch(k)] = ops[k].astype(BF16)
            return [(lambda val, r=r0 + g * 16, i=i: task(val, r, i)) for i in outer for g in range(n // 16)]

        def prep_d2_tasks(r0, n, z):
            def task(val, r, i):
                anchor(rd, 2 * FC, val, z)
                y = [_combine(_B_TERMS[i],
                              lambda kp, nu: rd[pl.ds((2 * kp + ta) * NL + r, 16), ch(2 * nu + up, KQ)].astype(F32))
                     for ta in range(2) for up in range(2)]
                ops = _ops(_B_TERMS, *y)
                for k in range(7):
                    BD.at[7 * i + k][pl.ds(r, 16), :] = ops[k].astype(BF16)
            return [(lambda val, r=r0 + g * 16, i=i: task(val, r, i)) for g in range(n // 16) for i in range(7)]

        def first_half(Y, B0, BQ, rq):
            B0, BQ = B0.bitcast(BF16), BQ.bitcast(BF16)

            class cp_cols:
                def __init__(self, src, col0, dst, slot0, sem):
                    self.args = src, col0, dst, slot0, sem

                def start(self):
                    src, col0, dst, slot0, sem = self.args
                    for k in range(NCH):
                        pltpu.make_async_copy(src.at[:, pl.ds(col0 + k * NL, NL)],
                                              dst.at[slot0 + k, pl.ds(0, D // 2), :].bitcast(BF16), sem).start()

                def wait(self):
                    _, _, dst, slot0, sem = self.args
                    whole = dst.at[pl.ds(slot0, NCH), pl.ds(0, D // 2), :]
                    pltpu.make_async_copy(whole, whole, sem).wait()

            def cp_q(m):
                return cp_cols(wqkv_hbm, m * D, rq, m * NCH, sem_q.at[m])

            def cp_o():
                return cp_cols(wo_hbm, 0, rq, 3 * NCH, sem_o.at[0])

            def ln_tasks(r0, n, z):
                def xrow(r):
                    return xbuf[pl.ds(r, 16), :].astype(F32)
                items = []
                for g in range(n // 16):
                    st = {}
                    for half in range(2):
                        def s0(val, r=half * HS + r0 + g * 16, st=st, half=half):
                            anchor(xbuf, S, val, z)
                            st["m", half] = jnp.sum(xrow(r), axis=-1, keepdims=True) * (1.0 / D)

                        def s1(val, r=half * HS + r0 + g * 16, st=st, half=half):
                            anchor(xbuf, S, val, z)
                            c = xrow(r) - st["m", half]
                            st["v", half] = lax.rsqrt(jnp.sum(c * c, axis=-1, keepdims=True) * (1.0 / D) + EPS)

                        def s01(val, r=half * HS + r0 + g * 16, st=st, half=half):
                            anchor(xbuf, S, val, z)
                            x = xrow(r)
                            m = jnp.sum(x, axis=-1, keepdims=True) * (1.0 / D)
                            e2 = jnp.sum(x * x, axis=-1, keepdims=True) * (1.0 / D)
                            st["m", half] = m
                            st["v", half] = lax.rsqrt(jnp.maximum(e2 - m * m, 0.0) + EPS)

                        def s2(val, r=r0 + g * 16, st=st, half=half):
                            for kc in (2 * half, 2 * half + 1):
                                anchor(xbuf, S, val, z)
                                pos = [(h, c) for h in range(2) for c in (kc, KC + kc)]
                                q = [(xbuf[pl.ds(h * HS + r, 16), ch(c)].astype(F32) - st["m", h]) * st["v", h]
                                     for h, c in pos]
                                for (h, c), y in zip(pos, q):
                                    Y[pl.ds(h * HS + r, 16), ch(c)] = y
                                for i, op in enumerate(_ops(_A_TERMS, *q)):
                                    XA.at[i][pl.ds(r, 16), ch(kc)] = op.astype(BF16)
                        stats = [s01] if ONEPASS else [s0, None, s1]
                        items.append(stats + [None] * (2 - half) + [s2])
                return _skew(items)

            def prep_g1_tasks(which, r0, n):
                for g in range(n // 16):
                    r = r0 + g * 16
                    top = rgu[0, which, pl.ds(r, 16), :].astype(F32)
                    bot = rgu[0, which, pl.ds(KH + r, 16), :].astype(F32)
                    for i, op in enumerate(_ops(_B_TERMS, top[:, :NL], top[:, NL:], bot[:, :NL], bot[:, NL:])):
                        B0.at[i][pl.ds(r, 16), ch(which)] = op.astype(BF16)

            def xb_tasks(r0, n, z):
                def task(val, r, kc, i):
                    anchor(Y, S, val, z)
                    x = [_combine(_A_TERMS[i],
                                  lambda sg, kp: Y[pl.ds((2 * sg + rho) * QS + r, 16), ch(4 * kp + 2 * ta + kc)])
                         for rho in range(2) for ta in range(2)]
                    ops = _ops(_A_TERMS, *x)
                    for k, slot in _XB_SLOT.items():
                        XB.at[5 * i + slot][pl.ds(r, 16), ch(kc)] = ops[k].astype(BF16)
                return [(lambda val, r=r0 + g * 16, kc=kc, i=i: task(val, r, kc, i))
                        for g in range(n // 16) for kc in range(2) for i in range(7)]

            def wide(w):
                return pltpu.bitcast(w, BF16).astype(F32)

            def prep_q_tasks(m, par, n, z):
                def perm_a(r):
                    y = [rq[m * NCH + k, pl.ds(r // 2, 8), :] for k in range(NCH)]
                    return [y[0]] + [pltpu.roll(y[k], 2 * k, 1) for k in range(1, NCH)]

                def perm_b(y):
                    lane = lax.broadcasted_iota(jnp.int32, (8, NL), 1)
                    sh = (((lane & 15) >> 1) - par) & 7
                    u = [y[(-j) % NCH] for j in range(NCH)]
                    b0, b1, b2 = (sh & 1) != 0, (sh & 2) != 0, (sh & 4) != 0
                    out = (2 * n, 2 * n + 4)
                    v = {j: jnp.where(b0, u[(j - 1) % NCH], u[j]) for j in (0, 2, 4, 6)}
                    v = {j: jnp.where(b1, v[(j - 2) % NCH], v[j]) for j in out}
                    v = {j: jnp.where(b2, v[(j - 4) % NCH], v[j]) for j in out}
                    return [pltpu.roll(v[j], (2 * NL - 2 * j - 2 * par) % NL, 1) for j in out]

                items = []
                for g in range(KH // 16):
                    st = {}
                    for half in range(2):
                        def s0(val, r=half * KH + g * 16, st=st, half=half):
                            anchor(rq.at[0], D // 2, val, z)
                            st["a", half] = perm_a(r)

                        def s1(val, st=st, half=half):
                            st["b", half] = perm_b(st["a", half])

                        def s2(val, r=g * 16, st=st):
                            ops = _ops(_B_TERMS, *[wide(w) for w in st["b", 0] + st["b", 1]])
                            for i in range(7):
                                BQ.at[i][pl.ds(r, 16), ch(n)] = ops[i].astype(BF16)
                        items.append([s0, s1] + ([s2] if half else []))
                flat = _skew(items)
                firsts = [j for j, t in enumerate(flat) if t.__name__ == "s0"] + [len(flat)]
                return [(lambda val, grp=flat[a:b]: [t(val) for t in grp]) for a, b in zip(firsts, firsts[1:])]

            def prep_o_tasks(src, n, z):
                def transpose(c, a):
                    sub = lax.broadcasted_iota(jnp.int32, (8, NL), 0)
                    y = [rq[src + c, pl.ds(64 * g + 8 * a, 8), :] for g in range(8)]
                    y = [y[0]] + [pltpu.roll(y[g], g, 0) for g in range(1, 8)]
                    v = [y[(-j) % 8] for j in range(8)]
                    for bit in (1, 2, 4):
                        v = [jnp.where((sub & bit) != 0, v[(j - bit) % 8], v[j]) for j in range(8)]
                    return [v[0]] + [pltpu.roll(v[j], 8 - j, 0) for j in range(1, 8)]

                tasks = []
                for a in range(8):
                    st = {}

                    def load(val, h, a=a, st=st):
                        anchor(rq.at[0], D // 2, val, z)
                        st[h] = transpose(h * KC + n, a)

                    def quad(val, jj, a=a, st=st):
                        q = [wide(st[h][kh * KC + jj]) for kh in range(2) for h in range(2)]
                        for i, op in enumerate(_ops(_B_TERMS, *q)):
                            BO.at[i][pl.ds(jj * NL + 16 * a, 16), ch(n)] = op.astype(BF16)
                    tasks += [lambda val, f=load: f(val, 0),
                              lambda val, f=load, g=quad: (f(val, 1), [g(val, jj) for jj in range(KC)])]
                return tasks

            def zero_p_tasks(u0, n, z):
                def task(val, u):
                    v = jnp.zeros((8, NL), F32) if val is None else jnp.where(z != 0, val, 0.0)
                    P[u // 32, pl.ds(pl.multiple_of((u % 32) * 32, 32), 32), :] = jnp.tile(v, (4, KC))
                return [(lambda val, u=u0 + j: task(val, u)) for j in range(n)]

            def up1(r0, m):
                g = {}

                def fin_u(k, u):
                    HF[pl.ds((k // 2) * HS + r0, m), ch(k % 2)] = gelu2(g[k], u)
                yield from _strassen(lambda i: _dot(XA[i, pl.ds(r0, m), :], B0[i, :, ch(0)]), g.__setitem__, RG)
                yield from _strassen(lambda i: _dot(XA[i, pl.ds(r0, m), :], B0[i, :, ch(1)]), fin_u, RU)

            with scope("start"):
                groups = [lambda: [cp_x(0, 0), cp_x(0, 1)], lambda: [cp_gu(0, 0, 0)], lambda: [cp_gu(0, 0, 1)]]
                groups += [(lambda i=i: [cp_x(i, 0), cp_x(i, 1)]) for i in range(1, NT0)]
                groups += [lambda: [cp_q(0)], lambda: [cp_gu(1, 1, 0), cp_gu(1, 1, 1), cp_d(0)],
                           lambda: [cp_q(1)], lambda: [cp_o()], lambda: [cp_q(2)]]

                def issue(k, c):
                    for g, cps in enumerate(groups):
                        when(k == g, lambda: [cp.start() for cp in cps()])
                    return c
                lax.fori_loop(0, len(groups), issue, 0)
                cp_x(0, 0).wait(); cp_x(0, 1).wait()

                def ln0(g, c):
                    for t in ln_tasks(pl.multiple_of(g * LN0, LN0), LN0, None):
                        t(None)
                    return c
                lax.fori_loop(0, T0 // LN0, ln0, 0)
                for which in range(2):
                    cp_gu(0, 0, which).wait()

                    def pg0(g, c):
                        prep_g1_tasks(which, pl.multiple_of(g * 64, 64), 64)
                        return c
                    lax.fori_loop(0, KH // 64, pg0, 0)

            def p0_body(i, c):
                cp_x(i + 1, 0).wait(); cp_x(i + 1, 1).wait()
                r0 = pl.multiple_of(i * T0, T0)
                _emit(LAG, up1(r0, T0), sum(RG) + sum(RU), (0.0, LNF, ln_tasks(r0 + T0, T0, zero(i))))
                return zero(i)
            with scope("p0"):
                z0 = lax.fori_loop(0, NT0 - 1, p0_body, 0)
            with scope("p0_last"):
                cp_q(0).wait()
                cp_gu(2, 0, 0).start(); cp_gu(2, 0, 1).start()
                _emit(LAG, up1(HS - T0, T0), sum(RG) + sum(RU), (0.0, 0.85, prep_q_tasks(0, 0, 0, z0)))

            def p1_body(b, c):
                with scope("p1i"):
                    return p1_body_(b, c)

            def p1_body_(b, c):
                when(b == 0, lambda: (cp_gu(1, 1, 0).wait(), cp_gu(1, 1, 1).wait(), cp_d(0).wait()))
                when(b == 1, lambda: cp_q(1).wait())
                when(b == 2, lambda: cp_o().wait())
                when(b == 3, lambda: cp_q(2).wait())
                m = b // 2
                par = b % 2

                def main():
                    for n in range(2):
                        for s in range(HS // RH):
                            r0 = s * RH

                            def fin(k, v):
                                j = m * NCH + par + 2 * n + 4 * (k % 2)
                                qkv[j, pl.ds(HALO + (k // 2) * HS + r0, RH), :] = v
                            yield from _strassen(lambda i: _dot(XA[i, pl.ds(r0, RH), :], BQ[i, :, ch(n)]), fin, (1,) * 7)
                piece = jnp.clip(b - 2, 0, 3)
                z = zero(b)
                _emit(LAG, main(), 14 * (HS // RH),
                      (0.0, P1A, prep_q_tasks(m, par, 1, z)),
                      (0.5, 0.5 + P1A, prep_q_tasks(jnp.minimum((b + 1) // 2, 2), (b + 1) % 2, 0, z)),
                      (0.0, 0.95, prep_g2_tasks(1, range(7), pl.multiple_of(jnp.minimum(b * 48, KQ - 48), 16), 48, z)),
                      (0.0, 0.95, xb_tasks(pl.multiple_of(jnp.minimum(b * 96, QS - 96), 32), 96, z)),
                      (0.0, 0.95, prep_d2_tasks(pl.multiple_of(jnp.minimum(b * 16, NL - PDN - 16), 16), 16, z)),
                      (0.0, 0.95, zero_p_tasks(jnp.minimum(b * 38, 224 - 38), 38, z)),
                      (0.0, 0.95, prep_o_tasks(jnp.where(b < 2, 0, 3 * NCH), piece, z)))
                return c
            with scope("p1"):
                lax.fori_loop(0, 6, p1_body, 0)
                for j in range(NCH, 3 * NCH):
                    qkv[j, 0:HALO, :] = jnp.broadcast_to(qkv[j, HALO:HALO + 1, :], (HALO, NL))

        def second_half(OA, HA, osc, obuf):
            OA, HA = OA.bitcast(BF16), HA.bitcast(BF16)

            def attn_unit(r0, masked, slot, z):
                st = {}

                def shifted(plane):
                    return [qkv[plane, pl.ds(r0 + HALO + 8 - DIL * k, 8), :] for k in range(12)]

                def logits(val, j):
                    anchor(qkv.at[0], HALO + S, val, z)
                    q = [qkv[j, pl.ds(r0 + HALO + 8 * g, 8), :] for g in range(2)]
                    kk = shifted(NCH + j)
                    for g in range(2):
                        for w in range(W):
                            t = q[g] * kk[w + 4 - 4 * g]
                            st[g, w] = t if j == 0 else st[g, w] + t
                    if j == NCH - 1:
                        softmax()

                def softmax():
                    lane = lax.broadcasted_iota(jnp.int32, (8, NL), 1)
                    odd = (lane & 1) != 0
                    hi = (lane & 16) != 0
                    keys = [(g, w) for g in range(2) for w in range(W)]
                    for k in keys:
                        a = st[k]
                        st[k] = a + jnp.where(odd, pltpu.roll(a, 1, 1), pltpu.roll(a, NL - 1, 1))
                    for k in keys:
                        a = st[k]
                        st[k] = a + jnp.where(hi, pltpu.roll(a, 16, 1), pltpu.roll(a, NL - 16, 1))
                    for g in range(2):
                        ls = [st[g, w] for w in range(W)]
                        if masked:
                            pos = r0 + 8 * g + lax.broadcasted_iota(jnp.int32, (8, NL), 0)
                            ls = [ls[0]] + [jnp.where(pos >= DIL * w, ls[w], NEG) for w in range(1, W)]
                        m = ls[0]
                        for w in range(1, W):
                            m = jnp.maximum(m, ls[w])
                        ps = [jnp.exp2((l - m) * EXP2_SCALE) for l in ls]
                        den = ps[0]
                        for w in range(1, W):
                            den = den + ps[w]
                        inv = 1.0 / den
                        for w in range(W):
                            st[g, w] = ps[w] * inv

                def pv(val, j):
                    anchor(qkv.at[0], HALO + S, val, z)
                    vv = shifted(2 * NCH + j)
                    for g in range(2):
                        a = st[g, 0] * vv[4 - 4 * g]
                        for w in range(1, W):
                            a = a + st[g, w] * vv[w + 4 - 4 * g]
                        osc[slot, j, pl.ds(8 * g, 8), :] = a

                return ([(lambda val, j=j: logits(val, j)) for j in range(NCH)] + [lambda val: None] * AGAP
                        + [(lambda val, j=j: pv(val, j)) for j in range(NCH)])

            def attn_tasks(t0, n, z):
                if 'noattn' in EXP or n == 0:
                    return []
                t0 = pl.multiple_of(jnp.minimum(t0, HS - n), 16)
                tasks = []
                for g in range(n // 16):
                    r = t0 + g * 16
                    tasks += attn_unit(r, g == 0, 2 * g, z) + attn_unit(HS + r, False, 2 * g + 1, z)

                    def oa(val, kc, g=g, r=r):
                        ops = _ops(_A_TERMS, osc[2 * g, kc], osc[2 * g, KC + kc],
                                   osc[2 * g + 1, kc], osc[2 * g + 1, KC + kc])
                        for i in range(7):
                            OA.at[i][pl.ds(r, 16), ch(kc)] = ops[i].astype(BF16)
                    tasks += [(lambda val, kc=kc, oa=oa: oa(val, kc)) for kc in range(KC)]
                return tasks

            def ha_task(val, r, i, z, have):
                anchor(HF, S, val, z)
                x = [_combine(_A_TERMS[i], lambda sg, kp: HF[pl.ds((2 * sg + rho) * QS + r, 16), ch(2 * kp + ta)])
                     for rho in range(2) for ta in range(2)]
                for k, op in enumerate(_ops(_A_TERMS, *x)):
                    HA[pl.ds(r, 16), ch(7 * i + k)] = op.astype(BF16)
                have.add((i, r))

            def up2(kp, free, on_half):
                def sub(r0, m):
                    hold, seen = {}, set()

                    def outer_fin(k, K, v):
                        if K in (2, 1):
                            hold[k] = v
                            return
                        sg = K // 2
                        HF[pl.ds((2 * sg + k // 2) * QS + r0, m), ch(2 * kp + k % 2)] = (
                            gelu2(hold[k], v) if K == 3 else gelu2(v, hold[k]))
                        seen.add((sg, k))
                        if all((sg, j) in seen for j in range(4)):
                            on_half(sg, r0, m)
                    folds = [_Fold(lambda K, v, k=k: outer_fin(k, K, v)) for k in range(4)]

                    def lhs(i, k):
                        if k == 2:
                            return XA[i, pl.ds(r0, m), pl.ds(0, KQ)]
                        if k == 3:
                            return XA[i, pl.ds(QS + r0, m), pl.ds(KQ, KQ)]
                        return XB[5 * i + _XB_SLOT[k], pl.ds(r0, m), :]
                    return lambda i: _strassen(lambda k: _dot(lhs(i, k), BG[i, :, ch(k)]),
                                               lambda k, v: folds[k](i, v), R2H if i in (2, 6) else R2L)
                subs = [sub(s * RH2, RH2) for s in range(QS // RH2)]
                for i in _ORDER:
                    for sb in subs:
                        yield from sb(i)
                    free.add(i)

            nsub = QS // RH2
            g_room = (5 * sum(R2L) + 2 * sum(R2H)) * nsub
            d_unit = RD2 * MD * ND / (RH2 * KQ)

            ends = [sum(sum(R2H if i in (2, 6) else R2L) for i in _ORDER[:j + 1]) * nsub for j in range(7)]

            def bg_sides(slot, total, z, free, n):
                return [((ends[j] + 1) / total, (ends[j + 1] if j < 6 else ends[6] + ends[0]) / total - 0.01,
                         prep_g2_tasks(slot, _ORDER[j:j + 1], 0, KQ, z, free)) for j in range(n)]

            def block_b(k):
                when(k < NP - 1, lambda: (cp_gu(0, 0, 0).wait(), cp_gu(0, 0, 1).wait()))

                def prefetch(val):
                    when(k < NP - 1, lambda: (cp_gu(2 * k + 3, 1, 0).start(), cp_gu(2 * k + 3, 1, 1).start(),
                                              cp_d(k + 1).start()))
                z = zero(k)
                free, have, halves = set(), set(), set()

                def on_half(sg, r0, m):
                    if r0 + m == QS:
                        halves.add(sg)

                def ha_tasks(outer, need):
                    def task(val, r, i):
                        assert need <= halves
                        ha_task(val, r, i, z, have)
                    return [(lambda val, r=r, i=i: task(val, r, i)) for i in outer for r in range(0, QS, 16)]

                def main():
                    yield from up2(1, free, on_half)
                    for i in (2, 5, 1, 3, 0, 4, 6):
                        assert all((i, r) in have for r in range(0, QS, 16))
                        for r0 in range(0, QS, MD):
                            for c in range(KQ // ND):
                                def fin(q, v):
                                    P[i, pl.ds((q // 2) * QS + r0, MD), pl.ds((q % 2) * KQ + c * ND, ND)] += v
                                yield from _strassen(
                                    lambda j: _dot(HA[pl.ds(r0, MD), ch(7 * i + j)], BD[7 * i + j, :, ch(c, ND)]),
                                    fin, (d_unit,) * 7)
                total = g_room + 49 * (QS // MD) * (KQ // ND) * d_unit
                gf = g_room / total
                df = (1 - gf) / 7
                att = attn_tasks(k * (APA + APB), APB, z)
                if ATS is None:
                    att_sides = [(0.0, ATB, att)]
                else:
                    cut = len(att) * ATS // (APB // 16)
                    att_sides = [(0.0, ATE * gf, att[:cut]), (gf + HA2 * df, ATB, att[cut:])]
                _emit(LAG2, main(), total, *bg_sides(0, total, z, free, 7),
                      (0.0, ends[0] / total, prep_g2_tasks(1, _ORDER[6:], 0, KQ, z)),
                      (0.0, HAF * gf, ha_tasks((2, 5), set())),
                      ((ends[4] + 1) / total, gf + HA1 * df, ha_tasks((1, 3, 0), {1})),
                      (gf + HA1 * df, gf + HA2 * df, ha_tasks((4, 6), {0, 1})),
                      (0.0, PDB * gf, prep_d2_tasks(NL - PDN, PDN, z)),
                      *att_sides,
                      (gf, gf + 0.01, [prefetch]))

            def block_a(k):
                cp_gu(0, 1, 0).wait(); cp_gu(0, 1, 1).wait(); cp_d(0).wait()

                def prefetch(val):
                    when(k < NP - 2, lambda: (cp_gu(2 * k + 4, 0, 0).start(), cp_gu(2 * k + 4, 0, 1).start()))
                z = zero(k)
                free = set()
                _emit(LAG2, up2(0, free, lambda *a: None), g_room, *bg_sides(1, g_room, z, free, 6),
                      (0.0, 0.95, prep_d2_tasks(0, NL - PDN, z)),
                      (0.0, 0.95, attn_tasks(k * (APA + APB) + APB, APA, z)),
                      (0.01, 0.02, [prefetch]))

            def p2_body(k, carry):
                with scope("b"):
                    block_b(k)
                with scope("a"):
                    when(k < NP - 1, lambda: block_a(k))
                return carry
            with scope("p2"):
                lax.fori_loop(0, NP, p2_body, 0)

            def cp_out(t, half, s):
                return pltpu.make_async_copy(obuf.at[t % 2, half, pl.ds(s * M3, M3), :],
                                             out_hbm.at[pl.ds(half * HS + t * T3 + s * M3, M3), :], sem_out.at[t % 2])

            def wait_out(t):
                pltpu.make_async_copy(obuf.at[t % 2], obuf.at[t % 2], sem_out.at[t % 2]).wait()

            def p3_body(t, carry):
                when(t >= 2, lambda: wait_out(t - 2))
                for s in range(T3 // M3):
                    r0 = pl.multiple_of(t * T3 + s * M3, M3)
                    for n in range(KC):
                        def fin(k, sq):
                            (j0, _), *rest = _C_TERMS[k]
                            f = P[j0, pl.ds(r0, M3), ch(n)]
                            for j, sign in rest:
                                f = f + P[j, pl.ds(r0, M3), ch(n)] if sign > 0 else f - P[j, pl.ds(r0, M3), ch(n)]
                            y = f * 0.25
                            half, col = k // 2, (k % 2) * KC + n
                            x = xbuf[pl.ds(half * HS + r0, M3), ch(col)].astype(F32)
                            obuf.at[t % 2, half][pl.ds(s * M3, M3), ch(col)] = (
                                x + sq * (y + y * jnp.tanh(y))).astype(BF16)
                        for step, _ in enumerate(_strassen(
                                lambda i: _dot(OA[i, pl.ds(r0, M3), :], BO[i, :, ch(n)]), fin, (1,) * 7)):
                            if s > 0 and n == 0 and step == OUTK:
                                cp_out(t, 0, s - 1).start(); cp_out(t, 1, s - 1).start()
                cp_out(t, 0, T3 // M3 - 1).start(); cp_out(t, 1, T3 // M3 - 1).start()
                return carry
            with scope("p3"):
                lax.fori_loop(0, NT3, p3_body, 0)
            with scope("end"):
                for t in range(NT3 - 2, NT3):
                    wait_out(t)

        pl.run_scoped(first_half,
                      pltpu.VMEM((S + SPARE, D), F32),
                      pltpu.VMEM((7, KH // 2, 2 * NL), U32),
                      pltpu.VMEM((7, KH // 2, 2 * NL), U32),
                      pltpu.VMEM((4 * NCH, D // 2 + SPARE, NL), U32))
        pl.run_scoped(second_half,
                      pltpu.VMEM((7, HS // 2, KH), U32),
                      pltpu.VMEM((QS // 2, 49 * NL), U32),
                      pltpu.VMEM((max(APA, APB) // 8, NCH, 16, NL), F32),
                      pltpu.VMEM((2, 2, T3, D), BF16))

    def fn(A_x, A_wqkv, A_wo, B_x, B_w_gate, B_w_up, B_w_down):
        x = A_x.reshape(S, D)
        anyspec = pl.BlockSpec(memory_space=pl.ANY)
        out = pl.pallas_call(
            kernel,
            in_specs=[anyspec] * 6,
            out_specs=anyspec,
            out_shape=jax.ShapeDtypeStruct((S, D), BF16),
            scratch_shapes=[
                pltpu.VMEM((S + SPARE, D), BF16),
                pltpu.VMEM((7, HS // 2, KH), U32),
                pltpu.VMEM((35, QS // 2, KQ), U32),
                pltpu.VMEM((3 * NCH, HALO + S + SPARE, NL), F32),
                pltpu.VMEM((7, HS, KH), F32),
                pltpu.VMEM((S + SPARE, 2 * FC), F32),
                pltpu.VMEM((7, KQ // 2, 7 * NL), U32),
                pltpu.VMEM((49, NL // 2, KQ), U32),
                pltpu.VMEM((7, KH // 2, KH), U32),
                pltpu.VMEM((2, 2, D + SPARE, FC), BF16),
                pltpu.VMEM((2 * FC + SPARE, D), BF16),
                pltpu.SemaphoreType.DMA((NT0, 2)),
                pltpu.SemaphoreType.DMA((2, 2)),
                pltpu.SemaphoreType.DMA((1,)),
                pltpu.SemaphoreType.DMA((3,)),
                pltpu.SemaphoreType.DMA((1,)),
                pltpu.SemaphoreType.DMA((2,)),
            ],
            compiler_params=pltpu.CompilerParams(vmem_limit_bytes=124 * 2 ** 20, disable_bounds_checks=True),
        )(x, A_wqkv, A_wo, B_w_gate, B_w_up, B_w_down)
        return out.reshape(1, S, D)
    return jax.jit(fn)


_IMPL = make()


@jax.jit
def pallas_recurrent_scan__sliding_local_dilated__geglu_ffn__prompt_kernel(
    A_x: jax.Array,
    A_wqkv: jax.Array,
    A_wo: jax.Array,
    B_x: jax.Array,
    B_w_gate: jax.Array,
    B_w_up: jax.Array,
    B_w_down: jax.Array,
):
    return _IMPL(A_x, A_wqkv, A_wo, B_x, B_w_gate, B_w_up, B_w_down)
```

```python
import contextlib
import math

import jax
import jax.numpy as jnp
from jax import lax
import jax.experimental.pallas as pl
import jax.experimental.pallas.tpu as pltpu

S, D, F = 2048, 1024, 3584
H, DH, W, DIL = 32, 32, 8, 2
NL = 128
NCH = D // NL
HS = S // 2
KH = D // 2
KC = KH // NL
QS = S // 4
KQ = D // 4
FC = 256
NP = F // (2 * FC)
HALO = 16
SPARE = 48
F32, BF16, U32 = jnp.float32, jnp.bfloat16, jnp.uint32
EPS = 1e-5
GELU_C0 = math.sqrt(2.0 / math.pi)
GELU_C1 = GELU_C0 * 0.044715
EXP2_SCALE = (DH ** -0.5) * math.log2(math.e)
NEG = -1e9 / (DH ** -0.5)

_A_TERMS = (((0, 0, 1), (1, 1, 1)), ((1, 0, 1), (1, 1, 1)), ((0, 0, 1),), ((1, 1, 1),),
            ((0, 0, 1), (0, 1, 1)), ((1, 0, 1), (0, 0, -1)), ((0, 1, 1), (1, 1, -1)))
_B_TERMS = (((0, 0, 1), (1, 1, 1)), ((0, 0, 1),), ((0, 1, 1), (1, 1, -1)), ((1, 0, 1), (0, 0, -1)),
            ((1, 1, 1),), ((0, 0, 1), (0, 1, 1)), ((1, 0, 1), (1, 1, 1)))
_C_TERMS = (((0, 1), (3, 1), (4, -1), (6, 1)), ((2, 1), (4, 1)), ((1, 1), (3, 1)), ((0, 1), (1, -1), (2, 1), (5, 1)))
_ORDER = (1, 3, 0, 5, 2, 4, 6)
_XB_SLOT = {0: 0, 1: 1, 4: 2, 5: 3, 6: 4}


def _combine(terms, get):
    (r, c, _), *rest = terms
    v = get(r, c)
    for r, c, sign in rest:
        v = v + get(r, c) if sign > 0 else v - get(r, c)
    return v


def _ops(terms, q11, q12, q21, q22):
    q = ((q11, q12), (q21, q22))
    return [_combine(t, lambda r, c: q[r][c]) for t in terms]


def _dot(a, b):
    return jnp.dot(a, b, preferred_element_type=F32)


class _Fold:
    def __init__(self, fin):
        self.fin = fin

    def __call__(self, i, m):
        if i == 1:
            self.m1 = m
        elif i == 3:
            self.fin(2, self.m1 + m)
            self.t11 = m
        elif i == 0:
            self.t11 = self.t11 + m
            self.t22 = m - self.m1
        elif i == 5:
            self.t22 = self.t22 + m
        elif i == 2:
            self.fin(3, self.t22 + m)
            self.m2 = m
        elif i == 4:
            self.fin(1, self.m2 + m)
            self.t11 = self.t11 - m
        else:
            self.fin(0, self.t11 + m)


def _strassen(prod, fin, room):
    fold = _Fold(fin)
    for step, i in enumerate(_ORDER):
        m = prod(i)
        fold(i, m)
        yield room[step], m


def _emit(lag, main, total, *sides, dyn=None, dyn_rate=0, dyn_delay=0):
    done = [0] * len(sides)
    acc = step = 0

    def flush(frac, val):
        due = []
        for k, (f0, f1, tasks) in enumerate(sides):
            want = len(tasks) if frac >= f1 else int(max(0.0, (frac - f0) / (f1 - f0)) * len(tasks) + 0.5)
            n = min(want, len(tasks)) - done[k]
            due += [((j + 0.5) / n, k, tasks[done[k] + j]) for j in range(n)]
            done[k] += max(n, 0)
        if dyn:
            rate = dyn_rate
            ready = [e for e in dyn if e[0] + dyn_delay <= step][:rate]
            for j, e in enumerate(ready):
                dyn.remove(e)
                due.append(((j + 0.5) / len(ready), -1, e[1]))
        due.sort(key=lambda e: e[:2])
        for j, (_, _, task) in enumerate(due):
            if val is None:
                task(None)
            else:
                r = (val.shape[0] // 8) * j // len(due) * 8
                task(val[r:r + 8, 0:NL])

    hist = [(0, None)] * lag
    for item in main:
        step += 1
        for e in dyn or ():
            if e[0] is None:
                e[0] = step
        hist.append(item)
        room, val = hist.pop(0)
        acc += room
        if room:
            flush(acc / total, val)
    acc += sum(h[0] for h in hist)
    assert abs(acc - total) < 1e-6 and not dyn, (acc, total)
    flush(2.0, hist[-1][1] if hist else val)


def _skew(items):
    depth = max(len(st) for st in items)
    return [items[t - k][k] for t in range(len(items) + depth - 1) for k in range(depth)
            if 0 <= t - k < len(items) and k < len(items[t - k]) and items[t - k][k] is not None]


def make(EXP='', ONEPASS=True, T0=128, LN0=64, LNF=0.8, RG=(2,) * 7, RU=(2, 1, 2, 2, 1, 1, 1),
         RH=256, LAG=1, P1A=0.44,
         RH2=64, LAG2=4, PG0=1.5, R2L=(2,) * 7, R2H=(2, 0, 2, 2, 0, 0, 0), MD=128, ND=128, RD2=2, DRATE=2, DDELAY=4,
         APA=32, APB=128, AP3=0, AT3=0.93, AGAP=4, HAF=0.6, HA1=2.0, HA2=4.6, ATS=None, ATE=0.75, ATB=0.97, PDN=32, PDB=0.8,
         M3=64, OUTK=1, LAG3=2, scopes=False):
    NT0 = HS // T0
    T3 = 256
    NT3 = HS // T3
    assert NL - PDN <= 96
    assert (NP - 1) * APA + NP * APB + (NT3 - 1) * AP3 >= HS and (NT3 - 1) * AP3 <= T3 and APA % 16 == 0 and APB % 16 == 0

    def scope(name):
        return jax.named_scope(name) if scopes else contextlib.nullcontext()

    def kernel(x_hbm, wqkv_hbm, wo_hbm, wg_hbm, wu_hbm, wd_hbm, out_hbm,
               xbuf, XA, XB, qkv, P, HF, BG, BD, BO, rgu, rd, Y, rq, OA32,
               sem_x, sem_gu, sem_d, sem_q, sem_o, sem_out):

        XA, XB, BG, BD, BO = [r.bitcast(BF16) for r in (XA, XB, BG, BD, BO)]

        def ch(n, w=NL):
            return pl.ds(n * w, w) if isinstance(n, int) else pl.ds(pl.multiple_of(n * w, w), w)

        def zero(i):
            return i % 2 + (i + 1) % 2 - 1

        def when(pred, fn):
            pl.when(pred)(lambda: (fn(), None)[1])

        def cp_x(i, half):
            r = half * HS + i * T0
            return pltpu.make_async_copy(x_hbm.at[pl.ds(r, T0), :], xbuf.at[pl.ds(r, T0), :], sem_x.at[i, half])

        def cp_gu(c, slot, which):
            src = wg_hbm if which == 0 else wu_hbm
            return pltpu.make_async_copy(src.at[:, pl.ds(c * FC, FC)], rgu.at[slot, which, pl.ds(0, D), :],
                                         sem_gu.at[slot, which])

        def cp_d(p):
            return pltpu.make_async_copy(wd_hbm.at[pl.ds(p * 2 * FC, 2 * FC), :], rd.at[pl.ds(0, 2 * FC), :],
                                         sem_d.at[0])

        def anchor(dst, row, val, z):
            if val is not None and z is not None:
                r = pl.multiple_of(row + 16 + z * 16, 8)
                dst[pl.ds(r, 8), pl.ds(0, NL)] = pltpu.bitcast(val, U32) if dst.dtype == U32 else val.astype(dst.dtype)

        def gelu2(g, u):
            t = jnp.tanh(g * (GELU_C0 + GELU_C1 * (g * g)))
            p = g * u
            return p + p * t

        def prep_g2_tasks(slot, outer, r0, n, z, free=None):
            def task(val, r, i):
                assert free is None or i in free
                anchor(rgu.at[0, 0], D, val, z)
                y = [_combine(_B_TERMS[i], lambda kp, mu: rgu[slot, mu, pl.ds((2 * kp + ta) * KQ + r, 16), :].astype(F32))
                     for ta in range(2)]
                ops = _ops(_B_TERMS, y[0][:, :NL], y[0][:, NL:], y[1][:, :NL], y[1][:, NL:])
                for k in range(7):
                    BG.at[i][pl.ds(r, 16), ch(k)] = ops[k].astype(BF16)
            return [(lambda val, r=r0 + g * 16, i=i: task(val, r, i)) for i in outer for g in range(n // 16)]

        def prep_d2_tasks(r0, n, z):
            def task(val, r, i):
                anchor(rd, 2 * FC, val, z)
                y = [_combine(_B_TERMS[i],
                              lambda kp, nu: rd[pl.ds((2 * kp + ta) * NL + r, 16), ch(2 * nu + up, KQ)].astype(F32))
                     for ta in range(2) for up in range(2)]
                ops = _ops(_B_TERMS, *y)
                for k in range(7):
                    BD.at[7 * i + k][pl.ds(r, 16), :] = ops[k].astype(BF16)
            return [(lambda val, r=r0 + g * 16, i=i: task(val, r, i)) for g in range(n // 16) for i in range(7)]

        def first_half(B0, BQ):
            B0, BQ = B0.bitcast(BF16), BQ.bitcast(BF16)

            class cp_cols:
                def __init__(self, src, col0, dst, slot0, sem):
                    self.args = src, col0, dst, slot0, sem

                def start(self):
                    src, col0, dst, slot0, sem = self.args
                    for k in range(NCH):
                        pltpu.make_async_copy(src.at[:, pl.ds(col0 + k * NL, NL)],
                                              dst.at[slot0 + k, pl.ds(0, D // 2), :].bitcast(BF16), sem).start()

                def wait(self):
                    _, _, dst, slot0, sem = self.args
                    whole = dst.at[pl.ds(slot0, NCH), pl.ds(0, D // 2), :]
                    pltpu.make_async_copy(whole, whole, sem).wait()

            def cp_q(m):
                return cp_cols(wqkv_hbm, m * D, rq, m * NCH, sem_q.at[m])

            def cp_o():
                return cp_cols(wo_hbm, 0, rq, 3 * NCH, sem_o.at[0])

            def ln_tasks(r0, n, z):
                def xrow(r):
                    return xbuf[pl.ds(r, 16), :].astype(F32)
                items = []
                for g in range(n // 16):
                    st = {}
                    for half in range(2):
                        def s0(val, r=half * HS + r0 + g * 16, st=st, half=half):
                            anchor(xbuf, S, val, z)
                            st["m", half] = jnp.sum(xrow(r), axis=-1, keepdims=True) * (1.0 / D)

                        def s1(val, r=half * HS + r0 + g * 16, st=st, half=half):
                            anchor(xbuf, S, val, z)
                            c = xrow(r) - st["m", half]
                            st["v", half] = lax.rsqrt(jnp.sum(c * c, axis=-1, keepdims=True) * (1.0 / D) + EPS)

                        def s01(val, r=half * HS + r0 + g * 16, st=st, half=half):
                            anchor(xbuf, S, val, z)
                            x = xrow(r)
                            m = jnp.sum(x, axis=-1, keepdims=True) * (1.0 / D)
                            e2 = jnp.sum(x * x, axis=-1, keepdims=True) * (1.0 / D)
                            st["m", half] = m
                            st["v", half] = lax.rsqrt(jnp.maximum(e2 - m * m, 0.0) + EPS)

                        def s2(val, r=r0 + g * 16, st=st, half=half):
                            for kc in (2 * half, 2 * half + 1):
                                anchor(xbuf, S, val, z)
                                pos = [(h, c) for h in range(2) for c in (kc, KC + kc)]
                                q = [(xbuf[pl.ds(h * HS + r, 16), ch(c)].astype(F32) - st["m", h]) * st["v", h]
                                     for h, c in pos]
                                for (h, c), y in zip(pos, q):
                                    Y[pl.ds(h * HS + r, 16), ch(c)] = y
                                for i, op in enumerate(_ops(_A_TERMS, *q)):
                                    XA.at[i][pl.ds(r, 16), ch(kc)] = op.astype(BF16)
                        stats = [s01] if ONEPASS else [s0, None, s1]
                        items.append(stats + [None] * (2 - half) + [s2])
                return _skew(items)

            def prep_g1_tasks(which, r0, n):
                for g in range(n // 16):
                    r = r0 + g * 16
                    top = rgu[0, which, pl.ds(r, 16), :].astype(F32)
                    bot = rgu[0, which, pl.ds(KH + r, 16), :].astype(F32)
                    for i, op in enumerate(_ops(_B_TERMS, top[:, :NL], top[:, NL:], bot[:, :NL], bot[:, NL:])):
                        B0.at[i][pl.ds(r, 16), ch(which)] = op.astype(BF16)

            def xb_tasks(r0, n, z):
                def task(val, r, kc, i):
                    anchor(Y, S, val, z)
                    x = [_combine(_A_TERMS[i],
                                  lambda sg, kp: Y[pl.ds((2 * sg + rho) * QS + r, 16), ch(4 * kp + 2 * ta + kc)])
                         for rho in range(2) for ta in range(2)]
                    ops = _ops(_A_TERMS, *x)
                    for k, slot in _XB_SLOT.items():
                        XB.at[5 * i + slot][pl.ds(r, 16), ch(kc)] = ops[k].astype(BF16)
                return [(lambda val, r=r0 + g * 16, kc=kc, i=i: task(val, r, kc, i))
                        for g in range(n // 16) for kc in range(2) for i in range(7)]

            def wide(w):
                return pltpu.bitcast(w, BF16).astype(F32)

            def prep_q_tasks(m, par, n, z):
                def perm_a(r):
                    y = [rq[m * NCH + k, pl.ds(r // 2, 8), :] for k in range(NCH)]
                    return [y[0]] + [pltpu.roll(y[k], 2 * k, 1) for k in range(1, NCH)]

                def perm_b(y):
                    lane = lax.broadcasted_iota(jnp.int32, (8, NL), 1)
                    sh = (((lane & 15) >> 1) - par) & 7
                    u = [y[(-j) % NCH] for j in range(NCH)]
                    b0, b1, b2 = (sh & 1) != 0, (sh & 2) != 0, (sh & 4) != 0
                    out = (2 * n, 2 * n + 4)
                    v = {j: jnp.where(b0, u[(j - 1) % NCH], u[j]) for j in (0, 2, 4, 6)}
                    v = {j: jnp.where(b1, v[(j - 2) % NCH], v[j]) for j in out}
                    v = {j: jnp.where(b2, v[(j - 4) % NCH], v[j]) for j in out}
                    return [pltpu.roll(v[j], (2 * NL - 2 * j - 2 * par) % NL, 1) for j in out]

                items = []
                for g in range(KH // 16):
                    st = {}
                    for half in range(2):
                        def s0(val, r=half * KH + g * 16, st=st, half=half):
                            anchor(rq.at[0], D // 2, val, z)
                            st["a", half] = perm_a(r)

                        def s1(val, st=st, half=half):
                            st["b", half] = perm_b(st["a", half])

                        def s2(val, r=g * 16, st=st):
                            ops = _ops(_B_TERMS, *[wide(w) for w in st["b", 0] + st["b", 1]])
                            for i in range(7):
                                BQ.at[i][pl.ds(r, 16), ch(n)] = ops[i].astype(BF16)
                        items.append([s0, s1] + ([s2] if half else []))
                flat = _skew(items)
                firsts = [j for j, t in enumerate(flat) if t.__name__ == "s0"] + [len(flat)]
                return [(lambda val, grp=flat[a:b]: [t(val) for t in grp]) for a, b in zip(firsts, firsts[1:])]

            def prep_o_tasks(src, n, z):
                def transpose(c, a):
                    sub = lax.broadcasted_iota(jnp.int32, (8, NL), 0)
                    y = [rq[src + c, pl.ds(64 * g + 8 * a, 8), :] for g in range(8)]
                    y = [y[0]] + [pltpu.roll(y[g], g, 0) for g in range(1, 8)]
                    v = [y[(-j) % 8] for j in range(8)]
                    for bit in (1, 2, 4):
                        v = [jnp.where((sub & bit) != 0, v[(j - bit) % 8], v[j]) for j in range(8)]
                    return [v[0]] + [pltpu.roll(v[j], 8 - j, 0) for j in range(1, 8)]

                tasks = []
                for a in range(8):
                    st = {}

                    def load(val, h, a=a, st=st):
                        anchor(rq.at[0], D // 2, val, z)
                        st[h] = transpose(h * KC + n, a)

                    def quad(val, jj, a=a, st=st):
                        q = [wide(st[h][kh * KC + jj]) for kh in range(2) for h in range(2)]
                        for i, op in enumerate(_ops(_B_TERMS, *q)):
                            BO.at[i][pl.ds(jj * NL + 16 * a, 16), ch(n)] = op.astype(BF16)
                    tasks += [lambda val, f=load: f(val, 0),
                              lambda val, f=load, g=quad: (f(val, 1), [g(val, jj) for jj in range(KC)])]
                return tasks

            def zero_p_tasks(u0, n, z):
                def task(val, u):
                    v = jnp.zeros((8, NL), F32) if val is None else jnp.where(z != 0, val, 0.0)
                    P[u // 32, pl.ds(pl.multiple_of((u % 32) * 32, 32), 32), :] = jnp.tile(v, (4, KC))
                return [(lambda val, u=u0 + j: task(val, u)) for j in range(n)]

            def up1(r0, m):
                g = {}

                def fin_u(k, u):
                    HF[pl.ds((k // 2) * HS + r0, m), ch(k % 2)] = gelu2(g[k], u)
                yield from _strassen(lambda i: _dot(XA[i, pl.ds(r0, m), :], B0[i, :, ch(0)]), g.__setitem__, RG)
                yield from _strassen(lambda i: _dot(XA[i, pl.ds(r0, m), :], B0[i, :, ch(1)]), fin_u, RU)

            with scope("start"):
                groups = [lambda: [cp_x(0, 0), cp_x(0, 1)], lambda: [cp_gu(0, 0, 0)], lambda: [cp_gu(0, 0, 1)]]
                groups += [(lambda i=i: [cp_x(i, 0), cp_x(i, 1)]) for i in range(1, NT0)]
                groups += [lambda: [cp_q(0)], lambda: [cp_gu(1, 1, 0), cp_gu(1, 1, 1), cp_d(0)],
                           lambda: [cp_q(1)], lambda: [cp_o()], lambda: [cp_q(2)]]

                def issue(k, c):
                    for g, cps in enumerate(groups):
                        when(k == g, lambda: [cp.start() for cp in cps()])
                    return c
                lax.fori_loop(0, len(groups), issue, 0)
                cp_x(0, 0).wait(); cp_x(0, 1).wait()

                def ln0(g, c):
                    for t in ln_tasks(pl.multiple_of(g * LN0, LN0), LN0, None):
                        t(None)
                    return c
                lax.fori_loop(0, T0 // LN0, ln0, 0)
                for which in range(2):
                    cp_gu(0, 0, which).wait()

                    def pg0(g, c):
                        prep_g1_tasks(which, pl.multiple_of(g * 64, 64), 64)
                        return c
                    lax.fori_loop(0, KH // 64, pg0, 0)

            def p0_body(i, c):
                cp_x(i + 1, 0).wait(); cp_x(i + 1, 1).wait()
                r0 = pl.multiple_of(i * T0, T0)
                _emit(LAG, up1(r0, T0), sum(RG) + sum(RU), (0.0, LNF, ln_tasks(r0 + T0, T0, zero(i))))
                return zero(i)
            with scope("p0"):
                z0 = lax.fori_loop(0, NT0 - 1, p0_body, 0)
            with scope("p0_last"):
                cp_q(0).wait()
                cp_gu(2, 0, 0).start(); cp_gu(2, 0, 1).start()
                _emit(LAG, up1(HS - T0, T0), sum(RG) + sum(RU), (0.0, 0.85, prep_q_tasks(0, 0, 0, z0)))

            def p1_body(b, c):
                with scope("p1i"):
                    return p1_body_(b, c)

            def p1_body_(b, c):
                when(b == 0, lambda: (cp_gu(1, 1, 0).wait(), cp_gu(1, 1, 1).wait(), cp_d(0).wait()))
                when(b == 1, lambda: cp_q(1).wait())
                when(b == 2, lambda: cp_o().wait())
                when(b == 3, lambda: cp_q(2).wait())
                m = b // 2
                par = b % 2

                def main():
                    for n in range(2):
                        for s in range(HS // RH):
                            r0 = s * RH

                            def fin(k, v):
                                j = m * NCH + par + 2 * n + 4 * (k % 2)
                                qkv[j, pl.ds(HALO + (k // 2) * HS + r0, RH), :] = v
                            yield from _strassen(lambda i: _dot(XA[i, pl.ds(r0, RH), :], BQ[i, :, ch(n)]), fin, (1,) * 7)
                piece = jnp.clip(b - 2, 0, 3)
                z = zero(b)
                _emit(LAG, main(), 14 * (HS // RH),
                      (0.0, P1A, prep_q_tasks(m, par, 1, z)),
                      (0.5, 0.5 + P1A, prep_q_tasks(jnp.minimum((b + 1) // 2, 2), (b + 1) % 2, 0, z)),
                      (0.0, 0.95, prep_g2_tasks(1, range(7), pl.multiple_of(jnp.minimum(b * 48, KQ - 48), 16), 48, z)),
                      (0.0, 0.95, xb_tasks(pl.multiple_of(jnp.minimum(b * 96, QS - 96), 32), 96, z)),
                      (0.0, 0.95, prep_d2_tasks(pl.multiple_of(jnp.minimum(b * 16, NL - PDN - 16), 16), 16, z)),
                      (0.0, 0.95, zero_p_tasks(jnp.minimum(b * 38, 224 - 38), 38, z)),
                      (0.0, 0.95, prep_o_tasks(jnp.where(b < 2, 0, 3 * NCH), piece, z)))
                return c
            with scope("p1"):
                lax.fori_loop(0, 6, p1_body, 0)
                for j in range(NCH, 3 * NCH):
                    qkv[j, 0:HALO, :] = jnp.broadcast_to(qkv[j, HALO:HALO + 1, :], (HALO, NL))

        def second_half(HA, osc, obuf, OB32):
            OA, HA, OB = OA32.bitcast(BF16), HA.bitcast(BF16), OB32.bitcast(BF16)

            def attn_unit(r0, masked, slot, z):
                st = {}

                def shifted(plane):
                    return [qkv[plane, pl.ds(r0 + HALO + 8 - DIL * k, 8), :] for k in range(12)]

                def logits(val, j):
                    anchor(qkv.at[0], HALO + S, val, z)
                    q = [qkv[j, pl.ds(r0 + HALO + 8 * g, 8), :] for g in range(2)]
                    kk = shifted(NCH + j)
                    for g in range(2):
                        for w in range(W):
                            t = q[g] * kk[w + 4 - 4 * g]
                            st[g, w] = t if j == 0 else st[g, w] + t
                    if j == NCH - 1:
                        softmax()

                def softmax():
                    lane = lax.broadcasted_iota(jnp.int32, (8, NL), 1)
                    odd = (lane & 1) != 0
                    hi = (lane & 16) != 0
                    keys = [(g, w) for g in range(2) for w in range(W)]
                    for k in keys:
                        a = st[k]
                        st[k] = a + jnp.where(odd, pltpu.roll(a, 1, 1), pltpu.roll(a, NL - 1, 1))
                    for k in keys:
                        a = st[k]
                        st[k] = a + jnp.where(hi, pltpu.roll(a, 16, 1), pltpu.roll(a, NL - 16, 1))
                    for g in range(2):
                        ls = [st[g, w] for w in range(W)]
                        if masked:
                            pos = r0 + 8 * g + lax.broadcasted_iota(jnp.int32, (8, NL), 0)
                            ls = [ls[0]] + [jnp.where(pos >= DIL * w, ls[w], NEG) for w in range(1, W)]
                        m = ls[0]
                        for w in range(1, W):
                            m = jnp.maximum(m, ls[w])
                        ps = [jnp.exp2((l - m) * EXP2_SCALE) for l in ls]
                        den = ps[0]
                        for w in range(1, W):
                            den = den + ps[w]
                        inv = 1.0 / den
                        for w in range(W):
                            st[g, w] = ps[w] * inv

                def pv(val, j):
                    anchor(qkv.at[0], HALO + S, val, z)
                    vv = shifted(2 * NCH + j)
                    for g in range(2):
                        a = st[g, 0] * vv[4 - 4 * g]
                        for w in range(1, W):
                            a = a + st[g, w] * vv[w + 4 - 4 * g]
                        osc[slot, j, pl.ds(8 * g, 8), :] = a

                return ([(lambda val, j=j: logits(val, j)) for j in range(NCH)] + [lambda val: None] * AGAP
                        + [(lambda val, j=j: pv(val, j)) for j in range(NCH)])

            def attn_tasks(t0, n, z, staged=False):
                if 'noattn' in EXP or n == 0:
                    return []
                t0 = pl.multiple_of(jnp.minimum(t0, HS - n), 16)
                tasks = []
                for g in range(n // 16):
                    r = t0 + g * 16
                    tasks += attn_unit(r, g == 0, 2 * g, z) + attn_unit(HS + r, False, 2 * g + 1, z)

                    def oa(val, kc, g=g, r=r):
                        ops = _ops(_A_TERMS, osc[2 * g, kc], osc[2 * g, KC + kc],
                                   osc[2 * g + 1, kc], osc[2 * g + 1, KC + kc])
                        for i in range(7):
                            dst, row = (OB, g * 16) if staged else (OA, r)
                            dst.at[i][pl.ds(row, 16), ch(kc)] = ops[i].astype(BF16)
                    tasks += [(lambda val, kc=kc, oa=oa: oa(val, kc)) for kc in range(KC)]
                return tasks

            def ha_task(val, r, i, z, have):
                anchor(HF, S, val, z)
                x = [_combine(_A_TERMS[i], lambda sg, kp: HF[pl.ds((2 * sg + rho) * QS + r, 16), ch(2 * kp + ta)])
                     for rho in range(2) for ta in range(2)]
                for k, op in enumerate(_ops(_A_TERMS, *x)):
                    HA[pl.ds(r, 16), ch(7 * i + k)] = op.astype(BF16)
                have.add((i, r))

            def up2(kp, free, on_half):
                def sub(r0, m):
                    hold, seen = {}, set()

                    def outer_fin(k, K, v):
                        if K in (2, 1):
                            hold[k] = v
                            return
                        sg = K // 2
                        HF[pl.ds((2 * sg + k // 2) * QS + r0, m), ch(2 * kp + k % 2)] = (
                            gelu2(hold[k], v) if K == 3 else gelu2(v, hold[k]))
                        seen.add((sg, k))
                        if all((sg, j) in seen for j in range(4)):
                            on_half(sg, r0, m)
                    folds = [_Fold(lambda K, v, k=k: outer_fin(k, K, v)) for k in range(4)]

                    def lhs(i, k):
                        if k == 2:
                            return XA[i, pl.ds(r0, m), pl.ds(0, KQ)]
                        if k == 3:
                            return XA[i, pl.ds(QS + r0, m), pl.ds(KQ, KQ)]
                        return XB[5 * i + _XB_SLOT[k], pl.ds(r0, m), :]
                    return lambda i: _strassen(lambda k: _dot(lhs(i, k), BG[i, :, ch(k)]),
                                               lambda k, v: folds[k](i, v), R2H if i in (2, 6) else R2L)
                subs = [sub(s * RH2, RH2) for s in range(QS // RH2)]
                for i in _ORDER:
                    for sb in subs:
                        yield from sb(i)
                    free.add(i)

            nsub = QS // RH2
            g_room = (5 * sum(R2L) + 2 * sum(R2H)) * nsub
            d_unit = RD2 * MD * ND / (RH2 * KQ)

            ends = [sum(sum(R2H if i in (2, 6) else R2L) for i in _ORDER[:j + 1]) * nsub for j in range(7)]

            def bg_sides(slot, total, z, free, n):
                return [((ends[j] + 1) / total, (ends[j + 1] if j < 6 else ends[6] + ends[0]) / total - 0.01,
                         prep_g2_tasks(slot, _ORDER[j:j + 1], 0, KQ, z, free)) for j in range(n)]

            def block_b(k):
                when(k < NP - 1, lambda: (cp_gu(0, 0, 0).wait(), cp_gu(0, 0, 1).wait()))

                def prefetch(val):
                    when(k < NP - 1, lambda: (cp_gu(2 * k + 3, 1, 0).start(), cp_gu(2 * k + 3, 1, 1).start(),
                                              cp_d(k + 1).start()))
                z = zero(k)
                free, have, halves = set(), set(), set()

                def on_half(sg, r0, m):
                    if r0 + m == QS:
                        halves.add(sg)

                def ha_tasks(outer, need):
                    def task(val, r, i):
                        assert need <= halves
                        ha_task(val, r, i, z, have)
                    return [(lambda val, r=r, i=i: task(val, r, i)) for i in outer for r in range(0, QS, 16)]

                def main():
                    yield from up2(1, free, on_half)
                    for i in (2, 5, 1, 3, 0, 4, 6):
                        assert all((i, r) in have for r in range(0, QS, 16))
                        for r0 in range(0, QS, MD):
                            for c in range(KQ // ND):
                                def fin(q, v):
                                    P[i, pl.ds((q // 2) * QS + r0, MD), pl.ds((q % 2) * KQ + c * ND, ND)] += v
                                yield from _strassen(
                                    lambda j: _dot(HA[pl.ds(r0, MD), ch(7 * i + j)], BD[7 * i + j, :, ch(c, ND)]),
                                    fin, (d_unit,) * 7)
                total = g_room + 49 * (QS // MD) * (KQ // ND) * d_unit
                gf = g_room / total
                df = (1 - gf) / 7
                att = attn_tasks(k * (APA + APB), APB, z)
                if ATS is None:
                    att_sides = [(0.0, ATB, att)]
                else:
                    cut = len(att) * ATS // (APB // 16)
                    att_sides = [(0.0, ATE * gf, att[:cut]), (gf + HA2 * df, ATB, att[cut:])]
                _emit(LAG2, main(), total, *bg_sides(0, total, z, free, 7),
                      (0.0, ends[0] / total, prep_g2_tasks(1, _ORDER[6:], 0, KQ, z)),
                      (0.0, HAF * gf, ha_tasks((2, 5), set())),
                      ((ends[4] + 1) / total, gf + HA1 * df, ha_tasks((1, 3, 0), {1})),
                      (gf + HA1 * df, gf + HA2 * df, ha_tasks((4, 6), {0, 1})),
                      (0.0, PDB * gf, prep_d2_tasks(NL - PDN, PDN, z)),
                      *att_sides,
                      (gf, gf + 0.01, [prefetch]))

            def block_a(k):
                cp_gu(0, 1, 0).wait(); cp_gu(0, 1, 1).wait(); cp_d(0).wait()

                def prefetch(val):
                    when(k < NP - 2, lambda: (cp_gu(2 * k + 4, 0, 0).start(), cp_gu(2 * k + 4, 0, 1).start()))
                z = zero(k)
                free = set()
                _emit(LAG2, up2(0, free, lambda *a: None), g_room, *bg_sides(1, g_room, z, free, 6),
                      (0.0, 0.95, prep_d2_tasks(0, NL - PDN, z)),
                      (0.0, 0.95, attn_tasks(k * (APA + APB) + APB, APA, z)),
                      (0.01, 0.02, [prefetch]))

            def p2_body(k, carry):
                with scope("b"):
                    block_b(k)
                with scope("a"):
                    when(k < NP - 1, lambda: block_a(k))
                return carry
            with scope("p2"):
                lax.fori_loop(0, NP, p2_body, 0)

            def cp_out(t, half, s):
                return pltpu.make_async_copy(obuf.at[t % 2, half, pl.ds(s * M3, M3), :],
                                             out_hbm.at[pl.ds(half * HS + t * T3 + s * M3, M3), :], sem_out.at[t % 2])

            def wait_out(t):
                pltpu.make_async_copy(obuf.at[t % 2], obuf.at[t % 2], sem_out.at[t % 2]).wait()

            def cp_late(t):
                r = pl.multiple_of((HS - (NT3 - 1 - t) * AP3) // 2, 8)
                return pltpu.make_async_copy(OB32, OA32.at[:, pl.ds(r, AP3 // 2), :], sem_o.at[0])

            def p3_body(t, carry):
                when(t >= 2, lambda: wait_out(t - 2))
                if AP3:
                    when(t >= 1, lambda: cp_late(t - 1).wait())

                def main():
                    for s in range(T3 // M3):
                        r0 = pl.multiple_of(t * T3 + s * M3, M3)
                        for n in range(KC):
                            def fin(k, sq):
                                (j0, _), *rest = _C_TERMS[k]
                                f = P[j0, pl.ds(r0, M3), ch(n)]
                                for j, sign in rest:
                                    f = f + P[j, pl.ds(r0, M3), ch(n)] if sign > 0 else f - P[j, pl.ds(r0, M3), ch(n)]
                                y = f * 0.25
                                half, col = k // 2, (k % 2) * KC + n
                                x = xbuf[pl.ds(half * HS + r0, M3), ch(col)].astype(F32)
                                obuf.at[t % 2, half][pl.ds(s * M3, M3), ch(col)] = (
                                    x + sq * (y + y * jnp.tanh(y))).astype(BF16)
                            for step, item in enumerate(_strassen(
                                    lambda i: _dot(OA[i, pl.ds(r0, M3), :], BO[i, :, ch(n)]), fin, (1,) * 7)):
                                yield item
                                if s > 0 and n == 0 and step == OUTK:
                                    cp_out(t, 0, s - 1).start(); cp_out(t, 1, s - 1).start()
                _emit(LAG3, main(), 7 * KC * (T3 // M3),
                      (0.0, AT3, attn_tasks(HS - (NT3 - 1 - t) * AP3, AP3, zero(t), staged=True)))
                if AP3:
                    when(t < NT3 - 1, lambda: cp_late(t).start())
                cp_out(t, 0, T3 // M3 - 1).start(); cp_out(t, 1, T3 // M3 - 1).start()
                return carry
            with scope("p3"):
                lax.fori_loop(0, NT3, p3_body, 0)
            with scope("end"):
                for t in range(NT3 - 2, NT3):
                    wait_out(t)

        pl.run_scoped(first_half,
                      pltpu.VMEM((7, KH // 2, 2 * NL), U32),
                      pltpu.VMEM((7, KH // 2, 2 * NL), U32))
        pl.run_scoped(second_half,
                      pltpu.VMEM((QS // 2, 49 * NL), U32),
                      pltpu.VMEM((max(APA, APB, AP3) // 8, NCH, 16, NL), F32),
                      pltpu.VMEM((2, 2, T3, D), BF16),
                      pltpu.VMEM((7, max(AP3, 16) // 2, KH), U32))

    def fn(A_x, A_wqkv, A_wo, B_x, B_w_gate, B_w_up, B_w_down):
        x = A_x.reshape(S, D)
        anyspec = pl.BlockSpec(memory_space=pl.ANY)
        out = pl.pallas_call(
            kernel,
            in_specs=[anyspec] * 6,
            out_specs=anyspec,
            out_shape=jax.ShapeDtypeStruct((S, D), BF16),
            scratch_shapes=[
                pltpu.VMEM((S + SPARE, D), BF16),
                pltpu.VMEM((7, HS // 2, KH), U32),
                pltpu.VMEM((35, QS // 2, KQ), U32),
                pltpu.VMEM((3 * NCH, HALO + S + SPARE, NL), F32),
                pltpu.VMEM((7, HS, KH), F32),
                pltpu.VMEM((S + SPARE, 2 * FC), F32),
                pltpu.VMEM((7, KQ // 2, 7 * NL), U32),
                pltpu.VMEM((49, NL // 2, KQ), U32),
                pltpu.VMEM((7, KH // 2, KH), U32),
                pltpu.VMEM((2, 2, D + SPARE, FC), BF16),
                pltpu.VMEM((2 * FC + SPARE, D), BF16),
                pltpu.VMEM((S + SPARE, D), F32),
                pltpu.VMEM((4 * NCH, D // 2 + 64, NL), U32),
                pltpu.VMEM((7, HS // 2, KH), U32),
                pltpu.SemaphoreType.DMA((NT0, 2)),
                pltpu.SemaphoreType.DMA((2, 2)),
                pltpu.SemaphoreType.DMA((1,)),
                pltpu.SemaphoreType.DMA((3,)),
                pltpu.SemaphoreType.DMA((1,)),
                pltpu.SemaphoreType.DMA((2,)),
            ],
            compiler_params=pltpu.CompilerParams(vmem_limit_bytes=124 * 2 ** 20, disable_bounds_checks=True),
        )(x, A_wqkv, A_wo, B_w_gate, B_w_up, B_w_down)
        return out.reshape(1, S, D)
    return jax.jit(fn)


_IMPL = make(AP3=0)


@jax.jit
def pallas_recurrent_scan__sliding_local_dilated__geglu_ffn__prompt_kernel(
    A_x: jax.Array,
    A_wqkv: jax.Array,
    A_wo: jax.Array,
    B_x: jax.Array,
    B_w_gate: jax.Array,
    B_w_up: jax.Array,
    B_w_down: jax.Array,
):
    return _IMPL(A_x, A_wqkv, A_wo, B_x, B_w_gate, B_w_up, B_w_down)
```

```python
import contextlib
import math

import jax
import jax.numpy as jnp
from jax import lax
import jax.experimental.pallas as pl
import jax.experimental.pallas.tpu as pltpu

S, D, F = 2048, 1024, 3584
H, DH, W, DIL = 32, 32, 8, 2
NL = 128
NCH = D // NL
HS = S // 2
KH = D // 2
KC = KH // NL
QS = S // 4
KQ = D // 4
FC = 256
NP = F // (2 * FC)
HALO = 16
SPARE = 48
F32, BF16, U32 = jnp.float32, jnp.bfloat16, jnp.uint32
EPS = 1e-5
GELU_C0 = math.sqrt(2.0 / math.pi)
GELU_C1 = GELU_C0 * 0.044715
EXP2_SCALE = (DH ** -0.5) * math.log2(math.e)
NEG = -1e9 / (DH ** -0.5)

_A_TERMS = (((0, 0, 1), (1, 1, 1)), ((1, 0, 1), (1, 1, 1)), ((0, 0, 1),), ((1, 1, 1),),
            ((0, 0, 1), (0, 1, 1)), ((1, 0, 1), (0, 0, -1)), ((0, 1, 1), (1, 1, -1)))
_B_TERMS = (((0, 0, 1), (1, 1, 1)), ((0, 0, 1),), ((0, 1, 1), (1, 1, -1)), ((1, 0, 1), (0, 0, -1)),
            ((1, 1, 1),), ((0, 0, 1), (0, 1, 1)), ((1, 0, 1), (1, 1, 1)))
_C_TERMS = (((0, 1), (3, 1), (4, -1), (6, 1)), ((2, 1), (4, 1)), ((1, 1), (3, 1)), ((0, 1), (1, -1), (2, 1), (5, 1)))
_ORDER = (1, 3, 0, 5, 2, 4, 6)
_XB_SLOT = {0: 0, 1: 1, 4: 2, 5: 3, 6: 4}


def _combine(terms, get):
    (r, c, _), *rest = terms
    v = get(r, c)
    for r, c, sign in rest:
        v = v + get(r, c) if sign > 0 else v - get(r, c)
    return v


def _ops(terms, q11, q12, q21, q22):
    q = ((q11, q12), (q21, q22))
    return [_combine(t, lambda r, c: q[r][c]) for t in terms]


def _dot(a, b):
    return jnp.dot(a, b, preferred_element_type=F32)


class _Fold:
    def __init__(self, fin):
        self.fin = fin

    def __call__(self, i, m):
        if i == 1:
            self.m1 = m
        elif i == 3:
            self.fin(2, self.m1 + m)
            self.t11 = m
        elif i == 0:
            self.t11 = self.t11 + m
            self.t22 = m - self.m1
        elif i == 5:
            self.t22 = self.t22 + m
        elif i == 2:
            self.fin(3, self.t22 + m)
            self.m2 = m
        elif i == 4:
            self.fin(1, self.m2 + m)
            self.t11 = self.t11 - m
        else:
            self.fin(0, self.t11 + m)


def _strassen(prod, fin, room):
    fold = _Fold(fin)
    for step, i in enumerate(_ORDER):
        m = prod(i)
        fold(i, m)
        yield room[step], m


def _emit(lag, main, total, *sides):
    done = [0] * len(sides)
    acc = 0

    def flush(frac, val):
        due = []
        for k, (f0, f1, tasks) in enumerate(sides):
            want = len(tasks) if frac >= f1 else int(max(0.0, (frac - f0) / (f1 - f0)) * len(tasks) + 0.5)
            n = min(want, len(tasks)) - done[k]
            due += [((j + 0.5) / n, k, tasks[done[k] + j]) for j in range(n)]
            done[k] += max(n, 0)
        due.sort(key=lambda e: e[:2])
        for j, (_, _, task) in enumerate(due):
            r = (val.shape[0] // 8) * j // len(due) * 8
            task(val[r:r + 8, 0:NL])

    hist = [(0, None)] * lag
    for item in main:
        hist.append(item)
        room, val = hist.pop(0)
        acc += room
        if room:
            flush(acc / total, val)
    assert abs(acc + sum(h[0] for h in hist) - total) < 1e-6
    flush(2.0, hist[-1][1])


def _skew(items):
    depth = max(len(st) for st in items)
    return [items[t - k][k] for t in range(len(items) + depth - 1) for k in range(depth)
            if 0 <= t - k < len(items) and k < len(items[t - k]) and items[t - k][k] is not None]


def make(ONEPASS=True, T0=128, LN0=64, LNF=0.85, RG=(2,) * 7, RU=(2, 2, 2, 2, 1, 1, 1), LAG0=2,
         RH=256, LAG=1, P1A=0.46, XBF=0.95,
         RH2=64, LAG2=4, R2L=(2,) * 7, R2H=(2, 0, 2, 2, 0, 0, 0), MD=128, ND=128, RD2=2,
         APA=32, APB=128, AGAP=4, HAF=0.6, HA1=2.0, HA2=4.6, ATB=0.97, PDN=32, PDB=0.8,
         M3=64, OUTK=1, scopes=False):
    NT0 = HS // T0
    T3 = 256
    NT3 = HS // T3
    assert NL - PDN <= 96
    assert (NP - 1) * APA + NP * APB >= HS and (APA + APB) % 32 == 0 and APA % 16 == 0 and APB % 16 == 0

    def scope(name):
        return jax.named_scope(name) if scopes else contextlib.nullcontext()

    def kernel(x_hbm, wqkv_hbm, wo_hbm, wg_hbm, wu_hbm, wd_hbm, out_hbm,
               xbuf, XA, XB, qkv, P, HF, BG, BD, BO, rgu, rd, Y, rq, OA,
               sem_x, sem_gu, sem_d, sem_q, sem_o, sem_out):

        XA, XB, BG, BD, BO, OA = [r.bitcast(BF16) for r in (XA, XB, BG, BD, BO, OA)]

        def ch(n, w=NL):
            return pl.ds(n * w, w) if isinstance(n, int) else pl.ds(pl.multiple_of(n * w, w), w)

        def zero(i):
            return i % 2 + (i + 1) % 2 - 1

        def when(pred, fn):
            pl.when(pred)(lambda: (fn(), None)[1])

        def cp_x(i, half):
            r = half * HS + i * T0
            return pltpu.make_async_copy(x_hbm.at[pl.ds(r, T0), :], xbuf.at[pl.ds(r, T0), :], sem_x.at[i, half])

        def cp_gu(c, slot, which):
            src = wg_hbm if which == 0 else wu_hbm
            return pltpu.make_async_copy(src.at[:, pl.ds(c * FC, FC)], rgu.at[slot, which, pl.ds(0, D), :],
                                         sem_gu.at[slot, which])

        def cp_d(p):
            return pltpu.make_async_copy(wd_hbm.at[pl.ds(p * 2 * FC, 2 * FC), :], rd.at[pl.ds(0, 2 * FC), :],
                                         sem_d.at[0])

        def anchor(dst, row, val, z):
            if val is not None and z is not None:
                r = pl.multiple_of(row + 16 + z * 16, 8)
                dst[pl.ds(r, 8), pl.ds(0, NL)] = pltpu.bitcast(val, U32) if dst.dtype == U32 else val.astype(dst.dtype)

        def gelu2(g, u):
            t = jnp.tanh(g * (GELU_C0 + GELU_C1 * (g * g)))
            p = g * u
            return p + p * t

        def prep_g2_tasks(slot, outer, r0, n, z, free=None):
            def task(val, r, i):
                assert free is None or i in free
                anchor(rgu.at[0, 0], D, val, z)
                y = [_combine(_B_TERMS[i], lambda kp, mu: rgu[slot, mu, pl.ds((2 * kp + ta) * KQ + r, 16), :].astype(F32))
                     for ta in range(2)]
                ops = _ops(_B_TERMS, y[0][:, :NL], y[0][:, NL:], y[1][:, :NL], y[1][:, NL:])
                for k in range(7):
                    BG.at[i][pl.ds(r, 16), ch(k)] = ops[k].astype(BF16)
            return [(lambda val, r=r0 + g * 16, i=i: task(val, r, i)) for i in outer for g in range(n // 16)]

        def prep_d2_tasks(r0, n, z):
            def task(val, r, i):
                anchor(rd, 2 * FC, val, z)
                y = [_combine(_B_TERMS[i],
                              lambda kp, nu: rd[pl.ds((2 * kp + ta) * NL + r, 16), ch(2 * nu + up, KQ)].astype(F32))
                     for ta in range(2) for up in range(2)]
                ops = _ops(_B_TERMS, *y)
                for k in range(7):
                    BD.at[7 * i + k][pl.ds(r, 16), :] = ops[k].astype(BF16)
            return [(lambda val, r=r0 + g * 16, i=i: task(val, r, i)) for g in range(n // 16) for i in range(7)]

        def first_half(B0, BQ):
            B0, BQ = B0.bitcast(BF16), BQ.bitcast(BF16)

            class cp_cols:
                def __init__(self, src, col0, dst, slot0, sem):
                    self.args = src, col0, dst, slot0, sem

                def start(self):
                    src, col0, dst, slot0, sem = self.args
                    for k in range(NCH):
                        pltpu.make_async_copy(src.at[:, pl.ds(col0 + k * NL, NL)],
                                              dst.at[slot0 + k, pl.ds(0, D // 2), :].bitcast(BF16), sem).start()

                def wait(self):
                    _, _, dst, slot0, sem = self.args
                    whole = dst.at[pl.ds(slot0, NCH), pl.ds(0, D // 2), :]
                    pltpu.make_async_copy(whole, whole, sem).wait()

            def cp_q(m):
                return cp_cols(wqkv_hbm, m * D, rq, m * NCH, sem_q.at[m])

            def cp_o():
                return cp_cols(wo_hbm, 0, rq, 3 * NCH, sem_o.at[0])

            def ln_tasks(r0, n, z):
                def xrow(r):
                    return xbuf[pl.ds(r, 16), :].astype(F32)
                items = []
                for g in range(n // 16):
                    st = {}
                    for half in range(2):
                        def s0(val, r=half * HS + r0 + g * 16, st=st, half=half):
                            anchor(xbuf, S, val, z)
                            st["m", half] = jnp.sum(xrow(r), axis=-1, keepdims=True) * (1.0 / D)

                        def s1(val, r=half * HS + r0 + g * 16, st=st, half=half):
                            anchor(xbuf, S, val, z)
                            c = xrow(r) - st["m", half]
                            st["v", half] = lax.rsqrt(jnp.sum(c * c, axis=-1, keepdims=True) * (1.0 / D) + EPS)

                        def s01(val, r=half * HS + r0 + g * 16, st=st, half=half):
                            anchor(xbuf, S, val, z)
                            x = xrow(r)
                            m = jnp.sum(x, axis=-1, keepdims=True) * (1.0 / D)
                            e2 = jnp.sum(x * x, axis=-1, keepdims=True) * (1.0 / D)
                            st["m", half] = m
                            st["v", half] = lax.rsqrt(jnp.maximum(e2 - m * m, 0.0) + EPS)

                        def s2(val, r=r0 + g * 16, st=st, half=half):
                            for kc in (2 * half, 2 * half + 1):
                                anchor(xbuf, S, val, z)
                                pos = [(h, c) for h in range(2) for c in (kc, KC + kc)]
                                q = [(xbuf[pl.ds(h * HS + r, 16), ch(c)].astype(F32) - st["m", h]) * st["v", h]
                                     for h, c in pos]
                                for (h, c), y in zip(pos, q):
                                    Y[pl.ds(h * HS + r, 16), ch(c)] = y
                                for i, op in enumerate(_ops(_A_TERMS, *q)):
                                    XA.at[i][pl.ds(r, 16), ch(kc)] = op.astype(BF16)
                        stats = [s01] if ONEPASS else [s0, None, s1]
                        items.append(stats + [None] * (2 - half) + [s2])
                return _skew(items)

            def prep_g1_tasks(which, r0, n):
                for g in range(n // 16):
                    r = r0 + g * 16
                    top = rgu[0, which, pl.ds(r, 16), :].astype(F32)
                    bot = rgu[0, which, pl.ds(KH + r, 16), :].astype(F32)
                    for i, op in enumerate(_ops(_B_TERMS, top[:, :NL], top[:, NL:], bot[:, :NL], bot[:, NL:])):
                        B0.at[i][pl.ds(r, 16), ch(which)] = op.astype(BF16)

            def xb_tasks(r0, n, z):
                def task(val, r, kc, i):
                    anchor(Y, S, val, z)
                    x = [_combine(_A_TERMS[i],
                                  lambda sg, kp: Y[pl.ds((2 * sg + rho) * QS + r, 16), ch(4 * kp + 2 * ta + kc)])
                         for rho in range(2) for ta in range(2)]
                    ops = _ops(_A_TERMS, *x)
                    for k, slot in _XB_SLOT.items():
                        XB.at[5 * i + slot][pl.ds(r, 16), ch(kc)] = ops[k].astype(BF16)
                return [(lambda val, r=r0 + g * 16, kc=kc, i=i: task(val, r, kc, i))
                        for g in range(n // 16) for kc in range(2) for i in range(7)]

            def wide(w):
                return pltpu.bitcast(w, BF16).astype(F32)

            def prep_q_tasks(m, par, n, z, chain=True):
                def perm_a(r):
                    y = [rq[m * NCH + k, pl.ds(r // 2, 8), :] for k in range(NCH)]
                    return [y[0]] + [pltpu.roll(y[k], 2 * k, 1) for k in range(1, NCH)]

                def perm_b(y):
                    lane = lax.broadcasted_iota(jnp.int32, (8, NL), 1)
                    sh = (((lane & 15) >> 1) - par) & 7
                    u = [y[(-j) % NCH] for j in range(NCH)]
                    b0, b1, b2 = (sh & 1) != 0, (sh & 2) != 0, (sh & 4) != 0
                    out = (2 * n, 2 * n + 4)
                    v = {j: jnp.where(b0, u[(j - 1) % NCH], u[j]) for j in (0, 2, 4, 6)}
                    v = {j: jnp.where(b1, v[(j - 2) % NCH], v[j]) for j in out}
                    v = {j: jnp.where(b2, v[(j - 4) % NCH], v[j]) for j in out}
                    return [pltpu.roll(v[j], (2 * NL - 2 * j - 2 * par) % NL, 1) for j in out]

                items = []
                for g in range(KH // 16):
                    st = {}
                    for half in range(2):
                        def s0(val, r=half * KH + g * 16, st=st, half=half):
                            anchor(rq.at[0], D // 2, val, z)
                            st["a", half] = perm_a(r)

                        def s1(val, st=st, half=half):
                            st["b", half] = perm_b(st["a", half])

                        def s2(val, r=g * 16, st=st):
                            ops = _ops(_B_TERMS, *[wide(w) for w in st["b", 0] + st["b", 1]])
                            for i in range(7):
                                BQ.at[i][pl.ds(r, 16), ch(n)] = ops[i].astype(BF16)
                            if chain:
                                anchor(rq.at[0], D // 2, (ops[5] + ops[6])[0:8], z)
                        items.append([s0, s1] + ([s2] if half else []))
                flat = _skew(items)
                firsts = [j for j, t in enumerate(flat) if t.__name__ == "s0"] + [len(flat)]
                return [(lambda val, grp=flat[a:b]: [t(val) for t in grp]) for a, b in zip(firsts, firsts[1:])]

            def prep_o_tasks(src, n, z):
                def transpose(c, a):
                    sub = lax.broadcasted_iota(jnp.int32, (8, NL), 0)
                    y = [rq[src + c, pl.ds(64 * g + 8 * a, 8), :] for g in range(8)]
                    y = [y[0]] + [pltpu.roll(y[g], g, 0) for g in range(1, 8)]
                    v = [y[(-j) % 8] for j in range(8)]
                    for bit in (1, 2, 4):
                        v = [jnp.where((sub & bit) != 0, v[(j - bit) % 8], v[j]) for j in range(8)]
                    return [v[0]] + [pltpu.roll(v[j], 8 - j, 0) for j in range(1, 8)]

                tasks = []
                for a in range(8):
                    st = {}

                    def load(val, h, a=a, st=st):
                        anchor(rq.at[0], D // 2, val, z)
                        st[h] = transpose(h * KC + n, a)

                    def quad(val, jj, a=a, st=st):
                        q = [wide(st[h][kh * KC + jj]) for kh in range(2) for h in range(2)]
                        for i, op in enumerate(_ops(_B_TERMS, *q)):
                            BO.at[i][pl.ds(jj * NL + 16 * a, 16), ch(n)] = op.astype(BF16)
                    tasks += [lambda val, f=load: f(val, 0),
                              lambda val, f=load, g=quad: (f(val, 1), [g(val, jj) for jj in range(KC)])]
                return tasks

            def zero_p_tasks(u0, n, z):
                def task(val, u):
                    v = jnp.zeros((8, NL), F32) if val is None else jnp.where(z != 0, val, 0.0)
                    P[u // 32, pl.ds(pl.multiple_of((u % 32) * 32, 32), 32), :] = jnp.tile(v, (4, KC))
                return [(lambda val, u=u0 + j: task(val, u)) for j in range(n)]

            def up1(r0, m):
                g = {}

                def fin_u(k, u):
                    HF[pl.ds((k // 2) * HS + r0, m), ch(k % 2)] = gelu2(g[k], u)
                yield from _strassen(lambda i: _dot(XA[i, pl.ds(r0, m), :], B0[i, :, ch(0)]), g.__setitem__, RG)
                yield from _strassen(lambda i: _dot(XA[i, pl.ds(r0, m), :], B0[i, :, ch(1)]), fin_u, RU)

            with scope("start"):
                groups = [lambda: [cp_x(0, 0), cp_x(0, 1)], lambda: [cp_gu(0, 0, 0)], lambda: [cp_gu(0, 0, 1)]]
                groups += [(lambda i=i: [cp_x(i, 0), cp_x(i, 1)]) for i in range(1, NT0)]
                groups += [lambda: [cp_q(0)], lambda: [cp_gu(1, 1, 0), cp_gu(1, 1, 1), cp_d(0)],
                           lambda: [cp_q(1)], lambda: [cp_o()], lambda: [cp_q(2)]]

                def issue(k, c):
                    for g, cps in enumerate(groups):
                        when(k == g, lambda: [cp.start() for cp in cps()])
                    return c
                lax.fori_loop(0, len(groups), issue, 0)
                cp_x(0, 0).wait(); cp_x(0, 1).wait()

                def ln0(g, c):
                    for t in ln_tasks(pl.multiple_of(g * LN0, LN0), LN0, None):
                        t(None)
                    return c
                lax.fori_loop(0, T0 // LN0, ln0, 0)
                for which in range(2):
                    cp_gu(0, 0, which).wait()

                    def pg0(g, c):
                        prep_g1_tasks(which, pl.multiple_of(g * 64, 64), 64)
                        return c
                    lax.fori_loop(0, KH // 64, pg0, 0)

            def p0_body(i, c):
                cp_x(i + 1, 0).wait(); cp_x(i + 1, 1).wait()
                r0 = pl.multiple_of(i * T0, T0)
                _emit(LAG0, up1(r0, T0), sum(RG) + sum(RU), (0.0, LNF, ln_tasks(r0 + T0, T0, zero(i))))
                return zero(i)
            with scope("p0"):
                z0 = lax.fori_loop(0, NT0 - 1, p0_body, 0)
            with scope("p0_last"):
                cp_q(0).wait()
                cp_gu(2, 0, 0).start(); cp_gu(2, 0, 1).start()
                _emit(LAG, up1(HS - T0, T0), sum(RG) + sum(RU), (0.0, 0.85, prep_q_tasks(0, 0, 0, z0, chain=False)))

            def p1_body(b, c):
                when(b == 0, lambda: (cp_gu(1, 1, 0).wait(), cp_gu(1, 1, 1).wait(), cp_d(0).wait()))
                when(b == 1, lambda: cp_q(1).wait())
                when(b == 2, lambda: cp_o().wait())
                when(b == 3, lambda: cp_q(2).wait())
                m = b // 2
                par = b % 2

                def main():
                    for n in range(2):
                        for s in range(HS // RH):
                            r0 = s * RH

                            def fin(k, v):
                                j = m * NCH + par + 2 * n + 4 * (k % 2)
                                qkv[j, pl.ds(HALO + (k // 2) * HS + r0, RH), :] = v
                            yield from _strassen(lambda i: _dot(XA[i, pl.ds(r0, RH), :], BQ[i, :, ch(n)]), fin, (1,) * 7)
                piece = jnp.clip(b - 2, 0, 3)
                z = zero(b)
                _emit(LAG, main(), 14 * (HS // RH),
                      (0.0, P1A, prep_q_tasks(m, par, 1, z)),
                      (0.5, 0.5 + P1A, prep_q_tasks(jnp.minimum((b + 1) // 2, 2), (b + 1) % 2, 0, z)),
                      (0.0, 0.95, prep_g2_tasks(1, range(7), pl.multiple_of(jnp.minimum(b * 48, KQ - 48), 16), 48, z)),
                      (0.0, XBF, xb_tasks(pl.multiple_of(jnp.minimum(b * 96, QS - 96), 32), 96, z)),
                      (0.0, 0.95, prep_d2_tasks(pl.multiple_of(jnp.minimum(b * 16, NL - PDN - 16), 16), 16, z)),
                      (0.0, 0.95, zero_p_tasks(jnp.minimum(b * 38, 224 - 38), 38, z)),
                      (0.0, 0.95, prep_o_tasks(jnp.where(b < 2, 0, 3 * NCH), piece, z)))
                return c
            with scope("p1"):
                lax.fori_loop(0, 6, p1_body, 0)
                for j in range(NCH, 3 * NCH):
                    qkv[j, 0:HALO, :] = jnp.broadcast_to(qkv[j, HALO:HALO + 1, :], (HALO, NL))

        def second_half(HA, osc, obuf):
            HA = HA.bitcast(BF16)

            def attn_unit(t0, r0, masked, slot, z):
                st = {}

                def shifted(plane):
                    return [qkv[plane, pl.ds(t0 + (r0 + HALO + 8 - DIL * k), 8), :] for k in range(12)]

                def logits(val, j):
                    anchor(qkv.at[0], HALO + S, val, z)
                    q = [qkv[j, pl.ds(t0 + (r0 + HALO + 8 * g), 8), :] for g in range(2)]
                    kk = shifted(NCH + j)
                    for g in range(2):
                        for w in range(W):
                            t = q[g] * kk[w + 4 - 4 * g]
                            st[g, w] = t if j == 0 else st[g, w] + t
                    if j == NCH - 1:
                        softmax()

                def softmax():
                    lane = lax.broadcasted_iota(jnp.int32, (8, NL), 1)
                    odd = (lane & 1) != 0
                    hi = (lane & 16) != 0
                    keys = [(g, w) for g in range(2) for w in range(W)]
                    for k in keys:
                        a = st[k]
                        st[k] = a + jnp.where(odd, pltpu.roll(a, 1, 1), pltpu.roll(a, NL - 1, 1))
                    for k in keys:
                        a = st[k]
                        st[k] = a + jnp.where(hi, pltpu.roll(a, 16, 1), pltpu.roll(a, NL - 16, 1))
                    for g in range(2):
                        ls = [st[g, w] for w in range(W)]
                        if masked:
                            pos = t0 + (r0 + 8 * g) + lax.broadcasted_iota(jnp.int32, (8, NL), 0)
                            ls = [ls[0]] + [jnp.where(pos >= DIL * w, ls[w], NEG) for w in range(1, W)]
                        m = ls[0]
                        for w in range(1, W):
                            m = jnp.maximum(m, ls[w])
                        ps = [jnp.exp2((l - m) * EXP2_SCALE) for l in ls]
                        den = ps[0]
                        for w in range(1, W):
                            den = den + ps[w]
                        inv = 1.0 / den
                        for w in range(W):
                            st[g, w] = ps[w] * inv

                def pv(val, j):
                    anchor(qkv.at[0], HALO + S, val, z)
                    vv = shifted(2 * NCH + j)
                    for g in range(2):
                        a = st[g, 0] * vv[4 - 4 * g]
                        for w in range(1, W):
                            a = a + st[g, w] * vv[w + 4 - 4 * g]
                        osc[slot, j, pl.ds(8 * g, 8), :] = a

                return ([(lambda val, j=j: logits(val, j)) for j in range(NCH)] + [lambda val: None] * AGAP
                        + [(lambda val, j=j: pv(val, j)) for j in range(NCH)])

            def attn_tasks(t0, off, n, z):
                t0 = pl.multiple_of(jnp.minimum(t0 + off // 32 * 32, HS - n - off % 32), 16)
                tasks = []
                for g in range(n // 16):
                    r = off % 32 + g * 16
                    tasks += attn_unit(t0, r, g == 0, 2 * g, z) + attn_unit(t0, HS + r, False, 2 * g + 1, z)

                    def oa(val, kc, g=g, r=r):
                        ops = _ops(_A_TERMS, osc[2 * g, kc], osc[2 * g, KC + kc],
                                   osc[2 * g + 1, kc], osc[2 * g + 1, KC + kc])
                        for i in range(7):
                            OA.at[i][pl.ds(t0 + r, 16), ch(kc)] = ops[i].astype(BF16)
                    tasks += [(lambda val, kc=kc, oa=oa: oa(val, kc)) for kc in range(KC)]
                return tasks

            def ha_task(val, r, i, z, have):
                anchor(HF, S, val, z)
                x = [_combine(_A_TERMS[i], lambda sg, kp: HF[pl.ds((2 * sg + rho) * QS + r, 16), ch(2 * kp + ta)])
                     for rho in range(2) for ta in range(2)]
                for k, op in enumerate(_ops(_A_TERMS, *x)):
                    HA[pl.ds(r, 16), ch(7 * i + k)] = op.astype(BF16)
                have.add((i, r))

            def up2(kp, free, on_half):
                def sub(r0, m):
                    hold, seen = {}, set()

                    def outer_fin(k, K, v):
                        if K in (2, 1):
                            hold[k] = v
                            return
                        sg = K // 2
                        HF[pl.ds((2 * sg + k // 2) * QS + r0, m), ch(2 * kp + k % 2)] = (
                            gelu2(hold[k], v) if K == 3 else gelu2(v, hold[k]))
                        seen.add((sg, k))
                        if all((sg, j) in seen for j in range(4)):
                            on_half(sg, r0, m)
                    folds = [_Fold(lambda K, v, k=k: outer_fin(k, K, v)) for k in range(4)]

                    def lhs(i, k):
                        if k == 2:
                            return XA[i, pl.ds(r0, m), pl.ds(0, KQ)]
                        if k == 3:
                            return XA[i, pl.ds(QS + r0, m), pl.ds(KQ, KQ)]
                        return XB[5 * i + _XB_SLOT[k], pl.ds(r0, m), :]
                    return lambda i: _strassen(lambda k: _dot(lhs(i, k), BG[i, :, ch(k)]),
                                               lambda k, v: folds[k](i, v), R2H if i in (2, 6) else R2L)
                subs = [sub(s * RH2, RH2) for s in range(QS // RH2)]
                for i in _ORDER:
                    for sb in subs:
                        yield from sb(i)
                    free.add(i)

            nsub = QS // RH2
            g_room = (5 * sum(R2L) + 2 * sum(R2H)) * nsub
            d_unit = RD2 * MD * ND / (RH2 * KQ)

            ends = [sum(sum(R2H if i in (2, 6) else R2L) for i in _ORDER[:j + 1]) * nsub for j in range(7)]

            def bg_sides(slot, total, z, free, n):
                return [((ends[j] + 1) / total, (ends[j + 1] if j < 6 else ends[6] + ends[0]) / total - 0.01,
                         prep_g2_tasks(slot, _ORDER[j:j + 1], 0, KQ, z, free)) for j in range(n)]

            def block_b(k):
                when(k < NP - 1, lambda: (cp_gu(0, 0, 0).wait(), cp_gu(0, 0, 1).wait()))

                def prefetch(val):
                    when(k < NP - 1, lambda: (cp_gu(2 * k + 3, 1, 0).start(), cp_gu(2 * k + 3, 1, 1).start(),
                                              cp_d(k + 1).start()))
                z = zero(k)
                free, have, halves = set(), set(), set()

                def on_half(sg, r0, m):
                    if r0 + m == QS:
                        halves.add(sg)

                def ha_tasks(outer, need):
                    def task(val, r, i):
                        assert need <= halves
                        ha_task(val, r, i, z, have)
                    return [(lambda val, r=r, i=i: task(val, r, i)) for i in outer for r in range(0, QS, 16)]

                def main():
                    yield from up2(1, free, on_half)
                    for i in (2, 5, 1, 3, 0, 4, 6):
                        assert all((i, r) in have for r in range(0, QS, 16))
                        for r0 in range(0, QS, MD):
                            for c in range(KQ // ND):
                                def fin(q, v):
                                    P[i, pl.ds((q // 2) * QS + r0, MD), pl.ds((q % 2) * KQ + c * ND, ND)] += v
                                yield from _strassen(
                                    lambda j: _dot(HA[pl.ds(r0, MD), ch(7 * i + j)], BD[7 * i + j, :, ch(c, ND)]),
                                    fin, (d_unit,) * 7)
                total = g_room + 49 * (QS // MD) * (KQ // ND) * d_unit
                gf = g_room / total
                df = (1 - gf) / 7
                _emit(LAG2, main(), total, *bg_sides(0, total, z, free, 7),
                      (0.0, ends[0] / total, prep_g2_tasks(1, _ORDER[6:], 0, KQ, z)),
                      (0.0, HAF * gf, ha_tasks((2, 5), set())),
                      ((ends[4] + 1) / total, gf + HA1 * df, ha_tasks((1, 3, 0), {1})),
                      (gf + HA1 * df, gf + HA2 * df, ha_tasks((4, 6), {0, 1})),
                      (0.0, PDB * gf, prep_d2_tasks(NL - PDN, PDN, z)),
                      (0.0, ATB, attn_tasks(k * (APA + APB), 0, APB, z)),
                      (gf, gf + 0.01, [prefetch]))

            def block_a(k):
                cp_gu(0, 1, 0).wait(); cp_gu(0, 1, 1).wait(); cp_d(0).wait()

                def prefetch(val):
                    when(k < NP - 2, lambda: (cp_gu(2 * k + 4, 0, 0).start(), cp_gu(2 * k + 4, 0, 1).start()))
                z = zero(k)
                free = set()
                _emit(LAG2, up2(0, free, lambda *a: None), g_room, *bg_sides(1, g_room, z, free, 6),
                      (0.0, 0.95, prep_d2_tasks(0, NL - PDN, z)),
                      (0.0, 0.95, attn_tasks(k * (APA + APB), APB, APA, z)),
                      (0.01, 0.02, [prefetch]))

            def p2_body(k, carry):
                with scope("b"):
                    block_b(k)
                with scope("a"):
                    when(k < NP - 1, lambda: block_a(k))
                return carry
            with scope("p2"):
                lax.fori_loop(0, NP, p2_body, 0)

            def cp_out(t, half, s):
                return pltpu.make_async_copy(obuf.at[t % 2, half, pl.ds(s * M3, M3), :],
                                             out_hbm.at[pl.ds(half * HS + t * T3 + s * M3, M3), :], sem_out.at[t % 2])

            def wait_out(t):
                pltpu.make_async_copy(obuf.at[t % 2], obuf.at[t % 2], sem_out.at[t % 2]).wait()

            def p3_body(t, carry):
                when(t >= 2, lambda: wait_out(t - 2))
                for s in range(T3 // M3):
                    r0 = pl.multiple_of(t * T3 + s * M3, M3)
                    for n in range(KC):
                        def fin(k, sq):
                            (j0, _), *rest = _C_TERMS[k]
                            f = P[j0, pl.ds(r0, M3), ch(n)]
                            for j, sign in rest:
                                f = f + P[j, pl.ds(r0, M3), ch(n)] if sign > 0 else f - P[j, pl.ds(r0, M3), ch(n)]
                            y = f * 0.25
                            half, col = k // 2, (k % 2) * KC + n
                            x = xbuf[pl.ds(half * HS + r0, M3), ch(col)].astype(F32)
                            obuf.at[t % 2, half][pl.ds(s * M3, M3), ch(col)] = (
                                x + sq * (y + y * jnp.tanh(y))).astype(BF16)
                        for step, _ in enumerate(_strassen(
                                lambda i: _dot(OA[i, pl.ds(r0, M3), :], BO[i, :, ch(n)]), fin, (1,) * 7)):
                            if s > 0 and n == 0 and step == OUTK:
                                cp_out(t, 0, s - 1).start(); cp_out(t, 1, s - 1).start()
                cp_out(t, 0, T3 // M3 - 1).start(); cp_out(t, 1, T3 // M3 - 1).start()
                return carry
            with scope("p3"):
                lax.fori_loop(0, NT3, p3_body, 0)
            with scope("end"):
                for t in range(NT3 - 2, NT3):
                    wait_out(t)

        pl.run_scoped(first_half,
                      pltpu.VMEM((7, KH // 2, 2 * NL), U32),
                      pltpu.VMEM((7, KH // 2, 2 * NL), U32))
        pl.run_scoped(second_half,
                      pltpu.VMEM((QS // 2, 49 * NL), U32),
                      pltpu.VMEM((max(APA, APB) // 8, NCH, 16, NL), F32),
                      pltpu.VMEM((2, 2, T3, D), BF16))

    def fn(A_x, A_wqkv, A_wo, B_x, B_w_gate, B_w_up, B_w_down):
        x = A_x.reshape(S, D)
        anyspec = pl.BlockSpec(memory_space=pl.ANY)
        out = pl.pallas_call(
            kernel,
            in_specs=[anyspec] * 6,
            out_specs=anyspec,
            out_shape=jax.ShapeDtypeStruct((S, D), BF16),
            scratch_shapes=[
                pltpu.VMEM((S + SPARE, D), BF16),
                pltpu.VMEM((7, HS // 2, KH), U32),
                pltpu.VMEM((35, QS // 2, KQ), U32),
                pltpu.VMEM((3 * NCH, HALO + S + SPARE, NL), F32),
                pltpu.VMEM((7, HS, KH), F32),
                pltpu.VMEM((S + SPARE, 2 * FC), F32),
                pltpu.VMEM((7, KQ // 2, 7 * NL), U32),
                pltpu.VMEM((49, NL // 2, KQ), U32),
                pltpu.VMEM((7, KH // 2, KH), U32),
                pltpu.VMEM((2, 2, D + SPARE, FC), BF16),
                pltpu.VMEM((2 * FC + SPARE, D), BF16),
                pltpu.VMEM((S + SPARE, D), F32),
                pltpu.VMEM((4 * NCH, D // 2 + 64, NL), U32),
                pltpu.VMEM((7, HS // 2, KH), U32),
                pltpu.SemaphoreType.DMA((NT0, 2)),
                pltpu.SemaphoreType.DMA((2, 2)),
                pltpu.SemaphoreType.DMA((1,)),
                pltpu.SemaphoreType.DMA((3,)),
                pltpu.SemaphoreType.DMA((1,)),
                pltpu.SemaphoreType.DMA((2,)),
            ],
            compiler_params=pltpu.CompilerParams(vmem_limit_bytes=124 * 2 ** 20, disable_bounds_checks=True),
        )(x, A_wqkv, A_wo, B_w_gate, B_w_up, B_w_down)
        return out.reshape(1, S, D)
    return jax.jit(fn)


_IMPL = make()


@jax.jit
def pallas_recurrent_scan__sliding_local_dilated__geglu_ffn__prompt_kernel(
    A_x: jax.Array,
    A_wqkv: jax.Array,
    A_wo: jax.Array,
    B_x: jax.Array,
    B_w_gate: jax.Array,
    B_w_up: jax.Array,
    B_w_down: jax.Array,
):
    return _IMPL(A_x, A_wqkv, A_wo, B_x, B_w_gate, B_w_up, B_w_down)
```

```python
import contextlib
import math

import jax
import jax.numpy as jnp
from jax import lax
import jax.experimental.pallas as pl
import jax.experimental.pallas.tpu as pltpu

S, D, F = 2048, 1024, 3584
H, DH, W, DIL = 32, 32, 8, 2
NL = 128
NCH = D // NL
HS = S // 2
KH = D // 2
KC = KH // NL
QS = S // 4
KQ = D // 4
FC = 256
NP = F // (2 * FC)
HALO = 16
SPARE = 48
F32, BF16, U32 = jnp.float32, jnp.bfloat16, jnp.uint32
EPS = 1e-5
GELU_C0 = math.sqrt(2.0 / math.pi)
GELU_C1 = GELU_C0 * 0.044715
EXP2_SCALE = (DH ** -0.5) * math.log2(math.e)
NEG = -1e9 / (DH ** -0.5)

_A_TERMS = (((0, 0, 1), (1, 1, 1)), ((1, 0, 1), (1, 1, 1)), ((0, 0, 1),), ((1, 1, 1),),
            ((0, 0, 1), (0, 1, 1)), ((1, 0, 1), (0, 0, -1)), ((0, 1, 1), (1, 1, -1)))
_B_TERMS = (((0, 0, 1), (1, 1, 1)), ((0, 0, 1),), ((0, 1, 1), (1, 1, -1)), ((1, 0, 1), (0, 0, -1)),
            ((1, 1, 1),), ((0, 0, 1), (0, 1, 1)), ((1, 0, 1), (1, 1, 1)))
_C_TERMS = (((0, 1), (3, 1), (4, -1), (6, 1)), ((2, 1), (4, 1)), ((1, 1), (3, 1)), ((0, 1), (1, -1), (2, 1), (5, 1)))
_ORDER = (1, 3, 0, 5, 2, 4, 6)
_XB_SLOT = {0: 0, 1: 1, 4: 2, 5: 3, 6: 4}


def _combine(terms, get):
    (r, c, _), *rest = terms
    v = get(r, c)
    for r, c, sign in rest:
        v = v + get(r, c) if sign > 0 else v - get(r, c)
    return v


def _ops(terms, q11, q12, q21, q22):
    q = ((q11, q12), (q21, q22))
    return [_combine(t, lambda r, c: q[r][c]) for t in terms]


def _dot(a, b):
    return jnp.dot(a, b, preferred_element_type=F32)


class _Fold:
    def __init__(self, fin):
        self.fin = fin

    def __call__(self, i, m):
        if i == 1:
            self.m1 = m
        elif i == 3:
            self.fin(2, self.m1 + m)
            self.t11 = m
        elif i == 0:
            self.t11 = self.t11 + m
            self.t22 = m - self.m1
        elif i == 5:
            self.t22 = self.t22 + m
        elif i == 2:
            self.fin(3, self.t22 + m)
            self.m2 = m
        elif i == 4:
            self.fin(1, self.m2 + m)
            self.t11 = self.t11 - m
        else:
            self.fin(0, self.t11 + m)


def _strassen(prod, fin, room):
    fold = _Fold(fin)
    for step, i in enumerate(_ORDER):
        m = prod(i)
        fold(i, m)
        yield room[step], m


def _emit(lag, main, total, *sides):
    done = [0] * len(sides)
    acc = 0

    def flush(frac, val):
        due = []
        for k, (f0, f1, tasks) in enumerate(sides):
            want = len(tasks) if frac >= f1 else int(max(0.0, (frac - f0) / (f1 - f0)) * len(tasks) + 0.5)
            n = min(want, len(tasks)) - done[k]
            due += [((j + 0.5) / n, k, tasks[done[k] + j]) for j in range(n)]
            done[k] += max(n, 0)
        due.sort(key=lambda e: e[:2])
        for j, (_, _, task) in enumerate(due):
            r = (val.shape[0] // 8) * j // len(due) * 8
            task(val[r:r + 8, 0:NL])

    hist = [(0, None)] * lag
    for item in main:
        hist.append(item)
        room, val = hist.pop(0)
        acc += room
        if room:
            flush(acc / total, val)
    assert abs(acc + sum(h[0] for h in hist) - total) < 1e-6
    flush(2.0, hist[-1][1])


def _skew(items):
    depth = max(len(st) for st in items)
    return [items[t - k][k] for t in range(len(items) + depth - 1) for k in range(depth)
            if 0 <= t - k < len(items) and k < len(items[t - k]) and items[t - k][k] is not None]


def make(ONEPASS=True, T0=128, LN0=64, LNF=0.85, RG=(2,) * 7, RU=(2, 2, 2, 2, 1, 1, 1), LAG0=2,
         RH=256, LAG=1, P1A=0.46, XBF=0.95,
         RH2=64, LAG2=5, LAGA=5, R2L=(2,) * 7, R2H=(2, 0, 2, 2, 0, 0, 0), MD=128, ND=128, RD2=2.5,
         APA=64, APB=96, AGAP=5, HAF=0.9, HA1=1.8, HA2=5.3, ATB=0.98, ATA=0.95, PDN=32, PDB=0.9, PDA=0.95,
         M3=64, OUTK=1, scopes=False):
    NT0 = HS // T0
    T3 = 256
    NT3 = HS // T3
    assert NL - PDN <= 96
    assert (NP - 1) * APA + NP * APB >= HS and (APA + APB) % 32 == 0 and APA % 16 == 0 and APB % 16 == 0

    def scope(name):
        return jax.named_scope(name) if scopes else contextlib.nullcontext()

    def kernel(x_hbm, wqkv_hbm, wo_hbm, wg_hbm, wu_hbm, wd_hbm, out_hbm,
               xbuf, XA, XB, qkv, P, HF, BG, BD, BO, rw, Y, rq, OA,
               sem_x, sem_gu, sem_d, sem_q, sem_o, sem_out):

        XA, XB, BG, BD, BO, OA = [r.bitcast(BF16) for r in (XA, XB, BG, BD, BO, OA)]

        def ch(n, w=NL):
            return pl.ds(n * w, w) if isinstance(n, int) else pl.ds(pl.multiple_of(n * w, w), w)

        def zero(i):
            return i % 2 + (i + 1) % 2 - 1

        def when(pred, fn):
            pl.when(pred)(lambda: (fn(), None)[1])

        def cp_x(i, half):
            r = half * HS + i * T0
            return pltpu.make_async_copy(x_hbm.at[pl.ds(r, T0), :], xbuf.at[pl.ds(r, T0), :], sem_x.at[i, half])

        def cp_gu(c, slot, which):
            src = wg_hbm if which == 0 else wu_hbm
            return pltpu.make_async_copy(src.at[:, pl.ds(c * FC, FC)], rw.at[2 * slot + which, pl.ds(0, D), :],
                                         sem_gu.at[slot, which])

        class cp_d:
            def __init__(self, p):
                self.p = p

            def start(self):
                for q in range(4):
                    pltpu.make_async_copy(wd_hbm.at[pl.ds(self.p * 2 * FC, 2 * FC), pl.ds(q * KQ, KQ)],
                                          rw.at[4 + q // 2, pl.ds((q % 2) * 2 * FC, 2 * FC), :], sem_d.at[0]).start()

            def wait(self):
                whole = rw.at[pl.ds(4, 2), pl.ds(0, D), :]
                pltpu.make_async_copy(whole, whole, sem_d.at[0]).wait()

        def anchor(dst, row, val, z):
            if val is not None and z is not None:
                r = pl.multiple_of(row + 16 + z * 16, 8)
                dst[pl.ds(r, 8), pl.ds(0, NL)] = pltpu.bitcast(val, U32) if dst.dtype == U32 else val.astype(dst.dtype)

        def gelu2(g, u):
            t = jnp.tanh(g * (GELU_C0 + GELU_C1 * (g * g)))
            p = g * u
            return p + p * t

        def prep_g2_tasks(slot, outer, r0, n, z, free=None):
            def task(val, r, i):
                assert free is None or i in free
                anchor(rw.at[0], D, val, z)
                y = [_combine(_B_TERMS[i], lambda kp, mu: rw[2 * slot + mu, pl.ds((2 * kp + ta) * KQ + r, 16), :].astype(F32))
                     for ta in range(2)]
                ops = _ops(_B_TERMS, y[0][:, :NL], y[0][:, NL:], y[1][:, :NL], y[1][:, NL:])
                for k in range(7):
                    BG.at[i][pl.ds(r, 16), ch(k)] = ops[k].astype(BF16)
            return [(lambda val, r=r0 + g * 16, i=i: task(val, r, i)) for i in outer for g in range(n // 16)]

        def prep_d2_tasks(r0, n, z):
            def task(val, r, i):
                anchor(rw.at[0], D, val, z)
                y = [_combine(_B_TERMS[i],
                              lambda kp, nu: rw[4 + nu, pl.ds(up * 2 * FC + (2 * kp + ta) * NL + r, 16), :].astype(F32))
                     for ta in range(2) for up in range(2)]
                ops = _ops(_B_TERMS, *y)
                for k in range(7):
                    BD.at[7 * i + k][pl.ds(r, 16), :] = ops[k].astype(BF16)
            return [(lambda val, r=r0 + g * 16, i=i: task(val, r, i)) for g in range(n // 16) for i in range(7)]

        def first_half(B0, BQ):
            B0, BQ = B0.bitcast(BF16), BQ.bitcast(BF16)

            class cp_cols:
                def __init__(self, src, col0, dst, slot0, sem):
                    self.args = src, col0, dst, slot0, sem

                def start(self):
                    src, col0, dst, slot0, sem = self.args
                    for k in range(NCH):
                        pltpu.make_async_copy(src.at[:, pl.ds(col0 + k * NL, NL)],
                                              dst.at[slot0 + k, pl.ds(0, D // 2), :].bitcast(BF16), sem).start()

                def wait(self):
                    _, _, dst, slot0, sem = self.args
                    whole = dst.at[pl.ds(slot0, NCH), pl.ds(0, D // 2), :]
                    pltpu.make_async_copy(whole, whole, sem).wait()

            def cp_q(m):
                return cp_cols(wqkv_hbm, m * D, rq, m * NCH, sem_q.at[m])

            def cp_o():
                return cp_cols(wo_hbm, 0, rq, 3 * NCH, sem_o.at[0])

            def ln_tasks(r0, n, z):
                def xrow(r):
                    return xbuf[pl.ds(r, 16), :].astype(F32)
                items = []
                for g in range(n // 16):
                    st = {}
                    for half in range(2):
                        def s0(val, r=half * HS + r0 + g * 16, st=st, half=half):
                            anchor(xbuf, S, val, z)
                            st["m", half] = jnp.sum(xrow(r), axis=-1, keepdims=True) * (1.0 / D)

                        def s1(val, r=half * HS + r0 + g * 16, st=st, half=half):
                            anchor(xbuf, S, val, z)
                            c = xrow(r) - st["m", half]
                            st["v", half] = lax.rsqrt(jnp.sum(c * c, axis=-1, keepdims=True) * (1.0 / D) + EPS)

                        def s01(val, r=half * HS + r0 + g * 16, st=st, half=half):
                            anchor(xbuf, S, val, z)
                            x = xrow(r)
                            m = jnp.sum(x, axis=-1, keepdims=True) * (1.0 / D)
                            e2 = jnp.sum(x * x, axis=-1, keepdims=True) * (1.0 / D)
                            st["m", half] = m
                            st["v", half] = lax.rsqrt(jnp.maximum(e2 - m * m, 0.0) + EPS)

                        def s2(val, r=r0 + g * 16, st=st, half=half):
                            for kc in (2 * half, 2 * half + 1):
                                anchor(xbuf, S, val, z)
                                pos = [(h, c) for h in range(2) for c in (kc, KC + kc)]
                                q = [(xbuf[pl.ds(h * HS + r, 16), ch(c)].astype(F32) - st["m", h]) * st["v", h]
                                     for h, c in pos]
                                for (h, c), y in zip(pos, q):
                                    Y[pl.ds(h * HS + r, 16), ch(c)] = y
                                for i, op in enumerate(_ops(_A_TERMS, *q)):
                                    XA.at[i][pl.ds(r, 16), ch(kc)] = op.astype(BF16)
                        stats = [s01] if ONEPASS else [s0, None, s1]
                        items.append(stats + [None] * (2 - half) + [s2])
                return _skew(items)

            def prep_g1_tasks(which, r0, n):
                for g in range(n // 16):
                    r = r0 + g * 16
                    top = rw[which, pl.ds(r, 16), :].astype(F32)
                    bot = rw[which, pl.ds(KH + r, 16), :].astype(F32)
                    for i, op in enumerate(_ops(_B_TERMS, top[:, :NL], top[:, NL:], bot[:, :NL], bot[:, NL:])):
                        B0.at[i][pl.ds(r, 16), ch(which)] = op.astype(BF16)

            def xb_tasks(r0, n, z):
                def task(val, r, kc, i):
                    anchor(Y, S, val, z)
                    x = [_combine(_A_TERMS[i],
                                  lambda sg, kp: Y[pl.ds((2 * sg + rho) * QS + r, 16), ch(4 * kp + 2 * ta + kc)])
                         for rho in range(2) for ta in range(2)]
                    ops = _ops(_A_TERMS, *x)
                    for k, slot in _XB_SLOT.items():
                        XB.at[5 * i + slot][pl.ds(r, 16), ch(kc)] = ops[k].astype(BF16)
                return [(lambda val, r=r0 + g * 16, kc=kc, i=i: task(val, r, kc, i))
                        for g in range(n // 16) for kc in range(2) for i in range(7)]

            def wide(w):
                return pltpu.bitcast(w, BF16).astype(F32)

            def prep_q_tasks(m, par, n, z, chain=True):
                def perm_a(r):
                    y = [rq[m * NCH + k, pl.ds(r // 2, 8), :] for k in range(NCH)]
                    return [y[0]] + [pltpu.roll(y[k], 2 * k, 1) for k in range(1, NCH)]

                def perm_b(y):
                    lane = lax.broadcasted_iota(jnp.int32, (8, NL), 1)
                    sh = (((lane & 15) >> 1) - par) & 7
                    u = [y[(-j) % NCH] for j in range(NCH)]
                    b0, b1, b2 = (sh & 1) != 0, (sh & 2) != 0, (sh & 4) != 0
                    out = (2 * n, 2 * n + 4)
                    v = {j: jnp.where(b0, u[(j - 1) % NCH], u[j]) for j in (0, 2, 4, 6)}
                    v = {j: jnp.where(b1, v[(j - 2) % NCH], v[j]) for j in out}
                    v = {j: jnp.where(b2, v[(j - 4) % NCH], v[j]) for j in out}
                    return [pltpu.roll(v[j], (2 * NL - 2 * j - 2 * par) % NL, 1) for j in out]

                items = []
                for g in range(KH // 16):
                    st = {}
                    for half in range(2):
                        def s0(val, r=half * KH + g * 16, st=st, half=half):
                            anchor(rq.at[0], D // 2, val, z)
                            st["a", half] = perm_a(r)

                        def s1(val, st=st, half=half):
                            st["b", half] = perm_b(st["a", half])

                        def s2(val, r=g * 16, st=st):
                            ops = _ops(_B_TERMS, *[wide(w) for w in st["b", 0] + st["b", 1]])
                            for i in range(7):
                                BQ.at[i][pl.ds(r, 16), ch(n)] = ops[i].astype(BF16)
                            if chain:
                                anchor(rq.at[0], D // 2, (ops[5] + ops[6])[0:8], z)
                        items.append([s0, s1] + ([s2] if half else []))
                flat = _skew(items)
                firsts = [j for j, t in enumerate(flat) if t.__name__ == "s0"] + [len(flat)]
                return [(lambda val, grp=flat[a:b]: [t(val) for t in grp]) for a, b in zip(firsts, firsts[1:])]

            def prep_o_tasks(src, n, z):
                def transpose(c, a):
                    sub = lax.broadcasted_iota(jnp.int32, (8, NL), 0)
                    y = [rq[src + c, pl.ds(64 * g + 8 * a, 8), :] for g in range(8)]
                    y = [y[0]] + [pltpu.roll(y[g], g, 0) for g in range(1, 8)]
                    v = [y[(-j) % 8] for j in range(8)]
                    for bit in (1, 2, 4):
                        v = [jnp.where((sub & bit) != 0, v[(j - bit) % 8], v[j]) for j in range(8)]
                    return [v[0]] + [pltpu.roll(v[j], 8 - j, 0) for j in range(1, 8)]

                tasks = []
                for a in range(8):
                    st = {}

                    def load(val, h, a=a, st=st):
                        anchor(rq.at[0], D // 2, val, z)
                        st[h] = transpose(h * KC + n, a)

                    def quad(val, jj, a=a, st=st):
                        q = [wide(st[h][kh * KC + jj]) for kh in range(2) for h in range(2)]
                        for i, op in enumerate(_ops(_B_TERMS, *q)):
                            BO.at[i][pl.ds(jj * NL + 16 * a, 16), ch(n)] = op.astype(BF16)
                    tasks += [lambda val, f=load: f(val, 0),
                              lambda val, f=load, g=quad: (f(val, 1), [g(val, jj) for jj in range(KC)])]
                return tasks

            def zero_p_tasks(u0, n, z):
                def task(val, u):
                    v = jnp.zeros((8, NL), F32) if val is None else jnp.where(z != 0, val, 0.0)
                    P[u // 32, pl.ds(pl.multiple_of((u % 32) * 32, 32), 32), :] = jnp.tile(v, (4, KC))
                return [(lambda val, u=u0 + j: task(val, u)) for j in range(n)]

            def up1(r0, m):
                g = {}

                def fin_u(k, u):
                    HF[pl.ds((k // 2) * HS + r0, m), ch(k % 2)] = gelu2(g[k], u)
                yield from _strassen(lambda i: _dot(XA[i, pl.ds(r0, m), :], B0[i, :, ch(0)]), g.__setitem__, RG)
                yield from _strassen(lambda i: _dot(XA[i, pl.ds(r0, m), :], B0[i, :, ch(1)]), fin_u, RU)

            with scope("start"):
                groups = [lambda: [cp_x(0, 0), cp_x(0, 1)], lambda: [cp_gu(0, 0, 0)], lambda: [cp_gu(0, 0, 1)]]
                groups += [(lambda i=i: [cp_x(i, 0), cp_x(i, 1)]) for i in range(1, NT0)]
                groups += [lambda: [cp_q(0)], lambda: [cp_gu(1, 1, 0), cp_gu(1, 1, 1), cp_d(0)],
                           lambda: [cp_q(1)], lambda: [cp_o()], lambda: [cp_q(2)]]

                def issue(k, c):
                    for g, cps in enumerate(groups):
                        when(k == g, lambda: [cp.start() for cp in cps()])
                    return c
                lax.fori_loop(0, len(groups), issue, 0)
                cp_x(0, 0).wait(); cp_x(0, 1).wait()

                def ln0(g, c):
                    for t in ln_tasks(pl.multiple_of(g * LN0, LN0), LN0, None):
                        t(None)
                    return c
                lax.fori_loop(0, T0 // LN0, ln0, 0)
                for which in range(2):
                    cp_gu(0, 0, which).wait()

                    def pg0(g, c):
                        prep_g1_tasks(which, pl.multiple_of(g * 64, 64), 64)
                        return c
                    lax.fori_loop(0, KH // 64, pg0, 0)

            def p0_body(i, c):
                cp_x(i + 1, 0).wait(); cp_x(i + 1, 1).wait()
                r0 = pl.multiple_of(i * T0, T0)
                _emit(LAG0, up1(r0, T0), sum(RG) + sum(RU), (0.0, LNF, ln_tasks(r0 + T0, T0, zero(i))))
                return zero(i)
            with scope("p0"):
                z0 = lax.fori_loop(0, NT0 - 1, p0_body, 0)
            with scope("p0_last"):
                cp_q(0).wait()
                cp_gu(2, 0, 0).start(); cp_gu(2, 0, 1).start()
                _emit(LAG, up1(HS - T0, T0), sum(RG) + sum(RU), (0.0, 0.85, prep_q_tasks(0, 0, 0, z0, chain=False)))

            def p1_body(b, c):
                when(b == 0, lambda: (cp_gu(1, 1, 0).wait(), cp_gu(1, 1, 1).wait(), cp_d(0).wait()))
                when(b == 1, lambda: cp_q(1).wait())
                when(b == 2, lambda: cp_o().wait())
                when(b == 3, lambda: cp_q(2).wait())
                m = b // 2
                par = b % 2

                def main():
                    for n in range(2):
                        for s in range(HS // RH):
                            r0 = s * RH

                            def fin(k, v):
                                j = m * NCH + par + 2 * n + 4 * (k % 2)
                                qkv[j, pl.ds(HALO + (k // 2) * HS + r0, RH), :] = v
                            yield from _strassen(lambda i: _dot(XA[i, pl.ds(r0, RH), :], BQ[i, :, ch(n)]), fin, (1,) * 7)
                piece = jnp.clip(b - 2, 0, 3)
                z = zero(b)
                _emit(LAG, main(), 14 * (HS // RH),
                      (0.0, P1A, prep_q_tasks(m, par, 1, z)),
                      (0.5, 0.5 + P1A, prep_q_tasks(jnp.minimum((b + 1) // 2, 2), (b + 1) % 2, 0, z)),
                      (0.0, 0.95, prep_g2_tasks(1, range(7), pl.multiple_of(jnp.minimum(b * 48, KQ - 48), 16), 48, z)),
                      (0.0, XBF, xb_tasks(pl.multiple_of(jnp.minimum(b * 96, QS - 96), 32), 96, z)),
                      (0.0, 0.95, prep_d2_tasks(pl.multiple_of(jnp.clip(b * 16, 0, max(NL - PDN - 16, 0)), 16), min(16, NL - PDN), z)),
                      (0.0, 0.95, zero_p_tasks(jnp.minimum(b * 38, 224 - 38), 38, z)),
                      (0.0, 0.95, prep_o_tasks(jnp.where(b < 2, 0, 3 * NCH), piece, z)))
                return c
            with scope("p1"):
                lax.fori_loop(0, 6, p1_body, 0)
                for j in range(NCH, 3 * NCH):
                    qkv[j, 0:HALO, :] = jnp.broadcast_to(qkv[j, HALO:HALO + 1, :], (HALO, NL))

        def second_half(HA, osc, obuf):
            HA = HA.bitcast(BF16)

            def attn_unit(t0, r0, masked, slot, z):
                st = {}

                def shifted(plane):
                    return [qkv[plane, pl.ds(t0 + (r0 + HALO + 8 - DIL * k), 8), :] for k in range(12)]

                def logits(val, j):
                    anchor(qkv.at[0], HALO + S, val, z)
                    q = [qkv[j, pl.ds(t0 + (r0 + HALO + 8 * g), 8), :] for g in range(2)]
                    kk = shifted(NCH + j)
                    for g in range(2):
                        for w in range(W):
                            t = q[g] * kk[w + 4 - 4 * g]
                            st[g, w] = t if j == 0 else st[g, w] + t
                    if j == NCH - 1:
                        softmax()

                def softmax():
                    lane = lax.broadcasted_iota(jnp.int32, (8, NL), 1)
                    odd = (lane & 1) != 0
                    hi = (lane & 16) != 0
                    keys = [(g, w) for g in range(2) for w in range(W)]
                    for k in keys:
                        a = st[k]
                        st[k] = a + jnp.where(odd, pltpu.roll(a, 1, 1), pltpu.roll(a, NL - 1, 1))
                    for k in keys:
                        a = st[k]
                        st[k] = a + jnp.where(hi, pltpu.roll(a, 16, 1), pltpu.roll(a, NL - 16, 1))
                    for g in range(2):
                        ls = [st[g, w] for w in range(W)]
                        if masked:
                            pos = t0 + (r0 + 8 * g) + lax.broadcasted_iota(jnp.int32, (8, NL), 0)
                            ls = [ls[0]] + [jnp.where(pos >= DIL * w, ls[w], NEG) for w in range(1, W)]
                        m = ls[0]
                        for w in range(1, W):
                            m = jnp.maximum(m, ls[w])
                        ps = [jnp.exp2((l - m) * EXP2_SCALE) for l in ls]
                        den = ps[0]
                        for w in range(1, W):
                            den = den + ps[w]
                        inv = 1.0 / den
                        for w in range(W):
                            st[g, w] = ps[w] * inv

                def pv(val, j):
                    anchor(qkv.at[0], HALO + S, val, z)
                    vv = shifted(2 * NCH + j)
                    for g in range(2):
                        a = st[g, 0] * vv[4 - 4 * g]
                        for w in range(1, W):
                            a = a + st[g, w] * vv[w + 4 - 4 * g]
                        osc[slot, j, pl.ds(8 * g, 8), :] = a

                return ([(lambda val, j=j: logits(val, j)) for j in range(NCH)] + [lambda val: None] * AGAP
                        + [(lambda val, j=j: pv(val, j)) for j in range(NCH)])

            def attn_tasks(t0, off, n, z):
                t0 = pl.multiple_of(jnp.minimum(t0 + off // 32 * 32, HS - n - off % 32), 16)
                tasks = []
                for g in range(n // 16):
                    r = off % 32 + g * 16
                    tasks += attn_unit(t0, r, g == 0, 2 * g, z) + attn_unit(t0, HS + r, False, 2 * g + 1, z)

                    def oa(val, kc, g=g, r=r):
                        ops = _ops(_A_TERMS, osc[2 * g, kc], osc[2 * g, KC + kc],
                                   osc[2 * g + 1, kc], osc[2 * g + 1, KC + kc])
                        for i in range(7):
                            OA.at[i][pl.ds(t0 + r, 16), ch(kc)] = ops[i].astype(BF16)
                    tasks += [(lambda val, kc=kc, oa=oa: oa(val, kc)) for kc in range(KC)]
                return tasks

            def ha_task(val, r, i, z, have):
                anchor(HF, S, val, z)
                x = [_combine(_A_TERMS[i], lambda sg, kp: HF[pl.ds((2 * sg + rho) * QS + r, 16), ch(2 * kp + ta)])
                     for rho in range(2) for ta in range(2)]
                for k, op in enumerate(_ops(_A_TERMS, *x)):
                    HA[pl.ds(r, 16), ch(7 * i + k)] = op.astype(BF16)
                have.add((i, r))

            def up2(kp, free, on_half):
                def sub(r0, m):
                    hold, seen = {}, set()

                    def outer_fin(k, K, v):
                        if K in (2, 1):
                            hold[k] = v
                            return
                        sg = K // 2
                        HF[pl.ds((2 * sg + k // 2) * QS + r0, m), ch(2 * kp + k % 2)] = (
                            gelu2(hold[k], v) if K == 3 else gelu2(v, hold[k]))
                        seen.add((sg, k))
                        if all((sg, j) in seen for j in range(4)):
                            on_half(sg, r0, m)
                    folds = [_Fold(lambda K, v, k=k: outer_fin(k, K, v)) for k in range(4)]

                    def lhs(i, k):
                        if k == 2:
                            return XA[i, pl.ds(r0, m), pl.ds(0, KQ)]
                        if k == 3:
                            return XA[i, pl.ds(QS + r0, m), pl.ds(KQ, KQ)]
                        return XB[5 * i + _XB_SLOT[k], pl.ds(r0, m), :]
                    return lambda i: _strassen(lambda k: _dot(lhs(i, k), BG[i, :, ch(k)]),
                                               lambda k, v: folds[k](i, v), R2H if i in (2, 6) else R2L)
                subs = [sub(s * RH2, RH2) for s in range(QS // RH2)]
                for i in _ORDER:
                    for sb in subs:
                        yield from sb(i)
                    free.add(i)

            nsub = QS // RH2
            g_room = (5 * sum(R2L) + 2 * sum(R2H)) * nsub
            d_unit = RD2 * MD * ND / (RH2 * KQ)

            ends = [sum(sum(R2H if i in (2, 6) else R2L) for i in _ORDER[:j + 1]) * nsub for j in range(7)]

            def bg_sides(slot, total, z, free, n):
                return [((ends[j] + 1) / total, (ends[j + 1] if j < 6 else ends[6] + ends[0]) / total - 0.01,
                         prep_g2_tasks(slot, _ORDER[j:j + 1], 0, KQ, z, free)) for j in range(n)]

            def block_b(k):
                when(k < NP - 1, lambda: (cp_gu(0, 0, 0).wait(), cp_gu(0, 0, 1).wait()))

                def prefetch(val):
                    when(k < NP - 1, lambda: (cp_gu(2 * k + 3, 1, 0).start(), cp_gu(2 * k + 3, 1, 1).start(),
                                              cp_d(k + 1).start()))
                z = zero(k)
                free, have, halves = set(), set(), set()

                def on_half(sg, r0, m):
                    if r0 + m == QS:
                        halves.add(sg)

                def ha_tasks(outer, need):
                    def task(val, r, i):
                        assert need <= halves
                        ha_task(val, r, i, z, have)
                    return [(lambda val, r=r, i=i: task(val, r, i)) for i in outer for r in range(0, QS, 16)]

                def main():
                    yield from up2(1, free, on_half)
                    for i in (2, 5, 1, 3, 0, 4, 6):
                        assert all((i, r) in have for r in range(0, QS, 16))
                        for r0 in range(0, QS, MD):
                            for c in range(KQ // ND):
                                def fin(q, v):
                                    P[i, pl.ds((q // 2) * QS + r0, MD), pl.ds((q % 2) * KQ + c * ND, ND)] += v
                                yield from _strassen(
                                    lambda j: _dot(HA[pl.ds(r0, MD), ch(7 * i + j)], BD[7 * i + j, :, ch(c, ND)]),
                                    fin, (d_unit,) * 7)
                total = g_room + 49 * (QS // MD) * (KQ // ND) * d_unit
                gf = g_room / total
                df = (1 - gf) / 7
                _emit(LAG2, main(), total, *bg_sides(0, total, z, free, 7),
                      (0.0, ends[0] / total, prep_g2_tasks(1, _ORDER[6:], 0, KQ, z)),
                      (0.0, HAF * gf, ha_tasks((2, 5), set())),
                      ((ends[4] + 1) / total, gf + HA1 * df, ha_tasks((1, 3, 0), {1})),
                      (gf + HA1 * df, gf + HA2 * df, ha_tasks((4, 6), {0, 1})),
                      (0.0, PDB * gf, prep_d2_tasks(NL - PDN, PDN, z)),
                      (0.0, ATB, attn_tasks(k * (APA + APB), 0, APB, z)),
                      (gf, gf + 0.01, [prefetch]))

            def block_a(k):
                cp_gu(0, 1, 0).wait(); cp_gu(0, 1, 1).wait(); cp_d(0).wait()

                def prefetch(val):
                    when(k < NP - 2, lambda: (cp_gu(2 * k + 4, 0, 0).start(), cp_gu(2 * k + 4, 0, 1).start()))
                z = zero(k)
                free = set()
                _emit(LAGA, up2(0, free, lambda *a: None), g_room, *bg_sides(1, g_room, z, free, 6),
                      (0.0, PDA, prep_d2_tasks(0, NL - PDN, z)),
                      (0.0, ATA, attn_tasks(k * (APA + APB), APB, APA, z)),
                      (0.01, 0.02, [prefetch]))

            def p2_body(k, carry):
                with scope("b"):
                    block_b(k)
                with scope("a"):
                    when(k < NP - 1, lambda: block_a(k))
                return carry
            with scope("p2"):
                lax.fori_loop(0, NP, p2_body, 0)

            def cp_out(t, half, s):
                return pltpu.make_async_copy(obuf.at[t % 2, half, pl.ds(s * M3, M3), :],
                                             out_hbm.at[pl.ds(half * HS + t * T3 + s * M3, M3), :], sem_out.at[t % 2])

            def wait_out(t):
                pltpu.make_async_copy(obuf.at[t % 2], obuf.at[t % 2], sem_out.at[t % 2]).wait()

            def p3_body(t, carry):
                when(t >= 2, lambda: wait_out(t - 2))
                for s in range(T3 // M3):
                    r0 = pl.multiple_of(t * T3 + s * M3, M3)
                    for n in range(KC):
                        def fin(k, sq):
                            (j0, _), *rest = _C_TERMS[k]
                            f = P[j0, pl.ds(r0, M3), ch(n)]
                            for j, sign in rest:
                                f = f + P[j, pl.ds(r0, M3), ch(n)] if sign > 0 else f - P[j, pl.ds(r0, M3), ch(n)]
                            y = f * 0.25
                            half, col = k // 2, (k % 2) * KC + n
                            x = xbuf[pl.ds(half * HS + r0, M3), ch(col)].astype(F32)
                            obuf.at[t % 2, half][pl.ds(s * M3, M3), ch(col)] = (
                                x + sq * (y + y * jnp.tanh(y))).astype(BF16)
                        for step, _ in enumerate(_strassen(
                                lambda i: _dot(OA[i, pl.ds(r0, M3), :], BO[i, :, ch(n)]), fin, (1,) * 7)):
                            if s > 0 and n == 0 and step == OUTK:
                                cp_out(t, 0, s - 1).start(); cp_out(t, 1, s - 1).start()
                cp_out(t, 0, T3 // M3 - 1).start(); cp_out(t, 1, T3 // M3 - 1).start()
                return carry
            with scope("p3"):
                lax.fori_loop(0, NT3, p3_body, 0)
            with scope("end"):
                for t in range(NT3 - 2, NT3):
                    wait_out(t)

        pl.run_scoped(first_half,
                      pltpu.VMEM((7, KH // 2, 2 * NL), U32),
                      pltpu.VMEM((7, KH // 2, 2 * NL), U32))
        pl.run_scoped(second_half,
                      pltpu.VMEM((QS // 2, 49 * NL), U32),
                      pltpu.VMEM((max(APA, APB) // 8, NCH, 16, NL), F32),
                      pltpu.VMEM((2, 2, T3, D), BF16))

    def fn(A_x, A_wqkv, A_wo, B_x, B_w_gate, B_w_up, B_w_down):
        x = A_x.reshape(S, D)
        anyspec = pl.BlockSpec(memory_space=pl.ANY)
        out = pl.pallas_call(
            kernel,
            in_specs=[anyspec] * 6,
            out_specs=anyspec,
            out_shape=jax.ShapeDtypeStruct((S, D), BF16),
            scratch_shapes=[
                pltpu.VMEM((S + SPARE, D), BF16),
                pltpu.VMEM((7, HS // 2, KH), U32),
                pltpu.VMEM((35, QS // 2, KQ), U32),
                pltpu.VMEM((3 * NCH, HALO + S + SPARE, NL), F32),
                pltpu.VMEM((7, HS, KH), F32),
                pltpu.VMEM((S + SPARE, 2 * FC), F32),
                pltpu.VMEM((7, KQ // 2, 7 * NL), U32),
                pltpu.VMEM((49, NL // 2, KQ), U32),
                pltpu.VMEM((7, KH // 2, KH), U32),
                pltpu.VMEM((6, D + 64, FC), BF16),
                pltpu.VMEM((S + SPARE, D), F32),
                pltpu.VMEM((4 * NCH, D // 2 + 64, NL), U32),
                pltpu.VMEM((7, HS // 2, KH), U32),
                pltpu.SemaphoreType.DMA((NT0, 2)),
                pltpu.SemaphoreType.DMA((2, 2)),
                pltpu.SemaphoreType.DMA((1,)),
                pltpu.SemaphoreType.DMA((3,)),
                pltpu.SemaphoreType.DMA((1,)),
                pltpu.SemaphoreType.DMA((2,)),
            ],
            compiler_params=pltpu.CompilerParams(vmem_limit_bytes=124 * 2 ** 20, disable_bounds_checks=True),
        )(x, A_wqkv, A_wo, B_w_gate, B_w_up, B_w_down)
        return out.reshape(1, S, D)
    return jax.jit(fn)


_IMPL = make()


@jax.jit
def pallas_recurrent_scan__sliding_local_dilated__geglu_ffn__prompt_kernel(
    A_x: jax.Array,
    A_wqkv: jax.Array,
    A_wo: jax.Array,
    B_x: jax.Array,
    B_w_gate: jax.Array,
    B_w_up: jax.Array,
    B_w_down: jax.Array,
):
    return _IMPL(A_x, A_wqkv, A_wo, B_x, B_w_gate, B_w_up, B_w_down)
```

```python
import contextlib
import math

import jax
import jax.numpy as jnp
from jax import lax
import jax.experimental.pallas as pl
import jax.experimental.pallas.tpu as pltpu

S, D, F = 2048, 1024, 3584
H, DH, W, DIL = 32, 32, 8, 2
NL = 128
NCH = D // NL
HS = S // 2
KH = D // 2
KC = KH // NL
QS = S // 4
KQ = D // 4
FC = 256
NP = F // (2 * FC)
HALO = 16
SPARE = 48
F32, BF16, U32 = jnp.float32, jnp.bfloat16, jnp.uint32
EPS = 1e-5
GELU_C0 = math.sqrt(2.0 / math.pi)
GELU_C1 = GELU_C0 * 0.044715
EXP2_SCALE = (DH ** -0.5) * math.log2(math.e)
NEG = -1e9 / (DH ** -0.5)

_A_TERMS = (((0, 0, 1), (1, 1, 1)), ((1, 0, 1), (1, 1, 1)), ((0, 0, 1),), ((1, 1, 1),),
            ((0, 0, 1), (0, 1, 1)), ((1, 0, 1), (0, 0, -1)), ((0, 1, 1), (1, 1, -1)))
_B_TERMS = (((0, 0, 1), (1, 1, 1)), ((0, 0, 1),), ((0, 1, 1), (1, 1, -1)), ((1, 0, 1), (0, 0, -1)),
            ((1, 1, 1),), ((0, 0, 1), (0, 1, 1)), ((1, 0, 1), (1, 1, 1)))
_C_TERMS = (((0, 1), (3, 1), (4, -1), (6, 1)), ((2, 1), (4, 1)), ((1, 1), (3, 1)), ((0, 1), (1, -1), (2, 1), (5, 1)))
_ORDER = (1, 3, 0, 5, 2, 4, 6)
_XB_SLOT = {0: 0, 1: 1, 4: 2, 5: 3, 6: 4}


def _combine(terms, get):
    (r, c, _), *rest = terms
    v = get(r, c)
    for r, c, sign in rest:
        v = v + get(r, c) if sign > 0 else v - get(r, c)
    return v


def _ops(terms, q11, q12, q21, q22):
    q = ((q11, q12), (q21, q22))
    return [_combine(t, lambda r, c: q[r][c]) for t in terms]


def _dot(a, b):
    return jnp.dot(a, b, preferred_element_type=F32)


class _Fold:
    def __init__(self, fin, lazy=False):
        self.fin, self.lazy = fin, lazy

    def __call__(self, i, m):
        if self.lazy and i in (0, 5, 4):
            if i == 0:
                self.m0 = m
            elif i == 5:
                self.t22 = (m + self.m0) - self.m1
            else:
                self.fin(1, self.m2 + m)
                self.t11 = (self.m0 - m) + self.t11
        elif i == 1:
            self.m1 = m
        elif i == 3:
            self.fin(2, self.m1 + m)
            self.t11 = m
        elif i == 0:
            self.t11 = self.t11 + m
            self.t22 = m - self.m1
        elif i == 5:
            self.t22 = self.t22 + m
        elif i == 2:
            self.fin(3, self.t22 + m)
            self.m2 = m
        elif i == 4:
            self.fin(1, self.m2 + m)
            self.t11 = self.t11 - m
        else:
            self.fin(0, self.t11 + m)


def _strassen(prod, fin, room, lazy=False):
    fold = _Fold(fin, lazy)
    for step, i in enumerate(_ORDER):
        m = prod(i)
        fold(i, m)
        yield room[step], m


def _emit(lag, main, total, *sides):
    done = [0] * len(sides)
    acc = 0

    def flush(frac, val):
        due = []
        for k, (f0, f1, tasks) in enumerate(sides):
            want = len(tasks) if frac >= f1 else int(max(0.0, (frac - f0) / (f1 - f0)) * len(tasks) + 0.5)
            n = min(want, len(tasks)) - done[k]
            due += [((j + 0.5) / n, k, tasks[done[k] + j]) for j in range(n)]
            done[k] += max(n, 0)
        due.sort(key=lambda e: e[:2])
        for j, (_, _, task) in enumerate(due):
            r = (val.shape[0] // 8) * j // len(due) * 8
            task(val[r:r + 8, 0:NL])

    hist = [(0, None)] * lag
    for item in main:
        hist.append(item)
        room, val = hist.pop(0)
        acc += room
        if room:
            flush(acc / total, val)
    assert abs(acc + sum(h[0] for h in hist) - total) < 1e-6
    flush(2.0, hist[-1][1])


def _skew(items):
    depth = max(len(st) for st in items)
    return [items[t - k][k] for t in range(len(items) + depth - 1) for k in range(depth)
            if 0 <= t - k < len(items) and k < len(items[t - k]) and items[t - k][k] is not None]


def make(AGB=1, GAPB=10, AGA=2, GAPA=5, AJ=1, LAZY='og', ONEPASS=True, T0=128, LN0=64, LNF=0.85, RG=(2,) * 7, RU=(2, 2, 2, 2, 1, 1, 1), LAG0=2,
         RH=256, LAG=1, P1A=0.46, XBF=0.95,
         RH2=64, LAG2=5, LAGA=4, R2L=(2,) * 7, R2H=(2, 0, 2, 2, 0, 0, 0), MD=128, ND=128, RD2=2.5,
         APA=64, APB=96, HAF=0.9, HA1=1.6, HA2=5.5, ATB=0.98, ATA=0.95, PDN=32, PDB=0.9, PDA=0.7,
         M3=64, OUTK=1, scopes=False):
    NT0 = HS // T0
    T3 = 256
    NT3 = HS // T3
    assert NL - PDN <= 96
    assert (NP - 1) * APA + NP * APB >= HS and (APA + APB) % 32 == 0 and APA % 16 == 0 and APB % 16 == 0

    def scope(name):
        return jax.named_scope(name) if scopes else contextlib.nullcontext()

    def kernel(x_hbm, wqkv_hbm, wo_hbm, wg_hbm, wu_hbm, wd_hbm, out_hbm,
               xbuf, XA, XB, qkv, P, HF, BG, BD, BO, rw, Y, rq, OA,
               sem_x, sem_gu, sem_d, sem_q, sem_o, sem_out):

        XA, XB, BG, BD, BO, OA = [r.bitcast(BF16) for r in (XA, XB, BG, BD, BO, OA)]

        def ch(n, w=NL):
            return pl.ds(n * w, w) if isinstance(n, int) else pl.ds(pl.multiple_of(n * w, w), w)

        def zero(i):
            return i % 2 + (i + 1) % 2 - 1

        def when(pred, fn):
            pl.when(pred)(lambda: (fn(), None)[1])

        def cp_x(i, half):
            r = half * HS + i * T0
            return pltpu.make_async_copy(x_hbm.at[pl.ds(r, T0), :], xbuf.at[pl.ds(r, T0), :], sem_x.at[i, half])

        def cp_gu(c, slot, which):
            src = wg_hbm if which == 0 else wu_hbm
            return pltpu.make_async_copy(src.at[:, pl.ds(c * FC, FC)], rw.at[2 * slot + which, pl.ds(0, D), :],
                                         sem_gu.at[slot, which])

        class cp_d:
            def __init__(self, p):
                self.p = p

            def start(self):
                for q in range(4):
                    pltpu.make_async_copy(wd_hbm.at[pl.ds(self.p * 2 * FC, 2 * FC), pl.ds(q * KQ, KQ)],
                                          rw.at[4 + q // 2, pl.ds((q % 2) * 2 * FC, 2 * FC), :], sem_d.at[0]).start()

            def wait(self):
                whole = rw.at[pl.ds(4, 2), pl.ds(0, D), :]
                pltpu.make_async_copy(whole, whole, sem_d.at[0]).wait()

        def anchor(dst, row, val, z):
            if val is not None and z is not None:
                r = pl.multiple_of(row + 16 + z * 16, 8)
                dst[pl.ds(r, 8), pl.ds(0, NL)] = pltpu.bitcast(val, U32) if dst.dtype == U32 else val.astype(dst.dtype)

        def gelu2(g, u):
            t = jnp.tanh(g * (GELU_C0 + GELU_C1 * (g * g)))
            p = g * u
            return p + p * t

        def prep_g2_tasks(slot, outer, r0, n, z, free=None):
            def task(val, r, i):
                assert free is None or i in free
                anchor(rw.at[0], D, val, z)
                y = [_combine(_B_TERMS[i], lambda kp, mu: rw[2 * slot + mu, pl.ds((2 * kp + ta) * KQ + r, 16), :].astype(F32))
                     for ta in range(2)]
                ops = _ops(_B_TERMS, y[0][:, :NL], y[0][:, NL:], y[1][:, :NL], y[1][:, NL:])
                for k in range(7):
                    BG.at[i][pl.ds(r, 16), ch(k)] = ops[k].astype(BF16)
            return [(lambda val, r=r0 + g * 16, i=i: task(val, r, i)) for i in outer for g in range(n // 16)]

        def prep_d2_tasks(r0, n, z):
            def task(val, r, i):
                anchor(rw.at[0], D, val, z)
                y = [_combine(_B_TERMS[i],
                              lambda kp, nu: rw[4 + nu, pl.ds(up * 2 * FC + (2 * kp + ta) * NL + r, 16), :].astype(F32))
                     for ta in range(2) for up in range(2)]
                ops = _ops(_B_TERMS, *y)
                for k in range(7):
                    BD.at[7 * i + k][pl.ds(r, 16), :] = ops[k].astype(BF16)
            return [(lambda val, r=r0 + g * 16, i=i: task(val, r, i)) for g in range(n // 16) for i in range(7)]

        def first_half(B0, BQ):
            B0, BQ = B0.bitcast(BF16), BQ.bitcast(BF16)

            class cp_cols:
                def __init__(self, src, col0, dst, slot0, sem):
                    self.args = src, col0, dst, slot0, sem

                def start(self):
                    src, col0, dst, slot0, sem = self.args
                    for k in range(NCH):
                        pltpu.make_async_copy(src.at[:, pl.ds(col0 + k * NL, NL)],
                                              dst.at[slot0 + k, pl.ds(0, D // 2), :].bitcast(BF16), sem).start()

                def wait(self):
                    _, _, dst, slot0, sem = self.args
                    whole = dst.at[pl.ds(slot0, NCH), pl.ds(0, D // 2), :]
                    pltpu.make_async_copy(whole, whole, sem).wait()

            def cp_q(m):
                return cp_cols(wqkv_hbm, m * D, rq, m * NCH, sem_q.at[m])

            def cp_o():
                return cp_cols(wo_hbm, 0, rq, 3 * NCH, sem_o.at[0])

            def ln_tasks(r0, n, z):
                def xrow(r):
                    return xbuf[pl.ds(r, 16), :].astype(F32)
                items = []
                for g in range(n // 16):
                    st = {}
                    for half in range(2):
                        def s0(val, r=half * HS + r0 + g * 16, st=st, half=half):
                            anchor(xbuf, S, val, z)
                            st["m", half] = jnp.sum(xrow(r), axis=-1, keepdims=True) * (1.0 / D)

                        def s1(val, r=half * HS + r0 + g * 16, st=st, half=half):
                            anchor(xbuf, S, val, z)
                            c = xrow(r) - st["m", half]
                            st["v", half] = lax.rsqrt(jnp.sum(c * c, axis=-1, keepdims=True) * (1.0 / D) + EPS)

                        def s01(val, r=half * HS + r0 + g * 16, st=st, half=half):
                            anchor(xbuf, S, val, z)
                            x = xrow(r)
                            m = jnp.sum(x, axis=-1, keepdims=True) * (1.0 / D)
                            e2 = jnp.sum(x * x, axis=-1, keepdims=True) * (1.0 / D)
                            st["m", half] = m
                            st["v", half] = lax.rsqrt(jnp.maximum(e2 - m * m, 0.0) + EPS)

                        def s2(val, r=r0 + g * 16, st=st, half=half):
                            for kc in (2 * half, 2 * half + 1):
                                anchor(xbuf, S, val, z)
                                pos = [(h, c) for h in range(2) for c in (kc, KC + kc)]
                                q = [(xbuf[pl.ds(h * HS + r, 16), ch(c)].astype(F32) - st["m", h]) * st["v", h]
                                     for h, c in pos]
                                for (h, c), y in zip(pos, q):
                                    Y[pl.ds(h * HS + r, 16), ch(c)] = y
                                for i, op in enumerate(_ops(_A_TERMS, *q)):
                                    XA.at[i][pl.ds(r, 16), ch(kc)] = op.astype(BF16)
                        stats = [s01] if ONEPASS else [s0, None, s1]
                        items.append(stats + [None] * (2 - half) + [s2])
                return _skew(items)

            def prep_g1_tasks(which, r0, n):
                for g in range(n // 16):
                    r = r0 + g * 16
                    top = rw[which, pl.ds(r, 16), :].astype(F32)
                    bot = rw[which, pl.ds(KH + r, 16), :].astype(F32)
                    for i, op in enumerate(_ops(_B_TERMS, top[:, :NL], top[:, NL:], bot[:, :NL], bot[:, NL:])):
                        B0.at[i][pl.ds(r, 16), ch(which)] = op.astype(BF16)

            def xb_tasks(r0, n, z):
                def task(val, r, kc, i):
                    anchor(Y, S, val, z)
                    x = [_combine(_A_TERMS[i],
                                  lambda sg, kp: Y[pl.ds((2 * sg + rho) * QS + r, 16), ch(4 * kp + 2 * ta + kc)])
                         for rho in range(2) for ta in range(2)]
                    ops = _ops(_A_TERMS, *x)
                    for k, slot in _XB_SLOT.items():
                        XB.at[5 * i + slot][pl.ds(r, 16), ch(kc)] = ops[k].astype(BF16)
                return [(lambda val, r=r0 + g * 16, kc=kc, i=i: task(val, r, kc, i))
                        for g in range(n // 16) for kc in range(2) for i in range(7)]

            def wide(w):
                return pltpu.bitcast(w, BF16).astype(F32)

            def prep_q_tasks(m, par, n, z, chain=True):
                def perm_a(r):
                    y = [rq[m * NCH + k, pl.ds(r // 2, 8), :] for k in range(NCH)]
                    return [y[0]] + [pltpu.roll(y[k], 2 * k, 1) for k in range(1, NCH)]

                def perm_b(y):
                    lane = lax.broadcasted_iota(jnp.int32, (8, NL), 1)
                    sh = (((lane & 15) >> 1) - par) & 7
                    u = [y[(-j) % NCH] for j in range(NCH)]
                    b0, b1, b2 = (sh & 1) != 0, (sh & 2) != 0, (sh & 4) != 0
                    out = (2 * n, 2 * n + 4)
                    v = {j: jnp.where(b0, u[(j - 1) % NCH], u[j]) for j in (0, 2, 4, 6)}
                    v = {j: jnp.where(b1, v[(j - 2) % NCH], v[j]) for j in out}
                    v = {j: jnp.where(b2, v[(j - 4) % NCH], v[j]) for j in out}
                    return [pltpu.roll(v[j], (2 * NL - 2 * j - 2 * par) % NL, 1) for j in out]

                items = []
                for g in range(KH // 16):
                    st = {}
                    for half in range(2):
                        def s0(val, r=half * KH + g * 16, st=st, half=half):
                            anchor(rq.at[0], D // 2, val, z)
                            st["a", half] = perm_a(r)

                        def s1(val, st=st, half=half):
                            st["b", half] = perm_b(st["a", half])

                        def s2(val, r=g * 16, st=st):
                            ops = _ops(_B_TERMS, *[wide(w) for w in st["b", 0] + st["b", 1]])
                            for i in range(7):
                                BQ.at[i][pl.ds(r, 16), ch(n)] = ops[i].astype(BF16)
                            if chain:
                                anchor(rq.at[0], D // 2, (ops[5] + ops[6])[0:8], z)
                        items.append([s0, s1] + ([s2] if half else []))
                flat = _skew(items)
                firsts = [j for j, t in enumerate(flat) if t.__name__ == "s0"] + [len(flat)]
                return [(lambda val, grp=flat[a:b]: [t(val) for t in grp]) for a, b in zip(firsts, firsts[1:])]

            def prep_o_tasks(src, n, z):
                def transpose(c, a):
                    sub = lax.broadcasted_iota(jnp.int32, (8, NL), 0)
                    y = [rq[src + c, pl.ds(64 * g + 8 * a, 8), :] for g in range(8)]
                    y = [y[0]] + [pltpu.roll(y[g], g, 0) for g in range(1, 8)]
                    v = [y[(-j) % 8] for j in range(8)]
                    for bit in (1, 2, 4):
                        v = [jnp.where((sub & bit) != 0, v[(j - bit) % 8], v[j]) for j in range(8)]
                    return [v[0]] + [pltpu.roll(v[j], 8 - j, 0) for j in range(1, 8)]

                tasks = []
                for a in range(8):
                    st = {}

                    def load(val, h, a=a, st=st):
                        anchor(rq.at[0], D // 2, val, z)
                        st[h] = transpose(h * KC + n, a)

                    def quad(val, jj, a=a, st=st):
                        q = [wide(st[h][kh * KC + jj]) for kh in range(2) for h in range(2)]
                        for i, op in enumerate(_ops(_B_TERMS, *q)):
                            BO.at[i][pl.ds(jj * NL + 16 * a, 16), ch(n)] = op.astype(BF16)
                    tasks += [lambda val, f=load: f(val, 0),
                              lambda val, f=load, g=quad: (f(val, 1), [g(val, jj) for jj in range(KC)])]
                return tasks

            def zero_p_tasks(u0, n, z):
                def task(val, u):
                    v = jnp.zeros((8, NL), F32) if val is None else jnp.where(z != 0, val, 0.0)
                    P[u // 32, pl.ds(pl.multiple_of((u % 32) * 32, 32), 32), :] = jnp.tile(v, (4, KC))
                return [(lambda val, u=u0 + j: task(val, u)) for j in range(n)]

            def up1(r0, m):
                g = {}

                def fin_u(k, u):
                    HF[pl.ds((k // 2) * HS + r0, m), ch(k % 2)] = gelu2(g[k], u)
                yield from _strassen(lambda i: _dot(XA[i, pl.ds(r0, m), :], B0[i, :, ch(0)]), g.__setitem__, RG, 'g' in LAZY)
                yield from _strassen(lambda i: _dot(XA[i, pl.ds(r0, m), :], B0[i, :, ch(1)]), fin_u, RU, 'g' in LAZY)

            with scope("start"):
                groups = [lambda: [cp_x(0, 0), cp_x(0, 1)], lambda: [cp_gu(0, 0, 0)], lambda: [cp_gu(0, 0, 1)]]
                groups += [(lambda i=i: [cp_x(i, 0), cp_x(i, 1)]) for i in range(1, NT0)]
                groups += [lambda: [cp_q(0)], lambda: [cp_gu(1, 1, 0), cp_gu(1, 1, 1), cp_d(0)],
                           lambda: [cp_q(1)], lambda: [cp_o()], lambda: [cp_q(2)]]

                def issue(k, c):
                    for g, cps in enumerate(groups):
                        when(k == g, lambda: [cp.start() for cp in cps()])
                    return c
                lax.fori_loop(0, len(groups), issue, 0)
                cp_x(0, 0).wait(); cp_x(0, 1).wait()

                def ln0(g, c):
                    for t in ln_tasks(pl.multiple_of(g * LN0, LN0), LN0, None):
                        t(None)
                    return c
                lax.fori_loop(0, T0 // LN0, ln0, 0)
                for which in range(2):
                    cp_gu(0, 0, which).wait()

                    def pg0(g, c):
                        prep_g1_tasks(which, pl.multiple_of(g * 64, 64), 64)
                        return c
                    lax.fori_loop(0, KH // 64, pg0, 0)

            def p0_body(i, c):
                cp_x(i + 1, 0).wait(); cp_x(i + 1, 1).wait()
                r0 = pl.multiple_of(i * T0, T0)
                _emit(LAG0, up1(r0, T0), sum(RG) + sum(RU), (0.0, LNF, ln_tasks(r0 + T0, T0, zero(i))))
                return zero(i)
            with scope("p0"):
                z0 = lax.fori_loop(0, NT0 - 1, p0_body, 0)
            with scope("p0_last"):
                cp_q(0).wait()
                cp_gu(2, 0, 0).start(); cp_gu(2, 0, 1).start()
                _emit(LAG, up1(HS - T0, T0), sum(RG) + sum(RU), (0.0, 0.85, prep_q_tasks(0, 0, 0, z0, chain=False)))

            def p1_body(b, c):
                when(b == 0, lambda: (cp_gu(1, 1, 0).wait(), cp_gu(1, 1, 1).wait(), cp_d(0).wait()))
                when(b == 1, lambda: cp_q(1).wait())
                when(b == 2, lambda: cp_o().wait())
                when(b == 3, lambda: cp_q(2).wait())
                m = b // 2
                par = b % 2

                def main():
                    for n in range(2):
                        for s in range(HS // RH):
                            r0 = s * RH

                            def fin(k, v):
                                j = m * NCH + par + 2 * n + 4 * (k % 2)
                                qkv[j, pl.ds(HALO + (k // 2) * HS + r0, RH), :] = v
                            yield from _strassen(lambda i: _dot(XA[i, pl.ds(r0, RH), :], BQ[i, :, ch(n)]), fin, (1,) * 7, 'q' in LAZY)
                piece = jnp.clip(b - 2, 0, 3)
                z = zero(b)
                _emit(LAG, main(), 14 * (HS // RH),
                      (0.0, P1A, prep_q_tasks(m, par, 1, z)),
                      (0.5, 0.5 + P1A, prep_q_tasks(jnp.minimum((b + 1) // 2, 2), (b + 1) % 2, 0, z)),
                      (0.0, 0.95, prep_g2_tasks(1, range(7), pl.multiple_of(jnp.minimum(b * 48, KQ - 48), 16), 48, z)),
                      (0.0, XBF, xb_tasks(pl.multiple_of(jnp.minimum(b * 96, QS - 96), 32), 96, z)),
                      (0.0, 0.95, prep_d2_tasks(pl.multiple_of(jnp.clip(b * 16, 0, max(NL - PDN - 16, 0)), 16), min(16, NL - PDN), z)),
                      (0.0, 0.95, zero_p_tasks(jnp.minimum(b * 38, 224 - 38), 38, z)),
                      (0.0, 0.95, prep_o_tasks(jnp.where(b < 2, 0, 3 * NCH), piece, z)))
                return c
            with scope("p1"):
                lax.fori_loop(0, 6, p1_body, 0)
                for j in range(NCH, 3 * NCH):
                    qkv[j, 0:HALO, :] = jnp.broadcast_to(qkv[j, HALO:HALO + 1, :], (HALO, NL))

        def second_half(HA, osc, obuf):
            HA = HA.bitcast(BF16)

            def attn_unit(t0, r0, masked, slot, z, G, g0, gap):
                st = {}
                sh = 4 * (G - 1)

                def shifted(plane):
                    return [qkv[plane, pl.ds(t0 + (r0 + HALO + 2 * sh - DIL * k), 8), :] for k in range(W + sh)]

                def logits(val, js):
                    anchor(qkv.at[0], HALO + S, val, z)
                    for j in js:
                        q = [qkv[j, pl.ds(t0 + (r0 + HALO + 8 * g), 8), :] for g in range(G)]
                        kk = shifted(NCH + j)
                        for g in range(G):
                            for w in range(W):
                                t = q[g] * kk[w + sh - 4 * g]
                                st[g, w] = t if j == 0 else st[g, w] + t
                    if j == NCH - 1:
                        softmax()

                def softmax():
                    lane = lax.broadcasted_iota(jnp.int32, (8, NL), 1)
                    odd = (lane & 1) != 0
                    hi = (lane & 16) != 0
                    keys = [(g, w) for g in range(G) for w in range(W)]
                    for k in keys:
                        a = st[k]
                        st[k] = a + jnp.where(odd, pltpu.roll(a, 1, 1), pltpu.roll(a, NL - 1, 1))
                    for k in keys:
                        a = st[k]
                        st[k] = a + jnp.where(hi, pltpu.roll(a, 16, 1), pltpu.roll(a, NL - 16, 1))
                    for g in range(G):
                        ls = [st[g, w] for w in range(W)]
                        if masked:
                            pos = t0 + (r0 + 8 * g) + lax.broadcasted_iota(jnp.int32, (8, NL), 0)
                            ls = [ls[0]] + [jnp.where(pos >= DIL * w, ls[w], NEG) for w in range(1, W)]
                        m = ls[0]
                        for w in range(1, W):
                            m = jnp.maximum(m, ls[w])
                        ps = [jnp.exp2((l - m) * EXP2_SCALE) for l in ls]
                        den = ps[0]
                        for w in range(1, W):
                            den = den + ps[w]
                        inv = 1.0 / den
                        for w in range(W):
                            st[g, w] = ps[w] * inv

                def pv(val, js):
                    anchor(qkv.at[0], HALO + S, val, z)
                    for j in js:
                        vv = shifted(2 * NCH + j)
                        for g in range(G):
                            a = st[g, 0] * vv[sh - 4 * g]
                            for w in range(1, W):
                                a = a + st[g, w] * vv[w + sh - 4 * g]
                            osc[slot, j, pl.ds(8 * (g0 + g), 8), :] = a

                jss = [range(j, j + AJ) for j in range(0, NCH, AJ)]
                return ([(lambda val, js=js: logits(val, js)) for js in jss] + [lambda val: None] * gap
                        + [(lambda val, js=js: pv(val, js)) for js in jss])

            def attn_tasks(t0, off, n, z, G, gap):
                t0 = pl.multiple_of(jnp.minimum(t0 + off // 32 * 32, HS - n - off % 32), 16)
                tasks = []
                for g in range(n // 16):
                    r = off % 32 + g * 16
                    for half in range(2):
                        for g0 in range(0, 2, G):
                            tasks += attn_unit(t0, half * HS + r + 8 * g0, g == 0 and half == 0, 2 * g + half, z, G, g0, gap)

                    def oa(val, kc, g=g, r=r):
                        ops = _ops(_A_TERMS, osc[2 * g, kc], osc[2 * g, KC + kc],
                                   osc[2 * g + 1, kc], osc[2 * g + 1, KC + kc])
                        for i in range(7):
                            OA.at[i][pl.ds(t0 + r, 16), ch(kc)] = ops[i].astype(BF16)
                    tasks += [(lambda val, kc=kc, oa=oa: oa(val, kc)) for kc in range(KC)]
                return tasks

            def ha_task(val, r, i, z, have):
                anchor(HF, S, val, z)
                x = [_combine(_A_TERMS[i], lambda sg, kp: HF[pl.ds((2 * sg + rho) * QS + r, 16), ch(2 * kp + ta)])
                     for rho in range(2) for ta in range(2)]
                for k, op in enumerate(_ops(_A_TERMS, *x)):
                    HA[pl.ds(r, 16), ch(7 * i + k)] = op.astype(BF16)
                have.add((i, r))

            def up2(kp, free, on_half):
                def sub(r0, m):
                    hold, seen = {}, set()

                    def outer_fin(k, K, v):
                        if K in (2, 1):
                            hold[k] = v
                            return
                        sg = K // 2
                        HF[pl.ds((2 * sg + k // 2) * QS + r0, m), ch(2 * kp + k % 2)] = (
                            gelu2(hold[k], v) if K == 3 else gelu2(v, hold[k]))
                        seen.add((sg, k))
                        if all((sg, j) in seen for j in range(4)):
                            on_half(sg, r0, m)
                    folds = [_Fold(lambda K, v, k=k: outer_fin(k, K, v), 'o' in LAZY) for k in range(4)]

                    def lhs(i, k):
                        if k == 2:
                            return XA[i, pl.ds(r0, m), pl.ds(0, KQ)]
                        if k == 3:
                            return XA[i, pl.ds(QS + r0, m), pl.ds(KQ, KQ)]
                        return XB[5 * i + _XB_SLOT[k], pl.ds(r0, m), :]
                    return lambda i: _strassen(lambda k: _dot(lhs(i, k), BG[i, :, ch(k)]),
                                               lambda k, v: folds[k](i, v), R2H if i in (2, 6) else R2L, 'i' in LAZY)
                subs = [sub(s * RH2, RH2) for s in range(QS // RH2)]
                for i in _ORDER:
                    for sb in subs:
                        yield from sb(i)
                    free.add(i)

            nsub = QS // RH2
            g_room = (5 * sum(R2L) + 2 * sum(R2H)) * nsub
            d_unit = RD2 * MD * ND / (RH2 * KQ)

            ends = [sum(sum(R2H if i in (2, 6) else R2L) for i in _ORDER[:j + 1]) * nsub for j in range(7)]

            def bg_sides(slot, total, z, free, n):
                return [((ends[j] + 1) / total, (ends[j + 1] if j < 6 else ends[6] + ends[0]) / total - 0.01,
                         prep_g2_tasks(slot, _ORDER[j:j + 1], 0, KQ, z, free)) for j in range(n)]

            def block_b(k):
                when(k < NP - 1, lambda: (cp_gu(0, 0, 0).wait(), cp_gu(0, 0, 1).wait()))

                def prefetch(val):
                    when(k < NP - 1, lambda: (cp_gu(2 * k + 3, 1, 0).start(), cp_gu(2 * k + 3, 1, 1).start(),
                                              cp_d(k + 1).start()))
                z = zero(k)
                free, have, halves = set(), set(), set()

                def on_half(sg, r0, m):
                    if r0 + m == QS:
                        halves.add(sg)

                def ha_tasks(outer, need):
                    def task(val, r, i):
                        assert need <= halves
                        ha_task(val, r, i, z, have)
                    return [(lambda val, r=r, i=i: task(val, r, i)) for i in outer for r in range(0, QS, 16)]

                def main():
                    yield from up2(1, free, on_half)
                    for i in (2, 5, 1, 3, 0, 4, 6):
                        assert all((i, r) in have for r in range(0, QS, 16))
                        for r0 in range(0, QS, MD):
                            for c in range(KQ // ND):
                                def fin(q, v):
                                    P[i, pl.ds((q // 2) * QS + r0, MD), pl.ds((q % 2) * KQ + c * ND, ND)] += v
                                yield from _strassen(
                                    lambda j: _dot(HA[pl.ds(r0, MD), ch(7 * i + j)], BD[7 * i + j, :, ch(c, ND)]),
                                    fin, (d_unit,) * 7, 'd' in LAZY)
                total = g_room + 49 * (QS // MD) * (KQ // ND) * d_unit
                gf = g_room / total
                df = (1 - gf) / 7
                _emit(LAG2, main(), total, *bg_sides(0, total, z, free, 7),
                      (0.0, ends[0] / total, prep_g2_tasks(1, _ORDER[6:], 0, KQ, z)),
                      (0.0, HAF * gf, ha_tasks((2, 5), set())),
                      ((ends[4] + 1) / total, gf + HA1 * df, ha_tasks((1, 3, 0), {1})),
                      (gf + HA1 * df, gf + HA2 * df, ha_tasks((4, 6), {0, 1})),
                      (0.0, PDB * gf, prep_d2_tasks(NL - PDN, PDN, z)),
                      (0.0, ATB, attn_tasks(k * (APA + APB), 0, APB, z, AGB, GAPB)),
                      (gf, gf + 0.01, [prefetch]))

            def block_a(k):
                cp_gu(0, 1, 0).wait(); cp_gu(0, 1, 1).wait(); cp_d(0).wait()

                def prefetch(val):
                    when(k < NP - 2, lambda: (cp_gu(2 * k + 4, 0, 0).start(), cp_gu(2 * k + 4, 0, 1).start()))
                z = zero(k)
                free = set()
                _emit(LAGA, up2(0, free, lambda *a: None), g_room, *bg_sides(1, g_room, z, free, 6),
                      (0.0, PDA, prep_d2_tasks(0, NL - PDN, z)),
                      (0.0, ATA, attn_tasks(k * (APA + APB), APB, APA, z, AGA, GAPA)),
                      (0.01, 0.02, [prefetch]))

            def p2_body(k, carry):
                with scope("b"):
                    block_b(k)
                with scope("a"):
                    when(k < NP - 1, lambda: block_a(k))
                return carry
            with scope("p2"):
                lax.fori_loop(0, NP, p2_body, 0)

            def cp_out(t, half, s):
                return pltpu.make_async_copy(obuf.at[t % 2, half, pl.ds(s * M3, M3), :],
                                             out_hbm.at[pl.ds(half * HS + t * T3 + s * M3, M3), :], sem_out.at[t % 2])

            def wait_out(t):
                pltpu.make_async_copy(obuf.at[t % 2], obuf.at[t % 2], sem_out.at[t % 2]).wait()

            def p3_body(t, carry):
                when(t >= 2, lambda: wait_out(t - 2))
                for s in range(T3 // M3):
                    r0 = pl.multiple_of(t * T3 + s * M3, M3)
                    for n in range(KC):
                        def fin(k, sq):
                            (j0, _), *rest = _C_TERMS[k]
                            f = P[j0, pl.ds(r0, M3), ch(n)]
                            for j, sign in rest:
                                f = f + P[j, pl.ds(r0, M3), ch(n)] if sign > 0 else f - P[j, pl.ds(r0, M3), ch(n)]
                            y = f * 0.25
                            half, col = k // 2, (k % 2) * KC + n
                            x = xbuf[pl.ds(half * HS + r0, M3), ch(col)].astype(F32)
                            obuf.at[t % 2, half][pl.ds(s * M3, M3), ch(col)] = (
                                x + sq * (y + y * jnp.tanh(y))).astype(BF16)
                        for step, _ in enumerate(_strassen(
                                lambda i: _dot(OA[i, pl.ds(r0, M3), :], BO[i, :, ch(n)]), fin, (1,) * 7)):
                            if s > 0 and n == 0 and step == OUTK:
                                cp_out(t, 0, s - 1).start(); cp_out(t, 1, s - 1).start()
                cp_out(t, 0, T3 // M3 - 1).start(); cp_out(t, 1, T3 // M3 - 1).start()
                return carry
            with scope("p3"):
                lax.fori_loop(0, NT3, p3_body, 0)
            with scope("end"):
                for t in range(NT3 - 2, NT3):
                    wait_out(t)

        pl.run_scoped(first_half,
                      pltpu.VMEM((7, KH // 2, 2 * NL), U32),
                      pltpu.VMEM((7, KH // 2, 2 * NL), U32))
        pl.run_scoped(second_half,
                      pltpu.VMEM((QS // 2, 49 * NL), U32),
                      pltpu.VMEM((max(APA, APB) // 8, NCH, 16, NL), F32),
                      pltpu.VMEM((2, 2, T3, D), BF16))

    def fn(A_x, A_wqkv, A_wo, B_x, B_w_gate, B_w_up, B_w_down):
        x = A_x.reshape(S, D)
        anyspec = pl.BlockSpec(memory_space=pl.ANY)
        out = pl.pallas_call(
            kernel,
            in_specs=[anyspec] * 6,
            out_specs=anyspec,
            out_shape=jax.ShapeDtypeStruct((S, D), BF16),
            scratch_shapes=[
                pltpu.VMEM((S + SPARE, D), BF16),
                pltpu.VMEM((7, HS // 2, KH), U32),
                pltpu.VMEM((35, QS // 2, KQ), U32),
                pltpu.VMEM((3 * NCH, HALO + S + SPARE, NL), F32),
                pltpu.VMEM((7, HS, KH), F32),
                pltpu.VMEM((S + SPARE, 2 * FC), F32),
                pltpu.VMEM((7, KQ // 2, 7 * NL), U32),
                pltpu.VMEM((49, NL // 2, KQ), U32),
                pltpu.VMEM((7, KH // 2, KH), U32),
                pltpu.VMEM((6, D + 64, FC), BF16),
                pltpu.VMEM((S + SPARE, D), F32),
                pltpu.VMEM((4 * NCH, D // 2 + 64, NL), U32),
                pltpu.VMEM((7, HS // 2, KH), U32),
                pltpu.SemaphoreType.DMA((NT0, 2)),
                pltpu.SemaphoreType.DMA((2, 2)),
                pltpu.SemaphoreType.DMA((1,)),
                pltpu.SemaphoreType.DMA((3,)),
                pltpu.SemaphoreType.DMA((1,)),
                pltpu.SemaphoreType.DMA((2,)),
            ],
            compiler_params=pltpu.CompilerParams(vmem_limit_bytes=124 * 2 ** 20, disable_bounds_checks=True),
        )(x, A_wqkv, A_wo, B_w_gate, B_w_up, B_w_down)
        return out.reshape(1, S, D)
    return jax.jit(fn)


_IMPL = make()


@jax.jit
def pallas_recurrent_scan__sliding_local_dilated__geglu_ffn__prompt_kernel(
    A_x: jax.Array,
    A_wqkv: jax.Array,
    A_wo: jax.Array,
    B_x: jax.Array,
    B_w_gate: jax.Array,
    B_w_up: jax.Array,
    B_w_down: jax.Array,
):
    return _IMPL(A_x, A_wqkv, A_wo, B_x, B_w_gate, B_w_up, B_w_down)
```

```python
import math

import jax
import jax.numpy as jnp
from jax import lax
import jax.experimental.pallas as pl
import jax.experimental.pallas.tpu as pltpu

S, D, F = 2048, 1024, 3584
H, DH, W, DIL = 32, 32, 8, 2
NL = 128
NCH = D // NL
HS = S // 2
KH = D // 2
KC = KH // NL
QS = S // 4
KQ = D // 4
FC = 256
NP = F // (2 * FC)
HALO = 16
SPARE = 48
F32, BF16, U32 = jnp.float32, jnp.bfloat16, jnp.uint32
EPS = 1e-5
GELU_C0 = math.sqrt(2.0 / math.pi)
GELU_C1 = GELU_C0 * 0.044715
EXP2_SCALE = (DH ** -0.5) * math.log2(math.e)
NEG = -1e9 / (DH ** -0.5)

_A_TERMS = (((0, 0, 1), (1, 1, 1)), ((1, 0, 1), (1, 1, 1)), ((0, 0, 1),), ((1, 1, 1),),
            ((0, 0, 1), (0, 1, 1)), ((1, 0, 1), (0, 0, -1)), ((0, 1, 1), (1, 1, -1)))
_B_TERMS = (((0, 0, 1), (1, 1, 1)), ((0, 0, 1),), ((0, 1, 1), (1, 1, -1)), ((1, 0, 1), (0, 0, -1)),
            ((1, 1, 1),), ((0, 0, 1), (0, 1, 1)), ((1, 0, 1), (1, 1, 1)))
_C_TERMS = (((0, 1), (3, 1), (4, -1), (6, 1)), ((2, 1), (4, 1)), ((1, 1), (3, 1)), ((0, 1), (1, -1), (2, 1), (5, 1)))
_ORDER = (1, 3, 0, 5, 2, 4, 6)
_XB_SLOT = {0: 0, 1: 1, 4: 2, 5: 3, 6: 4}


def _combine(terms, get):
    (r, c, _), *rest = terms
    v = get(r, c)
    for r, c, sign in rest:
        v = v + get(r, c) if sign > 0 else v - get(r, c)
    return v


def _ops(terms, q11, q12, q21, q22):
    q = ((q11, q12), (q21, q22))
    return [_combine(t, lambda r, c: q[r][c]) for t in terms]


def _dot(a, b):
    return jnp.dot(a, b, preferred_element_type=F32)


class _Fold:
    def __init__(self, fin, lazy=False):
        self.fin, self.lazy = fin, lazy

    def __call__(self, i, m):
        if self.lazy and i in (0, 5, 4):
            if i == 0:
                self.m0 = m
            elif i == 5:
                self.t22 = (m + self.m0) - self.m1
            else:
                self.fin(1, self.m2 + m)
                self.t11 = (self.m0 - m) + self.t11
        elif i == 1:
            self.m1 = m
        elif i == 3:
            self.fin(2, self.m1 + m)
            self.t11 = m
        elif i == 0:
            self.t11 = self.t11 + m
            self.t22 = m - self.m1
        elif i == 5:
            self.t22 = self.t22 + m
        elif i == 2:
            self.fin(3, self.t22 + m)
            self.m2 = m
        elif i == 4:
            self.fin(1, self.m2 + m)
            self.t11 = self.t11 - m
        else:
            self.fin(0, self.t11 + m)


def _strassen(prod, fin, room, lazy=False):
    fold = _Fold(fin, lazy)
    for step, i in enumerate(_ORDER):
        m = prod(i)
        fold(i, m)
        yield room[step], m


def _emit(lag, main, total, *sides):
    done = [0] * len(sides)
    acc = 0

    def flush(frac, val):
        due = []
        for k, (f0, f1, tasks) in enumerate(sides):
            want = len(tasks) if frac >= f1 else int(max(0.0, (frac - f0) / (f1 - f0)) * len(tasks) + 0.5)
            n = min(want, len(tasks)) - done[k]
            due += [((j + 0.5) / n, k, tasks[done[k] + j]) for j in range(n)]
            done[k] += max(n, 0)
        due.sort(key=lambda e: e[:2])
        for j, (_, _, task) in enumerate(due):
            r = (val.shape[0] // 8) * j // len(due) * 8
            task(val[r:r + 8, 0:NL])

    hist = [(0, None)] * lag
    for item in main:
        hist.append(item)
        room, val = hist.pop(0)
        acc += room
        if room:
            flush(acc / total, val)
    assert abs(acc + sum(h[0] for h in hist) - total) < 1e-6
    flush(2.0, hist[-1][1])


def _skew(items):
    depth = max(len(st) for st in items)
    return [items[t - k][k] for t in range(len(items) + depth - 1) for k in range(depth)
            if 0 <= t - k < len(items) and k < len(items[t - k]) and items[t - k][k] is not None]


T0, NT0 = 128, 8
RH = 256
RH2 = 64
MD, ND = 128, 128
T3, NT3, M3 = 256, 4, 64
APB, APA = 96, 64
PDN = 32
ROOM_G, ROOM_U = (2,) * 7, (2, 2, 2, 2, 1, 1, 1)
ROOM_L, ROOM_H = (2,) * 7, (2, 0, 2, 2, 0, 0, 0)
assert (NP - 1) * APA + NP * APB >= HS and APA % 32 == 0 and APB % 32 == 0


def _kernel(x_hbm, wqkv_hbm, wo_hbm, wg_hbm, wu_hbm, wd_hbm, out_hbm,
            xbuf, XA, XB, qkv, P, HF, BG, BD, BO, rw, Y, rq, OA,
            sem_x, sem_gu, sem_d, sem_q, sem_o, sem_out):

    XA, XB, BG, BD, BO, OA = [r.bitcast(BF16) for r in (XA, XB, BG, BD, BO, OA)]

    def ch(n, w=NL):
        return pl.ds(n * w, w) if isinstance(n, int) else pl.ds(pl.multiple_of(n * w, w), w)

    def zero(i):
        return i % 2 + (i + 1) % 2 - 1

    def when(pred, fn):
        pl.when(pred)(lambda: (fn(), None)[1])

    def cp_x(i, half):
        r = half * HS + i * T0
        return pltpu.make_async_copy(x_hbm.at[pl.ds(r, T0), :], xbuf.at[pl.ds(r, T0), :], sem_x.at[i, half])

    def cp_gu(c, slot, which):
        src = wg_hbm if which == 0 else wu_hbm
        return pltpu.make_async_copy(src.at[:, pl.ds(c * FC, FC)], rw.at[2 * slot + which, pl.ds(0, D), :],
                                     sem_gu.at[slot, which])

    class cp_d:
        def __init__(self, p):
            self.p = p

        def start(self):
            for q in range(4):
                pltpu.make_async_copy(wd_hbm.at[pl.ds(self.p * 2 * FC, 2 * FC), pl.ds(q * KQ, KQ)],
                                      rw.at[4 + q // 2, pl.ds((q % 2) * 2 * FC, 2 * FC), :], sem_d.at[0]).start()

        def wait(self):
            whole = rw.at[pl.ds(4, 2), pl.ds(0, D), :]
            pltpu.make_async_copy(whole, whole, sem_d.at[0]).wait()

    def anchor(dst, row, val, z):
        if val is not None and z is not None:
            r = pl.multiple_of(row + 16 + z * 16, 8)
            dst[pl.ds(r, 8), pl.ds(0, NL)] = pltpu.bitcast(val, U32) if dst.dtype == U32 else val.astype(dst.dtype)

    def gelu2(g, u):
        t = jnp.tanh(g * (GELU_C0 + GELU_C1 * (g * g)))
        p = g * u
        return p + p * t

    def prep_g2_tasks(slot, outer, r0, n, z, free=None):
        def task(val, r, i):
            assert free is None or i in free
            anchor(rw.at[0], D, val, z)
            y = [_combine(_B_TERMS[i], lambda kp, mu: rw[2 * slot + mu, pl.ds((2 * kp + ta) * KQ + r, 16), :].astype(F32))
                 for ta in range(2)]
            ops = _ops(_B_TERMS, y[0][:, :NL], y[0][:, NL:], y[1][:, :NL], y[1][:, NL:])
            for k in range(7):
                BG.at[i][pl.ds(r, 16), ch(k)] = ops[k].astype(BF16)
        return [(lambda val, r=r0 + g * 16, i=i: task(val, r, i)) for i in outer for g in range(n // 16)]

    def prep_d2_tasks(r0, n, z):
        def task(val, r, i):
            anchor(rw.at[0], D, val, z)
            y = [_combine(_B_TERMS[i],
                          lambda kp, nu: rw[4 + nu, pl.ds(up * 2 * FC + (2 * kp + ta) * NL + r, 16), :].astype(F32))
                 for ta in range(2) for up in range(2)]
            ops = _ops(_B_TERMS, *y)
            for k in range(7):
                BD.at[7 * i + k][pl.ds(r, 16), :] = ops[k].astype(BF16)
        return [(lambda val, r=r0 + g * 16, i=i: task(val, r, i)) for g in range(n // 16) for i in range(7)]

    def first_half(B0, BQ):
        B0, BQ = B0.bitcast(BF16), BQ.bitcast(BF16)

        class cp_cols:
            def __init__(self, src, col0, dst, slot0, sem):
                self.args = src, col0, dst, slot0, sem

            def start(self):
                src, col0, dst, slot0, sem = self.args
                for k in range(NCH):
                    pltpu.make_async_copy(src.at[:, pl.ds(col0 + k * NL, NL)],
                                          dst.at[slot0 + k, pl.ds(0, D // 2), :].bitcast(BF16), sem).start()

            def wait(self):
                _, _, dst, slot0, sem = self.args
                whole = dst.at[pl.ds(slot0, NCH), pl.ds(0, D // 2), :]
                pltpu.make_async_copy(whole, whole, sem).wait()

        def cp_q(m):
            return cp_cols(wqkv_hbm, m * D, rq, m * NCH, sem_q.at[m])

        def cp_o():
            return cp_cols(wo_hbm, 0, rq, 3 * NCH, sem_o.at[0])

        def ln_tasks(r0, n, z):
            def xrow(r):
                return xbuf[pl.ds(r, 16), :].astype(F32)
            items = []
            for g in range(n // 16):
                st = {}
                for half in range(2):
                    def stats(val, r=half * HS + r0 + g * 16, st=st, half=half):
                        anchor(xbuf, S, val, z)
                        x = xrow(r)
                        m = jnp.sum(x, axis=-1, keepdims=True) * (1.0 / D)
                        e2 = jnp.sum(x * x, axis=-1, keepdims=True) * (1.0 / D)
                        st["m", half] = m
                        st["v", half] = lax.rsqrt(jnp.maximum(e2 - m * m, 0.0) + EPS)

                    def apply(val, r=r0 + g * 16, st=st, half=half):
                        for kc in (2 * half, 2 * half + 1):
                            anchor(xbuf, S, val, z)
                            pos = [(h, c) for h in range(2) for c in (kc, KC + kc)]
                            q = [(xbuf[pl.ds(h * HS + r, 16), ch(c)].astype(F32) - st["m", h]) * st["v", h]
                                 for h, c in pos]
                            for (h, c), y in zip(pos, q):
                                Y[pl.ds(h * HS + r, 16), ch(c)] = y
                            for i, op in enumerate(_ops(_A_TERMS, *q)):
                                XA.at[i][pl.ds(r, 16), ch(kc)] = op.astype(BF16)
                    items.append([stats] + [None] * (2 - half) + [apply])
            return _skew(items)

        def prep_g1(which, r0, n):
            for g in range(n // 16):
                r = r0 + g * 16
                top = rw[which, pl.ds(r, 16), :].astype(F32)
                bot = rw[which, pl.ds(KH + r, 16), :].astype(F32)
                for i, op in enumerate(_ops(_B_TERMS, top[:, :NL], top[:, NL:], bot[:, :NL], bot[:, NL:])):
                    B0.at[i][pl.ds(r, 16), ch(which)] = op.astype(BF16)

        def xb_tasks(r0, n, z):
            def task(val, r, kc, i):
                anchor(Y, S, val, z)
                x = [_combine(_A_TERMS[i],
                              lambda sg, kp: Y[pl.ds((2 * sg + rho) * QS + r, 16), ch(4 * kp + 2 * ta + kc)])
                     for rho in range(2) for ta in range(2)]
                ops = _ops(_A_TERMS, *x)
                for k, slot in _XB_SLOT.items():
                    XB.at[5 * i + slot][pl.ds(r, 16), ch(kc)] = ops[k].astype(BF16)
            return [(lambda val, r=r0 + g * 16, kc=kc, i=i: task(val, r, kc, i))
                    for g in range(n // 16) for kc in range(2) for i in range(7)]

        def wide(w):
            return pltpu.bitcast(w, BF16).astype(F32)

        def prep_q_tasks(m, par, n, z, chain=True):
            def perm_a(r):
                y = [rq[m * NCH + k, pl.ds(r // 2, 8), :] for k in range(NCH)]
                return [y[0]] + [pltpu.roll(y[k], 2 * k, 1) for k in range(1, NCH)]

            def perm_b(y):
                lane = lax.broadcasted_iota(jnp.int32, (8, NL), 1)
                sh = (((lane & 15) >> 1) - par) & 7
                u = [y[(-j) % NCH] for j in range(NCH)]
                b0, b1, b2 = (sh & 1) != 0, (sh & 2) != 0, (sh & 4) != 0
                out = (2 * n, 2 * n + 4)
                v = {j: jnp.where(b0, u[(j - 1) % NCH], u[j]) for j in (0, 2, 4, 6)}
                v = {j: jnp.where(b1, v[(j - 2) % NCH], v[j]) for j in out}
                v = {j: jnp.where(b2, v[(j - 4) % NCH], v[j]) for j in out}
                return [pltpu.roll(v[j], (2 * NL - 2 * j - 2 * par) % NL, 1) for j in out]

            items = []
            for g in range(KH // 16):
                st = {}
                for half in range(2):
                    def s0(val, r=half * KH + g * 16, st=st, half=half):
                        anchor(rq.at[0], D // 2, val, z)
                        st["a", half] = perm_a(r)

                    def s1(val, st=st, half=half):
                        st["b", half] = perm_b(st["a", half])

                    def s2(val, r=g * 16, st=st):
                        ops = _ops(_B_TERMS, *[wide(w) for w in st["b", 0] + st["b", 1]])
                        for i in range(7):
                            BQ.at[i][pl.ds(r, 16), ch(n)] = ops[i].astype(BF16)
                        if chain:
                            anchor(rq.at[0], D // 2, (ops[5] + ops[6])[0:8], z)
                    items.append([s0, s1] + ([s2] if half else []))
            flat = _skew(items)
            firsts = [j for j, t in enumerate(flat) if t.__name__ == "s0"] + [len(flat)]
            return [(lambda val, grp=flat[a:b]: [t(val) for t in grp]) for a, b in zip(firsts, firsts[1:])]

        def prep_o_tasks(src, n, z):
            def transpose(c, a):
                sub = lax.broadcasted_iota(jnp.int32, (8, NL), 0)
                y = [rq[src + c, pl.ds(64 * g + 8 * a, 8), :] for g in range(8)]
                y = [y[0]] + [pltpu.roll(y[g], g, 0) for g in range(1, 8)]
                v = [y[(-j) % 8] for j in range(8)]
                for bit in (1, 2, 4):
                    v = [jnp.where((sub & bit) != 0, v[(j - bit) % 8], v[j]) for j in range(8)]
                return [v[0]] + [pltpu.roll(v[j], 8 - j, 0) for j in range(1, 8)]

            tasks = []
            for a in range(8):
                st = {}

                def load(val, h, a=a, st=st):
                    anchor(rq.at[0], D // 2, val, z)
                    st[h] = transpose(h * KC + n, a)

                def quad(val, jj, a=a, st=st):
                    q = [wide(st[h][kh * KC + jj]) for kh in range(2) for h in range(2)]
                    for i, op in enumerate(_ops(_B_TERMS, *q)):
                        BO.at[i][pl.ds(jj * NL + 16 * a, 16), ch(n)] = op.astype(BF16)
                tasks += [lambda val, f=load: f(val, 0),
                          lambda val, f=load, g=quad: (f(val, 1), [g(val, jj) for jj in range(KC)])]
            return tasks

        def zero_p_tasks(u0, n, z):
            def task(val, u):
                v = jnp.where(z != 0, val, 0.0)
                P[u // 32, pl.ds(pl.multiple_of((u % 32) * 32, 32), 32), :] = jnp.tile(v, (4, KC))
            return [(lambda val, u=u0 + j: task(val, u)) for j in range(n)]

        def up1(r0, m):
            g = {}

            def fin_u(k, u):
                HF[pl.ds((k // 2) * HS + r0, m), ch(k % 2)] = gelu2(g[k], u)
            yield from _strassen(lambda i: _dot(XA[i, pl.ds(r0, m), :], B0[i, :, ch(0)]), g.__setitem__, ROOM_G, lazy=True)
            yield from _strassen(lambda i: _dot(XA[i, pl.ds(r0, m), :], B0[i, :, ch(1)]), fin_u, ROOM_U, lazy=True)

        groups = [lambda: [cp_x(0, 0), cp_x(0, 1)], lambda: [cp_gu(0, 0, 0)], lambda: [cp_gu(0, 0, 1)]]
        groups += [(lambda i=i: [cp_x(i, 0), cp_x(i, 1)]) for i in range(1, NT0)]
        groups += [lambda: [cp_q(0)], lambda: [cp_gu(1, 1, 0), cp_gu(1, 1, 1), cp_d(0)],
                   lambda: [cp_q(1)], lambda: [cp_o()], lambda: [cp_q(2)]]

        def issue(k, c):
            for g, cps in enumerate(groups):
                when(k == g, lambda: [cp.start() for cp in cps()])
            return c
        lax.fori_loop(0, len(groups), issue, 0)
        cp_x(0, 0).wait(); cp_x(0, 1).wait()

        def ln0(g, c):
            for t in ln_tasks(pl.multiple_of(g * 64, 64), 64, None):
                t(None)
            return c
        lax.fori_loop(0, T0 // 64, ln0, 0)
        for which in range(2):
            cp_gu(0, 0, which).wait()

            def pg0(g, c):
                prep_g1(which, pl.multiple_of(g * 64, 64), 64)
                return c
            lax.fori_loop(0, KH // 64, pg0, 0)

        def p0_body(i, c):
            cp_x(i + 1, 0).wait(); cp_x(i + 1, 1).wait()
            r0 = pl.multiple_of(i * T0, T0)
            _emit(2, up1(r0, T0), sum(ROOM_G) + sum(ROOM_U), (0.0, 0.85, ln_tasks(r0 + T0, T0, zero(i))))
            return zero(i)
        z0 = lax.fori_loop(0, NT0 - 1, p0_body, 0)
        cp_q(0).wait()
        cp_gu(2, 0, 0).start(); cp_gu(2, 0, 1).start()
        _emit(1, up1(HS - T0, T0), sum(ROOM_G) + sum(ROOM_U), (0.0, 0.85, prep_q_tasks(0, 0, 0, z0, chain=False)))

        def p1_body(b, c):
            when(b == 0, lambda: (cp_gu(1, 1, 0).wait(), cp_gu(1, 1, 1).wait(), cp_d(0).wait()))
            when(b == 1, lambda: cp_q(1).wait())
            when(b == 2, lambda: cp_o().wait())
            when(b == 3, lambda: cp_q(2).wait())
            m = b // 2
            par = b % 2

            def main():
                for n in range(2):
                    for s in range(HS // RH):
                        r0 = s * RH

                        def fin(k, v):
                            j = m * NCH + par + 2 * n + 4 * (k % 2)
                            qkv[j, pl.ds(HALO + (k // 2) * HS + r0, RH), :] = v
                        yield from _strassen(lambda i: _dot(XA[i, pl.ds(r0, RH), :], BQ[i, :, ch(n)]), fin, (1,) * 7)
            piece = jnp.clip(b - 2, 0, 3)
            z = zero(b)
            _emit(1, main(), 14 * (HS // RH),
                  (0.0, 0.46, prep_q_tasks(m, par, 1, z)),
                  (0.5, 0.96, prep_q_tasks(jnp.minimum((b + 1) // 2, 2), (b + 1) % 2, 0, z)),
                  (0.0, 0.95, prep_g2_tasks(1, range(7), pl.multiple_of(jnp.minimum(b * 48, KQ - 48), 16), 48, z)),
                  (0.0, 0.95, xb_tasks(pl.multiple_of(jnp.minimum(b * 96, QS - 96), 32), 96, z)),
                  (0.0, 0.95, prep_d2_tasks(pl.multiple_of(jnp.clip(b * 16, 0, NL - PDN - 16), 16), 16, z)),
                  (0.0, 0.95, zero_p_tasks(jnp.minimum(b * 38, 224 - 38), 38, z)),
                  (0.0, 0.95, prep_o_tasks(jnp.where(b < 2, 0, 3 * NCH), piece, z)))
            return c
        lax.fori_loop(0, 6, p1_body, 0)
        for j in range(NCH, 3 * NCH):
            qkv[j, 0:HALO, :] = jnp.broadcast_to(qkv[j, HALO:HALO + 1, :], (HALO, NL))

    def second_half(HA, osc, obuf):
        HA = HA.bitcast(BF16)

        def attn_unit(t0, r0, masked, slot, z, G, g0, gap):
            st = {}
            sh = 4 * (G - 1)

            def shifted(plane):
                return [qkv[plane, pl.ds(t0 + (r0 + HALO + 2 * sh - DIL * k), 8), :] for k in range(W + sh)]

            def logits(val, j):
                anchor(qkv.at[0], HALO + S, val, z)
                q = [qkv[j, pl.ds(t0 + (r0 + HALO + 8 * g), 8), :] for g in range(G)]
                kk = shifted(NCH + j)
                for g in range(G):
                    for w in range(W):
                        t = q[g] * kk[w + sh - 4 * g]
                        st[g, w] = t if j == 0 else st[g, w] + t
                if j == NCH - 1:
                    softmax()

            def softmax():
                lane = lax.broadcasted_iota(jnp.int32, (8, NL), 1)
                odd = (lane & 1) != 0
                hi = (lane & 16) != 0
                keys = [(g, w) for g in range(G) for w in range(W)]
                for k in keys:
                    a = st[k]
                    st[k] = a + jnp.where(odd, pltpu.roll(a, 1, 1), pltpu.roll(a, NL - 1, 1))
                for k in keys:
                    a = st[k]
                    st[k] = a + jnp.where(hi, pltpu.roll(a, 16, 1), pltpu.roll(a, NL - 16, 1))
                for g in range(G):
                    ls = [st[g, w] for w in range(W)]
                    if masked:
                        pos = t0 + (r0 + 8 * g) + lax.broadcasted_iota(jnp.int32, (8, NL), 0)
                        ls = [ls[0]] + [jnp.where(pos >= DIL * w, ls[w], NEG) for w in range(1, W)]
                    m = ls[0]
                    for w in range(1, W):
                        m = jnp.maximum(m, ls[w])
                    ps = [jnp.exp2((l - m) * EXP2_SCALE) for l in ls]
                    den = ps[0]
                    for w in range(1, W):
                        den = den + ps[w]
                    inv = 1.0 / den
                    for w in range(W):
                        st[g, w] = ps[w] * inv

            def pv(val, j):
                anchor(qkv.at[0], HALO + S, val, z)
                vv = shifted(2 * NCH + j)
                for g in range(G):
                    a = st[g, 0] * vv[sh - 4 * g]
                    for w in range(1, W):
                        a = a + st[g, w] * vv[w + sh - 4 * g]
                    osc[slot, j, pl.ds(8 * (g0 + g), 8), :] = a

            return ([(lambda val, j=j: logits(val, j)) for j in range(NCH)] + [lambda val: None] * gap
                    + [(lambda val, j=j: pv(val, j)) for j in range(NCH)])

        def attn_tasks(t0, n, z, G, gap):
            t0 = pl.multiple_of(jnp.minimum(t0, HS - n), 16)
            tasks = []
            for g in range(n // 16):
                r = g * 16
                for half in range(2):
                    for g0 in range(0, 2, G):
                        tasks += attn_unit(t0, half * HS + r + 8 * g0, g == 0 and half == 0, 2 * g + half, z, G, g0, gap)

                def oa(val, kc, g=g, r=r):
                    ops = _ops(_A_TERMS, osc[2 * g, kc], osc[2 * g, KC + kc],
                               osc[2 * g + 1, kc], osc[2 * g + 1, KC + kc])
                    for i in range(7):
                        OA.at[i][pl.ds(t0 + r, 16), ch(kc)] = ops[i].astype(BF16)
                tasks += [(lambda val, kc=kc, oa=oa: oa(val, kc)) for kc in range(KC)]
            return tasks

        def ha_task(val, r, i, z, have):
            anchor(HF, S, val, z)
            x = [_combine(_A_TERMS[i], lambda sg, kp: HF[pl.ds((2 * sg + rho) * QS + r, 16), ch(2 * kp + ta)])
                 for rho in range(2) for ta in range(2)]
            for k, op in enumerate(_ops(_A_TERMS, *x)):
                HA[pl.ds(r, 16), ch(7 * i + k)] = op.astype(BF16)
            have.add((i, r))

        def up2(kp, free, on_half):
            def sub(r0, m):
                hold, seen = {}, set()

                def outer_fin(k, K, v):
                    if K in (2, 1):
                        hold[k] = v
                        return
                    sg = K // 2
                    HF[pl.ds((2 * sg + k // 2) * QS + r0, m), ch(2 * kp + k % 2)] = (
                        gelu2(hold[k], v) if K == 3 else gelu2(v, hold[k]))
                    seen.add((sg, k))
                    if all((sg, j) in seen for j in range(4)):
                        on_half(sg, r0, m)
                folds = [_Fold(lambda K, v, k=k: outer_fin(k, K, v), lazy=True) for k in range(4)]

                def lhs(i, k):
                    if k == 2:
                        return XA[i, pl.ds(r0, m), pl.ds(0, KQ)]
                    if k == 3:
                        return XA[i, pl.ds(QS + r0, m), pl.ds(KQ, KQ)]
                    return XB[5 * i + _XB_SLOT[k], pl.ds(r0, m), :]
                return lambda i: _strassen(lambda k: _dot(lhs(i, k), BG[i, :, ch(k)]),
                                           lambda k, v: folds[k](i, v), ROOM_H if i in (2, 6) else ROOM_L)
            subs = [sub(s * RH2, RH2) for s in range(QS // RH2)]
            for i in _ORDER:
                for sb in subs:
                    yield from sb(i)
                free.add(i)

        nsub = QS // RH2
        g_room = (5 * sum(ROOM_L) + 2 * sum(ROOM_H)) * nsub
        d_unit = 2.5 * MD * ND / (RH2 * KQ)

        ends = [sum(sum(ROOM_H if i in (2, 6) else ROOM_L) for i in _ORDER[:j + 1]) * nsub for j in range(7)]

        def bg_sides(slot, total, z, free, n):
            return [((ends[j] + 1) / total, (ends[j + 1] if j < 6 else ends[6] + ends[0]) / total - 0.01,
                     prep_g2_tasks(slot, _ORDER[j:j + 1], 0, KQ, z, free)) for j in range(n)]

        def block_b(k):
            when(k < NP - 1, lambda: (cp_gu(0, 0, 0).wait(), cp_gu(0, 0, 1).wait()))

            z = zero(k)
            free, have, halves, pending = set(), set(), set(), set()

            def reads_old(tasks):
                pending.update(tasks)
                return [(lambda val, t=t: (t(val), pending.discard(t))) for t in tasks]

            def prefetch(val):
                assert not pending
                when(k < NP - 1, lambda: (cp_gu(2 * k + 3, 1, 0).start(), cp_gu(2 * k + 3, 1, 1).start(),
                                          cp_d(k + 1).start()))

            def on_half(sg, r0, m):
                if r0 + m == QS:
                    halves.add(sg)

            def ha_tasks(outer, need):
                def task(val, r, i):
                    assert need <= halves
                    ha_task(val, r, i, z, have)
                return [(lambda val, r=r, i=i: task(val, r, i)) for i in outer for r in range(0, QS, 16)]

            def main():
                yield from up2(1, free, on_half)
                for i in (2, 5, 1, 3, 0, 4, 6):
                    assert all((i, r) in have for r in range(0, QS, 16))
                    for r0 in range(0, QS, MD):
                        for c in range(KQ // ND):
                            def fin(q, v):
                                P[i, pl.ds((q // 2) * QS + r0, MD), pl.ds((q % 2) * KQ + c * ND, ND)] += v
                            yield from _strassen(
                                lambda j: _dot(HA[pl.ds(r0, MD), ch(7 * i + j)], BD[7 * i + j, :, ch(c, ND)]),
                                fin, (d_unit,) * 7)
            total = g_room + 49 * (QS // MD) * (KQ // ND) * d_unit
            gf = g_room / total
            df = (1 - gf) / 7
            _emit(5, main(), total, *bg_sides(0, total, z, free, 7),
                  (0.0, ends[0] / total, reads_old(prep_g2_tasks(1, _ORDER[6:], 0, KQ, z))),
                  (0.0, 0.9 * gf, ha_tasks((2, 5), set())),
                  ((ends[4] + 1) / total, gf + 1.6 * df, ha_tasks((1, 3, 0), {1})),
                  (gf + 1.6 * df, gf + 5.5 * df, ha_tasks((4, 6), {0, 1})),
                  (0.0, 0.9 * gf, reads_old(prep_d2_tasks(NL - PDN, PDN, z))),
                  (0.0, 0.98, attn_tasks(k * (APA + APB), APB, z, 1, 10)),
                  (gf, gf + 0.01, [prefetch]))

        def block_a(k):
            cp_gu(0, 1, 0).wait(); cp_gu(0, 1, 1).wait(); cp_d(0).wait()

            def prefetch(val):
                when(k < NP - 2, lambda: (cp_gu(2 * k + 4, 0, 0).start(), cp_gu(2 * k + 4, 0, 1).start()))
            z = zero(k)
            free = set()
            _emit(4, up2(0, free, lambda *a: None), g_room, *bg_sides(1, g_room, z, free, 6),
                  (0.0, 0.7, prep_d2_tasks(0, NL - PDN, z)),
                  (0.0, 0.95, attn_tasks(k * (APA + APB) + APB, APA, z, 2, 5)),
                  (0.01, 0.02, [prefetch]))

        def p2_body(k, carry):
            block_b(k)
            when(k < NP - 1, lambda: block_a(k))
            return carry
        lax.fori_loop(0, NP, p2_body, 0)

        def cp_out(t, half, s):
            return pltpu.make_async_copy(obuf.at[t % 2, half, pl.ds(s * M3, M3), :],
                                         out_hbm.at[pl.ds(half * HS + t * T3 + s * M3, M3), :], sem_out.at[t % 2])

        def wait_out(t):
            pltpu.make_async_copy(obuf.at[t % 2], obuf.at[t % 2], sem_out.at[t % 2]).wait()

        def p3_body(t, carry):
            when(t >= 2, lambda: wait_out(t - 2))
            for s in range(T3 // M3):
                r0 = pl.multiple_of(t * T3 + s * M3, M3)
                for n in range(KC):
                    def fin(k, sq):
                        (j0, _), *rest = _C_TERMS[k]
                        f = P[j0, pl.ds(r0, M3), ch(n)]
                        for j, sign in rest:
                            f = f + P[j, pl.ds(r0, M3), ch(n)] if sign > 0 else f - P[j, pl.ds(r0, M3), ch(n)]
                        y = f * 0.25
                        half, col = k // 2, (k % 2) * KC + n
                        x = xbuf[pl.ds(half * HS + r0, M3), ch(col)].astype(F32)
                        obuf.at[t % 2, half][pl.ds(s * M3, M3), ch(col)] = (
                            x + sq * (y + y * jnp.tanh(y))).astype(BF16)
                    for step, _ in enumerate(_strassen(
                            lambda i: _dot(OA[i, pl.ds(r0, M3), :], BO[i, :, ch(n)]), fin, (1,) * 7)):
                        if s > 0 and n == 0 and step == 1:
                            cp_out(t, 0, s - 1).start(); cp_out(t, 1, s - 1).start()
            cp_out(t, 0, T3 // M3 - 1).start(); cp_out(t, 1, T3 // M3 - 1).start()
            return carry
        lax.fori_loop(0, NT3, p3_body, 0)
        for t in range(NT3 - 2, NT3):
            wait_out(t)

    pl.run_scoped(first_half,
                  pltpu.VMEM((7, KH // 2, 2 * NL), U32),
                  pltpu.VMEM((7, KH // 2, 2 * NL), U32))
    pl.run_scoped(second_half,
                  pltpu.VMEM((QS // 2, 49 * NL), U32),
                  pltpu.VMEM((max(APA, APB) // 8, NCH, 16, NL), F32),
                  pltpu.VMEM((2, 2, T3, D), BF16))


@jax.jit
def pallas_recurrent_scan__sliding_local_dilated__geglu_ffn__prompt_kernel(
    A_x: jax.Array,
    A_wqkv: jax.Array,
    A_wo: jax.Array,
    B_x: jax.Array,
    B_w_gate: jax.Array,
    B_w_up: jax.Array,
    B_w_down: jax.Array,
):
    del B_x
    x = A_x.reshape(S, D)
    anyspec = pl.BlockSpec(memory_space=pl.ANY)
    out = pl.pallas_call(
        _kernel,
        in_specs=[anyspec] * 6,
        out_specs=anyspec,
        out_shape=jax.ShapeDtypeStruct((S, D), BF16),
        scratch_shapes=[
            pltpu.VMEM((S + SPARE, D), BF16),
            pltpu.VMEM((7, HS // 2, KH), U32),
            pltpu.VMEM((35, QS // 2, KQ), U32),
            pltpu.VMEM((3 * NCH, HALO + S + SPARE, NL), F32),
            pltpu.VMEM((7, HS, KH), F32),
            pltpu.VMEM((S + SPARE, 2 * FC), F32),
            pltpu.VMEM((7, KQ // 2, 7 * NL), U32),
            pltpu.VMEM((49, NL // 2, KQ), U32),
            pltpu.VMEM((7, KH // 2, KH), U32),
            pltpu.VMEM((6, D + 64, FC), BF16),
            pltpu.VMEM((S + SPARE, D), F32),
            pltpu.VMEM((4 * NCH, D // 2 + 64, NL), U32),
            pltpu.VMEM((7, HS // 2, KH), U32),
            pltpu.SemaphoreType.DMA((NT0, 2)),
            pltpu.SemaphoreType.DMA((2, 2)),
            pltpu.SemaphoreType.DMA((1,)),
            pltpu.SemaphoreType.DMA((3,)),
            pltpu.SemaphoreType.DMA((1,)),
            pltpu.SemaphoreType.DMA((2,)),
        ],
        compiler_params=pltpu.CompilerParams(vmem_limit_bytes=124 * 2 ** 20, disable_bounds_checks=True),
    )(x, A_wqkv, A_wo, B_w_gate, B_w_up, B_w_down)
    return out.reshape(1, S, D)
```

```python
import math

import jax
import jax.numpy as jnp
from jax import lax
import jax.experimental.pallas as pl
import jax.experimental.pallas.tpu as pltpu

S, D, F = 2048, 1024, 3584
H, DH, W, DIL = 32, 32, 8, 2
NL = 128
NCH = D // NL
HS = S // 2
KH = D // 2
KC = KH // NL
QS = S // 4
KQ = D // 4
FC = 256
NP = F // (2 * FC)
HALO = 16
SPARE = 48
F32, BF16, U32 = jnp.float32, jnp.bfloat16, jnp.uint32
EPS = 1e-5
GELU_C0 = math.sqrt(2.0 / math.pi)
GELU_C1 = GELU_C0 * 0.044715
EXP2_SCALE = (DH ** -0.5) * math.log2(math.e)
NEG = -1e9 / (DH ** -0.5)

_A_TERMS = (((0, 0, 1), (1, 1, 1)), ((1, 0, 1), (1, 1, 1)), ((0, 0, 1),), ((1, 1, 1),),
            ((0, 0, 1), (0, 1, 1)), ((1, 0, 1), (0, 0, -1)), ((0, 1, 1), (1, 1, -1)))
_B_TERMS = (((0, 0, 1), (1, 1, 1)), ((0, 0, 1),), ((0, 1, 1), (1, 1, -1)), ((1, 0, 1), (0, 0, -1)),
            ((1, 1, 1),), ((0, 0, 1), (0, 1, 1)), ((1, 0, 1), (1, 1, 1)))
_C_TERMS = (((0, 1), (3, 1), (4, -1), (6, 1)), ((2, 1), (4, 1)), ((1, 1), (3, 1)), ((0, 1), (1, -1), (2, 1), (5, 1)))
_ORDER = (1, 3, 0, 5, 2, 4, 6)
_XB_SLOT = {0: 0, 1: 1, 4: 2, 5: 3, 6: 4}


def _combine(terms, get):
    (r, c, _), *rest = terms
    v = get(r, c)
    for r, c, sign in rest:
        v = v + get(r, c) if sign > 0 else v - get(r, c)
    return v


def _ops(terms, q11, q12, q21, q22):
    q = ((q11, q12), (q21, q22))
    return [_combine(t, lambda r, c: q[r][c]) for t in terms]


def _dot(a, b):
    return jnp.dot(a, b, preferred_element_type=F32)


class _Fold:
    def __init__(self, fin, lazy=False):
        self.fin, self.lazy = fin, lazy

    def __call__(self, i, m):
        if self.lazy and i in (0, 5, 4):
            if i == 0:
                self.m0 = m
            elif i == 5:
                self.t22 = (m + self.m0) - self.m1
            else:
                self.fin(1, self.m2 + m)
                self.t11 = (self.m0 - m) + self.t11
        elif i == 1:
            self.m1 = m
        elif i == 3:
            self.fin(2, self.m1 + m)
            self.t11 = m
        elif i == 0:
            self.t11 = self.t11 + m
            self.t22 = m - self.m1
        elif i == 5:
            self.t22 = self.t22 + m
        elif i == 2:
            self.fin(3, self.t22 + m)
            self.m2 = m
        elif i == 4:
            self.fin(1, self.m2 + m)
            self.t11 = self.t11 - m
        else:
            self.fin(0, self.t11 + m)


def _strassen(prod, fin, room, lazy=False):
    fold = _Fold(fin, lazy)
    for step, i in enumerate(_ORDER):
        m = prod(i)
        fold(i, m)
        yield room[step], m


def _emit(lag, main, total, *sides):
    done = [0] * len(sides)
    acc = 0

    def flush(frac, val):
        due = []
        for k, (f0, f1, tasks) in enumerate(sides):
            want = len(tasks) if frac >= f1 else int(max(0.0, (frac - f0) / (f1 - f0)) * len(tasks) + 0.5)
            n = min(want, len(tasks)) - done[k]
            due += [((j + 0.5) / n, k, tasks[done[k] + j]) for j in range(n)]
            done[k] += max(n, 0)
        due.sort(key=lambda e: e[:2])
        for j, (_, _, task) in enumerate(due):
            r = (val.shape[0] // 8) * j // len(due) * 8
            task(val[r:r + 8, 0:NL])

    hist = [(0, None)] * lag
    for item in main:
        hist.append(item)
        room, val = hist.pop(0)
        acc += room
        if room:
            flush(acc / total, val)
    assert abs(acc + sum(h[0] for h in hist) - total) < 1e-6
    flush(2.0, hist[-1][1])


def _skew(items):
    depth = max(len(st) for st in items)
    return [items[t - k][k] for t in range(len(items) + depth - 1) for k in range(depth)
            if 0 <= t - k < len(items) and k < len(items[t - k]) and items[t - k][k] is not None]


T0, NT0 = 128, 8
RH = 256
RH2 = 64
MD, ND = 128, 128
T3, NT3, M3 = 256, 4, 64
APB, APA = 96, 64
PDN = 32
ROOM_G, ROOM_U = (2,) * 7, (2, 2, 2, 2, 1, 1, 1)
ROOM_L, ROOM_H = (2,) * 7, (2, 0, 2, 2, 0, 0, 0)
assert (NP - 1) * APA + NP * APB >= HS and APA % 32 == 0 and APB % 32 == 0


def _kernel(x_hbm, wqkv_hbm, wo_hbm, wg_hbm, wu_hbm, wd_hbm, out_hbm,
            xbuf, XA, XB, qkv, P, HF, BG, BD, BO, rw, Y, rq, OA,
            sem_x, sem_gu, sem_d, sem_q, sem_o, sem_out):

    XA, XB, BG, BD, BO, OA = [r.bitcast(BF16) for r in (XA, XB, BG, BD, BO, OA)]

    def ch(n, w=NL):
        return pl.ds(n * w, w) if isinstance(n, int) else pl.ds(pl.multiple_of(n * w, w), w)

    def zero(i):
        return i % 2 + (i + 1) % 2 - 1

    def when(pred, fn):
        pl.when(pred)(lambda: (fn(), None)[1])

    def cp_x(i, half):
        r = half * HS + i * T0
        return pltpu.make_async_copy(x_hbm.at[pl.ds(r, T0), :], xbuf.at[pl.ds(r, T0), :], sem_x.at[i, half])

    def cp_gu(c, slot, which):
        src = wg_hbm if which == 0 else wu_hbm
        return pltpu.make_async_copy(src.at[:, pl.ds(c * FC, FC)], rw.at[2 * slot + which, pl.ds(0, D), :],
                                     sem_gu.at[slot, which])

    class cp_d:
        def __init__(self, p):
            self.p = p

        def start(self):
            for q in range(4):
                pltpu.make_async_copy(wd_hbm.at[pl.ds(self.p * 2 * FC, 2 * FC), pl.ds(q * KQ, KQ)],
                                      rw.at[4 + q // 2, pl.ds((q % 2) * 2 * FC, 2 * FC), :], sem_d.at[0]).start()

        def wait(self):
            whole = rw.at[pl.ds(4, 2), pl.ds(0, D), :]
            pltpu.make_async_copy(whole, whole, sem_d.at[0]).wait()

    def anchor(dst, row, val, z):
        if val is not None and z is not None:
            r = pl.multiple_of(row + 16 + z * 16, 8)
            dst[pl.ds(r, 8), pl.ds(0, NL)] = val.astype(dst.dtype)

    def gelu2(g, u):
        t = jnp.tanh(g * (GELU_C0 + GELU_C1 * (g * g)))
        p = g * u
        return p + p * t

    def prep_g2_tasks(slot, outer, r0, n, z, free=None):
        def task(val, r, i):
            assert free is None or i in free
            anchor(rw.at[0], D, val, z)
            y = [_combine(_B_TERMS[i], lambda kp, mu: rw[2 * slot + mu, pl.ds((2 * kp + ta) * KQ + r, 16), :].astype(F32))
                 for ta in range(2)]
            ops = _ops(_B_TERMS, y[0][:, :NL], y[0][:, NL:], y[1][:, :NL], y[1][:, NL:])
            for k in range(7):
                BG.at[i][pl.ds(r, 16), ch(k)] = ops[k].astype(BF16)
        return [(lambda val, r=r0 + g * 16, i=i: task(val, r, i)) for i in outer for g in range(n // 16)]

    def prep_d2_tasks(r0, n, z):
        def task(val, r, i):
            anchor(rw.at[0], D, val, z)
            y = [_combine(_B_TERMS[i],
                          lambda kp, nu: rw[4 + nu, pl.ds(up * 2 * FC + (2 * kp + ta) * NL + r, 16), :].astype(F32))
                 for ta in range(2) for up in range(2)]
            ops = _ops(_B_TERMS, *y)
            for k in range(7):
                BD.at[7 * i + k][pl.ds(r, 16), :] = ops[k].astype(BF16)
        return [(lambda val, r=r0 + g * 16, i=i: task(val, r, i)) for g in range(n // 16) for i in range(7)]

    def first_half(B0, BQ):
        B0, BQ = B0.bitcast(BF16), BQ.bitcast(BF16)

        class cp_cols:
            def __init__(self, src, col0, dst, slot0, sem):
                self.args = src, col0, dst, slot0, sem

            def start(self):
                src, col0, dst, slot0, sem = self.args
                for k in range(NCH):
                    pltpu.make_async_copy(src.at[:, pl.ds(col0 + k * NL, NL)],
                                          dst.at[slot0 + k, pl.ds(0, D), :], sem).start()

            def wait(self):
                _, _, dst, slot0, sem = self.args
                whole = dst.at[pl.ds(slot0, NCH), pl.ds(0, D), :]
                pltpu.make_async_copy(whole, whole, sem).wait()

        def cp_q(m):
            return cp_cols(wqkv_hbm, m * D, rq, m * NCH, sem_q.at[m])

        def cp_o():
            return cp_cols(wo_hbm, 0, rq, 3 * NCH, sem_o.at[0])

        def ln_tasks(r0, n, z):
            def xrow(r):
                return xbuf[pl.ds(r, 16), :].astype(F32)
            items = []
            for g in range(n // 16):
                st = {}
                for half in range(2):
                    def stats(val, r=half * HS + r0 + g * 16, st=st, half=half):
                        anchor(xbuf, S, val, z)
                        x = xrow(r)
                        m = jnp.sum(x, axis=-1, keepdims=True) * (1.0 / D)
                        e2 = jnp.sum(x * x, axis=-1, keepdims=True) * (1.0 / D)
                        st["m", half] = m
                        st["v", half] = lax.rsqrt(jnp.maximum(e2 - m * m, 0.0) + EPS)

                    def apply(val, r=r0 + g * 16, st=st, half=half):
                        for kc in (2 * half, 2 * half + 1):
                            anchor(xbuf, S, val, z)
                            pos = [(h, c) for h in range(2) for c in (kc, KC + kc)]
                            q = [(xbuf[pl.ds(h * HS + r, 16), ch(c)].astype(F32) - st["m", h]) * st["v", h]
                                 for h, c in pos]
                            for (h, c), y in zip(pos, q):
                                Y[pl.ds(h * HS + r, 16), ch(c)] = y
                            for i, op in enumerate(_ops(_A_TERMS, *q)):
                                XA.at[i][pl.ds(r, 16), ch(kc)] = op.astype(BF16)
                    items.append([stats] + [None] * (2 - half) + [apply])
            return _skew(items)

        def prep_g1(which, r0, n):
            for g in range(n // 16):
                r = r0 + g * 16
                top = rw[which, pl.ds(r, 16), :].astype(F32)
                bot = rw[which, pl.ds(KH + r, 16), :].astype(F32)
                for i, op in enumerate(_ops(_B_TERMS, top[:, :NL], top[:, NL:], bot[:, :NL], bot[:, NL:])):
                    B0.at[i][pl.ds(r, 16), ch(which)] = op.astype(BF16)

        def xb_tasks(r0, n, z):
            def task(val, r, kc, i):
                anchor(Y, S, val, z)
                x = [_combine(_A_TERMS[i],
                              lambda sg, kp: Y[pl.ds((2 * sg + rho) * QS + r, 16), ch(4 * kp + 2 * ta + kc)])
                     for rho in range(2) for ta in range(2)]
                ops = _ops(_A_TERMS, *x)
                for k, slot in _XB_SLOT.items():
                    XB.at[5 * i + slot][pl.ds(r, 16), ch(kc)] = ops[k].astype(BF16)
            return [(lambda val, r=r0 + g * 16, kc=kc, i=i: task(val, r, kc, i))
                    for g in range(n // 16) for kc in range(2) for i in range(7)]

        def wide(w):
            return pltpu.bitcast(w, BF16).astype(F32)

        def prep_q_tasks(m, par, n, z, chain=True):
            def perm_a(r):
                y = [pltpu.bitcast(rq[m * NCH + k, pl.ds(r, 16), :], U32) for k in range(NCH)]
                return [y[0]] + [pltpu.roll(y[k], 2 * k, 1) for k in range(1, NCH)]

            def perm_b(y):
                lane = lax.broadcasted_iota(jnp.int32, (8, NL), 1)
                sh = (((lane & 15) >> 1) - par) & 7
                u = [y[(-j) % NCH] for j in range(NCH)]
                b0, b1, b2 = (sh & 1) != 0, (sh & 2) != 0, (sh & 4) != 0
                out = (2 * n, 2 * n + 4)
                v = {j: jnp.where(b0, u[(j - 1) % NCH], u[j]) for j in (0, 2, 4, 6)}
                v = {j: jnp.where(b1, v[(j - 2) % NCH], v[j]) for j in out}
                v = {j: jnp.where(b2, v[(j - 4) % NCH], v[j]) for j in out}
                return [pltpu.roll(v[j], (2 * NL - 2 * j - 2 * par) % NL, 1) for j in out]

            items = []
            for g in range(KH // 16):
                st = {}
                for half in range(2):
                    def s0(val, r=half * KH + g * 16, st=st, half=half):
                        anchor(rq.at[0], D, val, z)
                        st["a", half] = perm_a(r)

                    def s1(val, st=st, half=half):
                        st["b", half] = perm_b(st["a", half])

                    def s2(val, r=g * 16, st=st):
                        ops = _ops(_B_TERMS, *[wide(w) for w in st["b", 0] + st["b", 1]])
                        for i in range(7):
                            BQ.at[i][pl.ds(r, 16), ch(n)] = ops[i].astype(BF16)
                        if chain:
                            anchor(rq.at[0], D, (ops[5] + ops[6])[0:8], z)
                    items.append([s0, s1] + ([s2] if half else []))
            flat = _skew(items)
            firsts = [j for j, t in enumerate(flat) if t.__name__ == "s0"] + [len(flat)]
            return [(lambda val, grp=flat[a:b]: [t(val) for t in grp]) for a, b in zip(firsts, firsts[1:])]

        def prep_o_tasks(src, n, z):
            def transpose(c, a):
                sub = lax.broadcasted_iota(jnp.int32, (8, NL), 0)
                y = [pltpu.bitcast(rq[src + c, pl.ds(128 * g + 16 * a, 16), :], U32) for g in range(8)]
                y = [y[0]] + [pltpu.roll(y[g], g, 0) for g in range(1, 8)]
                v = [y[(-j) % 8] for j in range(8)]
                for bit in (1, 2, 4):
                    v = [jnp.where((sub & bit) != 0, v[(j - bit) % 8], v[j]) for j in range(8)]
                return [v[0]] + [pltpu.roll(v[j], 8 - j, 0) for j in range(1, 8)]

            tasks = []
            for a in range(8):
                st = {}

                def load(val, h, a=a, st=st):
                    anchor(rq.at[0], D, val, z)
                    st[h] = transpose(h * KC + n, a)

                def quad(val, jj, a=a, st=st):
                    q = [wide(st[h][kh * KC + jj]) for kh in range(2) for h in range(2)]
                    for i, op in enumerate(_ops(_B_TERMS, *q)):
                        BO.at[i][pl.ds(jj * NL + 16 * a, 16), ch(n)] = op.astype(BF16)
                tasks += [lambda val, f=load: f(val, 0),
                          lambda val, f=load, g=quad: (f(val, 1), [g(val, jj) for jj in range(KC)])]
            return tasks

        def zero_p_tasks(u0, n, z):
            def task(val, u):
                v = jnp.where(z != 0, val, 0.0)
                P[u // 32, pl.ds(pl.multiple_of((u % 32) * 32, 32), 32), :] = jnp.tile(v, (4, KC))
            return [(lambda val, u=u0 + j: task(val, u)) for j in range(n)]

        def up1(r0, m):
            g = {}

            def fin_u(k, u):
                HF[pl.ds((k // 2) * HS + r0, m), ch(k % 2)] = gelu2(g[k], u)
            yield from _strassen(lambda i: _dot(XA[i, pl.ds(r0, m), :], B0[i, :, ch(0)]), g.__setitem__, ROOM_G, lazy=True)
            yield from _strassen(lambda i: _dot(XA[i, pl.ds(r0, m), :], B0[i, :, ch(1)]), fin_u, ROOM_U, lazy=True)

        groups = [lambda: [cp_x(0, 0), cp_x(0, 1)], lambda: [cp_gu(0, 0, 0)], lambda: [cp_gu(0, 0, 1)]]
        groups += [(lambda i=i: [cp_x(i, 0), cp_x(i, 1)]) for i in range(1, NT0)]
        groups += [lambda: [cp_q(0)], lambda: [cp_gu(1, 1, 0), cp_gu(1, 1, 1), cp_d(0)],
                   lambda: [cp_q(1)], lambda: [cp_o()], lambda: [cp_q(2)]]

        def issue(k, c):
            for g, cps in enumerate(groups):
                when(k == g, lambda: [cp.start() for cp in cps()])
            return c
        lax.fori_loop(0, len(groups), issue, 0)
        cp_x(0, 0).wait(); cp_x(0, 1).wait()

        def ln0(g, c):
            for t in ln_tasks(pl.multiple_of(g * 64, 64), 64, None):
                t(None)
            return c
        lax.fori_loop(0, T0 // 64, ln0, 0)
        for which in range(2):
            cp_gu(0, 0, which).wait()

            def pg0(g, c):
                prep_g1(which, pl.multiple_of(g * 64, 64), 64)
                return c
            lax.fori_loop(0, KH // 64, pg0, 0)

        def p0_body(i, c):
            cp_x(i + 1, 0).wait(); cp_x(i + 1, 1).wait()
            r0 = pl.multiple_of(i * T0, T0)
            _emit(2, up1(r0, T0), sum(ROOM_G) + sum(ROOM_U), (0.0, 0.85, ln_tasks(r0 + T0, T0, zero(i))))
            return zero(i)
        z0 = lax.fori_loop(0, NT0 - 1, p0_body, 0)
        cp_q(0).wait()
        cp_gu(2, 0, 0).start(); cp_gu(2, 0, 1).start()
        _emit(1, up1(HS - T0, T0), sum(ROOM_G) + sum(ROOM_U), (0.0, 0.9, prep_q_tasks(0, 0, 0, z0, chain=False)))

        def p1_body(b, c):
            when(b == 0, lambda: (cp_gu(1, 1, 0).wait(), cp_gu(1, 1, 1).wait(), cp_d(0).wait()))
            when(b == 1, lambda: cp_q(1).wait())
            when(b == 2, lambda: cp_o().wait())
            when(b == 3, lambda: cp_q(2).wait())
            m = b // 2
            par = b % 2

            def main():
                for n in range(2):
                    for s in range(HS // RH):
                        r0 = s * RH

                        def fin(k, v):
                            j = m * NCH + par + 2 * n + 4 * (k % 2)
                            qkv[j, pl.ds(HALO + (k // 2) * HS + r0, RH), :] = v
                        yield from _strassen(lambda i: _dot(XA[i, pl.ds(r0, RH), :], BQ[i, :, ch(n)]), fin, (1,) * 7)
            piece = jnp.clip(b - 2, 0, 3)
            z = zero(b)
            _emit(1, main(), 14 * (HS // RH),
                  (0.0, 0.48, prep_q_tasks(m, par, 1, z)),
                  (0.5, 0.98, prep_q_tasks(jnp.minimum((b + 1) // 2, 2), (b + 1) % 2, 0, z)),
                  (0.0, 0.95, prep_g2_tasks(1, range(7), pl.multiple_of(jnp.minimum(b * 48, KQ - 48), 16), 48, z)),
                  (0.0, 0.95, xb_tasks(pl.multiple_of(jnp.minimum(b * 96, QS - 96), 32), 96, z)),
                  (0.0, 0.95, prep_d2_tasks(pl.multiple_of(jnp.clip(b * 16, 0, NL - PDN - 16), 16), 16, z)),
                  (0.0, 0.95, zero_p_tasks(jnp.minimum(b * 38, 224 - 38), 38, z)),
                  (0.0, 0.95, prep_o_tasks(jnp.where(b < 2, 0, 3 * NCH), piece, z)))
            return c
        lax.fori_loop(0, 6, p1_body, 0)
        for j in range(NCH, 3 * NCH):
            qkv[j, 0:HALO, :] = jnp.broadcast_to(qkv[j, HALO:HALO + 1, :], (HALO, NL))

    def second_half(HA, osc, obuf):
        HA = HA.bitcast(BF16)

        def attn_unit(t0, r0, masked, slot, z, G, g0, gap):
            st = {}
            sh = 4 * (G - 1)

            def shifted(plane):
                return [qkv[plane, pl.ds(t0 + (r0 + HALO + 2 * sh - DIL * k), 8), :] for k in range(W + sh)]

            def logits(val, j):
                anchor(qkv.at[0], HALO + S, val, z)
                q = [qkv[j, pl.ds(t0 + (r0 + HALO + 8 * g), 8), :] for g in range(G)]
                kk = shifted(NCH + j)
                for g in range(G):
                    for w in range(W):
                        t = q[g] * kk[w + sh - 4 * g]
                        st[g, w] = t if j == 0 else st[g, w] + t
                if j == NCH - 1:
                    softmax()

            def softmax():
                lane = lax.broadcasted_iota(jnp.int32, (8, NL), 1)
                odd = (lane & 1) != 0
                hi = (lane & 16) != 0
                keys = [(g, w) for g in range(G) for w in range(W)]
                for k in keys:
                    a = st[k]
                    st[k] = a + jnp.where(odd, pltpu.roll(a, 1, 1), pltpu.roll(a, NL - 1, 1))
                for k in keys:
                    a = st[k]
                    st[k] = a + jnp.where(hi, pltpu.roll(a, 16, 1), pltpu.roll(a, NL - 16, 1))
                for g in range(G):
                    ls = [st[g, w] for w in range(W)]
                    if masked:
                        pos = t0 + (r0 + 8 * g) + lax.broadcasted_iota(jnp.int32, (8, NL), 0)
                        ls = [ls[0]] + [jnp.where(pos >= DIL * w, ls[w], NEG) for w in range(1, W)]
                    m = ls[0]
                    for w in range(1, W):
                        m = jnp.maximum(m, ls[w])
                    ps = [jnp.exp2((l - m) * EXP2_SCALE) for l in ls]
                    den = ps[0]
                    for w in range(1, W):
                        den = den + ps[w]
                    inv = 1.0 / den
                    for w in range(W):
                        st[g, w] = ps[w] * inv

            def pv(val, j):
                anchor(qkv.at[0], HALO + S, val, z)
                vv = shifted(2 * NCH + j)
                for g in range(G):
                    a = st[g, 0] * vv[sh - 4 * g]
                    for w in range(1, W):
                        a = a + st[g, w] * vv[w + sh - 4 * g]
                    osc[slot, j, pl.ds(8 * (g0 + g), 8), :] = a

            return ([(lambda val, j=j: logits(val, j)) for j in range(NCH)] + [lambda val: None] * gap
                    + [(lambda val, j=j: pv(val, j)) for j in range(NCH)])

        def attn_tasks(t0, n, z, G, gap):
            t0 = pl.multiple_of(jnp.minimum(t0, HS - n), 16)
            tasks = []
            for g in range(n // 16):
                r = g * 16
                for half in range(2):
                    for g0 in range(0, 2, G):
                        tasks += attn_unit(t0, half * HS + r + 8 * g0, g == 0 and half == 0, 2 * g + half, z, G, g0, gap)

                def oa(val, kc, g=g, r=r):
                    ops = _ops(_A_TERMS, osc[2 * g, kc], osc[2 * g, KC + kc],
                               osc[2 * g + 1, kc], osc[2 * g + 1, KC + kc])
                    for i in range(7):
                        OA.at[i][pl.ds(t0 + r, 16), ch(kc)] = ops[i].astype(BF16)
                tasks += [(lambda val, kc=kc, oa=oa: oa(val, kc)) for kc in range(KC)]
            return tasks

        def ha_task(val, r, i, z, have):
            anchor(HF, S, val, z)
            x = [_combine(_A_TERMS[i], lambda sg, kp: HF[pl.ds((2 * sg + rho) * QS + r, 16), ch(2 * kp + ta)])
                 for rho in range(2) for ta in range(2)]
            for k, op in enumerate(_ops(_A_TERMS, *x)):
                HA[pl.ds(r, 16), ch(7 * i + k)] = op.astype(BF16)
            have.add((i, r))

        def up2(kp, free, on_half):
            def sub(r0, m):
                hold, seen = {}, set()

                def outer_fin(k, K, v):
                    if K in (2, 1):
                        hold[k] = v
                        return
                    sg = K // 2
                    HF[pl.ds((2 * sg + k // 2) * QS + r0, m), ch(2 * kp + k % 2)] = (
                        gelu2(hold[k], v) if K == 3 else gelu2(v, hold[k]))
                    seen.add((sg, k))
                    if all((sg, j) in seen for j in range(4)):
                        on_half(sg, r0, m)
                folds = [_Fold(lambda K, v, k=k: outer_fin(k, K, v), lazy=True) for k in range(4)]

                def lhs(i, k):
                    if k == 2:
                        return XA[i, pl.ds(r0, m), pl.ds(0, KQ)]
                    if k == 3:
                        return XA[i, pl.ds(QS + r0, m), pl.ds(KQ, KQ)]
                    return XB[5 * i + _XB_SLOT[k], pl.ds(r0, m), :]
                return lambda i: _strassen(lambda k: _dot(lhs(i, k), BG[i, :, ch(k)]),
                                           lambda k, v: folds[k](i, v), ROOM_H if i in (2, 6) else ROOM_L)
            subs = [sub(s * RH2, RH2) for s in range(QS // RH2)]
            for i in _ORDER:
                for sb in subs:
                    yield from sb(i)
                free.add(i)

        nsub = QS // RH2
        g_room = (5 * sum(ROOM_L) + 2 * sum(ROOM_H)) * nsub
        d_unit = 2.5 * MD * ND / (RH2 * KQ)

        ends = [sum(sum(ROOM_H if i in (2, 6) else ROOM_L) for i in _ORDER[:j + 1]) * nsub for j in range(7)]

        def bg_sides(slot, total, z, free, n):
            return [((ends[j] + 1) / total, (ends[j + 1] if j < 6 else ends[6] + ends[0]) / total - 0.01,
                     prep_g2_tasks(slot, _ORDER[j:j + 1], 0, KQ, z, free)) for j in range(n)]

        def block_b(k):
            when(k < NP - 1, lambda: (cp_gu(0, 0, 0).wait(), cp_gu(0, 0, 1).wait()))

            z = zero(k)
            free, have, halves, pending = set(), set(), set(), set()

            def reads_old(tasks):
                pending.update(tasks)
                return [(lambda val, t=t: (t(val), pending.discard(t))) for t in tasks]

            def prefetch(val):
                assert not pending
                when(k < NP - 1, lambda: (cp_gu(2 * k + 3, 1, 0).start(), cp_gu(2 * k + 3, 1, 1).start(),
                                          cp_d(k + 1).start()))

            def on_half(sg, r0, m):
                if r0 + m == QS:
                    halves.add(sg)

            def ha_tasks(outer, need):
                def task(val, r, i):
                    assert need <= halves
                    ha_task(val, r, i, z, have)
                return [(lambda val, r=r, i=i: task(val, r, i)) for i in outer for r in range(0, QS, 16)]

            def main():
                yield from up2(1, free, on_half)
                for i in (2, 5, 1, 3, 0, 4, 6):
                    assert all((i, r) in have for r in range(0, QS, 16))
                    for r0 in range(0, QS, MD):
                        for c in range(KQ // ND):
                            def fin(q, v):
                                P[i, pl.ds((q // 2) * QS + r0, MD), pl.ds((q % 2) * KQ + c * ND, ND)] += v
                            yield from _strassen(
                                lambda j: _dot(HA[pl.ds(r0, MD), ch(7 * i + j)], BD[7 * i + j, :, ch(c, ND)]),
                                fin, (d_unit,) * 7)
            total = g_room + 49 * (QS // MD) * (KQ // ND) * d_unit
            gf = g_room / total
            df = (1 - gf) / 7
            _emit(5, main(), total, *bg_sides(0, total, z, free, 7),
                  (0.0, ends[0] / total, reads_old(prep_g2_tasks(1, _ORDER[6:], 0, KQ, z))),
                  (0.0, 0.9 * gf, ha_tasks((2, 5), set())),
                  ((ends[4] + 1) / total, gf + 1.6 * df, ha_tasks((1, 3, 0), {1})),
                  (gf + 1.6 * df, gf + 5.5 * df, ha_tasks((4, 6), {0, 1})),
                  (0.0, 0.9 * gf, reads_old(prep_d2_tasks(NL - PDN, PDN, z))),
                  (0.0, 0.98, attn_tasks(k * (APA + APB), APB, z, 1, 10)),
                  (gf, gf + 0.01, [prefetch]))

        def block_a(k):
            cp_gu(0, 1, 0).wait(); cp_gu(0, 1, 1).wait(); cp_d(0).wait()

            def prefetch(val):
                when(k < NP - 2, lambda: (cp_gu(2 * k + 4, 0, 0).start(), cp_gu(2 * k + 4, 0, 1).start()))
            z = zero(k)
            free = set()
            _emit(4, up2(0, free, lambda *a: None), g_room, *bg_sides(1, g_room, z, free, 6),
                  (0.0, 0.7, prep_d2_tasks(0, NL - PDN, z)),
                  (0.0, 0.95, attn_tasks(k * (APA + APB) + APB, APA, z, 2, 5)),
                  (0.01, 0.02, [prefetch]))

        def p2_body(k, carry):
            block_b(k)
            when(k < NP - 1, lambda: block_a(k))
            return carry
        lax.fori_loop(0, NP, p2_body, 0)

        def cp_out(t, half, s):
            return pltpu.make_async_copy(obuf.at[t % 2, half, pl.ds(s * M3, M3), :],
                                         out_hbm.at[pl.ds(half * HS + t * T3 + s * M3, M3), :], sem_out.at[t % 2])

        def wait_out(t):
            pltpu.make_async_copy(obuf.at[t % 2], obuf.at[t % 2], sem_out.at[t % 2]).wait()

        def p3_body(t, carry):
            when(t >= 2, lambda: wait_out(t - 2))
            for s in range(T3 // M3):
                r0 = pl.multiple_of(t * T3 + s * M3, M3)
                for n in range(KC):
                    def fin(k, sq):
                        (j0, _), *rest = _C_TERMS[k]
                        f = P[j0, pl.ds(r0, M3), ch(n)]
                        for j, sign in rest:
                            f = f + P[j, pl.ds(r0, M3), ch(n)] if sign > 0 else f - P[j, pl.ds(r0, M3), ch(n)]
                        y = f * 0.25
                        half, col = k // 2, (k % 2) * KC + n
                        x = xbuf[pl.ds(half * HS + r0, M3), ch(col)].astype(F32)
                        obuf.at[t % 2, half][pl.ds(s * M3, M3), ch(col)] = (
                            x + sq * (y + y * jnp.tanh(y))).astype(BF16)
                    for step, _ in enumerate(_strassen(
                            lambda i: _dot(OA[i, pl.ds(r0, M3), :], BO[i, :, ch(n)]), fin, (1,) * 7)):
                        if s > 0 and n == 0 and step == 1:
                            cp_out(t, 0, s - 1).start(); cp_out(t, 1, s - 1).start()
            cp_out(t, 0, T3 // M3 - 1).start(); cp_out(t, 1, T3 // M3 - 1).start()
            return carry
        lax.fori_loop(0, NT3, p3_body, 0)
        for t in range(NT3 - 2, NT3):
            wait_out(t)

    pl.run_scoped(first_half,
                  pltpu.VMEM((7, KH // 2, 2 * NL), U32),
                  pltpu.VMEM((7, KH // 2, 2 * NL), U32))
    pl.run_scoped(second_half,
                  pltpu.VMEM((QS // 2, 49 * NL), U32),
                  pltpu.VMEM((max(APA, APB) // 8, NCH, 16, NL), F32),
                  pltpu.VMEM((2, 2, T3, D), BF16))


@jax.jit
def pallas_recurrent_scan__sliding_local_dilated__geglu_ffn__prompt_kernel(
    A_x: jax.Array,
    A_wqkv: jax.Array,
    A_wo: jax.Array,
    B_x: jax.Array,
    B_w_gate: jax.Array,
    B_w_up: jax.Array,
    B_w_down: jax.Array,
):
    del B_x
    x = A_x.reshape(S, D)
    anyspec = pl.BlockSpec(memory_space=pl.ANY)
    out = pl.pallas_call(
        _kernel,
        in_specs=[anyspec] * 6,
        out_specs=anyspec,
        out_shape=jax.ShapeDtypeStruct((S, D), BF16),
        scratch_shapes=[
            pltpu.VMEM((S + SPARE, D), BF16),
            pltpu.VMEM((7, HS // 2, KH), U32),
            pltpu.VMEM((35, QS // 2, KQ), U32),
            pltpu.VMEM((3 * NCH, HALO + S + SPARE, NL), F32),
            pltpu.VMEM((7, HS, KH), F32),
            pltpu.VMEM((S + SPARE, 2 * FC), F32),
            pltpu.VMEM((7, KQ // 2, 7 * NL), U32),
            pltpu.VMEM((49, NL // 2, KQ), U32),
            pltpu.VMEM((7, KH // 2, KH), U32),
            pltpu.VMEM((6, D + 64, FC), BF16),
            pltpu.VMEM((S + SPARE, D), F32),
            pltpu.VMEM((4 * NCH, D + 64, NL), BF16),
            pltpu.VMEM((7, HS // 2, KH), U32),
            pltpu.SemaphoreType.DMA((NT0, 2)),
            pltpu.SemaphoreType.DMA((2, 2)),
            pltpu.SemaphoreType.DMA((1,)),
            pltpu.SemaphoreType.DMA((3,)),
            pltpu.SemaphoreType.DMA((1,)),
            pltpu.SemaphoreType.DMA((2,)),
        ],
        compiler_params=pltpu.CompilerParams(vmem_limit_bytes=124 * 2 ** 20, disable_bounds_checks=True),
    )(x, A_wqkv, A_wo, B_w_gate, B_w_up, B_w_down)
    return out.reshape(1, S, D)
```

```python
import math

import jax
import jax.numpy as jnp
from jax import lax
import jax.experimental.pallas as pl
import jax.experimental.pallas.tpu as pltpu

S, D, F = 2048, 1024, 3584
H, DH, W, DIL = 32, 32, 8, 2
NL = 128
NCH = D // NL
HS = S // 2
KH = D // 2
KC = KH // NL
QS = S // 4
KQ = D // 4
FC = 256
NP = F // (2 * FC)
HALO = 16
SPARE = 48
F32, BF16, U32 = jnp.float32, jnp.bfloat16, jnp.uint32
EPS = 1e-5
GELU_C0 = math.sqrt(2.0 / math.pi)
GELU_C1 = GELU_C0 * 0.044715
EXP2_SCALE = (DH ** -0.5) * math.log2(math.e)
NEG = -1e9 / (DH ** -0.5)

_A_TERMS = (((0, 0, 1), (1, 1, 1)), ((1, 0, 1), (1, 1, 1)), ((0, 0, 1),), ((1, 1, 1),),
            ((0, 0, 1), (0, 1, 1)), ((1, 0, 1), (0, 0, -1)), ((0, 1, 1), (1, 1, -1)))
_B_TERMS = (((0, 0, 1), (1, 1, 1)), ((0, 0, 1),), ((0, 1, 1), (1, 1, -1)), ((1, 0, 1), (0, 0, -1)),
            ((1, 1, 1),), ((0, 0, 1), (0, 1, 1)), ((1, 0, 1), (1, 1, 1)))
_C_TERMS = (((0, 1), (3, 1), (4, -1), (6, 1)), ((2, 1), (4, 1)), ((1, 1), (3, 1)), ((0, 1), (1, -1), (2, 1), (5, 1)))
_ORDER = (1, 3, 0, 5, 2, 4, 6)
_XB_SLOT = {0: 0, 1: 1, 4: 2, 5: 3, 6: 4}


def _combine(terms, get):
    (r, c, _), *rest = terms
    v = get(r, c)
    for r, c, sign in rest:
        v = v + get(r, c) if sign > 0 else v - get(r, c)
    return v


def _ops(terms, q11, q12, q21, q22):
    q = ((q11, q12), (q21, q22))
    return [_combine(t, lambda r, c: q[r][c]) for t in terms]


def _dot(a, b):
    return jnp.dot(a, b, preferred_element_type=F32)


class _Fold:
    def __init__(self, fin, lazy=False):
        self.fin, self.lazy = fin, lazy

    def __call__(self, i, m):
        if self.lazy and i in (0, 5, 4):
            if i == 0:
                self.m0 = m
            elif i == 5:
                self.t22 = (m + self.m0) - self.m1
            else:
                self.fin(1, self.m2 + m)
                self.t11 = (self.m0 - m) + self.t11
        elif i == 1:
            self.m1 = m
        elif i == 3:
            self.fin(2, self.m1 + m)
            self.t11 = m
        elif i == 0:
            self.t11 = self.t11 + m
            self.t22 = m - self.m1
        elif i == 5:
            self.t22 = self.t22 + m
        elif i == 2:
            self.fin(3, self.t22 + m)
            self.m2 = m
        elif i == 4:
            self.fin(1, self.m2 + m)
            self.t11 = self.t11 - m
        else:
            self.fin(0, self.t11 + m)


def _strassen(prod, fin, room, lazy=False):
    fold = _Fold(fin, lazy)
    for step, i in enumerate(_ORDER):
        m = prod(i)
        fold(i, m)
        yield room[step], m


def _emit(lag, main, total, *sides):
    done = [0] * len(sides)
    acc = 0

    def flush(frac, val):
        due = []
        for k, (f0, f1, tasks) in enumerate(sides):
            want = len(tasks) if frac >= f1 else int(max(0.0, (frac - f0) / (f1 - f0)) * len(tasks) + 0.5)
            n = min(want, len(tasks)) - done[k]
            due += [((j + 0.5) / n, k, tasks[done[k] + j]) for j in range(n)]
            done[k] += max(n, 0)
        due.sort(key=lambda e: e[:2])
        for j, (_, _, task) in enumerate(due):
            r = (val.shape[0] // 8) * j // len(due) * 8
            task(val[r:r + 8, 0:NL])

    hist = [(0, None)] * lag
    for item in main:
        hist.append(item)
        room, val = hist.pop(0)
        acc += room
        if room:
            flush(acc / total, val)
    assert abs(acc + sum(h[0] for h in hist) - total) < 1e-6
    flush(2.0, hist[-1][1])


def _skew(items):
    depth = max(len(st) for st in items)
    return [items[t - k][k] for t in range(len(items) + depth - 1) for k in range(depth)
            if 0 <= t - k < len(items) and k < len(items[t - k]) and items[t - k][k] is not None]


T0, NT0 = 128, 8
RH = 256
RH2 = 64
MD, ND = 128, 128
T3, NT3, M3 = 256, 4, 64
APB, APA = 96, 64
PDN = 48
ROOM_G, ROOM_U = (2,) * 7, (2, 2, 2, 2, 1, 1, 1)
ROOM_L, ROOM_H = (2,) * 7, (2, 0, 2, 2, 0, 0, 0)
assert (NP - 1) * APA + NP * APB >= HS and APA % 32 == 0 and APB % 32 == 0


def _kernel(x_hbm, wqkv_hbm, wo_hbm, wg_hbm, wu_hbm, wd_hbm, out_hbm,
            xbuf, XA, XB, qkv, P, HF, BG, BD, BO, rw, Y, rq, OA,
            sem_x, sem_gu, sem_d, sem_q, sem_o, sem_out):

    XA, XB, BG, BD, BO, OA = [r.bitcast(BF16) for r in (XA, XB, BG, BD, BO, OA)]

    def ch(n, w=NL):
        return pl.ds(n * w, w) if isinstance(n, int) else pl.ds(pl.multiple_of(n * w, w), w)

    def zero(i):
        return i % 2 + (i + 1) % 2 - 1

    def when(pred, fn):
        pl.when(pred)(lambda: (fn(), None)[1])

    def cp_x(i, half):
        r = half * HS + i * T0
        return pltpu.make_async_copy(x_hbm.at[pl.ds(r, T0), :], xbuf.at[pl.ds(r, T0), :], sem_x.at[i, half])

    def cp_gu(c, slot, which):
        src = wg_hbm if which == 0 else wu_hbm
        return pltpu.make_async_copy(src.at[:, pl.ds(c * FC, FC)], rw.at[2 * slot + which, pl.ds(0, D), :],
                                     sem_gu.at[slot, which])

    class cp_d:
        def __init__(self, p):
            self.p = p

        def start(self):
            for q in range(4):
                pltpu.make_async_copy(wd_hbm.at[pl.ds(self.p * 2 * FC, 2 * FC), pl.ds(q * KQ, KQ)],
                                      rw.at[4 + q // 2, pl.ds((q % 2) * 2 * FC, 2 * FC), :], sem_d.at[0]).start()

        def wait(self):
            whole = rw.at[pl.ds(4, 2), pl.ds(0, D), :]
            pltpu.make_async_copy(whole, whole, sem_d.at[0]).wait()

    def anchor(dst, row, val, z):
        if val is not None and z is not None:
            r = pl.multiple_of(row + 16 + z * 16, 8)
            dst[pl.ds(r, 8), pl.ds(0, NL)] = val.astype(dst.dtype)

    def gelu2(g, u):
        t = jnp.tanh(g * (GELU_C0 + GELU_C1 * (g * g)))
        p = g * u
        return p + p * t

    def prep_g2_tasks(slot, outer, r0, n, z, free=None):
        def task(val, r, i):
            assert free is None or i in free
            anchor(rw.at[0], D, val, z)
            y = [_combine(_B_TERMS[i], lambda kp, mu: rw[2 * slot + mu, pl.ds((2 * kp + ta) * KQ + r, 16), :].astype(F32))
                 for ta in range(2)]
            ops = _ops(_B_TERMS, y[0][:, :NL], y[0][:, NL:], y[1][:, :NL], y[1][:, NL:])
            for k in range(7):
                BG.at[i][pl.ds(r, 16), ch(k)] = ops[k].astype(BF16)
        return [(lambda val, r=r0 + g * 16, i=i: task(val, r, i)) for i in outer for g in range(n // 16)]

    def prep_d2_tasks(r0, n, z):
        def task(val, r, i, c):
            anchor(rw.at[0], D, val, z)
            y = [_combine(_B_TERMS[i],
                          lambda kp, nu: rw[4 + nu, pl.ds(up * 2 * FC + (2 * kp + ta) * NL + r, 16), ch(c)].astype(F32))
                 for ta in range(2) for up in range(2)]
            ops = _ops(_B_TERMS, *y)
            for k in range(7):
                BD.at[7 * i + k][pl.ds(r, 16), ch(c)] = ops[k].astype(BF16)
        return [(lambda val, r=r0 + g * 16, i=i, c=c: task(val, r, i, c))
                for g in range(n // 16) for i in range(7) for c in range(2)]

    def first_half(B0, BQ):
        B0, BQ = B0.bitcast(BF16), BQ.bitcast(BF16)

        class cp_cols:
            def __init__(self, src, col0, dst, slot0, sem):
                self.args = src, col0, dst, slot0, sem

            def start(self):
                src, col0, dst, slot0, sem = self.args
                for k in range(NCH):
                    pltpu.make_async_copy(src.at[:, pl.ds(col0 + k * NL, NL)],
                                          dst.at[slot0 + k, pl.ds(0, D), :], sem).start()

            def wait(self):
                _, _, dst, slot0, sem = self.args
                whole = dst.at[pl.ds(slot0, NCH), pl.ds(0, D), :]
                pltpu.make_async_copy(whole, whole, sem).wait()

        def cp_q(m):
            return cp_cols(wqkv_hbm, m * D, rq, m * NCH, sem_q.at[m])

        def cp_o():
            return cp_cols(wo_hbm, 0, rq, 3 * NCH, sem_o.at[0])

        def ln_tasks(r0, n, z):
            def xrow(r):
                return xbuf[pl.ds(r, 16), :].astype(F32)
            items = []
            for g in range(n // 16):
                st = {}
                for half in range(2):
                    def stats(val, r=half * HS + r0 + g * 16, st=st, half=half):
                        anchor(xbuf, S, val, z)
                        x = xrow(r)
                        m = jnp.sum(x, axis=-1, keepdims=True) * (1.0 / D)
                        e2 = jnp.sum(x * x, axis=-1, keepdims=True) * (1.0 / D)
                        st["m", half] = m
                        st["v", half] = lax.rsqrt(jnp.maximum(e2 - m * m, 0.0) + EPS)

                    def apply(val, r=r0 + g * 16, st=st, half=half):
                        for kc in (2 * half, 2 * half + 1):
                            anchor(xbuf, S, val, z)
                            pos = [(h, c) for h in range(2) for c in (kc, KC + kc)]
                            q = [(xbuf[pl.ds(h * HS + r, 16), ch(c)].astype(F32) - st["m", h]) * st["v", h]
                                 for h, c in pos]
                            for (h, c), y in zip(pos, q):
                                Y[pl.ds(h * HS + r, 16), ch(c)] = y
                            for i, op in enumerate(_ops(_A_TERMS, *q)):
                                XA.at[i][pl.ds(r, 16), ch(kc)] = op.astype(BF16)
                    items.append([stats] + [None] * (2 - half) + [apply])
            return _skew(items)

        def prep_g1(which, r0, n):
            for g in range(n // 16):
                r = r0 + g * 16
                top = rw[which, pl.ds(r, 16), :].astype(F32)
                bot = rw[which, pl.ds(KH + r, 16), :].astype(F32)
                for i, op in enumerate(_ops(_B_TERMS, top[:, :NL], top[:, NL:], bot[:, :NL], bot[:, NL:])):
                    B0.at[i][pl.ds(r, 16), ch(which)] = op.astype(BF16)

        def xb_tasks(r0, n, z):
            def task(val, r, kc, i):
                anchor(Y, S, val, z)
                x = [_combine(_A_TERMS[i],
                              lambda sg, kp: Y[pl.ds((2 * sg + rho) * QS + r, 16), ch(4 * kp + 2 * ta + kc)])
                     for rho in range(2) for ta in range(2)]
                ops = _ops(_A_TERMS, *x)
                for k, slot in _XB_SLOT.items():
                    XB.at[5 * i + slot][pl.ds(r, 16), ch(kc)] = ops[k].astype(BF16)
            return [(lambda val, r=r0 + g * 16, kc=kc, i=i: task(val, r, kc, i))
                    for g in range(n // 16) for kc in range(2) for i in range(7)]

        def wide(w):
            return pltpu.bitcast(w, BF16).astype(F32)

        def prep_q_tasks(m, par, n, z, chain=True):
            def perm_a(r):
                y = [pltpu.bitcast(rq[m * NCH + k, pl.ds(r, 16), :], U32) for k in range(NCH)]
                return [y[0]] + [pltpu.roll(y[k], 2 * k, 1) for k in range(1, NCH)]

            def perm_b(y):
                lane = lax.broadcasted_iota(jnp.int32, (8, NL), 1)
                sh = (((lane & 15) >> 1) - par) & 7
                u = [y[(-j) % NCH] for j in range(NCH)]
                b0, b1, b2 = (sh & 1) != 0, (sh & 2) != 0, (sh & 4) != 0
                out = (2 * n, 2 * n + 4)
                v = {j: jnp.where(b0, u[(j - 1) % NCH], u[j]) for j in (0, 2, 4, 6)}
                v = {j: jnp.where(b1, v[(j - 2) % NCH], v[j]) for j in out}
                v = {j: jnp.where(b2, v[(j - 4) % NCH], v[j]) for j in out}
                return [pltpu.roll(v[j], (2 * NL - 2 * j - 2 * par) % NL, 1) for j in out]

            items = []
            for g in range(KH // 16):
                st = {}
                for half in range(2):
                    def s0(val, r=half * KH + g * 16, st=st, half=half):
                        anchor(rq.at[0], D, val, z)
                        st["a", half] = perm_a(r)

                    def s1(val, st=st, half=half):
                        st["b", half] = perm_b(st["a", half])

                    def s2(val, r=g * 16, st=st):
                        ops = _ops(_B_TERMS, *[wide(w) for w in st["b", 0] + st["b", 1]])
                        for i in range(7):
                            BQ.at[i][pl.ds(r, 16), ch(n)] = ops[i].astype(BF16)
                        if chain:
                            anchor(rq.at[0], D, (ops[5] + ops[6])[0:8], z)
                    items.append([s0, s1] + ([s2] if half else []))
            flat = _skew(items)
            firsts = [j for j, t in enumerate(flat) if t.__name__ == "s0"] + [len(flat)]
            return [(lambda val, grp=flat[a:b]: [t(val) for t in grp]) for a, b in zip(firsts, firsts[1:])]

        def prep_o_tasks(src, n, z):
            def transpose(c, a):
                sub = lax.broadcasted_iota(jnp.int32, (8, NL), 0)
                y = [pltpu.bitcast(rq[src + c, pl.ds(128 * g + 16 * a, 16), :], U32) for g in range(8)]
                y = [y[0]] + [pltpu.roll(y[g], g, 0) for g in range(1, 8)]
                v = [y[(-j) % 8] for j in range(8)]
                for bit in (1, 2, 4):
                    v = [jnp.where((sub & bit) != 0, v[(j - bit) % 8], v[j]) for j in range(8)]
                return [v[0]] + [pltpu.roll(v[j], 8 - j, 0) for j in range(1, 8)]

            tasks = []
            for a in range(8):
                st = {}

                def load(val, h, a=a, st=st):
                    anchor(rq.at[0], D, val, z)
                    st[h] = transpose(h * KC + n, a)

                def quad(val, jj, a=a, st=st):
                    pace = jnp.where(z != 0, pltpu.bitcast(val, U32), jnp.uint32(0))
                    q = [wide(st[h][kh * KC + jj] | pace) for kh in range(2) for h in range(2)]
                    for i, op in enumerate(_ops(_B_TERMS, *q)):
                        BO.at[i][pl.ds(jj * NL + 16 * a, 16), ch(n)] = op.astype(BF16)
                tasks += [lambda val, f=load: f(val, 0), lambda val, f=load: f(val, 1)]
                tasks += [(lambda val, g=quad, jj=jj: g(val, jj)) for jj in range(KC)]
            return tasks

        def zero_p_tasks(u0, n, z):
            def task(val, u):
                v = jnp.where(z != 0, val, 0.0)
                P[u // 32, pl.ds(pl.multiple_of((u % 32) * 32, 32), 32), :] = jnp.tile(v, (4, KC))
            return [(lambda val, u=u0 + j: task(val, u)) for j in range(n)]

        def up1(r0, m):
            g = {}

            def fin_u(k, u):
                HF[pl.ds((k // 2) * HS + r0, m), ch(k % 2)] = gelu2(g[k], u)
            yield from _strassen(lambda i: _dot(XA[i, pl.ds(r0, m), :], B0[i, :, ch(0)]), g.__setitem__, ROOM_G, lazy=True)
            yield from _strassen(lambda i: _dot(XA[i, pl.ds(r0, m), :], B0[i, :, ch(1)]), fin_u, ROOM_U, lazy=True)

        groups = [lambda: [cp_x(0, 0), cp_x(0, 1)], lambda: [cp_gu(0, 0, 0)], lambda: [cp_gu(0, 0, 1)]]
        groups += [(lambda i=i: [cp_x(i, 0), cp_x(i, 1)]) for i in range(1, NT0)]
        groups += [lambda: [cp_q(0)], lambda: [cp_gu(1, 1, 0), cp_gu(1, 1, 1), cp_d(0)],
                   lambda: [cp_q(1)], lambda: [cp_o()], lambda: [cp_q(2)]]

        def issue(k, c):
            for g, cps in enumerate(groups):
                when(k == g, lambda: [cp.start() for cp in cps()])
            return c
        lax.fori_loop(0, len(groups), issue, 0)
        cp_x(0, 0).wait(); cp_x(0, 1).wait()

        def ln0(g, c):
            for t in ln_tasks(pl.multiple_of(g * 64, 64), 64, None):
                t(None)
            return c
        lax.fori_loop(0, T0 // 64, ln0, 0)
        for which in range(2):
            cp_gu(0, 0, which).wait()

            def pg0(g, c):
                prep_g1(which, pl.multiple_of(g * 64, 64), 64)
                return c
            lax.fori_loop(0, KH // 64, pg0, 0)

        def p0_body(i, c):
            cp_x(i + 1, 0).wait(); cp_x(i + 1, 1).wait()
            r0 = pl.multiple_of(i * T0, T0)
            _emit(2, up1(r0, T0), sum(ROOM_G) + sum(ROOM_U), (0.0, 0.85, ln_tasks(r0 + T0, T0, zero(i))))
            return zero(i)
        z0 = lax.fori_loop(0, NT0 - 1, p0_body, 0)
        cp_q(0).wait()
        cp_gu(2, 0, 0).start(); cp_gu(2, 0, 1).start()
        _emit(1, up1(HS - T0, T0), sum(ROOM_G) + sum(ROOM_U), (0.0, 0.9, prep_q_tasks(0, 0, 0, z0, chain=False)))

        def p1_body(b, c):
            when(b == 0, lambda: (cp_gu(1, 1, 0).wait(), cp_gu(1, 1, 1).wait(), cp_d(0).wait()))
            when(b == 1, lambda: cp_q(1).wait())
            when(b == 2, lambda: cp_o().wait())
            when(b == 3, lambda: cp_q(2).wait())
            m = b // 2
            par = b % 2

            def main():
                for n in range(2):
                    for s in range(HS // RH):
                        r0 = s * RH

                        def fin(k, v):
                            j = m * NCH + par + 2 * n + 4 * (k % 2)
                            qkv[j, pl.ds(HALO + (k // 2) * HS + r0, RH), :] = v
                        yield from _strassen(lambda i: _dot(XA[i, pl.ds(r0, RH), :], BQ[i, :, ch(n)]), fin, (1,) * 7)
            piece = jnp.clip(b - 2, 0, 3)
            z = zero(b)
            _emit(1, main(), 14 * (HS // RH),
                  (0.0, 0.48, prep_q_tasks(m, par, 1, z)),
                  (0.5, 0.98, prep_q_tasks(jnp.minimum((b + 1) // 2, 2), (b + 1) % 2, 0, z)),
                  (0.0, 0.95, prep_g2_tasks(1, range(7), pl.multiple_of(jnp.minimum(b * 48, KQ - 48), 16), 48, z)),
                  (0.0, 0.95, xb_tasks(pl.multiple_of(jnp.minimum(b * 96, QS - 96), 32), 96, z)),
                  (0.0, 0.95, prep_d2_tasks(pl.multiple_of(jnp.clip(b * 16, 0, NL - PDN - 16), 16), 16, z)),
                  (0.0, 0.95, zero_p_tasks(jnp.minimum(b * 38, 224 - 38), 38, z)),
                  (0.0, 0.95, prep_o_tasks(jnp.where(b < 2, 0, 3 * NCH), piece, z)))
            return c
        lax.fori_loop(0, 6, p1_body, 0)
        for j in range(NCH, 3 * NCH):
            qkv[j, 0:HALO, :] = jnp.broadcast_to(qkv[j, HALO:HALO + 1, :], (HALO, NL))

    def second_half(HA, osc, obuf):
        HA = HA.bitcast(BF16)

        def attn_unit(t0, r0, masked, slot, z, G, g0, gap):
            st = {}
            sh = 4 * (G - 1)

            def shifted(plane):
                return [qkv[plane, pl.ds(t0 + (r0 + HALO + 2 * sh - DIL * k), 8), :] for k in range(W + sh)]

            def logits(val, j):
                anchor(qkv.at[0], HALO + S, val, z)
                q = [qkv[j, pl.ds(t0 + (r0 + HALO + 8 * g), 8), :] for g in range(G)]
                kk = shifted(NCH + j)
                for g in range(G):
                    for w in range(W):
                        t = q[g] * kk[w + sh - 4 * g]
                        st[g, w] = t if j == 0 else st[g, w] + t
                if j == NCH - 1:
                    softmax()
                else:
                    vals = [st[0, W - 1]] if G == 1 else [st[g, w] for g in range(G) for w in range(0, W, 2)]
                    while len(vals) > 1:
                        vals = [vals[i] + vals[i + 1] for i in range(0, len(vals), 2)]
                    anchor(qkv.at[0], HALO + S + 8, vals[0], z)

            def softmax():
                lane = lax.broadcasted_iota(jnp.int32, (8, NL), 1)
                odd = (lane & 1) != 0
                hi = (lane & 16) != 0
                keys = [(g, w) for g in range(G) for w in range(W)]
                for k in keys:
                    a = st[k]
                    st[k] = a + jnp.where(odd, pltpu.roll(a, 1, 1), pltpu.roll(a, NL - 1, 1))
                for k in keys:
                    a = st[k]
                    st[k] = a + jnp.where(hi, pltpu.roll(a, 16, 1), pltpu.roll(a, NL - 16, 1))
                for g in range(G):
                    ls = [st[g, w] for w in range(W)]
                    if masked:
                        pos = t0 + (r0 + 8 * g) + lax.broadcasted_iota(jnp.int32, (8, NL), 0)
                        ls = [ls[0]] + [jnp.where(pos >= DIL * w, ls[w], NEG) for w in range(1, W)]
                    m = ls[0]
                    for w in range(1, W):
                        m = jnp.maximum(m, ls[w])
                    ps = [jnp.exp2((l - m) * EXP2_SCALE) for l in ls]
                    den = ps[0]
                    for w in range(1, W):
                        den = den + ps[w]
                    inv = 1.0 / den
                    for w in range(W):
                        st[g, w] = ps[w] * inv

            def pv(val, j):
                anchor(qkv.at[0], HALO + S, val, z)
                vv = shifted(2 * NCH + j)
                for g in range(G):
                    a = st[g, 0] * vv[sh - 4 * g]
                    for w in range(1, W):
                        a = a + st[g, w] * vv[w + sh - 4 * g]
                    osc[slot, j, pl.ds(8 * (g0 + g), 8), :] = a

            return ([(lambda val, j=j: logits(val, j)) for j in range(NCH)] + [lambda val: None] * gap
                    + [(lambda val, j=j: pv(val, j)) for j in range(NCH)])

        def attn_tasks(t0, n, z, G, gap):
            t0 = pl.multiple_of(jnp.minimum(t0, HS - n), 16)
            tasks = []
            for g in range(n // 16):
                r = g * 16
                for half in range(2):
                    for g0 in range(0, 2, G):
                        tasks += attn_unit(t0, half * HS + r + 8 * g0, g == 0 and half == 0, 2 * g + half, z, G, g0, gap)

                def oa(val, kc, g=g, r=r):
                    ops = _ops(_A_TERMS, osc[2 * g, kc], osc[2 * g, KC + kc],
                               osc[2 * g + 1, kc], osc[2 * g + 1, KC + kc])
                    for i in range(7):
                        OA.at[i][pl.ds(t0 + r, 16), ch(kc)] = ops[i].astype(BF16)
                tasks += [(lambda val, kc=kc, oa=oa: oa(val, kc)) for kc in range(KC)]
            return tasks

        def ha_task(val, r, i, z, have):
            anchor(HF, S, val, z)
            x = [_combine(_A_TERMS[i], lambda sg, kp: HF[pl.ds((2 * sg + rho) * QS + r, 16), ch(2 * kp + ta)])
                 for rho in range(2) for ta in range(2)]
            for k, op in enumerate(_ops(_A_TERMS, *x)):
                HA[pl.ds(r, 16), ch(7 * i + k)] = op.astype(BF16)
            have.add((i, r))

        def up2(kp, free, on_half):
            def sub(r0, m):
                hold, seen = {}, set()

                def outer_fin(k, K, v):
                    if K in (2, 1):
                        hold[k] = v
                        return
                    sg = K // 2
                    HF[pl.ds((2 * sg + k // 2) * QS + r0, m), ch(2 * kp + k % 2)] = (
                        gelu2(hold[k], v) if K == 3 else gelu2(v, hold[k]))
                    seen.add((sg, k))
                    if all((sg, j) in seen for j in range(4)):
                        on_half(sg, r0, m)
                folds = [_Fold(lambda K, v, k=k: outer_fin(k, K, v), lazy=True) for k in range(4)]

                def lhs(i, k):
                    if k == 2:
                        return XA[i, pl.ds(r0, m), pl.ds(0, KQ)]
                    if k == 3:
                        return XA[i, pl.ds(QS + r0, m), pl.ds(KQ, KQ)]
                    return XB[5 * i + _XB_SLOT[k], pl.ds(r0, m), :]
                return lambda i: _strassen(lambda k: _dot(lhs(i, k), BG[i, :, ch(k)]),
                                           lambda k, v: folds[k](i, v), ROOM_H if i in (2, 6) else ROOM_L)
            subs = [sub(s * RH2, RH2) for s in range(QS // RH2)]
            for i in _ORDER:
                for sb in subs:
                    yield from sb(i)
                free.add(i)

        nsub = QS // RH2
        g_room = (5 * sum(ROOM_L) + 2 * sum(ROOM_H)) * nsub
        d_unit = 2.5 * MD * ND / (RH2 * KQ)

        ends = [sum(sum(ROOM_H if i in (2, 6) else ROOM_L) for i in _ORDER[:j + 1]) * nsub for j in range(7)]

        def bg_sides(slot, total, z, free, n):
            return [((ends[j] + 1) / total, (ends[j + 1] if j < 6 else ends[6] + ends[0]) / total - 0.01,
                     prep_g2_tasks(slot, _ORDER[j:j + 1], 0, KQ, z, free)) for j in range(n)]

        def block_b(k):
            when(k < NP - 1, lambda: (cp_gu(0, 0, 0).wait(), cp_gu(0, 0, 1).wait()))

            z = zero(k)
            free, have, halves, pending = set(), set(), set(), set()

            def reads_old(tasks):
                pending.update(tasks)
                return [(lambda val, t=t: (t(val), pending.discard(t))) for t in tasks]

            def prefetch(val):
                assert not pending
                when(k < NP - 1, lambda: (cp_gu(2 * k + 3, 1, 0).start(), cp_gu(2 * k + 3, 1, 1).start(),
                                          cp_d(k + 1).start()))

            def on_half(sg, r0, m):
                if r0 + m == QS:
                    halves.add(sg)

            def ha_tasks(outer, need):
                def task(val, r, i):
                    assert need <= halves
                    ha_task(val, r, i, z, have)
                return [(lambda val, r=r, i=i: task(val, r, i)) for i in outer for r in range(0, QS, 16)]

            def main():
                yield from up2(1, free, on_half)
                for i in (2, 5, 1, 3, 0, 4, 6):
                    assert all((i, r) in have for r in range(0, QS, 16))
                    for r0 in range(0, QS, MD):
                        for c in range(KQ // ND):
                            def fin(q, v):
                                P[i, pl.ds((q // 2) * QS + r0, MD), pl.ds((q % 2) * KQ + c * ND, ND)] += v
                            yield from _strassen(
                                lambda j: _dot(HA[pl.ds(r0, MD), ch(7 * i + j)], BD[7 * i + j, :, ch(c, ND)]),
                                fin, (d_unit,) * 7)
            total = g_room + 49 * (QS // MD) * (KQ // ND) * d_unit
            gf = g_room / total
            df = (1 - gf) / 7
            _emit(5, main(), total, *bg_sides(0, total, z, free, 7),
                  (0.0, ends[0] / total, reads_old(prep_g2_tasks(1, _ORDER[6:], 0, KQ, z))),
                  (0.0, 0.9 * gf, ha_tasks((2, 5), set())),
                  ((ends[4] + 1) / total, gf + 1.6 * df, ha_tasks((1, 3, 0), {1})),
                  (gf + 1.6 * df, gf + 5.5 * df, ha_tasks((4, 6), {0, 1})),
                  (0.0, 0.8 * gf, reads_old(prep_d2_tasks(NL - PDN, PDN, z))),
                  (0.0, 0.98, attn_tasks(k * (APA + APB), APB, z, 1, 10)),
                  (gf, gf + 0.01, [prefetch]))

        def block_a(k):
            cp_gu(0, 1, 0).wait(); cp_gu(0, 1, 1).wait(); cp_d(0).wait()

            def prefetch(val):
                when(k < NP - 2, lambda: (cp_gu(2 * k + 4, 0, 0).start(), cp_gu(2 * k + 4, 0, 1).start()))
            z = zero(k)
            free = set()
            _emit(4, up2(0, free, lambda *a: None), g_room, *bg_sides(1, g_room, z, free, 6),
                  (0.0, 0.97, prep_d2_tasks(0, NL - PDN, z)),
                  (0.0, 0.95, attn_tasks(k * (APA + APB) + APB, APA, z, 2, 5)),
                  (0.01, 0.02, [prefetch]))

        def p2_body(k, carry):
            block_b(k)
            when(k < NP - 1, lambda: block_a(k))
            return carry
        lax.fori_loop(0, NP, p2_body, 0)

        def cp_out(t, half, s):
            return pltpu.make_async_copy(obuf.at[t % 2, half, pl.ds(s * M3, M3), :],
                                         out_hbm.at[pl.ds(half * HS + t * T3 + s * M3, M3), :], sem_out.at[t % 2])

        def wait_out(t):
            pltpu.make_async_copy(obuf.at[t % 2], obuf.at[t % 2], sem_out.at[t % 2]).wait()

        def p3_body(t, carry):
            when(t >= 2, lambda: wait_out(t - 2))
            for s in range(T3 // M3):
                r0 = pl.multiple_of(t * T3 + s * M3, M3)
                for n in range(KC):
                    def fin(k, sq):
                        (j0, _), *rest = _C_TERMS[k]
                        f = P[j0, pl.ds(r0, M3), ch(n)]
                        for j, sign in rest:
                            f = f + P[j, pl.ds(r0, M3), ch(n)] if sign > 0 else f - P[j, pl.ds(r0, M3), ch(n)]
                        y = f * 0.25
                        half, col = k // 2, (k % 2) * KC + n
                        x = xbuf[pl.ds(half * HS + r0, M3), ch(col)].astype(F32)
                        obuf.at[t % 2, half][pl.ds(s * M3, M3), ch(col)] = (
                            x + sq * (y + y * jnp.tanh(y))).astype(BF16)
                    for step, _ in enumerate(_strassen(
                            lambda i: _dot(OA[i, pl.ds(r0, M3), :], BO[i, :, ch(n)]), fin, (1,) * 7)):
                        if s > 0 and n == 0 and step == 1:
                            cp_out(t, 0, s - 1).start(); cp_out(t, 1, s - 1).start()
            cp_out(t, 0, T3 // M3 - 1).start(); cp_out(t, 1, T3 // M3 - 1).start()
            return carry
        lax.fori_loop(0, NT3, p3_body, 0)
        for t in range(NT3 - 2, NT3):
            wait_out(t)

    pl.run_scoped(first_half,
                  pltpu.VMEM((7, KH // 2, 2 * NL), U32),
                  pltpu.VMEM((7, KH // 2, 2 * NL), U32))
    pl.run_scoped(second_half,
                  pltpu.VMEM((QS // 2, 49 * NL), U32),
                  pltpu.VMEM((max(APA, APB) // 8, NCH, 16, NL), F32),
                  pltpu.VMEM((2, 2, T3, D), BF16))


@jax.jit
def pallas_recurrent_scan__sliding_local_dilated__geglu_ffn__prompt_kernel(
    A_x: jax.Array,
    A_wqkv: jax.Array,
    A_wo: jax.Array,
    B_x: jax.Array,
    B_w_gate: jax.Array,
    B_w_up: jax.Array,
    B_w_down: jax.Array,
):
    del B_x
    x = A_x.reshape(S, D)
    anyspec = pl.BlockSpec(memory_space=pl.ANY)
    out = pl.pallas_call(
        _kernel,
        in_specs=[anyspec] * 6,
        out_specs=anyspec,
        out_shape=jax.ShapeDtypeStruct((S, D), BF16),
        scratch_shapes=[
            pltpu.VMEM((S + SPARE, D), BF16),
            pltpu.VMEM((7, HS // 2, KH), U32),
            pltpu.VMEM((35, QS // 2, KQ), U32),
            pltpu.VMEM((3 * NCH, HALO + S + SPARE, NL), F32),
            pltpu.VMEM((7, HS, KH), F32),
            pltpu.VMEM((S + SPARE, 2 * FC), F32),
            pltpu.VMEM((7, KQ // 2, 7 * NL), U32),
            pltpu.VMEM((49, NL // 2, KQ), U32),
            pltpu.VMEM((7, KH // 2, KH), U32),
            pltpu.VMEM((6, D + 64, FC), BF16),
            pltpu.VMEM((S + SPARE, D), F32),
            pltpu.VMEM((4 * NCH, D + 64, NL), BF16),
            pltpu.VMEM((7, HS // 2, KH), U32),
            pltpu.SemaphoreType.DMA((NT0, 2)),
            pltpu.SemaphoreType.DMA((2, 2)),
            pltpu.SemaphoreType.DMA((1,)),
            pltpu.SemaphoreType.DMA((3,)),
            pltpu.SemaphoreType.DMA((1,)),
            pltpu.SemaphoreType.DMA((2,)),
        ],
        compiler_params=pltpu.CompilerParams(vmem_limit_bytes=124 * 2 ** 20, disable_bounds_checks=True),
    )(x, A_wqkv, A_wo, B_w_gate, B_w_up, B_w_down)
    return out.reshape(1, S, D)
```

```python
import math

import jax
import jax.numpy as jnp
from jax import lax
import jax.experimental.pallas as pl
import jax.experimental.pallas.tpu as pltpu

S, D, F = 2048, 1024, 3584
H, DH, W, DIL = 32, 32, 8, 2
NL = 128
NCH = D // NL
HS = S // 2
KH = D // 2
KC = KH // NL
QS = S // 4
KQ = D // 4
FC = 256
NP = F // (2 * FC)
HALO = 16
SPARE = 48
F32, BF16, U32 = jnp.float32, jnp.bfloat16, jnp.uint32
EPS = 1e-5
GELU_C0 = math.sqrt(2.0 / math.pi)
GELU_C1 = GELU_C0 * 0.044715
EXP2_SCALE = (DH ** -0.5) * math.log2(math.e)
NEG = -1e9 / (DH ** -0.5)

_A_TERMS = (((0, 0, 1), (1, 1, 1)), ((1, 0, 1), (1, 1, 1)), ((0, 0, 1),), ((1, 1, 1),),
            ((0, 0, 1), (0, 1, 1)), ((1, 0, 1), (0, 0, -1)), ((0, 1, 1), (1, 1, -1)))
_B_TERMS = (((0, 0, 1), (1, 1, 1)), ((0, 0, 1),), ((0, 1, 1), (1, 1, -1)), ((1, 0, 1), (0, 0, -1)),
            ((1, 1, 1),), ((0, 0, 1), (0, 1, 1)), ((1, 0, 1), (1, 1, 1)))
_C_TERMS = (((0, 1), (3, 1), (4, -1), (6, 1)), ((2, 1), (4, 1)), ((1, 1), (3, 1)), ((0, 1), (1, -1), (2, 1), (5, 1)))
_ORDER = (1, 3, 0, 5, 2, 4, 6)
_XB_SLOT = {0: 0, 1: 1, 4: 2, 5: 3, 6: 4}


def _combine(terms, get):
    (r, c, _), *rest = terms
    v = get(r, c)
    for r, c, sign in rest:
        v = v + get(r, c) if sign > 0 else v - get(r, c)
    return v


def _ops(terms, q11, q12, q21, q22):
    q = ((q11, q12), (q21, q22))
    return [_combine(t, lambda r, c: q[r][c]) for t in terms]


def _dot(a, b):
    return jnp.dot(a, b, preferred_element_type=F32)


class _Fold:
    def __init__(self, fin, lazy=False):
        self.fin, self.lazy = fin, lazy

    def __call__(self, i, m):
        if self.lazy and i in (0, 5, 4):
            if i == 0:
                self.m0 = m
            elif i == 5:
                self.t22 = (m + self.m0) - self.m1
            else:
                self.fin(1, self.m2 + m)
                self.t11 = (self.m0 - m) + self.t11
        elif i == 1:
            self.m1 = m
        elif i == 3:
            self.fin(2, self.m1 + m)
            self.t11 = m
        elif i == 0:
            self.t11 = self.t11 + m
            self.t22 = m - self.m1
        elif i == 5:
            self.t22 = self.t22 + m
        elif i == 2:
            self.fin(3, self.t22 + m)
            self.m2 = m
        elif i == 4:
            self.fin(1, self.m2 + m)
            self.t11 = self.t11 - m
        else:
            self.fin(0, self.t11 + m)


def _strassen(prod, fin, room, lazy=False):
    fold = _Fold(fin, lazy)
    for step, i in enumerate(_ORDER):
        m = prod(i)
        fold(i, m)
        yield room[step], m


def _emit(lag, main, total, *sides):
    done = [0] * len(sides)
    acc = 0

    def flush(frac, val):
        due = []
        for k, (f0, f1, tasks) in enumerate(sides):
            want = len(tasks) if frac >= f1 else int(max(0.0, (frac - f0) / (f1 - f0)) * len(tasks) + 0.5)
            n = min(want, len(tasks)) - done[k]
            due += [((j + 0.5) / n, k, tasks[done[k] + j]) for j in range(n)]
            done[k] += max(n, 0)
        due.sort(key=lambda e: e[:2])
        for j, (_, _, task) in enumerate(due):
            r = (val.shape[0] // 8) * j // len(due) * 8
            task(val[r:r + 8, 0:NL])

    hist = [(0, None)] * lag
    for item in main:
        hist.append(item)
        room, val = hist.pop(0)
        acc += room
        if room:
            flush(acc / total, val)
    assert abs(acc + sum(h[0] for h in hist) - total) < 1e-6
    flush(2.0, hist[-1][1])


def _skew(items):
    depth = max(len(st) for st in items)
    return [items[t - k][k] for t in range(len(items) + depth - 1) for k in range(depth)
            if 0 <= t - k < len(items) and k < len(items[t - k]) and items[t - k][k] is not None]


T0, NT0 = 128, 8
RH = 256
RH2 = 64
MD, ND = 128, 128
T3, NT3, M3 = 256, 4, 64
APB, APA = 96, 64
PDN = 48
ROOM_G, ROOM_U = (2,) * 7, (2, 2, 2, 2, 1, 1, 1)
ROOM_L, ROOM_H = (2,) * 7, (2, 0, 2, 2, 0, 0, 0)
assert (NP - 1) * APA + NP * APB >= HS and APA % 32 == 0 and APB % 32 == 0


def _kernel(x_hbm, wqkv_hbm, wo_hbm, wg_hbm, wu_hbm, wd_hbm, out_hbm,
            xbuf, XA, XB, qkv, P, HF, BG, BD, BO, rw, Y, rq, OA,
            sem_x, sem_gu, sem_d, sem_q, sem_o, sem_out):

    XA, XB, BG, BD, BO, OA = [r.bitcast(BF16) for r in (XA, XB, BG, BD, BO, OA)]

    def ch(n, w=NL):
        return pl.ds(n * w, w) if isinstance(n, int) else pl.ds(pl.multiple_of(n * w, w), w)

    def zero(i):
        return i % 2 + (i + 1) % 2 - 1

    def when(pred, fn):
        pl.when(pred)(lambda: (fn(), None)[1])

    def cp_x(i, half):
        r = half * HS + i * T0
        return pltpu.make_async_copy(x_hbm.at[pl.ds(r, T0), :], xbuf.at[pl.ds(r, T0), :], sem_x.at[i, half])

    def cp_gu(c, slot, which):
        src = wg_hbm if which == 0 else wu_hbm
        return pltpu.make_async_copy(src.at[:, pl.ds(c * FC, FC)], rw.at[2 * slot + which, pl.ds(0, D), :],
                                     sem_gu.at[slot, which])

    class cp_d:
        def __init__(self, p):
            self.p = p

        def start(self):
            for q in range(4):
                pltpu.make_async_copy(wd_hbm.at[pl.ds(self.p * 2 * FC, 2 * FC), pl.ds(q * KQ, KQ)],
                                      rw.at[4 + q // 2, pl.ds((q % 2) * 2 * FC, 2 * FC), :], sem_d.at[0]).start()

        def wait(self):
            whole = rw.at[pl.ds(4, 2), pl.ds(0, D), :]
            pltpu.make_async_copy(whole, whole, sem_d.at[0]).wait()

    def anchor(dst, row, val, z):
        if val is not None and z is not None:
            r = pl.multiple_of(row + 16 + z * 16, 8)
            dst[pl.ds(r, 8), pl.ds(0, NL)] = val.astype(dst.dtype)

    def gelu2(g, u):
        t = jnp.tanh(g * (GELU_C0 + GELU_C1 * (g * g)))
        p = g * u
        return p + p * t

    def prep_g2_tasks(slot, outer, r0, n, z, free=None):
        def task(val, r, i):
            assert free is None or i in free
            anchor(rw.at[0], D, val, z)
            y = [_combine(_B_TERMS[i], lambda kp, mu: rw[2 * slot + mu, pl.ds((2 * kp + ta) * KQ + r, 16), :].astype(F32))
                 for ta in range(2)]
            ops = _ops(_B_TERMS, y[0][:, :NL], y[0][:, NL:], y[1][:, :NL], y[1][:, NL:])
            for k in range(7):
                BG.at[i][pl.ds(r, 16), ch(k)] = ops[k].astype(BF16)
        return [(lambda val, r=r0 + g * 16, i=i: task(val, r, i)) for i in outer for g in range(n // 16)]

    def prep_d2_tasks(r0, n, z):
        def task(val, r, i, c):
            anchor(rw.at[0], D, val, z)
            y = [_combine(_B_TERMS[i],
                          lambda kp, nu: rw[4 + nu, pl.ds(up * 2 * FC + (2 * kp + ta) * NL + r, 16), ch(c)].astype(F32))
                 for ta in range(2) for up in range(2)]
            ops = _ops(_B_TERMS, *y)
            for k in range(7):
                BD.at[7 * i + k][pl.ds(r, 16), ch(c)] = ops[k].astype(BF16)
        return [(lambda val, r=r0 + g * 16, i=i, c=c: task(val, r, i, c))
                for g in range(n // 16) for i in range(7) for c in range(2)]

    def first_half(B0, BQ, WP):
        B0, BQ = B0.bitcast(BF16), BQ.bitcast(BF16)

        class cp_cols:
            def __init__(self, src, col0, dst, slot0, sem):
                self.args = src, col0, dst, slot0, sem

            def start(self):
                src, col0, dst, slot0, sem = self.args
                for k in range(NCH):
                    pltpu.make_async_copy(src.at[:, pl.ds(col0 + k * NL, NL)],
                                          dst.at[slot0 + k, pl.ds(0, D), :], sem).start()

            def wait(self):
                _, _, dst, slot0, sem = self.args
                whole = dst.at[pl.ds(slot0, NCH), pl.ds(0, D), :]
                pltpu.make_async_copy(whole, whole, sem).wait()

        def cp_q(m):
            return cp_cols(wqkv_hbm, m * D, rq, m * NCH, sem_q.at[m])

        def cp_o():
            return cp_cols(wo_hbm, 0, rq, 3 * NCH, sem_o.at[0])

        def ln_tasks(r0, n, z):
            def xrow(r):
                return xbuf[pl.ds(r, 16), :].astype(F32)
            items = []
            for g in range(n // 16):
                st = {}
                for half in range(2):
                    def stats(val, r=half * HS + r0 + g * 16, st=st, half=half):
                        anchor(xbuf, S, val, z)
                        x = xrow(r)
                        m = jnp.sum(x, axis=-1, keepdims=True) * (1.0 / D)
                        e2 = jnp.sum(x * x, axis=-1, keepdims=True) * (1.0 / D)
                        st["m", half] = m
                        st["v", half] = lax.rsqrt(jnp.maximum(e2 - m * m, 0.0) + EPS)

                    def apply(val, r=r0 + g * 16, st=st, half=half):
                        for kc in (2 * half, 2 * half + 1):
                            anchor(xbuf, S, val, z)
                            pos = [(h, c) for h in range(2) for c in (kc, KC + kc)]
                            q = [(xbuf[pl.ds(h * HS + r, 16), ch(c)].astype(F32) - st["m", h]) * st["v", h]
                                 for h, c in pos]
                            for (h, c), y in zip(pos, q):
                                Y[pl.ds(h * HS + r, 16), ch(c)] = y
                            for i, op in enumerate(_ops(_A_TERMS, *q)):
                                XA.at[i][pl.ds(r, 16), ch(kc)] = op.astype(BF16)
                    items.append([stats] + [None] * (2 - half) + [apply])
            return _skew(items)

        def prep_g1(which, r0, n):
            for g in range(n // 16):
                r = r0 + g * 16
                top = rw[which, pl.ds(r, 16), :].astype(F32)
                bot = rw[which, pl.ds(KH + r, 16), :].astype(F32)
                for i, op in enumerate(_ops(_B_TERMS, top[:, :NL], top[:, NL:], bot[:, :NL], bot[:, NL:])):
                    B0.at[i][pl.ds(r, 16), ch(which)] = op.astype(BF16)

        def xb_tasks(r0, n, z):
            def task(val, r, kc, i):
                anchor(Y, S, val, z)
                x = [_combine(_A_TERMS[i],
                              lambda sg, kp: Y[pl.ds((2 * sg + rho) * QS + r, 16), ch(4 * kp + 2 * ta + kc)])
                     for rho in range(2) for ta in range(2)]
                ops = _ops(_A_TERMS, *x)
                for k, slot in _XB_SLOT.items():
                    XB.at[5 * i + slot][pl.ds(r, 16), ch(kc)] = ops[k].astype(BF16)
            return [(lambda val, r=r0 + g * 16, kc=kc, i=i: task(val, r, kc, i))
                    for g in range(n // 16) for kc in range(2) for i in range(7)]

        def wide(w):
            return pltpu.bitcast(w, BF16).astype(F32)

        def prep_q_tasks(m, par, n, z, chain=True):
            def perm_a(r):
                y = [pltpu.bitcast(rq[m * NCH + k, pl.ds(r, 16), :], U32) for k in range(NCH)]
                return [y[0]] + [pltpu.roll(y[k], 2 * k, 1) for k in range(1, NCH)]

            def perm_b(y):
                lane = lax.broadcasted_iota(jnp.int32, (8, NL), 1)
                sh = (((lane & 15) >> 1) - par) & 7
                u = [y[(-j) % NCH] for j in range(NCH)]
                b0, b1, b2 = (sh & 1) != 0, (sh & 2) != 0, (sh & 4) != 0
                out = (2 * n, 2 * n + 4)
                v = {j: jnp.where(b0, u[(j - 1) % NCH], u[j]) for j in (0, 2, 4, 6)}
                v = {j: jnp.where(b1, v[(j - 2) % NCH], v[j]) for j in out}
                v = {j: jnp.where(b2, v[(j - 4) % NCH], v[j]) for j in out}
                return [pltpu.roll(v[j], (2 * NL - 2 * j - 2 * par) % NL, 1) for j in out]

            items = []
            for g in range(KH // 16):
                st = {}
                for half in range(2):
                    def s0(val, r=half * KH + g * 16, st=st, half=half):
                        anchor(rq.at[0], D, val, z)
                        st["a", half] = perm_a(r)

                    def s1(val, st=st, half=half):
                        st["b", half] = perm_b(st["a", half])

                    def s2(val, r=g * 16, st=st):
                        ops = _ops(_B_TERMS, *[wide(w) for w in st["b", 0] + st["b", 1]])
                        for i in range(7):
                            BQ.at[i][pl.ds(r, 16), ch(n)] = ops[i].astype(BF16)
                        if chain:
                            anchor(rq.at[0], D, (ops[5] + ops[6])[0:8], z)
                    items.append([s0, s1] + ([s2] if half else []))
            flat = _skew(items)
            firsts = [j for j, t in enumerate(flat) if t.__name__ == "s0"] + [len(flat)]
            return [(lambda val, grp=flat[a:b]: [t(val) for t in grp]) for a, b in zip(firsts, firsts[1:])]

        def prep_o_tasks(src, n, z):
            h, c = n // 2, n % 2

            def load(val, u, q):
                anchor(rq.at[0], D, val, z)
                sub = lax.broadcasted_iota(jnp.int32, (8, NL), 0)
                rows = rq.at[src + (2 * q + c), pl.ds(pl.multiple_of(h * 64, 64), D - 64), :]
                y = [pltpu.bitcast(rows[pl.ds(128 * g + 16 * u, 16), :], U32) for g in range(8)]
                y = [y[0]] + [pltpu.roll(y[g], g, 0) for g in range(1, 8)]
                v = [y[(-j) % 8] for j in range(8)]
                for bit in (1, 2, 4):
                    v = [jnp.where((sub & bit) != 0, v[(j - bit) % 8], v[j]) for j in range(8)]
                for j, w in enumerate([v[0]] + [pltpu.roll(v[j], 8 - j, 0) for j in range(1, 8)]):
                    WP[4 * u + q, pl.ds(8 * j, 8), :] = w

            def ops(val, u, jj, i):
                WP[16, pl.ds(pl.multiple_of(16 + z * 8, 8), 8), :] = pltpu.bitcast(val, U32)
                y = [_combine(_B_TERMS[i],
                              lambda kp, nu: wide(WP[4 * u + 2 * nu + up, pl.ds(8 * (4 * kp + 2 * ta + jj), 8), :]))
                     for ta in range(2) for up in range(2)]
                r = pl.multiple_of(h * 64, 64) + (jj * NL + 16 * u)
                for k, op in enumerate(_ops(_B_TERMS, *y)):
                    BO.at[7 * i + k][pl.ds(r, 16), ch(c)] = op.astype(BF16)

            tasks = []
            for u in range(4):
                tasks += [(lambda val, u=u, q=q: load(val, u, q)) for q in range(4)]
                tasks += [(lambda val, u=u, jj=jj, i=i: ops(val, u, jj, i)) for jj in range(2) for i in range(7)]
            return tasks

        def zero_p_tasks(u0, n, z):
            def task(val, u):
                v = jnp.where(z != 0, val, 0.0)
                P[u // 32, pl.ds(pl.multiple_of((u % 32) * 32, 32), 32), :] = jnp.tile(v, (4, KC))
            return [(lambda val, u=u0 + j: task(val, u)) for j in range(n)]

        def up1(r0, m):
            g = {}

            def fin_u(k, u):
                HF[pl.ds((k // 2) * HS + r0, m), ch(k % 2)] = gelu2(g[k], u)
            yield from _strassen(lambda i: _dot(XA[i, pl.ds(r0, m), :], B0[i, :, ch(0)]), g.__setitem__, ROOM_G, lazy=True)
            yield from _strassen(lambda i: _dot(XA[i, pl.ds(r0, m), :], B0[i, :, ch(1)]), fin_u, ROOM_U, lazy=True)

        groups = [lambda: [cp_x(0, 0), cp_x(0, 1)], lambda: [cp_gu(0, 0, 0)], lambda: [cp_gu(0, 0, 1)]]
        groups += [(lambda i=i: [cp_x(i, 0), cp_x(i, 1)]) for i in range(1, NT0)]
        groups += [lambda: [cp_q(0)], lambda: [cp_gu(1, 1, 0), cp_gu(1, 1, 1), cp_d(0)],
                   lambda: [cp_q(1)], lambda: [cp_o()], lambda: [cp_q(2)]]

        def issue(k, c):
            for g, cps in enumerate(groups):
                when(k == g, lambda: [cp.start() for cp in cps()])
            return c
        lax.fori_loop(0, len(groups), issue, 0)
        cp_x(0, 0).wait(); cp_x(0, 1).wait()

        def ln0(g, c):
            for t in ln_tasks(pl.multiple_of(g * 64, 64), 64, None):
                t(None)
            return c
        lax.fori_loop(0, T0 // 64, ln0, 0)
        for which in range(2):
            cp_gu(0, 0, which).wait()

            def pg0(g, c):
                prep_g1(which, pl.multiple_of(g * 64, 64), 64)
                return c
            lax.fori_loop(0, KH // 64, pg0, 0)

        def p0_body(i, c):
            cp_x(i + 1, 0).wait(); cp_x(i + 1, 1).wait()
            r0 = pl.multiple_of(i * T0, T0)
            _emit(2, up1(r0, T0), sum(ROOM_G) + sum(ROOM_U), (0.0, 0.85, ln_tasks(r0 + T0, T0, zero(i))))
            return zero(i)
        z0 = lax.fori_loop(0, NT0 - 1, p0_body, 0)
        cp_q(0).wait()
        cp_gu(2, 0, 0).start(); cp_gu(2, 0, 1).start()
        _emit(1, up1(HS - T0, T0), sum(ROOM_G) + sum(ROOM_U), (0.0, 0.9, prep_q_tasks(0, 0, 0, z0, chain=False)))

        def p1_body(b, c):
            when(b == 0, lambda: (cp_gu(1, 1, 0).wait(), cp_gu(1, 1, 1).wait(), cp_d(0).wait()))
            when(b == 1, lambda: cp_q(1).wait())
            when(b == 2, lambda: cp_o().wait())
            when(b == 3, lambda: cp_q(2).wait())
            m = b // 2
            par = b % 2

            def main():
                for n in range(2):
                    for s in range(HS // RH):
                        r0 = s * RH

                        def fin(k, v):
                            j = m * NCH + par + 2 * n + 4 * (k % 2)
                            qkv[j, pl.ds(HALO + (k // 2) * HS + r0, RH), :] = v
                        yield from _strassen(lambda i: _dot(XA[i, pl.ds(r0, RH), :], BQ[i, :, ch(n)]), fin, (1,) * 7)
            piece = jnp.clip(b - 2, 0, 3)
            z = zero(b)
            _emit(1, main(), 14 * (HS // RH),
                  (0.0, 0.48, prep_q_tasks(m, par, 1, z)),
                  (0.5, 0.98, prep_q_tasks(jnp.minimum((b + 1) // 2, 2), (b + 1) % 2, 0, z)),
                  (0.0, 0.95, prep_g2_tasks(1, range(7), pl.multiple_of(jnp.minimum(b * 48, KQ - 48), 16), 48, z)),
                  (0.0, 0.95, xb_tasks(pl.multiple_of(jnp.minimum(b * 96, QS - 96), 32), 96, z)),
                  (0.0, 0.95, prep_d2_tasks(pl.multiple_of(jnp.clip(b * 16, 0, NL - PDN - 16), 16), 16, z)),
                  (0.0, 0.95, zero_p_tasks(jnp.minimum(b * 38, 224 - 38), 38, z)),
                  (0.0, 0.95, prep_o_tasks(jnp.where(b < 2, 0, 3 * NCH), piece, z)))
            return c
        lax.fori_loop(0, 6, p1_body, 0)
        for j in range(NCH, 3 * NCH):
            qkv[j, 0:HALO, :] = jnp.broadcast_to(qkv[j, HALO:HALO + 1, :], (HALO, NL))

    def second_half(HA, osc, obuf):
        HA = HA.bitcast(BF16)

        def attn_unit(t0, r0, masked, slot, z, G, g0, gap):
            st = {}
            sh = 4 * (G - 1)

            def shifted(plane):
                return [qkv[plane, pl.ds(t0 + (r0 + HALO + 2 * sh - DIL * k), 8), :] for k in range(W + sh)]

            def logits(val, j):
                anchor(qkv.at[0], HALO + S, val, z)
                q = [qkv[j, pl.ds(t0 + (r0 + HALO + 8 * g), 8), :] for g in range(G)]
                kk = shifted(NCH + j)
                for g in range(G):
                    for w in range(W):
                        t = q[g] * kk[w + sh - 4 * g]
                        st[g, w] = t if j == 0 else st[g, w] + t
                if j == NCH - 1:
                    softmax()
                else:
                    vals = [st[0, W - 1]] if G == 1 else [st[g, w] for g in range(G) for w in range(0, W, 2)]
                    while len(vals) > 1:
                        vals = [vals[i] + vals[i + 1] for i in range(0, len(vals), 2)]
                    anchor(qkv.at[0], HALO + S + 8, vals[0], z)

            def softmax():
                lane = lax.broadcasted_iota(jnp.int32, (8, NL), 1)
                odd = (lane & 1) != 0
                hi = (lane & 16) != 0
                keys = [(g, w) for g in range(G) for w in range(W)]
                for k in keys:
                    a = st[k]
                    st[k] = a + jnp.where(odd, pltpu.roll(a, 1, 1), pltpu.roll(a, NL - 1, 1))
                for k in keys:
                    a = st[k]
                    st[k] = a + jnp.where(hi, pltpu.roll(a, 16, 1), pltpu.roll(a, NL - 16, 1))
                for g in range(G):
                    ls = [st[g, w] for w in range(W)]
                    if masked:
                        pos = t0 + (r0 + 8 * g) + lax.broadcasted_iota(jnp.int32, (8, NL), 0)
                        ls = [ls[0]] + [jnp.where(pos >= DIL * w, ls[w], NEG) for w in range(1, W)]
                    m = ls[0]
                    for w in range(1, W):
                        m = jnp.maximum(m, ls[w])
                    ps = [jnp.exp2((l - m) * EXP2_SCALE) for l in ls]
                    den = ps[0]
                    for w in range(1, W):
                        den = den + ps[w]
                    inv = 1.0 / den
                    for w in range(W):
                        st[g, w] = ps[w] * inv

            def pv(val, j):
                anchor(qkv.at[0], HALO + S, val, z)
                vv = shifted(2 * NCH + j)
                for g in range(G):
                    a = st[g, 0] * vv[sh - 4 * g]
                    for w in range(1, W):
                        a = a + st[g, w] * vv[w + sh - 4 * g]
                    osc[slot, j, pl.ds(8 * (g0 + g), 8), :] = a

            return ([(lambda val, j=j: logits(val, j)) for j in range(NCH)] + [lambda val: None] * gap
                    + [(lambda val, j=j: pv(val, j)) for j in range(NCH)])

        def attn_tasks(t0, n, z, G, gap):
            t0 = pl.multiple_of(jnp.minimum(t0, HS - n), 16)
            th = pl.multiple_of(t0 // 2, 16)

            def oa(val, u, kc, i):
                osc.at[osc.shape[0] - 1, 2 + z][pl.ds(0, 8), :] = val
                x = [_combine(_A_TERMS[i], lambda sg, kp: osc[2 * (2 * u + rho) + sg, 4 * kp + 2 * ta + kc])
                     for rho in range(2) for ta in range(2)]
                for k, op in enumerate(_ops(_A_TERMS, *x)):
                    OA.at[7 * i + k][pl.ds(th + u * 16, 16), ch(kc)] = op.astype(BF16)

            out, prev = [], []
            for u in range(n // 32):
                seg = [t for g in (2 * u, 2 * u + 1) for half in range(2) for g0 in range(0, 2, G)
                       for t in attn_unit(t0, half * HS + 16 * g + 8 * g0, g == 0 and half == 0, 2 * g + half,
                                          z, G, g0, gap)]
                for j, t in enumerate(seg):
                    out += [t] + prev[j * len(prev) // len(seg):(j + 1) * len(prev) // len(seg)]
                prev = [(lambda val, u=u, kc=kc, i=i: oa(val, u, kc, i)) for kc in range(2) for i in range(7)]
            return out + prev

        def ha_task(val, r, i, z, have):
            anchor(HF, S, val, z)
            x = [_combine(_A_TERMS[i], lambda sg, kp: HF[pl.ds((2 * sg + rho) * QS + r, 16), ch(2 * kp + ta)])
                 for rho in range(2) for ta in range(2)]
            for k, op in enumerate(_ops(_A_TERMS, *x)):
                HA[pl.ds(r, 16), ch(7 * i + k)] = op.astype(BF16)
            have.add((i, r))

        def up2(kp, free, on_half):
            def sub(r0, m):
                hold, seen = {}, set()

                def outer_fin(k, K, v):
                    if K in (2, 1):
                        hold[k] = v
                        return
                    sg = K // 2
                    HF[pl.ds((2 * sg + k // 2) * QS + r0, m), ch(2 * kp + k % 2)] = (
                        gelu2(hold[k], v) if K == 3 else gelu2(v, hold[k]))
                    seen.add((sg, k))
                    if all((sg, j) in seen for j in range(4)):
                        on_half(sg, r0, m)
                folds = [_Fold(lambda K, v, k=k: outer_fin(k, K, v), lazy=True) for k in range(4)]

                def lhs(i, k):
                    if k == 2:
                        return XA[i, pl.ds(r0, m), pl.ds(0, KQ)]
                    if k == 3:
                        return XA[i, pl.ds(QS + r0, m), pl.ds(KQ, KQ)]
                    return XB[5 * i + _XB_SLOT[k], pl.ds(r0, m), :]
                return lambda i: _strassen(lambda k: _dot(lhs(i, k), BG[i, :, ch(k)]),
                                           lambda k, v: folds[k](i, v), ROOM_H if i in (2, 6) else ROOM_L)
            subs = [sub(s * RH2, RH2) for s in range(QS // RH2)]
            for i in _ORDER:
                for sb in subs:
                    yield from sb(i)
                free.add(i)

        nsub = QS // RH2
        g_room = (5 * sum(ROOM_L) + 2 * sum(ROOM_H)) * nsub
        d_unit = 2.5 * MD * ND / (RH2 * KQ)

        ends = [sum(sum(ROOM_H if i in (2, 6) else ROOM_L) for i in _ORDER[:j + 1]) * nsub for j in range(7)]

        def bg_sides(slot, total, z, free, n):
            return [((ends[j] + 1) / total, (ends[j + 1] if j < 6 else ends[6] + ends[0]) / total - 0.01,
                     prep_g2_tasks(slot, _ORDER[j:j + 1], 0, KQ, z, free)) for j in range(n)]

        def block_b(k):
            when(k < NP - 1, lambda: (cp_gu(0, 0, 0).wait(), cp_gu(0, 0, 1).wait()))

            z = zero(k)
            free, have, halves, pending = set(), set(), set(), set()

            def reads_old(tasks):
                pending.update(tasks)
                return [(lambda val, t=t: (t(val), pending.discard(t))) for t in tasks]

            def prefetch(val):
                assert not pending
                when(k < NP - 1, lambda: (cp_gu(2 * k + 3, 1, 0).start(), cp_gu(2 * k + 3, 1, 1).start(),
                                          cp_d(k + 1).start()))

            def on_half(sg, r0, m):
                if r0 + m == QS:
                    halves.add(sg)

            def ha_tasks(outer, need):
                def task(val, r, i):
                    assert need <= halves
                    ha_task(val, r, i, z, have)
                return [(lambda val, r=r, i=i: task(val, r, i)) for i in outer for r in range(0, QS, 16)]

            def main():
                yield from up2(1, free, on_half)
                for i in (2, 5, 1, 3, 0, 4, 6):
                    assert all((i, r) in have for r in range(0, QS, 16))
                    for r0 in range(0, QS, MD):
                        for c in range(KQ // ND):
                            def fin(q, v):
                                P[i, pl.ds((q // 2) * QS + r0, MD), pl.ds((q % 2) * KQ + c * ND, ND)] += v
                            yield from _strassen(
                                lambda j: _dot(HA[pl.ds(r0, MD), ch(7 * i + j)], BD[7 * i + j, :, ch(c, ND)]),
                                fin, (d_unit,) * 7)
            total = g_room + 49 * (QS // MD) * (KQ // ND) * d_unit
            gf = g_room / total
            df = (1 - gf) / 7
            _emit(4, main(), total, *bg_sides(0, total, z, free, 7),
                  (0.0, ends[0] / total, reads_old(prep_g2_tasks(1, _ORDER[6:], 0, KQ, z))),
                  (0.0, 0.9 * gf, ha_tasks((2, 5), set())),
                  ((ends[4] + 1) / total, gf + 1.6 * df, ha_tasks((1, 3, 0), {1})),
                  (gf + 1.6 * df, gf + 5.5 * df, ha_tasks((4, 6), {0, 1})),
                  (0.0, 0.9 * gf, reads_old(prep_d2_tasks(NL - PDN, PDN, z))),
                  (0.0, 0.98, attn_tasks(k * (APA + APB), APB, z, 1, 10)),
                  (gf, gf + 0.01, [prefetch]))

        def block_a(k):
            cp_gu(0, 1, 0).wait(); cp_gu(0, 1, 1).wait(); cp_d(0).wait()

            def prefetch(val):
                when(k < NP - 2, lambda: (cp_gu(2 * k + 4, 0, 0).start(), cp_gu(2 * k + 4, 0, 1).start()))
            z = zero(k)
            free = set()
            _emit(4, up2(0, free, lambda *a: None), g_room, *bg_sides(1, g_room, z, free, 6),
                  (0.0, 0.97, prep_d2_tasks(0, NL - PDN, z)),
                  (0.0, 0.95, attn_tasks(k * (APA + APB) + APB, APA, z, 2, 5)),
                  (0.01, 0.02, [prefetch]))

        def p2_body(k, carry):
            block_b(k)
            when(k < NP - 1, lambda: block_a(k))
            return carry
        lax.fori_loop(0, NP, p2_body, 0)

        def cp_out(t, half, s):
            return pltpu.make_async_copy(obuf.at[t % 2, half, pl.ds(s * 2 * M3, 2 * M3), :],
                                         out_hbm.at[pl.ds(half * HS + t * T3 + s * 2 * M3, 2 * M3), :],
                                         sem_out.at[t % 2])

        def wait_out(t):
            pltpu.make_async_copy(obuf.at[t % 2], obuf.at[t % 2], sem_out.at[t % 2]).wait()

        def p3_body(t, carry):
            when(t >= 2, lambda: wait_out(t - 2))
            nsub3 = T3 // (2 * M3)
            for s in range(nsub3):
                ro = pl.multiple_of(t * (T3 // 2) + s * M3, M3)
                rh = pl.multiple_of(t * T3 + s * 2 * M3, 2 * M3)
                for c in range(2):
                    def outer_fin(k, K, v):
                        (j0, _), *rest = _C_TERMS[K]
                        half, pc = K // 2, 2 * (k % 2) + c
                        col = (K % 2) * KC + pc
                        for g in range(M3 // 16):
                            dr = 32 * g + 16 * (k // 2)
                            f = P[j0, pl.ds(rh + dr, 16), ch(pc)]
                            for j, sign in rest:
                                p = P[j, pl.ds(rh + dr, 16), ch(pc)]
                                f = f + p if sign > 0 else f - p
                            y = f * 0.25
                            x = xbuf[pl.ds(half * HS + rh + dr, 16), ch(col)].astype(F32)
                            obuf.at[t % 2, half][pl.ds(s * 2 * M3 + dr, 16), ch(col)] = (
                                x + v[16 * g:16 * g + 16] * (y + y * jnp.tanh(y))).astype(BF16)
                    folds = [_Fold(lambda K, v, k=k: outer_fin(k, K, v), lazy=True) for k in range(4)]
                    for step, i in enumerate(_ORDER):
                        for _ in _strassen(lambda k: _dot(OA[7 * i + k, pl.ds(ro, M3), :], BO[7 * i + k, :, ch(c)]),
                                           lambda k, v: folds[k](i, v), (1,) * 7):
                            pass
                        if c == 1 and step == 5:
                            cp_out(t, 1, s).start()
                        if c == 0 and step == 0 and s > 0:
                            cp_out(t, 0, s - 1).start()
            cp_out(t, 0, nsub3 - 1).start()
            return carry
        lax.fori_loop(0, NT3, p3_body, 0)
        for t in range(NT3 - 2, NT3):
            wait_out(t)

    pl.run_scoped(first_half,
                  pltpu.VMEM((7, KH // 2, 2 * NL), U32),
                  pltpu.VMEM((7, KH // 2, 2 * NL), U32),
                  pltpu.VMEM((17, 64, NL), U32))
    pl.run_scoped(second_half,
                  pltpu.VMEM((QS // 2, 49 * NL), U32),
                  pltpu.VMEM((max(APA, APB) // 8 + 1, NCH, 16, NL), F32),
                  pltpu.VMEM((2, 2, T3, D), BF16))


@jax.jit
def pallas_recurrent_scan__sliding_local_dilated__geglu_ffn__prompt_kernel(
    A_x: jax.Array,
    A_wqkv: jax.Array,
    A_wo: jax.Array,
    B_x: jax.Array,
    B_w_gate: jax.Array,
    B_w_up: jax.Array,
    B_w_down: jax.Array,
):
    del B_x
    x = A_x.reshape(S, D)
    anyspec = pl.BlockSpec(memory_space=pl.ANY)
    out = pl.pallas_call(
        _kernel,
        in_specs=[anyspec] * 6,
        out_specs=anyspec,
        out_shape=jax.ShapeDtypeStruct((S, D), BF16),
        scratch_shapes=[
            pltpu.VMEM((S + SPARE, D), BF16),
            pltpu.VMEM((7, HS // 2, KH), U32),
            pltpu.VMEM((35, QS // 2, KQ), U32),
            pltpu.VMEM((3 * NCH, HALO + S + SPARE, NL), F32),
            pltpu.VMEM((7, HS, KH), F32),
            pltpu.VMEM((S + SPARE, 2 * FC), F32),
            pltpu.VMEM((7, KQ // 2, 7 * NL), U32),
            pltpu.VMEM((49, NL // 2, KQ), U32),
            pltpu.VMEM((49, KQ // 2, KQ), U32),
            pltpu.VMEM((6, D + 64, FC), BF16),
            pltpu.VMEM((S + SPARE, D), F32),
            pltpu.VMEM((4 * NCH, D + 64, NL), BF16),
            pltpu.VMEM((49, QS // 2, KQ), U32),
            pltpu.SemaphoreType.DMA((NT0, 2)),
            pltpu.SemaphoreType.DMA((2, 2)),
            pltpu.SemaphoreType.DMA((1,)),
            pltpu.SemaphoreType.DMA((3,)),
            pltpu.SemaphoreType.DMA((1,)),
            pltpu.SemaphoreType.DMA((2,)),
        ],
        compiler_params=pltpu.CompilerParams(vmem_limit_bytes=126 * 2 ** 20, disable_bounds_checks=True),
    )(x, A_wqkv, A_wo, B_w_gate, B_w_up, B_w_down)
    return out.reshape(1, S, D)
```
